```python
import jax
import jax.numpy as jnp

def _softmax(x, axis=-1):
    return jax.nn.softmax(x, axis=axis)
def _gelu(x):
    return jax.nn.gelu(x, approximate=True)
def _silu(x):
    return jax.nn.silu(x)
def _sigmoid(x):
    return jax.nn.sigmoid(x)
def _layernorm(x, axis=-1, eps=1e-5):
    m = jnp.mean(x, axis=axis, keepdims=True)
    v = jnp.var(x, axis=axis, keepdims=True)
    return (x - m) / jnp.sqrt(v + eps)
def _scatter_add(tgt, idx, src, axis=0):
    return tgt.at[idx].add(src)
def _segment_sum(src, seg, n):
    return jax.ops.segment_sum(src, seg, n)
class _Rng:
    def __init__(self, key):
        self._k = key
    def _next(self):
        self._k, sub = jax.random.split(self._k)
        return sub
    def normal(self, shape):
        return jax.random.normal(self._next(), shape, dtype=jnp.bfloat16)
    def randint(self, lo, hi, shape):
        return jax.random.randint(self._next(), shape, lo, hi, dtype=jnp.int32)
    def uniform(self, shape, lo=0.0, hi=1.0):
        return jax.random.uniform(self._next(), shape, jnp.bfloat16, lo, hi)
    def permutation(self, n):
        return jax.random.permutation(self._next(), n)


kernel_name = 'concat_heads__spectral_gfnet__compressed_kv_cla__prompt'

def setup_inputs():
    _rng = _Rng(jax.random.key(int.from_bytes(__import__("os").urandom(4), "little")))
    _w = (lambda a: (lambda t: t.astype(jnp.bfloat16) if jnp.issubdtype(t.dtype, jnp.floating) else t)(jnp.asarray(a)))
    def _A_setup():
        B, S, D = 1, 2048, 448
        Df = D // 2 + 1
        return {
            "x": _w((lambda *s: _rng.normal(s) * 0.05)(B, S, D)),
            "w_r": _w((lambda *s: _rng.normal(s) * 0.05)(S, Df) * 0.02),
            "w_i": _w((lambda *s: _rng.normal(s) * 0.05)(S, Df) * 0.02),
        }
    _A_in = _A_setup()

    def _B_setup():
        B, H, Sq, Sk, D, M = 1, 16, 2048, 2048, 256, 448
        Dc = 4 * D
        return {
            "x": _w((lambda *s: _rng.normal(s) * 0.05)(B, Sq, M)),
            "c_kv": _w((lambda *s: _rng.normal(s) * 0.05)(B, Sk, Dc)),
            "w_q": _w((lambda *s: _rng.normal(s) * 0.05)(M, H, D) * (M ** -0.5)),
            "w_uk": _w((lambda *s: _rng.normal(s) * 0.05)(Dc, H, D) * (Dc ** -0.5)),
            "w_uv": _w((lambda *s: _rng.normal(s) * 0.05)(Dc, H, D) * (Dc ** -0.5)),
            "w_o": _w((lambda *s: _rng.normal(s) * 0.05)(H, D, M) * ((H * D) ** -0.5)),
        }
    _B_in = _B_setup()

    return {
        "A_x": _A_in["x"],
        "A_w_r": _A_in["w_r"],
        "A_w_i": _A_in["w_i"],
        "B_x": _B_in["x"],
        "B_c_kv": _B_in["c_kv"],
        "B_w_q": _B_in["w_q"],
        "B_w_uk": _B_in["w_uk"],
        "B_w_uv": _B_in["w_uv"],
        "B_w_o": _B_in["w_o"],
    }

def reference(A_x, A_w_r, A_w_i, B_x, B_c_kv, B_w_q, B_w_uk, B_w_uv, B_w_o):
    def _A_ref(x, w_r, w_i):
        B, S, D = x.shape
        X = (lambda x, axes=(-2,-1): jnp.fft.rfft2(x.astype(jnp.float32), axes=axes))(x, axes=(-2, -1))
        W = w_r + 1j * w_i
        X = X * W
        y = (lambda x, s, axes=(-2,-1): jnp.fft.irfft2(x, s=s, axes=axes).astype(jnp.bfloat16))(X, (S, D), axes=(-2, -1))
        return y

    def _B_ref(x, c_kv, w_q, w_uk, w_uv, w_o):
        B, Sq, M = x.shape[0], x.shape[1], x.shape[2]
        Sk = c_kv.shape[1]
        H, D = w_q.shape[1], w_q.shape[2]
        q = jnp.einsum("bqm,mhd->bhqd", x, w_q)
        k = jnp.einsum("bkc,chd->bhkd", c_kv, w_uk)
        v = jnp.einsum("bkc,chd->bhkd", c_kv, w_uv)
        scores = jnp.einsum("bhqd,bhkd->bhqk", q, k) * (D ** -0.5)
        off = Sk - Sq
        qi = jnp.arange(Sq)[:, None]
        kj = jnp.arange(Sk)[None, :]
        cmask = kj <= (qi + off)
        scores = jnp.where(cmask[None, None], scores, -1e9)
        p = _softmax(scores, axis=-1)
        ctx = jnp.einsum("bhqk,bhkd->bhqd", p, v)
        return jnp.einsum("bhqd,hdm->bqm", ctx, w_o)

    a = _A_ref(A_x, A_w_r, A_w_i)
    b = _B_ref(B_x, B_c_kv, B_w_q, B_w_uk, B_w_uv, B_w_o)
    return jnp.concatenate([a, b], axis=-1)
```

```python
import functools
import math

import jax
import jax.numpy as jnp
import numpy as np
import jax.experimental.pallas as pl
import jax.experimental.pallas.tpu as pltpu

f32 = jnp.float32
bf16 = jnp.bfloat16

NN = (((1,), (0,)), ((), ()))
NT = (((1,), (1,)), ((), ()))

S = 2048
DM = 448
J = DM // 2 + 1
JP = 232
H = 16
D = 256
DC = 1024
R16 = 16
LN = 128
TQ = 256
CCH = DC // H


def _dot(a, b, dn):
    return jax.lax.dot_general(a, b, dn, preferred_element_type=f32)


@functools.lru_cache(maxsize=None)
def _tables():
    j = np.arange(J)[:, None].astype(np.float64)
    d = np.arange(DM)[None, :].astype(np.float64)
    ang = 2.0 * np.pi * ((j * d) % DM) / DM
    fd = np.zeros((2 * JP, DM), np.float64)
    fd[:J] = np.cos(ang)
    fd[JP:JP + J] = -np.sin(ang)

    m = np.arange(LN)[:, None].astype(np.float64)
    l = np.arange(LN)[None, :].astype(np.float64)
    a128 = 2.0 * np.pi * ((m * l) % LN) / LN
    fr, fi = np.cos(a128), -np.sin(a128)
    l2 = np.block([[fr, -fi], [fi, fr]])

    r = np.arange(R16)[:, None].astype(np.float64)
    at = 2.0 * np.pi * (r * l) / S
    tw = np.stack([np.cos(at), -np.sin(at)])
    tw = np.broadcast_to(tw[:, :, None, :], (2, R16, 8, LN)).copy()

    l3 = np.zeros((R16, 2 * LN, 2 * LN), np.float64)
    for rr in range(R16):
        a3 = 2.0 * np.pi * ((m * (rr + R16 * l)) % S) / S
        nr, ni = np.cos(a3), np.sin(a3)
        l3[rr] = np.block([[nr, -ni], [ni, nr]])

    cj = np.full((J,), 2.0)
    cj[0] = 1.0
    cj[J - 1] = 1.0
    scale = cj[None, :] / float(S * DM)
    l4 = np.stack([np.cos(ang).T * scale, -np.sin(ang).T * scale])

    cast = lambda a, dt: np.asarray(a, np.float32).astype(dt)
    return (cast(fd, bf16), cast(l2, bf16), cast(tw, np.float32), cast(l3, bf16), cast(l4, bf16))


def _cmul_const(z, k, n, sign):
    re, im = z
    k = k % n
    if k == 0:
        return re, im
    if 4 * k == n:
        return (-im, re) if sign > 0 else (im, -re)
    if 8 * k == n:
        c = math.sqrt(0.5)
        return ((re - im) * c, (re + im) * c) if sign > 0 else ((re + im) * c, (im - re) * c)
    if 8 * k == 3 * n:
        c = math.sqrt(0.5)
        return ((re + im) * (-c), (re - im) * c) if sign > 0 else ((im - re) * c, (re + im) * (-c))
    c = math.cos(2.0 * math.pi * k / n)
    s = sign * math.sin(2.0 * math.pi * k / n)
    return re * c - im * s, re * s + im * c


def _fft(zs, sign):
    n = len(zs)
    if n == 1:
        return zs
    ev = _fft(zs[0::2], sign)
    od = _fft(zs[1::2], sign)
    out = [None] * n
    for k in range(n // 2):
        if 4 * k == n:
            (er, ei), (orr, oi) = ev[k], od[k]
            if sign > 0:
                out[k] = (er - oi, ei + orr)
                out[k + n // 2] = (er + oi, ei - orr)
            else:
                out[k] = (er + oi, ei - orr)
                out[k + n // 2] = (er - oi, ei + orr)
            continue
        tr, ti = _cmul_const(od[k], k, n, sign)
        er, ei = ev[k]
        out[k] = (er + tr, ei + ti)
        out[k + n // 2] = (er - tr, ei - ti)
    return out


def _kernel(axt_hbm, wrt_hbm, wit_hbm, bxt_hbm, ckv_hbm, wq_hbm, wuk_hbm, wuv_hbm, wot_hbm,
            fd_hbm, l2_hbm, tw_hbm, l3_hbm, l4_hbm,
            out_hbm,
            axt, wrt, wit, fd, l2, tw, l3, l4,
            bxt, xn, ckv, wq_raw, wq_s, wuk_raw, wuv_raw, wkv_s, wot, q_all,
            ot, obuf, sem, wsem, osem, *, do_a, do_b):
    simple = [(axt_hbm, axt), (fd_hbm, fd), (tw_hbm, tw), (l2_hbm, l2), (wrt_hbm, wrt), (wit_hbm, wit),
              (l3_hbm, l3), (l4_hbm, l4), (bxt_hbm, bxt), (wq_hbm, wq_raw), (ckv_hbm, ckv), (wot_hbm, wot)]
    cps = [pltpu.make_async_copy(s, d, sem.at[i]) for i, (s, d) in enumerate(simple)]
    (c_axt, c_fd, c_tw, c_l2, c_wrt, c_wit, c_l3, c_l4, c_bxt, c_wq, c_ckv, c_wot) = cps

    def wchunk(which, t):
        src, dst = ((wuk_hbm, wuk_raw), (wuv_hbm, wuv_raw))[which]
        return pltpu.make_async_copy(src.at[pl.ds(t * CCH, CCH)], dst.at[pl.ds(t * CCH, CCH)], wsem.at[which, t])

    for c in cps[:11]:
        c.start()
    for t in range(H):
        wchunk(0, t).start()
        wchunk(1, t).start()
    c_wot.start()

    def part_a(x1, rm, wf, cs, u):
        c_axt.wait()
        c_fd.wait()
        for c in range(4):
            x1[:, c * 512:(c + 1) * 512] = _dot(fd[...], axt[:, c * 512:(c + 1) * 512], NN)

        c_tw.wait()

        def fwd16(g, carry):
            r0 = pl.multiple_of(g * 8, 8)
            zs = [(x1[pl.ds(r0, 8), c * LN:(c + 1) * LN], x1[pl.ds(JP + r0, 8), c * LN:(c + 1) * LN])
                  for c in range(R16)]
            ys = _fft(zs, -1)
            for r in range(R16):
                re, im = ys[r]
                if r:
                    tr, ti = tw[0, r], tw[1, r]
                    re, im = re * tr - im * ti, re * ti + im * tr
                rm[r, pl.ds(r0, 8), 0:LN] = re
                rm[r, pl.ds(r0, 8), LN:2 * LN] = im
            return carry

        jax.lax.fori_loop(0, JP // 8, fwd16, 0)

        c_wrt.wait()
        c_wit.wait()
        row = jax.lax.broadcasted_iota(jnp.int32, (LN, LN), 0)
        col = jax.lax.broadcasted_iota(jnp.int32, (LN, LN), 1)
        perm = jnp.where(col == (row >> 3) + R16 * (row & 7), 1.0, 0.0).astype(bf16)
        for p, wt in enumerate((wrt, wit)):
            for c in range(R16):
                wf[p, c] = _dot(perm, wt[:, c * LN:(c + 1) * LN], NT)

        c_l2.wait()
        c_l3.wait()
        for r in range(R16):
            x = _dot(l2[...], rm[r, 0:J, :].astype(bf16), NT)
            xr, xi = x[0:LN], x[LN:2 * LN]
            wr = wf[0, :, 8 * r:8 * r + 8, :].reshape(LN, J)
            wi = wf[1, :, 8 * r:8 * r + 8, :].reshape(LN, J)
            g = jnp.concatenate([xr * wr - xi * wi, xr * wi + xi * wr], axis=0).astype(bf16)
            cs[r] = _dot(l3[r], g, NN)

        def inv16(g, carry):
            r0 = pl.multiple_of(g * 8, 8)
            for a, b in ((0, LN), (LN, J)):
                zs = [(cs[r, pl.ds(r0, 8), a:b], cs[r, pl.ds(LN + r0, 8), a:b]) for r in range(R16)]
                ys = _fft(zs, +1)
                for c in range(R16):
                    u[0, c, pl.ds(r0, 8), a:b] = ys[c][0]
                    u[1, c, pl.ds(r0, 8), a:b] = ys[c][1]
            return carry

        jax.lax.fori_loop(0, LN // 8, inv16, 0)

        c_l4.wait()
        for c in range(0, R16, 4):
            ur = u[0, c:c + 4].reshape(4 * LN, J).astype(bf16)
            ui = u[1, c:c + 4].reshape(4 * LN, J).astype(bf16)
            ot[0:DM, c * LN:(c + 4) * LN] = _dot(l4[0], ur, NT) + _dot(l4[1], ui, NT)

    if do_a:
        pl.run_scoped(part_a,
                      pltpu.VMEM((2 * JP, S), f32),
                      pltpu.VMEM((R16, JP, 2 * LN), f32),
                      pltpu.VMEM((2, R16, LN, J), f32),
                      pltpu.VMEM((R16, 2 * LN, J), f32),
                      pltpu.VMEM((2, R16, LN, J), f32))
    else:
        for c in (c_axt, c_fd, c_tw, c_wrt, c_wit, c_l2, c_l3, c_l4):
            c.wait()
        ot[0:DM, :] = jnp.zeros((DM, S), f32)

    c_bxt.wait()
    c_wq.wait()
    c_ckv.wait()
    c_wot.wait()
    ot[DM:2 * DM, :] = jnp.zeros((DM, S), f32)

    if do_b:
        for c in range(S // 256):
            xn[c * 256:(c + 1) * 256, :] = bxt[:, c * 256:(c + 1) * 256].T
        for c in range(DM // 64):
            wq_s[:, c * 64:(c + 1) * 64, :] = jnp.swapaxes(wq_raw[c * 64:(c + 1) * 64], 0, 1)

    qscale = (D ** -0.5) * math.log2(math.e)

    def qstep(t, carry):
        wchunk(0, t).wait()
        wchunk(1, t).wait()
        if do_b:
            r0 = pl.multiple_of(t * CCH, CCH)
            wkv_s[:, pl.ds(r0, CCH), 0:D] = jnp.swapaxes(wuk_raw[pl.ds(r0, CCH)], 0, 1)
            wkv_s[:, pl.ds(r0, CCH), D:2 * D] = jnp.swapaxes(wuv_raw[pl.ds(r0, CCH)], 0, 1)
            q_all[t] = (_dot(xn[...], wq_s[t], NN) * qscale).astype(bf16)
        return carry

    jax.lax.fori_loop(0, H, qstep, 0)

    def head(h, carry):
        kv = _dot(ckv[...], wkv_s[h], NN).astype(bf16)
        k = kv[:, 0:D]
        v = kv[:, D:2 * D]
        wo = wot[h]
        rr = jax.lax.broadcasted_iota(jnp.int32, (LN, LN), 0)
        cc = jax.lax.broadcasted_iota(jnp.int32, (LN, LN), 1)
        tri = cc <= rr
        neg = -1e30
        for i in reversed(range(S // TQ)):
            r0 = i * TQ
            lm = r0 + LN
            q = q_all[h, r0:r0 + TQ, :]
            s = _dot(q, k[0:lm], NT)
            sx = jnp.where(tri, _dot(q[LN:], k[lm:lm + LN], NT), neg)
            sd = jnp.where(tri, s[0:LN, r0:lm], neg)
            mt = jnp.max(sd, axis=1, keepdims=True)
            if i:
                st = s[0:LN, 0:r0]
                mt = jnp.maximum(mt, jnp.max(st, axis=1, keepdims=True))
                pt = jnp.concatenate([jnp.exp2(st - mt), jnp.exp2(sd - mt)], axis=1)
            else:
                pt = jnp.exp2(sd - mt)
            sb = s[LN:]
            mb = jnp.maximum(jnp.max(sb, axis=1, keepdims=True), jnp.max(sx, axis=1, keepdims=True))
            pb = jnp.exp2(sb - mb)
            px = jnp.exp2(sx - mb)
            lt = jnp.sum(pt, axis=1, keepdims=True)
            lb = jnp.sum(pb, axis=1, keepdims=True) + jnp.sum(px, axis=1, keepdims=True)
            p = jnp.concatenate([pt, pb], axis=0).astype(bf16)
            ctx = _dot(p, v[0:lm], NN)
            cx = _dot(px.astype(bf16), v[lm:lm + LN], NN)
            ctx = jnp.concatenate([ctx[0:LN] * (1.0 / lt), (ctx[LN:] + cx) * (1.0 / lb)], axis=0).astype(bf16)
            ot[DM:2 * DM, r0:r0 + TQ] += _dot(wo, ctx, NT)
        return carry

    if do_b:
        jax.lax.fori_loop(0, H, head, 0)

    ocp = [pltpu.make_async_copy(obuf.at[pl.ds(c * 256, 256)], out_hbm.at[pl.ds(c * 256, 256)], osem.at[c])
           for c in range(S // 256)]
    for c in range(S // 256):
        obuf[c * 256:(c + 1) * 256, :] = ot[:, c * 256:(c + 1) * 256].astype(bf16).T
        ocp[c].start()
    for c in ocp:
        c.wait()


def _build(do_a=True, do_b=True):
    def run(A_x, A_w_r, A_w_i, B_x, B_c_kv, B_w_q, B_w_uk, B_w_uv, B_w_o):
        axt = jnp.swapaxes(A_x, 1, 2).reshape(DM, S)
        bxt = jnp.swapaxes(B_x, 1, 2).reshape(DM, S)
        wrt = A_w_r.T
        wit = A_w_i.T
        ckv = B_c_kv.reshape(S, DC)
        wot = jnp.swapaxes(B_w_o, 1, 2)
        tabs = [jnp.asarray(t) for t in _tables()]
        args = (axt, wrt, wit, bxt, ckv, B_w_q, B_w_uk, B_w_uv, wot, *tabs)
        vm = pltpu.VMEM
        scratch = [
            vm((DM, S), bf16), vm((J, S), bf16), vm((J, S), bf16),
            vm(tabs[0].shape, bf16), vm(tabs[1].shape, bf16), vm(tabs[2].shape, f32),
            vm(tabs[3].shape, bf16), vm(tabs[4].shape, bf16),
            vm((DM, S), bf16), vm((S, DM), bf16), vm((S, DC), bf16),
            vm((DM, H, D), bf16), vm((H, DM, D), bf16),
            vm((DC, H, D), bf16), vm((DC, H, D), bf16), vm((H, DC, 2 * D), bf16),
            vm((H, DM, D), bf16), vm((H, S, D), bf16),
            vm((2 * DM, S), f32), vm((S, 2 * DM), bf16),
            pltpu.SemaphoreType.DMA((12,)), pltpu.SemaphoreType.DMA((2, H)),
            pltpu.SemaphoreType.DMA((S // 256,)),
        ]
        out = pl.pallas_call(
            functools.partial(_kernel, do_a=do_a, do_b=do_b),
            in_specs=[pl.BlockSpec(memory_space=pl.ANY)] * len(args),
            out_specs=pl.BlockSpec(memory_space=pl.ANY),
            out_shape=jax.ShapeDtypeStruct((S, 2 * DM), bf16),
            scratch_shapes=scratch,
            compiler_params=pltpu.CompilerParams(vmem_limit_bytes=120 * 2**20),
        )(*args)
        return out.reshape(1, S, 2 * DM)

    return run


_run = _build()


@jax.jit
def pallas_concat_heads__spectral_gfnet__compressed_kv_cla__prompt_kernel(
    A_x: jax.Array,
    A_w_r: jax.Array,
    A_w_i: jax.Array,
    B_x: jax.Array,
    B_c_kv: jax.Array,
    B_w_q: jax.Array,
    B_w_uk: jax.Array,
    B_w_uv: jax.Array,
    B_w_o: jax.Array,
):
    return _run(A_x, A_w_r, A_w_i, B_x, B_c_kv, B_w_q, B_w_uk, B_w_uv, B_w_o)
```

```python
import functools
import math

import jax
import jax.numpy as jnp
import numpy as np
import jax.experimental.pallas as pl
import jax.experimental.pallas.tpu as pltpu

f32 = jnp.float32
bf16 = jnp.bfloat16

NN = (((1,), (0,)), ((), ()))
NT = (((1,), (1,)), ((), ()))

S = 2048
DM = 448
J = DM // 2 + 1
JP = 232
H = 16
D = 256
DC = 1024
R16 = 16
LN = 128
TQ = 256
CCH = DC // H
LOOKAHEAD = 3


def _dot(a, b, dn):
    return jax.lax.dot_general(a, b, dn, preferred_element_type=f32)


@functools.lru_cache(maxsize=None)
def _tables():
    j = np.arange(J)[:, None].astype(np.float64)
    d = np.arange(DM)[None, :].astype(np.float64)
    ang = 2.0 * np.pi * ((j * d) % DM) / DM
    fd = np.zeros((2 * JP, DM), np.float64)
    fd[:J] = np.cos(ang)
    fd[JP:JP + J] = -np.sin(ang)

    m = np.arange(LN)[:, None].astype(np.float64)
    l = np.arange(LN)[None, :].astype(np.float64)
    a128 = 2.0 * np.pi * ((m * l) % LN) / LN
    fr, fi = np.cos(a128), -np.sin(a128)
    l2 = np.block([[fr, -fi], [fi, fr]])

    r = np.arange(R16)[:, None].astype(np.float64)
    at = 2.0 * np.pi * (r * l) / S
    tw = np.stack([np.cos(at), -np.sin(at)])
    tw = np.broadcast_to(tw[:, :, None, :], (2, R16, 8, LN)).copy()

    l3 = np.zeros((R16, 2 * LN, 2 * LN), np.float64)
    for rr in range(R16):
        a3 = 2.0 * np.pi * ((m * (rr + R16 * l)) % S) / S
        nr, ni = np.cos(a3), np.sin(a3)
        l3[rr] = np.block([[nr, -ni], [ni, nr]])

    cj = np.full((J,), 2.0)
    cj[0] = 1.0
    cj[J - 1] = 1.0
    scale = cj[None, :] / float(S * DM)
    l4 = np.stack([np.cos(ang).T * scale, -np.sin(ang).T * scale])

    cast = lambda a, dt: np.asarray(a, np.float32).astype(dt)
    return (cast(fd, bf16), cast(l2, bf16), cast(tw, np.float32), cast(l3, bf16), cast(l4, bf16))


def _cmul_const(z, k, n, sign):
    re, im = z
    k = k % n
    if k == 0:
        return re, im
    if 4 * k == n:
        return (-im, re) if sign > 0 else (im, -re)
    if 8 * k == n:
        c = math.sqrt(0.5)
        return ((re - im) * c, (re + im) * c) if sign > 0 else ((re + im) * c, (im - re) * c)
    if 8 * k == 3 * n:
        c = math.sqrt(0.5)
        return ((re + im) * (-c), (re - im) * c) if sign > 0 else ((im - re) * c, (re + im) * (-c))
    c = math.cos(2.0 * math.pi * k / n)
    s = sign * math.sin(2.0 * math.pi * k / n)
    return re * c - im * s, re * s + im * c


def _fft(zs, sign):
    n = len(zs)
    if n == 1:
        return zs
    ev = _fft(zs[0::2], sign)
    od = _fft(zs[1::2], sign)
    out = [None] * n
    for k in range(n // 2):
        if 4 * k == n:
            (er, ei), (orr, oi) = ev[k], od[k]
            if sign > 0:
                out[k] = (er - oi, ei + orr)
                out[k + n // 2] = (er + oi, ei - orr)
            else:
                out[k] = (er + oi, ei - orr)
                out[k + n // 2] = (er - oi, ei + orr)
            continue
        tr, ti = _cmul_const(od[k], k, n, sign)
        er, ei = ev[k]
        out[k] = (er + tr, ei + ti)
        out[k + n // 2] = (er - tr, ei - ti)
    return out


def _softmax_rows(segs):
    m = functools.reduce(jnp.maximum, [jnp.max(sg, axis=1, keepdims=True) for sg in segs])
    es = [jnp.exp2(sg - m) for sg in segs]
    l = functools.reduce(jnp.add, [jnp.sum(e, axis=1, keepdims=True) for e in es])
    return [e.astype(bf16) for e in es], l


def _kernel(axt_hbm, wrt_hbm, wit_hbm, bxt_hbm, ckv_hbm, wq_hbm, wuk_hbm, wuv_hbm, wot_hbm,
            fd_hbm, l2_hbm, tw_hbm, l3_hbm, l4_hbm,
            out_hbm,
            axt, wrt, wit, fd, l2, tw, l3, l4,
            bxt, xn, ckv, wq_raw, wq_s, wuk_raw, wuv_raw, wkv_s, wot, q_all,
            ot, obuf, sem, wsem, osem, *, do_a, do_b):
    simple = [(axt_hbm, axt), (fd_hbm, fd), (tw_hbm, tw), (l2_hbm, l2), (wrt_hbm, wrt), (wit_hbm, wit),
              (l3_hbm, l3), (l4_hbm, l4), (bxt_hbm, bxt), (wq_hbm, wq_raw), (ckv_hbm, ckv), (wot_hbm, wot)]
    cps = [pltpu.make_async_copy(s, d, sem.at[i]) for i, (s, d) in enumerate(simple)]
    (c_axt, c_fd, c_tw, c_l2, c_wrt, c_wit, c_l3, c_l4, c_bxt, c_wq, c_ckv, c_wot) = cps

    def wchunk(which, t):
        src, dst = ((wuk_hbm, wuk_raw), (wuv_hbm, wuv_raw))[which]
        return pltpu.make_async_copy(src.at[pl.ds(t * CCH, CCH)], dst.at[pl.ds(t * CCH, CCH)], wsem.at[which, t])

    c_axt.start()
    c_fd.start()

    def part_a(x1, rm, wf, cs, u):
        c_axt.wait()
        c_fd.wait()
        for c in (c_tw, c_l2, c_wrt, c_wit, c_l3, c_l4):
            c.start()
        for c in range(4):
            x1[:, c * 512:(c + 1) * 512] = _dot(fd[...], axt[:, c * 512:(c + 1) * 512], NN)

        c_tw.wait()

        def fwd16(g, carry):
            r0 = pl.multiple_of(g * 8, 8)
            zs = [(x1[pl.ds(r0, 8), c * LN:(c + 1) * LN], x1[pl.ds(JP + r0, 8), c * LN:(c + 1) * LN])
                  for c in range(R16)]
            ys = _fft(zs, -1)
            for r in range(R16):
                re, im = ys[r]
                if r:
                    tr, ti = tw[0, r], tw[1, r]
                    re, im = re * tr - im * ti, re * ti + im * tr
                rm[r, pl.ds(r0, 8), 0:LN] = re
                rm[r, pl.ds(r0, 8), LN:2 * LN] = im
            return carry

        jax.lax.fori_loop(0, JP // 8, fwd16, 0)

        c_wrt.wait()
        c_wit.wait()
        c_l2.wait()
        c_l3.wait()
        c_l4.wait()
        for c in (c_bxt, c_wq, c_ckv):
            c.start()
        row = jax.lax.broadcasted_iota(jnp.int32, (LN, LN), 0)
        col = jax.lax.broadcasted_iota(jnp.int32, (LN, LN), 1)
        perm = jnp.where(col == (row >> 3) + R16 * (row & 7), 1.0, 0.0).astype(bf16)
        for p, wt in enumerate((wrt, wit)):
            for c in range(R16):
                wf[p, c] = _dot(perm, wt[:, c * LN:(c + 1) * LN], NT)

        for r in range(R16):
            x = _dot(l2[...], rm[r, 0:J, :].astype(bf16), NT)
            xr, xi = x[0:LN], x[LN:2 * LN]
            wr = wf[0, :, 8 * r:8 * r + 8, :].reshape(LN, J)
            wi = wf[1, :, 8 * r:8 * r + 8, :].reshape(LN, J)
            g = jnp.concatenate([xr * wr - xi * wi, xr * wi + xi * wr], axis=0).astype(bf16)
            cs[r] = _dot(l3[r], g, NN)

        def inv16(g, carry):
            r0 = pl.multiple_of(g * 8, 8)
            for a, b in ((0, LN), (LN, J)):
                zs = [(cs[r, pl.ds(r0, 8), a:b], cs[r, pl.ds(LN + r0, 8), a:b]) for r in range(R16)]
                ys = _fft(zs, +1)
                for c in range(R16):
                    u[0, c, pl.ds(r0, 8), a:b] = ys[c][0]
                    u[1, c, pl.ds(r0, 8), a:b] = ys[c][1]
            return carry

        jax.lax.fori_loop(0, LN // 8, inv16, 0)

        for c in range(0, R16, 4):
            ur = u[0, c:c + 4].reshape(4 * LN, J).astype(bf16)
            ui = u[1, c:c + 4].reshape(4 * LN, J).astype(bf16)
            ot[0:DM, c * LN:(c + 4) * LN] = _dot(l4[0], ur, NT) + _dot(l4[1], ui, NT)

    if do_a:
        pl.run_scoped(part_a,
                      pltpu.VMEM((2 * JP, S), f32),
                      pltpu.VMEM((R16, JP, 2 * LN), f32),
                      pltpu.VMEM((2, R16, LN, J), f32),
                      pltpu.VMEM((R16, 2 * LN, J), f32),
                      pltpu.VMEM((2, R16, LN, J), f32))
    else:
        c_axt.wait()
        c_fd.wait()
        for c in (c_tw, c_l2, c_wrt, c_wit, c_l3, c_l4):
            c.start()
        for c in (c_tw, c_wrt, c_wit, c_l2, c_l3, c_l4):
            c.wait()
        for c in (c_bxt, c_wq, c_ckv):
            c.start()
        ot[0:DM, :] = jnp.zeros((DM, S), f32)

    c_bxt.wait()
    c_wq.wait()
    c_ckv.wait()
    for t in range(LOOKAHEAD):
        wchunk(0, t).start()
        wchunk(1, t).start()
    c_wot.start()
    ot[DM:2 * DM, :] = jnp.zeros((DM, S), f32)

    if do_b:
        for c in range(S // 256):
            xn[c * 256:(c + 1) * 256, :] = bxt[:, c * 256:(c + 1) * 256].T
        for c in range(DM // 64):
            wq_s[:, c * 64:(c + 1) * 64, :] = jnp.swapaxes(wq_raw[c * 64:(c + 1) * 64], 0, 1)

    qscale = (D ** -0.5) * math.log2(math.e)

    def qstep(t, carry):
        wchunk(0, t).wait()
        wchunk(1, t).wait()

        @pl.when(t + LOOKAHEAD < H)
        def _():
            wchunk(0, t + LOOKAHEAD).start()
            wchunk(1, t + LOOKAHEAD).start()

        if do_b:
            r0 = pl.multiple_of(t * CCH, CCH)
            wkv_s[:, pl.ds(r0, CCH), 0:D] = jnp.swapaxes(wuk_raw[pl.ds(r0, CCH)], 0, 1)
            wkv_s[:, pl.ds(r0, CCH), D:2 * D] = jnp.swapaxes(wuv_raw[pl.ds(r0, CCH)], 0, 1)
            q_all[t] = (_dot(xn[...], wq_s[t], NN) * qscale).astype(bf16)
        return carry

    jax.lax.fori_loop(0, H, qstep, 0)
    c_wot.wait()

    def head(h, carry):
        kv = _dot(ckv[...], wkv_s[h], NN).astype(bf16)
        k = kv[:, 0:D]
        v = kv[:, D:2 * D]
        wo = wot[h]
        rr = jax.lax.broadcasted_iota(jnp.int32, (LN, LN), 0)
        cc = jax.lax.broadcasted_iota(jnp.int32, (LN, LN), 1)
        tri = cc <= rr
        neg = -1e30
        ctxs = []
        for i in reversed(range(S // TQ)):
            r0 = i * TQ
            lm = r0 + LN
            q = q_all[h, r0:r0 + TQ, :]
            s = _dot(q, k[0:lm], NT)
            sx = jnp.where(tri, _dot(q[LN:], k[lm:lm + LN], NT), neg)
            sd = jnp.where(tri, s[0:LN, r0:lm], neg)
            pt, lt = _softmax_rows(([s[0:LN, 0:r0]] if i else []) + [sd])
            pb, lb = _softmax_rows([s[LN:], sx])
            pt = jnp.concatenate(pt, axis=1) if i else pt[0]
            ctx = _dot(jnp.concatenate([pt, pb[0]], axis=0), v[0:lm], NN)
            cx = _dot(pb[1], v[lm:lm + LN], NN)
            ctxs.append(jnp.concatenate([ctx[0:LN] * (1.0 / lt), (ctx[LN:] + cx) * (1.0 / lb)],
                                        axis=0).astype(bf16))
        res = _dot(wo, jnp.concatenate(ctxs, axis=0), NT)
        nb = S // TQ
        for n in range(nb):
            ot[DM:2 * DM, (nb - 1 - n) * TQ:(nb - n) * TQ] += res[:, n * TQ:(n + 1) * TQ]
        return carry

    if do_b:
        jax.lax.fori_loop(0, H, head, 0)

    ocp = [pltpu.make_async_copy(obuf.at[pl.ds(c * 256, 256)], out_hbm.at[pl.ds(c * 256, 256)], osem.at[c])
           for c in range(S // 256)]
    for c in range(S // 256):
        obuf[c * 256:(c + 1) * 256, :] = ot[:, c * 256:(c + 1) * 256].astype(bf16).T
        ocp[c].start()
    for c in ocp:
        c.wait()


def _build(do_a=True, do_b=True):
    def run(A_x, A_w_r, A_w_i, B_x, B_c_kv, B_w_q, B_w_uk, B_w_uv, B_w_o):
        axt = jnp.swapaxes(A_x, 1, 2).reshape(DM, S)
        bxt = jnp.swapaxes(B_x, 1, 2).reshape(DM, S)
        wrt = A_w_r.T
        wit = A_w_i.T
        ckv = B_c_kv.reshape(S, DC)
        wot = jnp.swapaxes(B_w_o, 1, 2)
        tabs = [jnp.asarray(t) for t in _tables()]
        args = (axt, wrt, wit, bxt, ckv, B_w_q, B_w_uk, B_w_uv, wot, *tabs)
        vm = pltpu.VMEM
        scratch = [
            vm((DM, S), bf16), vm((J, S), bf16), vm((J, S), bf16),
            vm(tabs[0].shape, bf16), vm(tabs[1].shape, bf16), vm(tabs[2].shape, f32),
            vm(tabs[3].shape, bf16), vm(tabs[4].shape, bf16),
            vm((DM, S), bf16), vm((S, DM), bf16), vm((S, DC), bf16),
            vm((DM, H, D), bf16), vm((H, DM, D), bf16),
            vm((DC, H, D), bf16), vm((DC, H, D), bf16), vm((H, DC, 2 * D), bf16),
            vm((H, DM, D), bf16), vm((H, S, D), bf16),
            vm((2 * DM, S), f32), vm((S, 2 * DM), bf16),
            pltpu.SemaphoreType.DMA((12,)), pltpu.SemaphoreType.DMA((2, H)),
            pltpu.SemaphoreType.DMA((S // 256,)),
        ]
        out = pl.pallas_call(
            functools.partial(_kernel, do_a=do_a, do_b=do_b),
            in_specs=[pl.BlockSpec(memory_space=pl.ANY)] * len(args),
            out_specs=pl.BlockSpec(memory_space=pl.ANY),
            out_shape=jax.ShapeDtypeStruct((S, 2 * DM), bf16),
            scratch_shapes=scratch,
            compiler_params=pltpu.CompilerParams(vmem_limit_bytes=120 * 2**20),
        )(*args)
        return out.reshape(1, S, 2 * DM)

    return run


_run = _build()


@jax.jit
def pallas_concat_heads__spectral_gfnet__compressed_kv_cla__prompt_kernel(
    A_x: jax.Array,
    A_w_r: jax.Array,
    A_w_i: jax.Array,
    B_x: jax.Array,
    B_c_kv: jax.Array,
    B_w_q: jax.Array,
    B_w_uk: jax.Array,
    B_w_uv: jax.Array,
    B_w_o: jax.Array,
):
    return _run(A_x, A_w_r, A_w_i, B_x, B_c_kv, B_w_q, B_w_uk, B_w_uv, B_w_o)
```

```python
import functools
import math

import jax
import jax.numpy as jnp
import numpy as np
import jax.experimental.pallas as pl
import jax.experimental.pallas.tpu as pltpu

f32 = jnp.float32
bf16 = jnp.bfloat16

NN = (((1,), (0,)), ((), ()))
NT = (((1,), (1,)), ((), ()))

S = 2048
DM = 448
J = DM // 2 + 1
JP = 232
H = 16
D = 256
DC = 1024
R16 = 16
LN = 128
TQ = 256
CCH = DC // H
QPIECES = 16
LOOKAHEAD = 3


def _dot(a, b, dn):
    return jax.lax.dot_general(a, b, dn, preferred_element_type=f32)


@functools.lru_cache(maxsize=None)
def _tables():
    j = np.arange(J)[:, None].astype(np.float64)
    d = np.arange(DM)[None, :].astype(np.float64)
    ang = 2.0 * np.pi * ((j * d) % DM) / DM
    fd = np.zeros((2 * JP, DM), np.float64)
    fd[:J] = np.cos(ang)
    fd[JP:JP + J] = -np.sin(ang)

    m = np.arange(LN)[:, None].astype(np.float64)
    l = np.arange(LN)[None, :].astype(np.float64)
    a128 = 2.0 * np.pi * ((m * l) % LN) / LN
    fr, fi = np.cos(a128), -np.sin(a128)
    l2 = np.block([[fr, -fi], [fi, fr]])

    r = np.arange(R16)[:, None].astype(np.float64)
    at = 2.0 * np.pi * (r * l) / S
    tw = np.stack([np.cos(at), -np.sin(at)])
    tw = np.broadcast_to(tw[:, :, None, :], (2, R16, 8, LN)).copy()

    l3 = np.zeros((R16, 2 * LN, 2 * LN), np.float64)
    for rr in range(R16):
        a3 = 2.0 * np.pi * ((m * (rr + R16 * l)) % S) / S
        nr, ni = np.cos(a3), np.sin(a3)
        l3[rr] = np.block([[nr, -ni], [ni, nr]])

    cj = np.full((J,), 2.0)
    cj[0] = 1.0
    cj[J - 1] = 1.0
    scale = cj[None, :] / float(S * DM)
    l4 = np.stack([np.cos(ang).T * scale, -np.sin(ang).T * scale])

    cast = lambda a, dt: np.asarray(a, np.float32).astype(dt)
    return (cast(fd, bf16), cast(l2, bf16), cast(tw, np.float32), cast(l3, bf16), cast(l4, bf16))


def _cmul_const(z, k, n, sign):
    re, im = z
    k = k % n
    if k == 0:
        return re, im
    if 4 * k == n:
        return (-im, re) if sign > 0 else (im, -re)
    if 8 * k == n:
        c = math.sqrt(0.5)
        return ((re - im) * c, (re + im) * c) if sign > 0 else ((re + im) * c, (im - re) * c)
    if 8 * k == 3 * n:
        c = math.sqrt(0.5)
        return ((re + im) * (-c), (re - im) * c) if sign > 0 else ((im - re) * c, (re + im) * (-c))
    c = math.cos(2.0 * math.pi * k / n)
    s = sign * math.sin(2.0 * math.pi * k / n)
    return re * c - im * s, re * s + im * c


def _fft(zs, sign):
    n = len(zs)
    if n == 1:
        return zs
    ev = _fft(zs[0::2], sign)
    od = _fft(zs[1::2], sign)
    out = [None] * n
    for k in range(n // 2):
        if 4 * k == n:
            (er, ei), (orr, oi) = ev[k], od[k]
            if sign > 0:
                out[k] = (er - oi, ei + orr)
                out[k + n // 2] = (er + oi, ei - orr)
            else:
                out[k] = (er + oi, ei - orr)
                out[k + n // 2] = (er - oi, ei + orr)
            continue
        tr, ti = _cmul_const(od[k], k, n, sign)
        er, ei = ev[k]
        out[k] = (er + tr, ei + ti)
        out[k + n // 2] = (er - tr, ei - ti)
    return out


def _softmax_rows(segs):
    m = functools.reduce(jnp.maximum, [jnp.max(sg, axis=1, keepdims=True) for sg in segs])
    es = [jnp.exp2(sg - m) for sg in segs]
    l = functools.reduce(jnp.add, [jnp.sum(e, axis=1, keepdims=True) for e in es])
    return [e.astype(bf16) for e in es], l


def _kernel(axt_hbm, wrt_hbm, wit_hbm, bxt_hbm, ckv_hbm, wq_hbm, wuk_hbm, wuv_hbm, wot_hbm,
            fd_hbm, l2_hbm, tw_hbm, l3_hbm, l4_hbm,
            out_hbm,
            axt, wrt, wit, fd, l2, tw, l3, l4,
            bxt, xn, ckv, wq_raw, wuk_raw, wuv_raw, wall, wot, q_all,
            ot, obuf, sem, wsem, osem, *, do_a, do_b):
    simple = [(axt_hbm, axt), (fd_hbm, fd), (tw_hbm, tw), (l2_hbm, l2), (wrt_hbm, wrt), (wit_hbm, wit),
              (l3_hbm, l3), (l4_hbm, l4), (bxt_hbm, bxt), (wq_hbm, wq_raw), (ckv_hbm, ckv), (wot_hbm, wot)]
    cps = [pltpu.make_async_copy(s, d, sem.at[i]) for i, (s, d) in enumerate(simple)]
    (c_axt, c_fd, c_tw, c_l2, c_wrt, c_wit, c_l3, c_l4, c_bxt, c_wq, c_ckv, c_wot) = cps

    def wchunk(which, t):
        src, dst = ((wuk_hbm, wuk_raw), (wuv_hbm, wuv_raw))[which]
        return pltpu.make_async_copy(src.at[pl.ds(t * CCH, CCH)], dst.at[pl.ds(t * CCH, CCH)], wsem.at[which, t])

    c_axt.start()
    c_fd.start()

    def part_a(x1, rm, wf, cs, u):
        c_axt.wait()
        c_fd.wait()
        for c in (c_tw, c_l2, c_wrt, c_wit, c_l3, c_l4):
            c.start()
        for c in range(4):
            x1[:, c * 512:(c + 1) * 512] = _dot(fd[...], axt[:, c * 512:(c + 1) * 512], NN)

        c_tw.wait()

        def fwd16(g, carry):
            r0 = pl.multiple_of(g * 8, 8)
            zs = [(x1[pl.ds(r0, 8), c * LN:(c + 1) * LN], x1[pl.ds(JP + r0, 8), c * LN:(c + 1) * LN])
                  for c in range(R16)]
            ys = _fft(zs, -1)
            for r in range(R16):
                re, im = ys[r]
                if r:
                    tr, ti = tw[0, r], tw[1, r]
                    re, im = re * tr - im * ti, re * ti + im * tr
                rm[r, pl.ds(r0, 8), 0:LN] = re
                rm[r, pl.ds(r0, 8), LN:2 * LN] = im
            return carry

        jax.lax.fori_loop(0, JP // 8, fwd16, 0)

        c_wrt.wait()
        c_wit.wait()
        c_l2.wait()
        c_l3.wait()
        c_l4.wait()
        for c in (c_bxt, c_wq):
            c.start()
        row = jax.lax.broadcasted_iota(jnp.int32, (LN, LN), 0)
        col = jax.lax.broadcasted_iota(jnp.int32, (LN, LN), 1)
        perm = jnp.where(col == (row >> 3) + R16 * (row & 7), 1.0, 0.0).astype(bf16)
        for p, wt in enumerate((wrt, wit)):
            for c in range(R16):
                wf[p, c] = _dot(perm, wt[:, c * LN:(c + 1) * LN], NT)

        for r in range(R16):
            x = _dot(l2[...], rm[r, 0:J, :].astype(bf16), NT)
            xr, xi = x[0:LN], x[LN:2 * LN]
            wr = wf[0, :, 8 * r:8 * r + 8, :].reshape(LN, J)
            wi = wf[1, :, 8 * r:8 * r + 8, :].reshape(LN, J)
            g = jnp.concatenate([xr * wr - xi * wi, xr * wi + xi * wr], axis=0).astype(bf16)
            cs[r] = _dot(l3[r], g, NN)

        def inv16(g, carry):
            r0 = pl.multiple_of(g * 8, 8)
            for a, b in ((0, LN), (LN, J)):
                zs = [(cs[r, pl.ds(r0, 8), a:b], cs[r, pl.ds(LN + r0, 8), a:b]) for r in range(R16)]
                ys = _fft(zs, +1)
                for c in range(R16):
                    u[0, c, pl.ds(r0, 8), a:b] = ys[c][0]
                    u[1, c, pl.ds(r0, 8), a:b] = ys[c][1]
            return carry

        jax.lax.fori_loop(0, LN // 8, inv16, 0)

        c_bxt.wait()
        c_wq.wait()
        for t in range(LOOKAHEAD):
            wchunk(0, t).start()
            wchunk(1, t).start()
        for c in range(0, R16, 4):
            ur = u[0, c:c + 4].reshape(4 * LN, J).astype(bf16)
            ui = u[1, c:c + 4].reshape(4 * LN, J).astype(bf16)
            ot[0:DM, c * LN:(c + 4) * LN] = _dot(l4[0], ur, NT) + _dot(l4[1], ui, NT)

    if do_a:
        pl.run_scoped(part_a,
                      pltpu.VMEM((2 * JP, S), f32),
                      pltpu.VMEM((R16, JP, 2 * LN), f32),
                      pltpu.VMEM((2, R16, LN, J), f32),
                      pltpu.VMEM((R16, 2 * LN, J), f32),
                      pltpu.VMEM((2, R16, LN, J), f32))
    else:
        c_axt.wait()
        c_fd.wait()
        for c in (c_tw, c_l2, c_wrt, c_wit, c_l3, c_l4):
            c.start()
        for c in (c_tw, c_wrt, c_wit, c_l2, c_l3, c_l4):
            c.wait()
        for c in (c_bxt, c_wq):
            c.start()
        c_bxt.wait()
        c_wq.wait()
        for t in range(LOOKAHEAD):
            wchunk(0, t).start()
            wchunk(1, t).start()
        ot[0:DM, :] = jnp.zeros((DM, S), f32)

    ot[DM:2 * DM, :] = jnp.zeros((DM, S), f32)

    if do_b:
        for c in range(S // 256):
            xn[c * 256:(c + 1) * 256, :] = bxt[:, c * 256:(c + 1) * 256].T
        for c in range(DM // 64):
            wall[:, c * 64:(c + 1) * 64, :] = jnp.swapaxes(wq_raw[c * 64:(c + 1) * 64], 0, 1)

    qscale = (D ** -0.5) * math.log2(math.e)

    wchunk(0, 0).wait()
    wchunk(1, 0).wait()

    def qstep(t, carry):
        if do_b:
            rq, rw = S // QPIECES, 2 * CCH // QPIECES
            for j in range(QPIECES):
                which, off = divmod(j * rw, CCH)
                r0 = pl.multiple_of(t * CCH + off, rw)
                src = (wuk_raw, wuv_raw)[which]
                wall[:, pl.ds(DM + which * DC + r0, rw), :] = jnp.swapaxes(src[pl.ds(r0, rw)], 0, 1)
                q_all[t, j * rq:(j + 1) * rq] = (_dot(xn[j * rq:(j + 1) * rq], wall[t, 0:DM, :], NN) * qscale).astype(bf16)

        @pl.when(t + LOOKAHEAD < H)
        def _():
            wchunk(0, t + LOOKAHEAD).start()
            wchunk(1, t + LOOKAHEAD).start()

        @pl.when(t == 1)
        def _():
            c_ckv.start()

        @pl.when(t == 6)
        def _():
            c_wot.start()

        @pl.when(t + 1 < H)
        def _():
            wchunk(0, t + 1).wait()
            wchunk(1, t + 1).wait()

        return carry

    jax.lax.fori_loop(0, H, qstep, 0)
    c_ckv.wait()
    c_wot.wait()

    def head(h, carry):
        wkv = jnp.concatenate([wall[h, DM:DM + DC, :], wall[h, DM + DC:DM + 2 * DC, :]], axis=1)
        kv = _dot(ckv[...], wkv, NN).astype(bf16)
        k = kv[:, 0:D]
        v = kv[:, D:2 * D]
        wo = wot[h]
        rr = jax.lax.broadcasted_iota(jnp.int32, (LN, LN), 0)
        cc = jax.lax.broadcasted_iota(jnp.int32, (LN, LN), 1)
        tri = cc <= rr
        neg = -1e30
        ctxs = []
        for i in reversed(range(S // TQ)):
            r0 = i * TQ
            lm = r0 + LN
            q = q_all[h, r0:r0 + TQ, :]
            s = _dot(q, k[0:lm], NT)
            sx = jnp.where(tri, _dot(q[LN:], k[lm:lm + LN], NT), neg)
            sd = jnp.where(tri, s[0:LN, r0:lm], neg)
            pt, lt = _softmax_rows(([s[0:LN, 0:r0]] if i else []) + [sd])
            pb, lb = _softmax_rows([s[LN:], sx])
            pt = jnp.concatenate(pt, axis=1) if i else pt[0]
            ctx = _dot(jnp.concatenate([pt, pb[0]], axis=0), v[0:lm], NN)
            cx = _dot(pb[1], v[lm:lm + LN], NN)
            ctxs.append(jnp.concatenate([ctx[0:LN] * (1.0 / lt), (ctx[LN:] + cx) * (1.0 / lb)],
                                        axis=0).astype(bf16))
        res = _dot(wo, jnp.concatenate(ctxs, axis=0), NT)
        nb = S // TQ
        for n in range(nb):
            ot[DM:2 * DM, (nb - 1 - n) * TQ:(nb - n) * TQ] += res[:, n * TQ:(n + 1) * TQ]
        return carry

    if do_b:
        jax.lax.fori_loop(0, H, head, 0)

    ocp = [pltpu.make_async_copy(obuf.at[pl.ds(c * 256, 256)], out_hbm.at[pl.ds(c * 256, 256)], osem.at[c])
           for c in range(S // 256)]
    for c in range(S // 256):
        obuf[c * 256:(c + 1) * 256, :] = ot[:, c * 256:(c + 1) * 256].astype(bf16).T
        ocp[c].start()
    for c in ocp:
        c.wait()


def _build(do_a=True, do_b=True):
    def run(A_x, A_w_r, A_w_i, B_x, B_c_kv, B_w_q, B_w_uk, B_w_uv, B_w_o):
        axt = jnp.swapaxes(A_x, 1, 2).reshape(DM, S)
        bxt = jnp.swapaxes(B_x, 1, 2).reshape(DM, S)
        wrt = A_w_r.T
        wit = A_w_i.T
        ckv = B_c_kv.reshape(S, DC)
        wot = jnp.swapaxes(B_w_o, 1, 2)
        tabs = [jnp.asarray(t) for t in _tables()]
        args = (axt, wrt, wit, bxt, ckv, B_w_q, B_w_uk, B_w_uv, wot, *tabs)
        vm = pltpu.VMEM
        scratch = [
            vm((DM, S), bf16), vm((J, S), bf16), vm((J, S), bf16),
            vm(tabs[0].shape, bf16), vm(tabs[1].shape, bf16), vm(tabs[2].shape, f32),
            vm(tabs[3].shape, bf16), vm(tabs[4].shape, bf16),
            vm((DM, S), bf16), vm((S, DM), bf16), vm((S, DC), bf16),
            vm((DM, H, D), bf16),
            vm((DC, H, D), bf16), vm((DC, H, D), bf16), vm((H, DM + 2 * DC, D), bf16),
            vm((H, DM, D), bf16), vm((H, S, D), bf16),
            vm((2 * DM, S), f32), vm((S, 2 * DM), bf16),
            pltpu.SemaphoreType.DMA((12,)), pltpu.SemaphoreType.DMA((2, H)),
            pltpu.SemaphoreType.DMA((S // 256,)),
        ]
        out = pl.pallas_call(
            functools.partial(_kernel, do_a=do_a, do_b=do_b),
            in_specs=[pl.BlockSpec(memory_space=pl.ANY)] * len(args),
            out_specs=pl.BlockSpec(memory_space=pl.ANY),
            out_shape=jax.ShapeDtypeStruct((S, 2 * DM), bf16),
            scratch_shapes=scratch,
            compiler_params=pltpu.CompilerParams(vmem_limit_bytes=120 * 2**20),
        )(*args)
        return out.reshape(1, S, 2 * DM)

    return run


_run = _build()


@jax.jit
def pallas_concat_heads__spectral_gfnet__compressed_kv_cla__prompt_kernel(
    A_x: jax.Array,
    A_w_r: jax.Array,
    A_w_i: jax.Array,
    B_x: jax.Array,
    B_c_kv: jax.Array,
    B_w_q: jax.Array,
    B_w_uk: jax.Array,
    B_w_uv: jax.Array,
    B_w_o: jax.Array,
):
    return _run(A_x, A_w_r, A_w_i, B_x, B_c_kv, B_w_q, B_w_uk, B_w_uv, B_w_o)
```

```python
import contextlib
import functools
import math

import jax
import jax.numpy as jnp
import numpy as np
import jax.experimental.pallas as pl
import jax.experimental.pallas.tpu as pltpu

f32 = jnp.float32
bf16 = jnp.bfloat16

NN = (((1,), (0,)), ((), ()))
NT = (((1,), (1,)), ((), ()))

S = 2048
DM = 448
J = DM // 2 + 1
JB = 104
H = 16
D = 256
DC = 1024
R16 = 16
LN = 128
TQ = 256
CCH = DC // H
OCH = 128
QPIECES = 16
LOOKAHEAD = 3


def _dot(a, b, dn):
    return jax.lax.dot_general(a, b, dn, preferred_element_type=f32)


@functools.lru_cache(maxsize=None)
def _tables():
    j = np.arange(J)[:, None].astype(np.float64)
    d = np.arange(DM)[None, :].astype(np.float64)
    ang = 2.0 * np.pi * ((j * d) % DM) / DM
    cos, sin = np.cos(ang), np.sin(ang)
    fd = np.zeros((2 * LN + 2 * JB, DM), np.float64)
    fd[0:LN] = cos[0:LN]
    fd[LN:2 * LN] = -sin[0:LN]
    fd[2 * LN:2 * LN + J - LN] = cos[LN:]
    fd[2 * LN + JB:2 * LN + JB + J - LN] = -sin[LN:]

    m = np.arange(LN)[:, None].astype(np.float64)
    l = np.arange(LN)[None, :].astype(np.float64)
    a128 = 2.0 * np.pi * ((m * l) % LN) / LN
    fr, fi = np.cos(a128), -np.sin(a128)
    l2 = np.block([[fr, -fi], [fi, fr]])

    r = np.arange(R16)[:, None].astype(np.float64)
    at = 2.0 * np.pi * (r * l) / S
    tw = np.stack([np.cos(at), -np.sin(at)])
    tw = np.broadcast_to(tw[:, :, None, :], (2, R16, 8, LN)).copy()

    l3 = np.zeros((R16, 2 * LN, 2 * LN), np.float64)
    for rr in range(R16):
        a3 = 2.0 * np.pi * ((m * (rr + R16 * l)) % S) / S
        nr, ni = np.cos(a3), np.sin(a3)
        l3[rr] = np.block([[nr, -ni], [ni, nr]])

    cj = np.full((J,), 2.0)
    cj[0] = 1.0
    cj[J - 1] = 1.0
    scale = cj[None, :] / float(S * DM)
    cr, ci = cos.T * scale, -sin.T * scale
    l4 = np.zeros((2, DM, 2 * LN), np.float64)
    l4[0, :, 0:LN] = cr[:, 0:LN]
    l4[0, :, LN:] = ci[:, 0:LN]
    l4[1, :, 0:J - LN] = cr[:, LN:]
    l4[1, :, LN:LN + J - LN] = ci[:, LN:]

    cast = lambda a, dt: np.asarray(a, np.float32).astype(dt)
    return (cast(fd, bf16), cast(l2, bf16), cast(tw, np.float32), cast(l3, bf16), cast(l4, bf16))


def _cmul_const(z, k, n, sign):
    re, im = z
    k = k % n
    if k == 0:
        return re, im
    if 4 * k == n:
        return (-im, re) if sign > 0 else (im, -re)
    if 8 * k == n:
        c = math.sqrt(0.5)
        return ((re - im) * c, (re + im) * c) if sign > 0 else ((re + im) * c, (im - re) * c)
    if 8 * k == 3 * n:
        c = math.sqrt(0.5)
        return ((re + im) * (-c), (re - im) * c) if sign > 0 else ((im - re) * c, (re + im) * (-c))
    c = math.cos(2.0 * math.pi * k / n)
    s = sign * math.sin(2.0 * math.pi * k / n)
    return re * c - im * s, re * s + im * c


def _fft(zs, sign):
    n = len(zs)
    if n == 1:
        return zs
    ev = _fft(zs[0::2], sign)
    od = _fft(zs[1::2], sign)
    out = [None] * n
    for k in range(n // 2):
        if 4 * k == n:
            (er, ei), (orr, oi) = ev[k], od[k]
            if sign > 0:
                out[k] = (er - oi, ei + orr)
                out[k + n // 2] = (er + oi, ei - orr)
            else:
                out[k] = (er + oi, ei - orr)
                out[k + n // 2] = (er - oi, ei + orr)
            continue
        tr, ti = _cmul_const(od[k], k, n, sign)
        er, ei = ev[k]
        out[k] = (er + tr, ei + ti)
        out[k + n // 2] = (er - tr, ei - ti)
    return out


def _softmax_rows(segs):
    m = functools.reduce(jnp.maximum, [jnp.max(sg, axis=1, keepdims=True) for sg in segs])
    es = [jnp.exp2(sg - m) for sg in segs]
    l = functools.reduce(jnp.add, [jnp.sum(e, axis=1, keepdims=True) for e in es])
    return [e.astype(bf16) for e in es], l


def _kernel(axt_hbm, wrt_hbm, wit_hbm, bxt_hbm, ckv_hbm, wq_hbm, wuk_hbm, wuv_hbm, wot_hbm,
            fd_hbm, l2_hbm, tw_hbm, l3_hbm, l4_hbm,
            out_hbm,
            axt, wrt, wit, fd, l2, tw, l3, l4,
            bxt, xn, ckv, wq_raw, wuk_raw, wuv_raw, wall, wot, q_all,
            ot, obuf, sem, wsem, osem, *, do_a, do_b, scopes):
    scope = jax.named_scope if scopes else (lambda name: contextlib.nullcontext())
    simple = [(axt_hbm, axt), (fd_hbm, fd), (tw_hbm, tw), (l2_hbm, l2), (wrt_hbm, wrt), (wit_hbm, wit),
              (l3_hbm, l3), (l4_hbm, l4), (bxt_hbm, bxt), (wq_hbm, wq_raw), (ckv_hbm, ckv), (wot_hbm, wot)]
    cps = [pltpu.make_async_copy(s, d, sem.at[i]) for i, (s, d) in enumerate(simple)]
    (c_axt, c_fd, c_tw, c_l2, c_wrt, c_wit, c_l3, c_l4, c_bxt, c_wq, c_ckv, c_wot) = cps

    def wchunk(which, t):
        src, dst = ((wuk_hbm, wuk_raw), (wuv_hbm, wuv_raw))[which]
        return pltpu.make_async_copy(src.at[pl.ds(t * CCH, CCH)], dst.at[pl.ds(t * CCH, CCH)], wsem.at[which, t])

    for c in (c_axt, c_fd, c_tw, c_l2):
        c.start()

    def zero(i, carry):
        ot[pl.ds(pl.multiple_of(DM + i * 64, 64), 64), :] = jnp.zeros((64, S), f32)
        return carry

    jax.lax.fori_loop(0, DM // 64, zero, 0)

    def b_prep():
        for c in range(S // 256):
            xn[c * 256:(c + 1) * 256, :] = bxt[:, c * 256:(c + 1) * 256].T
        for c in range(DM // 64):
            wall[:, c * 64:(c + 1) * 64, :] = jnp.swapaxes(wq_raw[c * 64:(c + 1) * 64], 0, 1)

    def part_a(x1a, x1b, rma, rmb, wsa, wsb, csa, csb, ua, ub):
        with scope('w0'):
            for c in (c_axt, c_fd, c_tw, c_l2):
                c.wait()
        c_wrt.start()
        c_wit.start()

        def stage1(x1, lo, hi):
            for c in range(4):
                x1[:, c * 512:(c + 1) * 512] = _dot(fd[lo:hi, :], axt[:, c * 512:(c + 1) * 512], NN)

        def fwd16(x1, rm, n):
            for r0 in range(0, n, 8):
                zs = [(x1[r0:r0 + 8, c * LN:(c + 1) * LN], x1[n + r0:n + r0 + 8, c * LN:(c + 1) * LN])
                      for c in range(R16)]
                ys = _fft(zs, -1)
                for r in range(R16):
                    re, im = ys[r]
                    if r:
                        tr, ti = tw[0, r], tw[1, r]
                        re, im = re * tr - im * ti, re * ti + im * tr
                    rm[r, r0:r0 + 8, 0:LN] = re
                    rm[r, r0:r0 + 8, LN:2 * LN] = im
            if n < LN:
                rm[:, n:LN, :] = jnp.zeros((R16, LN - n, 2 * LN), f32)

        def wprep(ws, lo, hi):
            for p, wt in enumerate((wrt, wit)):
                for c in range(R16):
                    t = wt[lo:hi, c * LN:(c + 1) * LN].astype(f32).T
                    if hi - lo < LN:
                        t = jnp.concatenate([t, jnp.zeros((LN, LN - (hi - lo)), f32)], axis=1)
                    ws[p, c * LN:(c + 1) * LN, :] = t

        def stage23(rm, ws, cs):
            x = _dot(l2[...], rm[...].reshape(R16 * LN, 2 * LN).astype(bf16), NT)
            for r in range(R16):
                xr, xi = x[0:LN, r * LN:(r + 1) * LN], x[LN:2 * LN, r * LN:(r + 1) * LN]
                wr = ws[0, pl.ds(r, LN, stride=R16), :]
                wi = ws[1, pl.ds(r, LN, stride=R16), :]
                g = jnp.concatenate([xr * wr - xi * wi, xr * wi + xi * wr], axis=0).astype(bf16)
                cs[r] = _dot(l3[r], g, NN)

        def inv16(cs, u):
            for r0 in range(0, LN, 8):
                zs = [(cs[r, r0:r0 + 8, :], cs[r, LN + r0:LN + r0 + 8, :]) for r in range(R16)]
                ys = _fft(zs, +1)
                for c in range(R16):
                    u[c, r0:r0 + 8, 0:LN] = ys[c][0]
                    u[c, r0:r0 + 8, LN:2 * LN] = ys[c][1]

        def stage4(u, half):
            for c in range(0, R16, 4):
                y = _dot(l4[half], u[c:c + 4].reshape(4 * LN, 2 * LN).astype(bf16), NT)
                if half:
                    ot[0:DM, c * LN:(c + 4) * LN] += y
                else:
                    ot[0:DM, c * LN:(c + 4) * LN] = y

        stage1(x1a, 0, 2 * LN)
        c_wrt.wait()
        c_wit.wait()
        c_l3.start()
        c_l4.start()
        stage1(x1b, 2 * LN, 2 * LN + 2 * JB)
        fwd16(x1a, rma, LN)
        wprep(wsa, 0, LN)
        c_l3.wait()
        c_l4.wait()
        c_bxt.start()
        c_wq.start()
        stage23(rma, wsa, csa)
        fwd16(x1b, rmb, JB)
        wprep(wsb, LN, J)
        stage23(rmb, wsb, csb)
        inv16(csa, ua)
        stage4(ua, 0)
        c_bxt.wait()
        c_wq.wait()
        for t in range(LOOKAHEAD):
            wchunk(0, t).start()
            wchunk(1, t).start()
        inv16(csb, ub)
        if do_b:
            b_prep()
        stage4(ub, 1)

    if do_a:
        pl.run_scoped(part_a,
                      pltpu.VMEM((2 * LN, S), f32), pltpu.VMEM((2 * JB, S), f32),
                      pltpu.VMEM((R16, LN, 2 * LN), f32), pltpu.VMEM((R16, LN, 2 * LN), f32),
                      pltpu.VMEM((2, S, LN), f32), pltpu.VMEM((2, S, LN), f32),
                      pltpu.VMEM((R16, 2 * LN, LN), f32), pltpu.VMEM((R16, 2 * LN, LN), f32),
                      pltpu.VMEM((R16, LN, 2 * LN), f32), pltpu.VMEM((R16, LN, 2 * LN), f32))
    else:
        for c in (c_axt, c_fd, c_tw, c_l2):
            c.wait()
        for c in (c_wrt, c_wit, c_l3, c_l4, c_bxt, c_wq):
            c.start()
        for c in (c_wrt, c_wit, c_l3, c_l4, c_bxt, c_wq):
            c.wait()
        for t in range(LOOKAHEAD):
            wchunk(0, t).start()
            wchunk(1, t).start()
        ot[0:DM, :] = jnp.zeros((DM, S), f32)
        if do_b:
            b_prep()

    qscale = (D ** -0.5) * math.log2(math.e)

    wchunk(0, 0).wait()
    wchunk(1, 0).wait()

    def qstep(t, carry):
        if do_b:
            rq, rw = S // QPIECES, 2 * CCH // QPIECES
            for j in range(QPIECES):
                which, off = divmod(j * rw, CCH)
                r0 = pl.multiple_of(t * CCH + off, rw)
                src = (wuk_raw, wuv_raw)[which]
                wall[:, pl.ds(DM + which * DC + r0, rw), :] = jnp.swapaxes(src[pl.ds(r0, rw)], 0, 1)
                q_all[t, j * rq:(j + 1) * rq] = (_dot(xn[j * rq:(j + 1) * rq], wall[t, 0:DM, :], NN) * qscale).astype(bf16)

        @pl.when(t + LOOKAHEAD < H)
        def _():
            wchunk(0, t + LOOKAHEAD).start()
            wchunk(1, t + LOOKAHEAD).start()

        @pl.when(t == 1)
        def _():
            c_ckv.start()

        @pl.when(t == 6)
        def _():
            c_wot.start()

        @pl.when(t + 1 < H)
        def _():
            wchunk(0, t + 1).wait()
            wchunk(1, t + 1).wait()

        return carry

    with scope('P2'):
        jax.lax.fori_loop(0, H, qstep, 0)
    c_ckv.wait()
    c_wot.wait()

    def head(h, carry):
        with scope('head'):
            return head_body(h, carry)

    def head_body(h, carry):
        wkv = jnp.concatenate([wall[h, DM:DM + DC, :], wall[h, DM + DC:DM + 2 * DC, :]], axis=1)
        kv = _dot(ckv[...], wkv, NN).astype(bf16)
        k = kv[:, 0:D]
        v = kv[:, D:2 * D]
        wo = wot[h]
        rr = jax.lax.broadcasted_iota(jnp.int32, (LN, LN), 0)
        cc = jax.lax.broadcasted_iota(jnp.int32, (LN, LN), 1)
        tri = cc <= rr
        neg = -1e30
        ctxs = []
        for i in reversed(range(S // TQ)):
            r0 = i * TQ
            lm = r0 + LN
            q = q_all[h, r0:r0 + TQ, :]
            s = _dot(q, k[0:lm], NT)
            sx = jnp.where(tri, _dot(q[LN:], k[lm:lm + LN], NT), neg)
            sd = jnp.where(tri, s[0:LN, r0:lm], neg)
            pt, lt = _softmax_rows(([s[0:LN, 0:r0]] if i else []) + [sd])
            pb, lb = _softmax_rows([s[LN:], sx])
            pt = jnp.concatenate(pt, axis=1) if i else pt[0]
            ctx = _dot(jnp.concatenate([pt, pb[0]], axis=0), v[0:lm], NN)
            cx = _dot(pb[1], v[lm:lm + LN], NN)
            ctxs.append(jnp.concatenate([ctx[0:LN] * (1.0 / lt), (ctx[LN:] + cx) * (1.0 / lb)],
                                        axis=0).astype(bf16))
        res = _dot(wo, jnp.concatenate(ctxs, axis=0), NT)
        nb = S // TQ
        for n in range(nb):
            ot[DM:2 * DM, (nb - 1 - n) * TQ:(nb - n) * TQ] += res[:, n * TQ:(n + 1) * TQ]
        return carry

    if do_b:
        with scope('P3'):
            jax.lax.fori_loop(0, H, head, 0)

    def ocopy(c):
        rows = pl.ds(pl.multiple_of(c * OCH, OCH), OCH)
        return pltpu.make_async_copy(obuf.at[rows], out_hbm.at[rows], osem.at[c])

    def ostep(c, carry):
        cols = pl.ds(pl.multiple_of(c * OCH, OCH), OCH)
        obuf[cols, :] = ot[:, cols].astype(bf16).T
        ocopy(c).start()
        return carry

    jax.lax.fori_loop(0, S // OCH, ostep, 0)
    for c in range(S // OCH):
        ocopy(c).wait()


def _build(do_a=True, do_b=True, scopes=False):
    def run(A_x, A_w_r, A_w_i, B_x, B_c_kv, B_w_q, B_w_uk, B_w_uv, B_w_o):
        axt = jnp.swapaxes(A_x, 1, 2).reshape(DM, S)
        bxt = jnp.swapaxes(B_x, 1, 2).reshape(DM, S)
        wrt = A_w_r.T
        wit = A_w_i.T
        ckv = B_c_kv.reshape(S, DC)
        wot = jnp.swapaxes(B_w_o, 1, 2)
        tabs = [jnp.asarray(t) for t in _tables()]
        args = (axt, wrt, wit, bxt, ckv, B_w_q, B_w_uk, B_w_uv, wot, *tabs)
        vm = pltpu.VMEM
        scratch = [
            vm((DM, S), bf16), vm((J, S), bf16), vm((J, S), bf16),
            vm(tabs[0].shape, bf16), vm(tabs[1].shape, bf16), vm(tabs[2].shape, f32),
            vm(tabs[3].shape, bf16), vm(tabs[4].shape, bf16),
            vm((DM, S), bf16), vm((S, DM), bf16), vm((S, DC), bf16),
            vm((DM, H, D), bf16),
            vm((DC, H, D), bf16), vm((DC, H, D), bf16), vm((H, DM + 2 * DC, D), bf16),
            vm((H, DM, D), bf16), vm((H, S, D), bf16),
            vm((2 * DM, S), f32), vm((S, 2 * DM), bf16),
            pltpu.SemaphoreType.DMA((12,)), pltpu.SemaphoreType.DMA((2, H)),
            pltpu.SemaphoreType.DMA((S // OCH,)),
        ]
        out = pl.pallas_call(
            functools.partial(_kernel, do_a=do_a, do_b=do_b, scopes=scopes),
            in_specs=[pl.BlockSpec(memory_space=pl.ANY)] * len(args),
            out_specs=pl.BlockSpec(memory_space=pl.ANY),
            out_shape=jax.ShapeDtypeStruct((S, 2 * DM), bf16),
            scratch_shapes=scratch,
            compiler_params=pltpu.CompilerParams(vmem_limit_bytes=120 * 2**20),
        )(*args)
        return out.reshape(1, S, 2 * DM)

    return run


_run = _build()


@jax.jit
def pallas_concat_heads__spectral_gfnet__compressed_kv_cla__prompt_kernel(
    A_x: jax.Array,
    A_w_r: jax.Array,
    A_w_i: jax.Array,
    B_x: jax.Array,
    B_c_kv: jax.Array,
    B_w_q: jax.Array,
    B_w_uk: jax.Array,
    B_w_uv: jax.Array,
    B_w_o: jax.Array,
):
    return _run(A_x, A_w_r, A_w_i, B_x, B_c_kv, B_w_q, B_w_uk, B_w_uv, B_w_o)
```

```python
import contextlib
import functools
import math

import jax
import jax.numpy as jnp
import numpy as np
import jax.experimental.pallas as pl
import jax.experimental.pallas.tpu as pltpu

f32 = jnp.float32
bf16 = jnp.bfloat16

NN = (((1,), (0,)), ((), ()))
NT = (((1,), (1,)), ((), ()))

S = 2048
DM = 448
J = DM // 2 + 1
JB = 104
H = 16
D = 256
DC = 1024
R16 = 16
LN = 128
TQ = 256
CCH = DC // H
PX = H
PU = H + 2
OCH = 128
QPIECES = 16


def _dot(a, b, dn):
    return jax.lax.dot_general(a, b, dn, preferred_element_type=f32)


@functools.lru_cache(maxsize=None)
def _tables():
    j = np.arange(J)[:, None].astype(np.float64)
    d = np.arange(DM)[None, :].astype(np.float64)
    ang = 2.0 * np.pi * ((j * d) % DM) / DM
    cos, sin = np.cos(ang), np.sin(ang)
    fd = np.zeros((2 * LN + 2 * JB, DM), np.float64)
    fd[0:LN] = cos[0:LN]
    fd[LN:2 * LN] = -sin[0:LN]
    fd[2 * LN:2 * LN + J - LN] = cos[LN:]
    fd[2 * LN + JB:2 * LN + JB + J - LN] = -sin[LN:]

    m = np.arange(LN)[:, None].astype(np.float64)
    l = np.arange(LN)[None, :].astype(np.float64)
    a128 = 2.0 * np.pi * ((m * l) % LN) / LN
    fr, fi = np.cos(a128), -np.sin(a128)
    l2 = np.block([[fr, -fi], [fi, fr]])

    r = np.arange(R16)[:, None].astype(np.float64)
    at = 2.0 * np.pi * (r * l) / S
    tw = np.stack([np.cos(at), -np.sin(at)])
    tw = np.broadcast_to(tw[:, :, None, :], (2, R16, 8, LN)).copy()

    l3 = np.zeros((R16, 2 * LN, 2 * LN), np.float64)
    for rr in range(R16):
        a3 = 2.0 * np.pi * ((m * (rr + R16 * l)) % S) / S
        nr, ni = np.cos(a3), np.sin(a3)
        l3[rr] = np.block([[nr, -ni], [ni, nr]])

    cj = np.full((J,), 2.0)
    cj[0] = 1.0
    cj[J - 1] = 1.0
    scale = cj[None, :] / float(S * DM)
    cr, ci = cos.T * scale, -sin.T * scale
    l4 = np.zeros((2, DM, 2 * LN), np.float64)
    l4[0, :, 0:LN] = cr[:, 0:LN]
    l4[0, :, LN:] = ci[:, 0:LN]
    l4[1, :, 0:J - LN] = cr[:, LN:]
    l4[1, :, LN:LN + J - LN] = ci[:, LN:]

    cast = lambda a, dt: np.asarray(a, np.float32).astype(dt)
    return (cast(fd, bf16), cast(l2, bf16), cast(tw, np.float32), cast(l3, bf16),
            cast(l4.reshape(2 * DM, 2 * LN), bf16))


def _cmul_const(z, k, n, sign):
    re, im = z
    k = k % n
    if k == 0:
        return re, im
    if 4 * k == n:
        return (-im, re) if sign > 0 else (im, -re)
    if 8 * k == n:
        c = math.sqrt(0.5)
        return ((re - im) * c, (re + im) * c) if sign > 0 else ((re + im) * c, (im - re) * c)
    if 8 * k == 3 * n:
        c = math.sqrt(0.5)
        return ((re + im) * (-c), (re - im) * c) if sign > 0 else ((im - re) * c, (re + im) * (-c))
    c = math.cos(2.0 * math.pi * k / n)
    s = sign * math.sin(2.0 * math.pi * k / n)
    return re * c - im * s, re * s + im * c


def _fft(zs, sign):
    n = len(zs)
    if n == 1:
        return zs
    ev = _fft(zs[0::2], sign)
    od = _fft(zs[1::2], sign)
    out = [None] * n
    for k in range(n // 2):
        if 4 * k == n:
            (er, ei), (orr, oi) = ev[k], od[k]
            if sign > 0:
                out[k] = (er - oi, ei + orr)
                out[k + n // 2] = (er + oi, ei - orr)
            else:
                out[k] = (er + oi, ei - orr)
                out[k + n // 2] = (er - oi, ei + orr)
            continue
        tr, ti = _cmul_const(od[k], k, n, sign)
        er, ei = ev[k]
        out[k] = (er + tr, ei + ti)
        out[k + n // 2] = (er - tr, ei - ti)
    return out


def _softmax_rows(segs):
    m = functools.reduce(jnp.maximum, [jnp.max(sg, axis=1, keepdims=True) for sg in segs])
    es = [jnp.exp2(sg - m) for sg in segs]
    l = functools.reduce(jnp.add, [jnp.sum(e, axis=1, keepdims=True) for e in es])
    return [e.astype(bf16) for e in es], l


def _kernel(axt_hbm, wrt_hbm, wit_hbm, bxt_hbm, ckv_hbm, wq_hbm, wuk_hbm, wuv_hbm, wot_hbm,
            fd_hbm, l2_hbm, tw_hbm, l3_hbm, l4_hbm,
            out_hbm,
            axt, wrt, wit, fd, l2, tw, l3, l4,
            bxt, ckv, wq_raw, wuk_raw, wuv_raw, wall, wot, q_all,
            ot, obuf, sem, wsem, osem, *, do_a, do_b, scopes):
    scope = jax.named_scope if scopes else (lambda name: contextlib.nullcontext())
    XC = S // 4
    simple = ([(fd_hbm.at[0:2 * LN], fd.at[0:2 * LN])]
              + [(axt_hbm.at[:, c * XC:(c + 1) * XC], axt.at[:, c * XC:(c + 1) * XC]) for c in range(4)]
              + [(fd_hbm.at[2 * LN:], fd.at[2 * LN:]), (tw_hbm, tw), (l2_hbm, l2), (wrt_hbm, wrt), (wit_hbm, wit),
                 (l3_hbm, l3), (bxt_hbm, bxt), (l4_hbm, l4), (wq_hbm, wq_raw), (ckv_hbm, ckv), (wot_hbm, wot)])
    cps = [pltpu.make_async_copy(s, d, sem.at[i]) for i, (s, d) in enumerate(simple)]
    c_fda, c_axt = cps[0], cps[1:5]
    (c_fdb, c_tw, c_l2, c_wrt, c_wit, c_l3, c_bxt, c_l4, c_wq, c_ckv, c_wot) = cps[5:]

    def wchunk(which, t):
        src, dst = ((wuk_hbm, wuk_raw), (wuv_hbm, wuv_raw))[which]
        return pltpu.make_async_copy(src.at[pl.ds(t * CCH, CCH)], dst.at[pl.ds(t * CCH, CCH)], wsem.at[which, t])

    def issue(lo, hi):
        def body(i, carry):
            for k in range(lo, hi):
                pl.when(i == k)(cps[k].start)
            return carry
        jax.lax.fori_loop(lo, hi, body, 0)

    def issue_w(t, carry):
        wchunk(0, t).start()
        wchunk(1, t).start()
        return carry

    issue(0, len(cps) - 2)
    jax.lax.fori_loop(0, H, issue_w, 0)
    issue(len(cps) - 2, len(cps))

    def zero(i, carry):
        ot[pl.ds(pl.multiple_of(DM + i * 64, 64), 64), :] = jnp.zeros((64, S), f32)
        return carry

    jax.lax.fori_loop(0, DM // 64, zero, 0)

    NPREP = 7

    def x_prep(k):
        n = 256
        for k0 in range(k * n, S if k == NPREP - 1 else (k + 1) * n, n):
            wall[PX, k0:k0 + n, :] = bxt[0:D, k0:k0 + n].T
            wall[PX + 1, k0:k0 + n, 0:DM - D] = bxt[D:DM, k0:k0 + n].T

    def wq_prep(k):
        n = DM // NPREP
        wall[0:H, k * n:(k + 1) * n, :] = jnp.swapaxes(wq_raw[k * n:(k + 1) * n], 0, 1)

    def part_a(x1a, x1b, rma, rmb, wsa, wsb, csa, csb):
        def stage1(x1, lo, hi, wait):
            for c in range(4):
                if wait:
                    c_axt[c].wait()
                x1[:, c * XC:(c + 1) * XC] = _dot(fd[lo:hi, :], axt[:, c * XC:(c + 1) * XC], NN)

        def fwd16(x1, rm, n, unroll):
            def group(r0):
                zs = [(x1[pl.ds(r0, 8), c * LN:(c + 1) * LN], x1[pl.ds(n + r0, 8), c * LN:(c + 1) * LN])
                      for c in range(R16)]
                ys = _fft(zs, -1)
                for r in range(R16):
                    re, im = ys[r]
                    if r:
                        tr, ti = tw[0, r], tw[1, r]
                        re, im = re * tr - im * ti, re * ti + im * tr
                    rm[r, pl.ds(r0, 8), 0:LN] = re
                    rm[r, pl.ds(r0, 8), LN:2 * LN] = im

            if unroll:
                for r0 in range(0, n, 8):
                    group(r0)
            else:
                def body(g, carry):
                    group(pl.multiple_of(g * 8, 8))
                    return carry
                jax.lax.fori_loop(0, n // 8, body, 0)
            if n < LN:
                rm[:, n:LN, :] = jnp.zeros((R16, LN - n, 2 * LN), f32)

        def wprep(ws, lo, hi):
            for p, wt in enumerate((wrt, wit)):
                for c in range(R16):
                    t = wt[lo:hi, c * LN:(c + 1) * LN].astype(f32).T
                    if hi - lo < LN:
                        t = jnp.concatenate([t, jnp.zeros((LN, LN - (hi - lo)), f32)], axis=1)
                    ws[p, c * LN:(c + 1) * LN, :] = t

        def stage23(rm, ws, cs):
            x = _dot(l2[...], rm[...].reshape(R16 * LN, 2 * LN).astype(bf16), NT)
            for r in range(R16):
                xr, xi = x[0:LN, r * LN:(r + 1) * LN], x[LN:2 * LN, r * LN:(r + 1) * LN]
                wr = ws[0, pl.ds(r, LN, stride=R16), :]
                wi = ws[1, pl.ds(r, LN, stride=R16), :]
                g = jnp.concatenate([xr * wr - xi * wi, xr * wi + xi * wr], axis=0).astype(bf16)
                cs[r] = _dot(l3[r], g, NN)

        def inv16(cs, half):
            for r0 in range(0, LN, 8):
                zs = [(cs[r, r0:r0 + 8, :], cs[r, LN + r0:LN + r0 + 8, :]) for r in range(R16)]
                ys = _fft(zs, +1)
                for c in range(R16):
                    wall[PU + half, c * LN + r0:c * LN + r0 + 8, 0:LN] = ys[c][0].astype(bf16)
                    wall[PU + half, c * LN + r0:c * LN + r0 + 8, LN:2 * LN] = ys[c][1].astype(bf16)

        def stage4(half):
            n = S // 4
            for k in range(4):
                y = _dot(l4[half * DM:(half + 1) * DM, :], wall[PU + half, k * n:(k + 1) * n, :], NT)
                if half:
                    ot[0:DM, k * n:(k + 1) * n] += y
                else:
                    ot[0:DM, k * n:(k + 1) * n] = y

        with scope('w0'):
            c_fda.wait()
        stage1(x1a, 0, 2 * LN, True)
        c_fdb.wait()
        c_tw.wait()
        stage1(x1b, 2 * LN, 2 * LN + 2 * JB, False)
        fwd16(x1a, rma, LN, False)
        c_l2.wait()
        c_wrt.wait()
        c_wit.wait()
        wprep(wsa, 0, LN)
        c_l3.wait()
        stage23(rma, wsa, csa)
        fwd16(x1b, rmb, JB, True)
        wprep(wsb, LN, J)
        stage23(rmb, wsb, csb)
        inv16(csa, 0)
        c_bxt.wait()
        c_l4.wait()
        c_wq.wait()
        stage4(0)
        inv16(csb, 1)
        if do_b:
            for k in range(NPREP):
                x_prep(k)
                wq_prep(k)
        stage4(1)

    if do_a:
        pl.run_scoped(part_a,
                      pltpu.VMEM((2 * LN, S), f32), pltpu.VMEM((2 * JB, S), f32),
                      pltpu.VMEM((R16, LN, 2 * LN), f32), pltpu.VMEM((R16, LN, 2 * LN), f32),
                      pltpu.VMEM((2, S, LN), f32), pltpu.VMEM((2, S, LN), f32),
                      pltpu.VMEM((R16, 2 * LN, LN), f32), pltpu.VMEM((R16, 2 * LN, LN), f32))
    else:
        for c in cps[:-2]:
            c.wait()
        ot[0:DM, :] = jnp.zeros((DM, S), f32)
        if do_b:
            for k in range(NPREP):
                x_prep(k)
                wq_prep(k)

    qscale = (D ** -0.5) * math.log2(math.e)

    wchunk(0, 0).wait()
    wchunk(1, 0).wait()

    def qstep(t, carry):
        if do_b:
            rq, rw = S // QPIECES, 2 * CCH // QPIECES
            for j in range(QPIECES):
                which, off = divmod(j * rw, CCH)
                r0 = pl.multiple_of(t * CCH + off, rw)
                src = (wuk_raw, wuv_raw)[which]
                wall[0:H, pl.ds(DM + which * DC + r0, rw), :] = jnp.swapaxes(src[pl.ds(r0, rw)], 0, 1)
                x = jnp.concatenate([wall[PX, j * rq:(j + 1) * rq, :], wall[PX + 1, j * rq:(j + 1) * rq, 0:DM - D]], axis=1)
                q_all[t, j * rq:(j + 1) * rq] = (_dot(x, wall[t, 0:DM, :], NN) * qscale).astype(bf16)

        @pl.when(t + 1 < H)
        def _():
            wchunk(0, t + 1).wait()
            wchunk(1, t + 1).wait()

        return carry

    with scope('P2'):
        jax.lax.fori_loop(0, H, qstep, 0)
    c_ckv.wait()
    c_wot.wait()

    def head(h, carry):
        with scope('head'):
            return head_body(h, carry)

    def head_body(h, carry):
        wkv = jnp.concatenate([wall[h, DM:DM + DC, :], wall[h, DM + DC:DM + 2 * DC, :]], axis=1)
        kv = _dot(ckv[...], wkv, NN).astype(bf16)
        k = kv[:, 0:D]
        v = kv[:, D:2 * D]
        wo = wot[h]
        rr = jax.lax.broadcasted_iota(jnp.int32, (LN, LN), 0)
        cc = jax.lax.broadcasted_iota(jnp.int32, (LN, LN), 1)
        tri = cc <= rr
        neg = -1e30
        ctxs = []
        for i in reversed(range(S // TQ)):
            r0 = i * TQ
            lm = r0 + LN
            q = q_all[h, r0:r0 + TQ, :]
            s = _dot(q, k[0:lm], NT)
            sx = jnp.where(tri, _dot(q[LN:], k[lm:lm + LN], NT), neg)
            sd = jnp.where(tri, s[0:LN, r0:lm], neg)
            pt, lt = _softmax_rows(([s[0:LN, 0:r0]] if i else []) + [sd])
            pb, lb = _softmax_rows([s[LN:], sx])
            pt = jnp.concatenate(pt, axis=1) if i else pt[0]
            ctx = _dot(jnp.concatenate([pt, pb[0]], axis=0), v[0:lm], NN)
            cx = _dot(pb[1], v[lm:lm + LN], NN)
            ctxs.append(jnp.concatenate([ctx[0:LN] * (1.0 / lt), (ctx[LN:] + cx) * (1.0 / lb)],
                                        axis=0).astype(bf16))
        res = _dot(wo, jnp.concatenate(ctxs, axis=0), NT)
        nb = S // TQ
        for n in range(nb):
            ot[DM:2 * DM, (nb - 1 - n) * TQ:(nb - n) * TQ] += res[:, n * TQ:(n + 1) * TQ]
        return carry

    if do_b:
        with scope('P3'):
            jax.lax.fori_loop(0, H, head, 0)

    def ocopy(c):
        rows = pl.ds(pl.multiple_of(c * OCH, OCH), OCH)
        return pltpu.make_async_copy(obuf.at[rows], out_hbm.at[rows], osem.at[c])

    def ostep(c, carry):
        cols = pl.ds(pl.multiple_of(c * OCH, OCH), OCH)
        obuf[cols, :] = ot[:, cols].astype(bf16).T
        ocopy(c).start()
        return carry

    jax.lax.fori_loop(0, S // OCH, ostep, 0)
    for c in range(S // OCH):
        ocopy(c).wait()


def _build(do_a=True, do_b=True, scopes=False):
    def run(A_x, A_w_r, A_w_i, B_x, B_c_kv, B_w_q, B_w_uk, B_w_uv, B_w_o):
        axt = jnp.swapaxes(A_x, 1, 2).reshape(DM, S)
        bxt = jnp.swapaxes(B_x, 1, 2).reshape(DM, S)
        wrt = A_w_r.T
        wit = A_w_i.T
        ckv = B_c_kv.reshape(S, DC)
        wot = jnp.swapaxes(B_w_o, 1, 2)
        tabs = [jnp.asarray(t) for t in _tables()]
        args = (axt, wrt, wit, bxt, ckv, B_w_q, B_w_uk, B_w_uv, wot, *tabs)
        vm = pltpu.VMEM
        scratch = [
            vm((DM, S), bf16), vm((J, S), bf16), vm((J, S), bf16),
            vm(tabs[0].shape, bf16), vm(tabs[1].shape, bf16), vm(tabs[2].shape, f32),
            vm(tabs[3].shape, bf16), vm(tabs[4].shape, bf16),
            vm((DM, S), bf16), vm((S, DC), bf16),
            vm((DM, H, D), bf16),
            vm((DC, H, D), bf16), vm((DC, H, D), bf16), vm((H + 4, DM + 2 * DC, D), bf16),
            vm((H, DM, D), bf16), vm((H, S, D), bf16),
            vm((2 * DM, S), f32), vm((S, 2 * DM), bf16),
            pltpu.SemaphoreType.DMA((16,)), pltpu.SemaphoreType.DMA((2, H)),
            pltpu.SemaphoreType.DMA((S // OCH,)),
        ]
        out = pl.pallas_call(
            functools.partial(_kernel, do_a=do_a, do_b=do_b, scopes=scopes),
            in_specs=[pl.BlockSpec(memory_space=pl.ANY)] * len(args),
            out_specs=pl.BlockSpec(memory_space=pl.ANY),
            out_shape=jax.ShapeDtypeStruct((S, 2 * DM), bf16),
            scratch_shapes=scratch,
            compiler_params=pltpu.CompilerParams(vmem_limit_bytes=120 * 2**20),
        )(*args)
        return out.reshape(1, S, 2 * DM)

    return run


_run = _build()


@jax.jit
def pallas_concat_heads__spectral_gfnet__compressed_kv_cla__prompt_kernel(
    A_x: jax.Array,
    A_w_r: jax.Array,
    A_w_i: jax.Array,
    B_x: jax.Array,
    B_c_kv: jax.Array,
    B_w_q: jax.Array,
    B_w_uk: jax.Array,
    B_w_uv: jax.Array,
    B_w_o: jax.Array,
):
    return _run(A_x, A_w_r, A_w_i, B_x, B_c_kv, B_w_q, B_w_uk, B_w_uv, B_w_o)
```

```python
import contextlib
import functools
import math

import jax
import jax.numpy as jnp
import numpy as np
import jax.experimental.pallas as pl
import jax.experimental.pallas.tpu as pltpu

f32 = jnp.float32
bf16 = jnp.bfloat16

NN = (((1,), (0,)), ((), ()))
NT = (((1,), (1,)), ((), ()))

S = 2048
DM = 448
J = DM // 2 + 1
JB = 104
H = 16
D = 256
DC = 1024
R16 = 16
LN = 128
TQ = 256
CCH = DC // H
PX = H
PU = H + 2
NP4 = 16
OCH = 128
QPIECES = 16


def _dot(a, b, dn):
    return jax.lax.dot_general(a, b, dn, preferred_element_type=f32)


@functools.lru_cache(maxsize=None)
def _tables():
    j = np.arange(J)[:, None].astype(np.float64)
    d = np.arange(DM)[None, :].astype(np.float64)
    ang = 2.0 * np.pi * ((j * d) % DM) / DM
    cos, sin = np.cos(ang), np.sin(ang)
    fd = np.zeros((2 * LN + 2 * JB, DM), np.float64)
    fd[0:LN] = cos[0:LN]
    fd[LN:2 * LN] = -sin[0:LN]
    fd[2 * LN:2 * LN + J - LN] = cos[LN:]
    fd[2 * LN + JB:2 * LN + JB + J - LN] = -sin[LN:]

    m = np.arange(LN)[:, None].astype(np.float64)
    l = np.arange(LN)[None, :].astype(np.float64)
    a128 = 2.0 * np.pi * ((m * l) % LN) / LN
    fr, fi = np.cos(a128), -np.sin(a128)
    l2 = np.block([[fr, -fi], [fi, fr]])

    r = np.arange(R16)[:, None].astype(np.float64)
    at = 2.0 * np.pi * (r * l) / S
    tw = np.stack([np.cos(at), -np.sin(at)])
    tw = np.broadcast_to(tw[:, :, None, :], (2, R16, 8, LN)).copy()

    l3 = np.zeros((R16, 2 * LN, 2 * LN), np.float64)
    for rr in range(R16):
        a3 = 2.0 * np.pi * ((m * (rr + R16 * l)) % S) / S
        nr, ni = np.cos(a3), np.sin(a3)
        l3[rr] = np.block([[nr, -ni], [ni, nr]])

    cj = np.full((J,), 2.0)
    cj[0] = 1.0
    cj[J - 1] = 1.0
    scale = cj[None, :] / float(S * DM)
    cr, ci = cos.T * scale, -sin.T * scale
    l4 = np.zeros((2, DM, 2 * LN), np.float64)
    l4[0, :, 0:LN] = cr[:, 0:LN]
    l4[0, :, LN:] = ci[:, 0:LN]
    l4[1, :, 0:J - LN] = cr[:, LN:]
    l4[1, :, LN:LN + J - LN] = ci[:, LN:]

    cast = lambda a, dt: np.asarray(a, np.float32).astype(dt)
    return (cast(fd, bf16), cast(l2, bf16), cast(tw, np.float32), cast(l3, bf16),
            cast(l4.reshape(2 * DM, 2 * LN), bf16))


def _cmul_const(z, k, n, sign):
    re, im = z
    k = k % n
    if k == 0:
        return re, im
    if 4 * k == n:
        return (-im, re) if sign > 0 else (im, -re)
    if 8 * k == n:
        c = math.sqrt(0.5)
        return ((re - im) * c, (re + im) * c) if sign > 0 else ((re + im) * c, (im - re) * c)
    if 8 * k == 3 * n:
        c = math.sqrt(0.5)
        return ((re + im) * (-c), (re - im) * c) if sign > 0 else ((im - re) * c, (re + im) * (-c))
    c = math.cos(2.0 * math.pi * k / n)
    s = sign * math.sin(2.0 * math.pi * k / n)
    return re * c - im * s, re * s + im * c


def _fft(zs, sign):
    n = len(zs)
    if n == 1:
        return zs
    ev = _fft(zs[0::2], sign)
    od = _fft(zs[1::2], sign)
    out = [None] * n
    for k in range(n // 2):
        if 4 * k == n:
            (er, ei), (orr, oi) = ev[k], od[k]
            if sign > 0:
                out[k] = (er - oi, ei + orr)
                out[k + n // 2] = (er + oi, ei - orr)
            else:
                out[k] = (er + oi, ei - orr)
                out[k + n // 2] = (er - oi, ei + orr)
            continue
        tr, ti = _cmul_const(od[k], k, n, sign)
        er, ei = ev[k]
        out[k] = (er + tr, ei + ti)
        out[k + n // 2] = (er - tr, ei - ti)
    return out


def _softmax_rows(segs):
    m = functools.reduce(jnp.maximum, [jnp.max(sg, axis=1, keepdims=True) for sg in segs])
    es = [jnp.exp2(sg - m) for sg in segs]
    l = functools.reduce(jnp.add, [jnp.sum(e, axis=1, keepdims=True) for e in es])
    return [e.astype(bf16) for e in es], l


def _kernel(axt_hbm, wrt_hbm, wit_hbm, bxt_hbm, ckv_hbm, wq_hbm, wuk_hbm, wuv_hbm, wot_hbm,
            fd_hbm, l2_hbm, tw_hbm, l3_hbm, l4_hbm,
            out_hbm,
            axt, wrt, wit, fd, l2, tw, l3, l4,
            bxt, ckv, wq_raw, wuk_raw, wuv_raw, wall, wot, q_all,
            ot, obuf, sem, wsem, osem, *, do_a, do_b, scopes):
    scope = jax.named_scope if scopes else (lambda name: contextlib.nullcontext())
    XC = S // 4
    simple = ([(fd_hbm.at[0:2 * LN], fd.at[0:2 * LN])]
              + [(axt_hbm.at[:, c * XC:(c + 1) * XC], axt.at[:, c * XC:(c + 1) * XC]) for c in range(4)]
              + [(fd_hbm.at[2 * LN:], fd.at[2 * LN:]), (tw_hbm, tw), (l2_hbm, l2), (wrt_hbm, wrt), (wit_hbm, wit),
                 (l3_hbm, l3), (bxt_hbm, bxt), (l4_hbm, l4), (wq_hbm, wq_raw), (ckv_hbm, ckv), (wot_hbm, wot)])
    cps = [pltpu.make_async_copy(s, d, sem.at[i]) for i, (s, d) in enumerate(simple)]
    c_fda, c_axt = cps[0], cps[1:5]
    (c_fdb, c_tw, c_l2, c_wrt, c_wit, c_l3, c_bxt, c_l4, c_wq, c_ckv, c_wot) = cps[5:]

    def wchunk(which, t):
        src, dst = ((wuk_hbm, wuk_raw), (wuv_hbm, wuv_raw))[which]
        return pltpu.make_async_copy(src.at[pl.ds(t * CCH, CCH)], dst.at[pl.ds(t * CCH, CCH)], wsem.at[which, t])

    def issue(lo, hi):
        def body(i, carry):
            for k in range(lo, hi):
                pl.when(i == k)(cps[k].start)
            return carry
        jax.lax.fori_loop(lo, hi, body, 0)

    def wait_all(cs):
        def body(i, carry):
            for k, c in enumerate(cs):
                pl.when(i == k)(c.wait)
            return carry
        jax.lax.fori_loop(0, len(cs), body, 0)

    def issue_w(t, carry):
        wchunk(0, t).start()
        wchunk(1, t).start()
        return carry

    issue(0, len(cps) - 2)
    jax.lax.fori_loop(0, H, issue_w, 0)
    issue(len(cps) - 2, len(cps))

    def zero(i, carry):
        ot[pl.ds(pl.multiple_of(DM + i * 64, 64), 64), :] = jnp.zeros((64, S), f32)
        return carry

    jax.lax.fori_loop(0, DM // 64, zero, 0)

    def x_prep(k, n):
        w = S // n
        wall[PX, k * w:(k + 1) * w, :] = bxt[0:D, k * w:(k + 1) * w].T
        wall[PX + 1, k * w:(k + 1) * w, 0:DM - D] = bxt[D:DM, k * w:(k + 1) * w].T

    def wq_prep(k, n):
        g = DM // 16
        lo, hi = 16 * (k * g // n), 16 * ((k + 1) * g // n)
        wall[0:H, lo:hi, :] = jnp.swapaxes(wq_raw[lo:hi], 0, 1)

    def part_a(x1a, x1b, rma, rmb, wsa, wsb, csa, csb):
        def stage1(x1, lo, hi, wait):
            def body(c, carry):
                cols = pl.ds(pl.multiple_of(c * XC, XC), XC)
                if wait:
                    pltpu.make_async_copy(axt_hbm.at[:, cols], axt.at[:, cols], sem.at[1 + c]).wait()
                x1[:, cols] = _dot(fd[lo:hi, :], axt[:, cols], NN)
                return carry
            if wait:
                jax.lax.fori_loop(0, 4, body, 0)
            else:
                for c in range(4):
                    x1[:, c * XC:(c + 1) * XC] = _dot(fd[lo:hi, :], axt[:, c * XC:(c + 1) * XC], NN)

        def fwd16(x1, rm, n, unroll):
            def group(r0):
                zs = [(x1[pl.ds(r0, 8), c * LN:(c + 1) * LN], x1[pl.ds(n + r0, 8), c * LN:(c + 1) * LN])
                      for c in range(R16)]
                ys = _fft(zs, -1)
                for r in range(R16):
                    re, im = ys[r]
                    if r:
                        tr, ti = tw[0, r], tw[1, r]
                        re, im = re * tr - im * ti, re * ti + im * tr
                    rm[r, pl.ds(r0, 8), 0:LN] = re
                    rm[r, pl.ds(r0, 8), LN:2 * LN] = im

            if unroll:
                for r0 in range(0, n, 8):
                    group(r0)
            else:
                def body(g, carry):
                    group(pl.multiple_of(g * 8, 8))
                    return carry
                jax.lax.fori_loop(0, n // 8, body, 0)
            if n < LN:
                rm[:, n:LN, :] = jnp.zeros((R16, LN - n, 2 * LN), f32)

        def wprep(ws, lo, hi):
            for p, wt in enumerate((wrt, wit)):
                for c in range(R16):
                    t = wt[lo:hi, c * LN:(c + 1) * LN].astype(f32).T
                    if hi - lo < LN:
                        t = jnp.concatenate([t, jnp.zeros((LN, LN - (hi - lo)), f32)], axis=1)
                    ws[p, c * LN:(c + 1) * LN, :] = t

        def stage23(rm, ws, cs):
            x = _dot(l2[...], rm[...].reshape(R16 * LN, 2 * LN).astype(bf16), NT)
            for r in range(R16):
                xr, xi = x[0:LN, r * LN:(r + 1) * LN], x[LN:2 * LN, r * LN:(r + 1) * LN]
                wr = ws[0, pl.ds(r, LN, stride=R16), :]
                wi = ws[1, pl.ds(r, LN, stride=R16), :]
                g = jnp.concatenate([xr * wr - xi * wi, xr * wi + xi * wr], axis=0).astype(bf16)
                cs[r] = _dot(l3[r], g, NN)

        def inv16(cs, half):
            for r0 in range(0, LN, 8):
                zs = [(cs[r, r0:r0 + 8, :], cs[r, LN + r0:LN + r0 + 8, :]) for r in range(R16)]
                ys = _fft(zs, +1)
                for c in range(R16):
                    wall[PU + half, c * LN + r0:c * LN + r0 + 8, 0:LN] = ys[c][0].astype(bf16)
                    wall[PU + half, c * LN + r0:c * LN + r0 + 8, LN:2 * LN] = ys[c][1].astype(bf16)

        def stage4(half, prep):
            n = S // NP4
            for k in range(NP4):
                if do_b:
                    prep(k, NP4)
                y = _dot(l4[half * DM:(half + 1) * DM, :], wall[PU + half, k * n:(k + 1) * n, :], NT)
                if half:
                    ot[0:DM, k * n:(k + 1) * n] += y
                else:
                    ot[0:DM, k * n:(k + 1) * n] = y

        with scope('w0'):
            c_fda.wait()
        stage1(x1a, 0, 2 * LN, True)
        wait_all([c_fdb, c_tw])
        stage1(x1b, 2 * LN, 2 * LN + 2 * JB, False)
        fwd16(x1a, rma, LN, False)
        wait_all([c_l2, c_wrt, c_wit, c_l3])
        wprep(wsa, 0, LN)
        stage23(rma, wsa, csa)
        fwd16(x1b, rmb, JB, True)
        wprep(wsb, LN, J)
        stage23(rmb, wsb, csb)
        inv16(csa, 0)
        wait_all([c_bxt, c_l4, c_wq])
        stage4(0, x_prep)
        inv16(csb, 1)
        stage4(1, wq_prep)

    if do_a:
        pl.run_scoped(part_a,
                      pltpu.VMEM((2 * LN, S), f32), pltpu.VMEM((2 * JB, S), f32),
                      pltpu.VMEM((R16, LN, 2 * LN), f32), pltpu.VMEM((R16, LN, 2 * LN), f32),
                      pltpu.VMEM((2, S, LN), f32), pltpu.VMEM((2, S, LN), f32),
                      pltpu.VMEM((R16, 2 * LN, LN), f32), pltpu.VMEM((R16, 2 * LN, LN), f32))
    else:
        for c in cps[:-2]:
            c.wait()
        ot[0:DM, :] = jnp.zeros((DM, S), f32)
        if do_b:
            for k in range(NP4):
                x_prep(k, NP4)
                wq_prep(k, NP4)

    qscale = (D ** -0.5) * math.log2(math.e)

    wchunk(0, 0).wait()
    wchunk(1, 0).wait()

    def qstep(t, carry):
        if do_b:
            rq, rw = S // QPIECES, 2 * CCH // QPIECES
            for j in range(QPIECES):
                which, off = divmod(j * rw, CCH)
                r0 = pl.multiple_of(t * CCH + off, rw)
                src = (wuk_raw, wuv_raw)[which]
                wall[0:H, pl.ds(DM + which * DC + r0, rw), :] = jnp.swapaxes(src[pl.ds(r0, rw)], 0, 1)
                x = jnp.concatenate([wall[PX, j * rq:(j + 1) * rq, :], wall[PX + 1, j * rq:(j + 1) * rq, 0:DM - D]], axis=1)
                q_all[t, j * rq:(j + 1) * rq] = (_dot(x, wall[t, 0:DM, :], NN) * qscale).astype(bf16)

        @pl.when(t + 1 < H)
        def _():
            wchunk(0, t + 1).wait()
            wchunk(1, t + 1).wait()

        return carry

    with scope('P2'):
        jax.lax.fori_loop(0, H, qstep, 0)
    c_ckv.wait()
    c_wot.wait()

    def head(h, carry):
        with scope('head'):
            return head_body(h, carry)

    def head_body(h, carry):
        wkv = jnp.concatenate([wall[h, DM:DM + DC, :], wall[h, DM + DC:DM + 2 * DC, :]], axis=1)
        kv = _dot(ckv[...], wkv, NN).astype(bf16)
        k = kv[:, 0:D]
        v = kv[:, D:2 * D]
        wo = wot[h]
        rr = jax.lax.broadcasted_iota(jnp.int32, (LN, LN), 0)
        cc = jax.lax.broadcasted_iota(jnp.int32, (LN, LN), 1)
        tri = cc <= rr
        neg = -1e30
        ctxs = []
        for i in reversed(range(S // TQ)):
            r0 = i * TQ
            lm = r0 + LN
            q = q_all[h, r0:r0 + TQ, :]
            s = _dot(q, k[0:lm], NT)
            sx = jnp.where(tri, _dot(q[LN:], k[lm:lm + LN], NT), neg)
            sd = jnp.where(tri, s[0:LN, r0:lm], neg)
            pt, lt = _softmax_rows(([s[0:LN, 0:r0]] if i else []) + [sd])
            pb, lb = _softmax_rows([s[LN:], sx])
            pt = jnp.concatenate(pt, axis=1) if i else pt[0]
            ctx = _dot(jnp.concatenate([pt, pb[0]], axis=0), v[0:lm], NN)
            cx = _dot(pb[1], v[lm:lm + LN], NN)
            ctxs.append(jnp.concatenate([ctx[0:LN] * (1.0 / lt), (ctx[LN:] + cx) * (1.0 / lb)],
                                        axis=0).astype(bf16))
        res = _dot(wo, jnp.concatenate(ctxs, axis=0), NT)
        nb = S // TQ
        for n in range(nb):
            ot[DM:2 * DM, (nb - 1 - n) * TQ:(nb - n) * TQ] += res[:, n * TQ:(n + 1) * TQ]
        return carry

    if do_b:
        with scope('P3'):
            jax.lax.fori_loop(0, H, head, 0)

    def ocopy(c):
        rows = pl.ds(pl.multiple_of(c * OCH, OCH), OCH)
        return pltpu.make_async_copy(obuf.at[rows], out_hbm.at[rows], osem.at[c])

    def ostep(c, carry):
        cols = pl.ds(pl.multiple_of(c * OCH, OCH), OCH)
        obuf[cols, :] = ot[:, cols].astype(bf16).T
        ocopy(c).start()
        return carry

    jax.lax.fori_loop(0, S // OCH, ostep, 0)
    for c in range(S // OCH):
        ocopy(c).wait()


def _build(do_a=True, do_b=True, scopes=False):
    def run(A_x, A_w_r, A_w_i, B_x, B_c_kv, B_w_q, B_w_uk, B_w_uv, B_w_o):
        axt = jnp.swapaxes(A_x, 1, 2).reshape(DM, S)
        bxt = jnp.swapaxes(B_x, 1, 2).reshape(DM, S)
        wrt = A_w_r.T
        wit = A_w_i.T
        ckv = B_c_kv.reshape(S, DC)
        wot = jnp.swapaxes(B_w_o, 1, 2)
        tabs = [jnp.asarray(t) for t in _tables()]
        args = (axt, wrt, wit, bxt, ckv, B_w_q, B_w_uk, B_w_uv, wot, *tabs)
        vm = pltpu.VMEM
        scratch = [
            vm((DM, S), bf16), vm((J, S), bf16), vm((J, S), bf16),
            vm(tabs[0].shape, bf16), vm(tabs[1].shape, bf16), vm(tabs[2].shape, f32),
            vm(tabs[3].shape, bf16), vm(tabs[4].shape, bf16),
            vm((DM, S), bf16), vm((S, DC), bf16),
            vm((DM, H, D), bf16),
            vm((DC, H, D), bf16), vm((DC, H, D), bf16), vm((H + 4, DM + 2 * DC, D), bf16),
            vm((H, DM, D), bf16), vm((H, S, D), bf16),
            vm((2 * DM, S), f32), vm((S, 2 * DM), bf16),
            pltpu.SemaphoreType.DMA((16,)), pltpu.SemaphoreType.DMA((2, H)),
            pltpu.SemaphoreType.DMA((S // OCH,)),
        ]
        out = pl.pallas_call(
            functools.partial(_kernel, do_a=do_a, do_b=do_b, scopes=scopes),
            in_specs=[pl.BlockSpec(memory_space=pl.ANY)] * len(args),
            out_specs=pl.BlockSpec(memory_space=pl.ANY),
            out_shape=jax.ShapeDtypeStruct((S, 2 * DM), bf16),
            scratch_shapes=scratch,
            compiler_params=pltpu.CompilerParams(vmem_limit_bytes=120 * 2**20),
        )(*args)
        return out.reshape(1, S, 2 * DM)

    return run


_run = _build()


@jax.jit
def pallas_concat_heads__spectral_gfnet__compressed_kv_cla__prompt_kernel(
    A_x: jax.Array,
    A_w_r: jax.Array,
    A_w_i: jax.Array,
    B_x: jax.Array,
    B_c_kv: jax.Array,
    B_w_q: jax.Array,
    B_w_uk: jax.Array,
    B_w_uv: jax.Array,
    B_w_o: jax.Array,
):
    return _run(A_x, A_w_r, A_w_i, B_x, B_c_kv, B_w_q, B_w_uk, B_w_uv, B_w_o)
```

```python
import contextlib
import functools
import math

import jax
import jax.numpy as jnp
import numpy as np
import jax.experimental.pallas as pl
import jax.experimental.pallas.tpu as pltpu

f32 = jnp.float32
bf16 = jnp.bfloat16

NN = (((1,), (0,)), ((), ()))
NT = (((1,), (1,)), ((), ()))

S = 2048
DM = 448
J = DM // 2 + 1
JB = 104
H = 16
D = 256
DC = 1024
R16 = 16
LN = 128
TQ = 256
CCH = DC // H
PX = H
PU = H + 2
YC = 384
NP4 = 16
OCH = 512
QPIECES = 16


def _dot(a, b, dn):
    return jax.lax.dot_general(a, b, dn, preferred_element_type=f32)


@functools.lru_cache(maxsize=None)
def _tables():
    j = np.arange(J)[:, None].astype(np.float64)
    d = np.arange(DM)[None, :].astype(np.float64)
    ang = 2.0 * np.pi * ((j * d) % DM) / DM
    cos, sin = np.cos(ang), np.sin(ang)
    fd = np.zeros((2 * LN + 2 * JB, DM), np.float64)
    fd[0:LN] = cos[0:LN]
    fd[LN:2 * LN] = -sin[0:LN]
    fd[2 * LN:2 * LN + J - LN] = cos[LN:]
    fd[2 * LN + JB:2 * LN + JB + J - LN] = -sin[LN:]

    m = np.arange(LN)[:, None].astype(np.float64)
    l = np.arange(LN)[None, :].astype(np.float64)
    a128 = 2.0 * np.pi * ((m * l) % LN) / LN
    fr, fi = np.cos(a128), -np.sin(a128)
    l2 = np.block([[fr, -fi], [fi, fr]])

    r = np.arange(R16)[:, None].astype(np.float64)
    at = 2.0 * np.pi * (r * l) / S
    tw = np.stack([np.cos(at), -np.sin(at)])
    tw = np.broadcast_to(tw[:, :, None, :], (2, R16, 8, LN)).copy()

    l3 = np.zeros((R16, 2 * LN, LN), np.float64)
    for rr in range(R16):
        a3 = 2.0 * np.pi * ((m * (rr + R16 * l)) % S) / S
        l3[rr] = np.concatenate([np.cos(a3), np.sin(a3)], axis=0)

    cj = np.full((J,), 2.0)
    cj[0] = 1.0
    cj[J - 1] = 1.0
    scale = cj[None, :] / float(S * DM)
    cr, ci = cos.T * scale, -sin.T * scale
    l4 = np.zeros((2, DM, 2 * LN), np.float64)
    l4[0, :, 0:LN] = cr[:, 0:LN]
    l4[0, :, LN:] = ci[:, 0:LN]
    l4[1, :, 0:J - LN] = cr[:, LN:]
    l4[1, :, LN:LN + J - LN] = ci[:, LN:]

    cast = lambda a, dt: np.asarray(a, np.float32).astype(dt)
    return (cast(fd, bf16), cast(l2, bf16), cast(tw, np.float32), cast(l3, bf16),
            cast(l4.reshape(2 * DM, 2 * LN), bf16))


def _cmul_const(z, k, n, sign):
    re, im = z
    k = k % n
    if k == 0:
        return re, im
    if 4 * k == n:
        return (-im, re) if sign > 0 else (im, -re)
    if 8 * k == n:
        c = math.sqrt(0.5)
        return ((re - im) * c, (re + im) * c) if sign > 0 else ((re + im) * c, (im - re) * c)
    if 8 * k == 3 * n:
        c = math.sqrt(0.5)
        return ((re + im) * (-c), (re - im) * c) if sign > 0 else ((im - re) * c, (re + im) * (-c))
    c = math.cos(2.0 * math.pi * k / n)
    s = sign * math.sin(2.0 * math.pi * k / n)
    return re * c - im * s, re * s + im * c


def _fft(zs, sign):
    n = len(zs)
    if n == 1:
        return zs
    ev = _fft(zs[0::2], sign)
    od = _fft(zs[1::2], sign)
    out = [None] * n
    for k in range(n // 2):
        if 4 * k == n:
            (er, ei), (orr, oi) = ev[k], od[k]
            if sign > 0:
                out[k] = (er - oi, ei + orr)
                out[k + n // 2] = (er + oi, ei - orr)
            else:
                out[k] = (er + oi, ei - orr)
                out[k + n // 2] = (er - oi, ei + orr)
            continue
        tr, ti = _cmul_const(od[k], k, n, sign)
        er, ei = ev[k]
        out[k] = (er + tr, ei + ti)
        out[k + n // 2] = (er - tr, ei - ti)
    return out


def _softmax_rows(segs):
    m = functools.reduce(jnp.maximum, [jnp.max(sg, axis=1, keepdims=True) for sg in segs])
    es = [jnp.exp2(sg - m) for sg in segs]
    l = functools.reduce(jnp.add, [jnp.sum(e, axis=1, keepdims=True) for e in es])
    return [e.astype(bf16) for e in es], l


def _kernel(axt_hbm, wrt_hbm, wit_hbm, bxt_hbm, ckv_hbm, wq_hbm, wuk_hbm, wuv_hbm, wot_hbm,
            fd_hbm, l2_hbm, tw_hbm, l3_hbm, l4_hbm,
            out_hbm,
            axt, wrt, wit, fd, l2, tw, l3, l4,
            bxt, ckv, wq_raw, wuk_raw, wuv_raw, wall, wot, q_all,
            ot, ybuf, obuf, sem, wsem, osem, ysem, *, do_a, do_b, scopes):
    scope = jax.named_scope if scopes else (lambda name: contextlib.nullcontext())
    XC = S // 4
    simple = ([(fd_hbm.at[0:2 * LN], fd.at[0:2 * LN])]
              + [(axt_hbm.at[:, c * XC:(c + 1) * XC], axt.at[:, c * XC:(c + 1) * XC]) for c in range(4)]
              + [(fd_hbm.at[2 * LN:], fd.at[2 * LN:]), (tw_hbm, tw), (l2_hbm, l2), (wrt_hbm, wrt), (wit_hbm, wit),
                 (l3_hbm, l3), (bxt_hbm, bxt), (l4_hbm, l4), (wq_hbm, wq_raw), (ckv_hbm, ckv), (wot_hbm, wot)])
    cps = [pltpu.make_async_copy(s, d, sem.at[i]) for i, (s, d) in enumerate(simple)]
    c_fda, c_axt = cps[0], cps[1:5]
    (c_fdb, c_tw, c_l2, c_wrt, c_wit, c_l3, c_bxt, c_l4, c_wq, c_ckv, c_wot) = cps[5:]

    def wchunk(which, t):
        src, dst = ((wuk_hbm, wuk_raw), (wuv_hbm, wuv_raw))[which]
        return pltpu.make_async_copy(src.at[pl.ds(t * CCH, CCH)], dst.at[pl.ds(t * CCH, CCH)], wsem.at[which, t])

    def issue(lo, hi):
        def body(i, carry):
            for k in range(lo, hi):
                pl.when(i == k)(cps[k].start)
            return carry
        jax.lax.fori_loop(lo, hi, body, 0)

    def wait_all(cs):
        def body(i, carry):
            for k, c in enumerate(cs):
                pl.when(i == k)(c.wait)
            return carry
        jax.lax.fori_loop(0, len(cs), body, 0)

    def issue_w(t, carry):
        wchunk(0, t).start()
        wchunk(1, t).start()
        return carry

    issue(0, len(cps) - 2)
    jax.lax.fori_loop(0, H, issue_w, 0)
    issue(len(cps) - 2, len(cps))

    def zero(i, carry):
        ot[pl.ds(pl.multiple_of(DM + i * 64, 64), 64), :] = jnp.zeros((64, S), f32)
        return carry

    jax.lax.fori_loop(0, DM // 64, zero, 0)

    def x_prep(k, n):
        w = S // n
        wall[PX, k * w:(k + 1) * w, :] = bxt[0:D, k * w:(k + 1) * w].T
        wall[PX + 1, k * w:(k + 1) * w, 0:DM - D] = bxt[D:DM, k * w:(k + 1) * w].T

    def wq_prep(k, n):
        g = DM // 16
        lo, hi = 16 * (k * g // n), 16 * ((k + 1) * g // n)
        wall[0:H, lo:hi, :] = jnp.swapaxes(wq_raw[lo:hi], 0, 1)

    def part_a(x1a, x1b, rma, rmb, wsa, wsb, csa, csb):
        def stage1(x1, lo, hi, wait):
            def body(c, carry):
                cols = pl.ds(pl.multiple_of(c * XC, XC), XC)
                if wait:
                    pltpu.make_async_copy(axt_hbm.at[:, cols], axt.at[:, cols], sem.at[1 + c]).wait()
                x1[:, cols] = _dot(fd[lo:hi, :], axt[:, cols], NN)
                return carry
            if wait:
                jax.lax.fori_loop(0, 4, body, 0)
            else:
                for c in range(4):
                    x1[:, c * XC:(c + 1) * XC] = _dot(fd[lo:hi, :], axt[:, c * XC:(c + 1) * XC], NN)

        def fwd16(x1, rm, n, unroll):
            def group(r0):
                zs = [(x1[pl.ds(r0, 8), c * LN:(c + 1) * LN], x1[pl.ds(n + r0, 8), c * LN:(c + 1) * LN])
                      for c in range(R16)]
                ys = _fft(zs, -1)
                for r in range(R16):
                    re, im = ys[r]
                    if r:
                        tr, ti = tw[0, r], tw[1, r]
                        re, im = re * tr - im * ti, re * ti + im * tr
                    rm[r, pl.ds(r0, 8), 0:LN] = re
                    rm[r, pl.ds(r0, 8), LN:2 * LN] = im

            if unroll:
                for r0 in range(0, n, 8):
                    group(r0)
            else:
                def body(g, carry):
                    group(pl.multiple_of(g * 8, 8))
                    return carry
                jax.lax.fori_loop(0, n // 8, body, 0)
            if n < LN:
                rm[:, n:LN, :] = jnp.zeros((R16, LN - n, 2 * LN), f32)

        def wprep(ws, lo, hi):
            for p, wt in enumerate((wrt, wit)):
                for c in range(R16):
                    t = wt[lo:hi, c * LN:(c + 1) * LN].astype(f32).T
                    if hi - lo < LN:
                        t = jnp.concatenate([t, jnp.zeros((LN, LN - (hi - lo)), f32)], axis=1)
                    ws[p, c * LN:(c + 1) * LN, :] = t

        def stage23(rm, ws, cs):
            x = _dot(l2[...], rm[...].reshape(R16 * LN, 2 * LN).astype(bf16), NT)
            for r in range(R16):
                xr, xi = x[0:LN, r * LN:(r + 1) * LN], x[LN:2 * LN, r * LN:(r + 1) * LN]
                wr = ws[0, pl.ds(r, LN, stride=R16), :]
                wi = ws[1, pl.ds(r, LN, stride=R16), :]
                g = jnp.concatenate([xr * wr - xi * wi, xr * wi + xi * wr], axis=1).astype(bf16)
                c = _dot(l3[r], g, NN)
                cs[r, 0:LN, :] = c[0:LN, 0:LN] - c[LN:2 * LN, LN:2 * LN]
                cs[r, LN:2 * LN, :] = c[LN:2 * LN, 0:LN] + c[0:LN, LN:2 * LN]

        def inv16(cs, half):
            for r0 in range(0, LN, 8):
                zs = [(cs[r, r0:r0 + 8, :], cs[r, LN + r0:LN + r0 + 8, :]) for r in range(R16)]
                ys = _fft(zs, +1)
                for c in range(R16):
                    wall[PU + half, c * LN + r0:c * LN + r0 + 8, 0:LN] = ys[c][0].astype(bf16)
                    wall[PU + half, c * LN + r0:c * LN + r0 + 8, LN:2 * LN] = ys[c][1].astype(bf16)

        def stage4(half, prep):
            n = S // NP4
            for k in range(NP4):
                if do_b:
                    prep(k, NP4)
                y = _dot(l4[half * DM:(half + 1) * DM, :], wall[PU + half, k * n:(k + 1) * n, :], NT)
                if half:
                    ot[0:DM, k * n:(k + 1) * n] += y
                else:
                    ot[0:DM, k * n:(k + 1) * n] = y

        with scope('w0'):
            c_fda.wait()
        stage1(x1a, 0, 2 * LN, True)
        wait_all([c_fdb, c_tw])
        stage1(x1b, 2 * LN, 2 * LN + 2 * JB, False)
        fwd16(x1a, rma, LN, False)
        wait_all([c_l2, c_wrt, c_wit, c_l3])
        wprep(wsa, 0, LN)
        stage23(rma, wsa, csa)
        fwd16(x1b, rmb, JB, True)
        wprep(wsb, LN, J)
        stage23(rmb, wsb, csb)
        inv16(csa, 0)
        wait_all([c_bxt, c_l4, c_wq])
        stage4(0, x_prep)
        inv16(csb, 1)
        stage4(1, wq_prep)

    if do_a:
        pl.run_scoped(part_a,
                      pltpu.VMEM((2 * LN, S), f32), pltpu.VMEM((2 * JB, S), f32),
                      pltpu.VMEM((R16, LN, 2 * LN), f32), pltpu.VMEM((R16, LN, 2 * LN), f32),
                      pltpu.VMEM((2, S, LN), f32), pltpu.VMEM((2, S, LN), f32),
                      pltpu.VMEM((R16, 2 * LN, LN), f32), pltpu.VMEM((R16, 2 * LN, LN), f32))
    else:
        for c in cps[:-2]:
            c.wait()
        ot[0:DM, :] = jnp.zeros((DM, S), f32)
        if do_b:
            for k in range(NP4):
                x_prep(k, NP4)
                wq_prep(k, NP4)

    def ystep(c, carry):
        for k in range(OCH // LN):
            cols = pl.ds(pl.multiple_of(c * OCH + k * LN, LN), LN)
            ybuf[cols, :] = ot[0:YC, cols].astype(bf16).T
        return carry

    jax.lax.fori_loop(0, S // OCH, ystep, 0)
    c_y = pltpu.make_async_copy(ybuf, out_hbm.at[:, 0:YC], ysem.at[0])
    c_y.start()

    qscale = (D ** -0.5) * math.log2(math.e)

    wchunk(0, 0).wait()
    wchunk(1, 0).wait()

    def qstep(t, carry):
        if do_b:
            rq, rw = S // QPIECES, 2 * CCH // QPIECES
            for j in range(QPIECES):
                which, off = divmod(j * rw, CCH)
                r0 = pl.multiple_of(t * CCH + off, rw)
                src = (wuk_raw, wuv_raw)[which]
                wall[0:H, pl.ds(DM + which * DC + r0, rw), :] = jnp.swapaxes(src[pl.ds(r0, rw)], 0, 1)
                x = jnp.concatenate([wall[PX, j * rq:(j + 1) * rq, :], wall[PX + 1, j * rq:(j + 1) * rq, 0:DM - D]], axis=1)
                q_all[t, j * rq:(j + 1) * rq] = (_dot(x, wall[t, 0:DM, :], NN) * qscale).astype(bf16)

        @pl.when(t + 1 < H)
        def _():
            wchunk(0, t + 1).wait()
            wchunk(1, t + 1).wait()

        return carry

    with scope('P2'):
        jax.lax.fori_loop(0, H, qstep, 0)
    c_ckv.wait()
    c_wot.wait()

    def head(h, carry):
        with scope('head'):
            return head_body(h, carry)

    def head_body(h, carry):
        wkv = jnp.concatenate([wall[h, DM:DM + DC, :], wall[h, DM + DC:DM + 2 * DC, :]], axis=1)
        kv = _dot(ckv[...], wkv, NN).astype(bf16)
        k = kv[:, 0:D]
        v = kv[:, D:2 * D]
        wo = wot[h]
        rr = jax.lax.broadcasted_iota(jnp.int32, (LN, LN), 0)
        cc = jax.lax.broadcasted_iota(jnp.int32, (LN, LN), 1)
        tri = cc <= rr
        neg = -1e30
        ctxs = []
        for i in reversed(range(S // TQ)):
            r0 = i * TQ
            lm = r0 + LN
            q = q_all[h, r0:r0 + TQ, :]
            s = _dot(q, k[0:lm], NT)
            sx = jnp.where(tri, _dot(q[LN:], k[lm:lm + LN], NT), neg)
            sd = jnp.where(tri, s[0:LN, r0:lm], neg)
            pt, lt = _softmax_rows(([s[0:LN, 0:r0]] if i else []) + [sd])
            pb, lb = _softmax_rows([s[LN:], sx])
            pt = jnp.concatenate(pt, axis=1) if i else pt[0]
            ctx = _dot(jnp.concatenate([pt, pb[0]], axis=0), v[0:lm], NN)
            cx = _dot(pb[1], v[lm:lm + LN], NN)
            ctxs.append(jnp.concatenate([ctx[0:LN] * (1.0 / lt), (ctx[LN:] + cx) * (1.0 / lb)],
                                        axis=0).astype(bf16))
        res = _dot(wo, jnp.concatenate(ctxs, axis=0), NT)
        nb = S // TQ
        for n in range(nb):
            ot[DM:2 * DM, (nb - 1 - n) * TQ:(nb - n) * TQ] += res[:, n * TQ:(n + 1) * TQ]
        return carry

    if do_b:
        with scope('P3'):
            jax.lax.fori_loop(0, H, head, 0)

    def ocopy(c):
        rows = pl.ds(pl.multiple_of(c * OCH, OCH), OCH)
        return pltpu.make_async_copy(obuf.at[rows], out_hbm.at[rows, YC:2 * DM], osem.at[c])

    def ostep(c, carry):
        for k in range(OCH // LN):
            cols = pl.ds(pl.multiple_of(c * OCH + k * LN, LN), LN)
            obuf[cols, :] = ot[YC:2 * DM, cols].astype(bf16).T
        ocopy(c).start()
        return carry

    jax.lax.fori_loop(0, S // OCH, ostep, 0)
    c_y.wait()
    for c in range(S // OCH):
        ocopy(c).wait()


def _build(do_a=True, do_b=True, scopes=False):
    def run(A_x, A_w_r, A_w_i, B_x, B_c_kv, B_w_q, B_w_uk, B_w_uv, B_w_o):
        axt = jnp.swapaxes(A_x, 1, 2).reshape(DM, S)
        bxt = jnp.swapaxes(B_x, 1, 2).reshape(DM, S)
        wrt = A_w_r.T
        wit = A_w_i.T
        ckv = B_c_kv.reshape(S, DC)
        wot = jnp.swapaxes(B_w_o, 1, 2)
        tabs = [jnp.asarray(t) for t in _tables()]
        args = (axt, wrt, wit, bxt, ckv, B_w_q, B_w_uk, B_w_uv, wot, *tabs)
        vm = pltpu.VMEM
        scratch = [
            vm((DM, S), bf16), vm((J, S), bf16), vm((J, S), bf16),
            vm(tabs[0].shape, bf16), vm(tabs[1].shape, bf16), vm(tabs[2].shape, f32),
            vm(tabs[3].shape, bf16), vm(tabs[4].shape, bf16),
            vm((DM, S), bf16), vm((S, DC), bf16),
            vm((DM, H, D), bf16),
            vm((DC, H, D), bf16), vm((DC, H, D), bf16), vm((H + 4, DM + 2 * DC, D), bf16),
            vm((H, DM, D), bf16), vm((H, S, D), bf16),
            vm((2 * DM, S), f32), vm((S, YC), bf16), vm((S, 2 * DM - YC), bf16),
            pltpu.SemaphoreType.DMA((16,)), pltpu.SemaphoreType.DMA((2, H)),
            pltpu.SemaphoreType.DMA((S // OCH,)), pltpu.SemaphoreType.DMA((1,)),
        ]
        out = pl.pallas_call(
            functools.partial(_kernel, do_a=do_a, do_b=do_b, scopes=scopes),
            in_specs=[pl.BlockSpec(memory_space=pl.ANY)] * len(args),
            out_specs=pl.BlockSpec(memory_space=pl.ANY),
            out_shape=jax.ShapeDtypeStruct((S, 2 * DM), bf16),
            scratch_shapes=scratch,
            compiler_params=pltpu.CompilerParams(vmem_limit_bytes=120 * 2**20),
        )(*args)
        return out.reshape(1, S, 2 * DM)

    return run


_run = _build()


@jax.jit
def pallas_concat_heads__spectral_gfnet__compressed_kv_cla__prompt_kernel(
    A_x: jax.Array,
    A_w_r: jax.Array,
    A_w_i: jax.Array,
    B_x: jax.Array,
    B_c_kv: jax.Array,
    B_w_q: jax.Array,
    B_w_uk: jax.Array,
    B_w_uv: jax.Array,
    B_w_o: jax.Array,
):
    return _run(A_x, A_w_r, A_w_i, B_x, B_c_kv, B_w_q, B_w_uk, B_w_uv, B_w_o)
```

```python
import contextlib
import functools
import math

import jax
import jax.numpy as jnp
import numpy as np
import jax.experimental.pallas as pl
import jax.experimental.pallas.tpu as pltpu

f32 = jnp.float32
bf16 = jnp.bfloat16

NN = (((1,), (0,)), ((), ()))
NT = (((1,), (1,)), ((), ()))

S = 2048
DM = 448
J = DM // 2 + 1
JB = 104
H = 16
D = 256
DC = 1024
R16 = 16
LN = 128
TQ = 256
CCH = DC // H
PX = H
PU = H + 2
YC = 384
HEAD_ORDER = ('K Q7 U S7 Q5 V7 S5 V5 Q6 S6 V6 Q4 S4 V4 Q3 S3 V3 Q2 Q1 Q0 S2 O7653 S1 V1 V2 O4 S0 V0 O210')
NP4 = 16
OCH = 512
QPIECES = 16


def _dot(a, b, dn):
    return jax.lax.dot_general(a, b, dn, preferred_element_type=f32)


@functools.lru_cache(maxsize=None)
def _tables():
    j = np.arange(J)[:, None].astype(np.float64)
    d = np.arange(DM)[None, :].astype(np.float64)
    ang = 2.0 * np.pi * ((j * d) % DM) / DM
    cos, sin = np.cos(ang), np.sin(ang)
    fd = np.zeros((2 * LN + 2 * JB, DM), np.float64)
    fd[0:LN] = cos[0:LN]
    fd[LN:2 * LN] = -sin[0:LN]
    fd[2 * LN:2 * LN + J - LN] = cos[LN:]
    fd[2 * LN + JB:2 * LN + JB + J - LN] = -sin[LN:]

    m = np.arange(LN)[:, None].astype(np.float64)
    l = np.arange(LN)[None, :].astype(np.float64)
    a128 = 2.0 * np.pi * ((m * l) % LN) / LN
    fr, fi = np.cos(a128), -np.sin(a128)
    l2 = np.block([[fr, -fi], [fi, fr]])

    r = np.arange(R16)[:, None].astype(np.float64)
    at = 2.0 * np.pi * (r * l) / S
    tw = np.stack([np.cos(at), -np.sin(at)])
    tw = np.broadcast_to(tw[:, :, None, :], (2, R16, 8, LN)).copy()

    l3 = np.zeros((R16, 2 * LN, LN), np.float64)
    for rr in range(R16):
        a3 = 2.0 * np.pi * ((m * (rr + R16 * l)) % S) / S
        l3[rr] = np.concatenate([np.cos(a3), np.sin(a3)], axis=0)

    cj = np.full((J,), 2.0)
    cj[0] = 1.0
    cj[J - 1] = 1.0
    scale = cj[None, :] / float(S * DM)
    cr, ci = cos.T * scale, -sin.T * scale
    l4 = np.zeros((2, DM, 2 * LN), np.float64)
    l4[0, :, 0:LN] = cr[:, 0:LN]
    l4[0, :, LN:] = ci[:, 0:LN]
    l4[1, :, 0:J - LN] = cr[:, LN:]
    l4[1, :, LN:LN + J - LN] = ci[:, LN:]

    cast = lambda a, dt: np.asarray(a, np.float32).astype(dt)
    return (cast(fd, bf16), cast(l2, bf16), cast(tw, np.float32), cast(l3, bf16),
            cast(l4.reshape(2 * DM, 2 * LN), bf16))


def _cmul_const(z, k, n, sign):
    re, im = z
    k = k % n
    if k == 0:
        return re, im
    if 4 * k == n:
        return (-im, re) if sign > 0 else (im, -re)
    if 8 * k == n:
        c = math.sqrt(0.5)
        return ((re - im) * c, (re + im) * c) if sign > 0 else ((re + im) * c, (im - re) * c)
    if 8 * k == 3 * n:
        c = math.sqrt(0.5)
        return ((re + im) * (-c), (re - im) * c) if sign > 0 else ((im - re) * c, (re + im) * (-c))
    c = math.cos(2.0 * math.pi * k / n)
    s = sign * math.sin(2.0 * math.pi * k / n)
    return re * c - im * s, re * s + im * c


def _fft(zs, sign):
    n = len(zs)
    if n == 1:
        return zs
    ev = _fft(zs[0::2], sign)
    od = _fft(zs[1::2], sign)
    out = [None] * n
    for k in range(n // 2):
        if 4 * k == n:
            (er, ei), (orr, oi) = ev[k], od[k]
            if sign > 0:
                out[k] = (er - oi, ei + orr)
                out[k + n // 2] = (er + oi, ei - orr)
            else:
                out[k] = (er + oi, ei - orr)
                out[k + n // 2] = (er - oi, ei + orr)
            continue
        tr, ti = _cmul_const(od[k], k, n, sign)
        er, ei = ev[k]
        out[k] = (er + tr, ei + ti)
        out[k + n // 2] = (er - tr, ei - ti)
    return out


def _softmax_rows(segs):
    m = functools.reduce(jnp.maximum, [jnp.max(sg, axis=1, keepdims=True) for sg in segs])
    ps = [jnp.exp2(sg - m).astype(bf16) for sg in segs]
    l = functools.reduce(jnp.add, [jnp.sum(p.astype(f32), axis=1, keepdims=True) for p in ps])
    return ps, l


def _cat(parts, axis):
    return jnp.concatenate(parts, axis=axis) if len(parts) > 1 else parts[0]


def _kernel(axt_hbm, wrt_hbm, wit_hbm, bxt_hbm, ckv_hbm, wq_hbm, wuk_hbm, wuv_hbm, wot_hbm,
            fd_hbm, l2_hbm, tw_hbm, l3_hbm, l4_hbm,
            out_hbm,
            axt, wrt, wit, fd, l2, tw, l3, l4,
            bxt, ckv, wq_raw, wuk_raw, wuv_raw, wall, wot, q_all,
            ot, ybuf, obuf, sem, wsem, osem, ysem, *, do_a, do_b, scopes):
    scope = jax.named_scope if scopes else (lambda name: contextlib.nullcontext())
    XC = S // 4
    simple = ([(fd_hbm.at[0:2 * LN], fd.at[0:2 * LN])]
              + [(axt_hbm.at[:, c * XC:(c + 1) * XC], axt.at[:, c * XC:(c + 1) * XC]) for c in range(4)]
              + [(fd_hbm.at[2 * LN:], fd.at[2 * LN:]), (tw_hbm, tw), (l2_hbm, l2), (wrt_hbm, wrt), (wit_hbm, wit),
                 (l3_hbm, l3), (bxt_hbm, bxt), (l4_hbm, l4), (wq_hbm, wq_raw), (ckv_hbm, ckv), (wot_hbm, wot)])
    cps = [pltpu.make_async_copy(s, d, sem.at[i]) for i, (s, d) in enumerate(simple)]
    c_fda, c_axt = cps[0], cps[1:5]
    (c_fdb, c_tw, c_l2, c_wrt, c_wit, c_l3, c_bxt, c_l4, c_wq, c_ckv, c_wot) = cps[5:]

    def wchunk(which, t):
        src, dst = ((wuk_hbm, wuk_raw), (wuv_hbm, wuv_raw))[which]
        return pltpu.make_async_copy(src.at[pl.ds(t * CCH, CCH)], dst.at[pl.ds(t * CCH, CCH)], wsem.at[which, t])

    def issue(lo, hi):
        def body(i, carry):
            for k in range(lo, hi):
                pl.when(i == k)(cps[k].start)
            return carry
        jax.lax.fori_loop(lo, hi, body, 0)

    def wait_all(cs):
        def body(i, carry):
            for k, c in enumerate(cs):
                pl.when(i == k)(c.wait)
            return carry
        jax.lax.fori_loop(0, len(cs), body, 0)

    def issue_w(t, carry):
        wchunk(0, t).start()
        wchunk(1, t).start()
        return carry

    issue(0, len(cps) - 2)
    jax.lax.fori_loop(0, H, issue_w, 0)
    issue(len(cps) - 2, len(cps))

    def zero(i, carry):
        ot[pl.ds(pl.multiple_of(DM + i * 64, 64), 64), :] = jnp.zeros((64, S), f32)
        return carry

    jax.lax.fori_loop(0, DM // 64, zero, 0)

    def x_prep(k, n):
        w = S // n
        wall[PX, k * w:(k + 1) * w, :] = bxt[0:D, k * w:(k + 1) * w].T
        wall[PX + 1, k * w:(k + 1) * w, 0:DM - D] = bxt[D:DM, k * w:(k + 1) * w].T

    def wq_prep(k, n):
        g = DM // 16
        lo, hi = 16 * (k * g // n), 16 * ((k + 1) * g // n)
        wall[0:H, lo:hi, :] = jnp.swapaxes(wq_raw[lo:hi], 0, 1)

    def part_a(x1a, x1b, rma, rmb, wsa, wsb, csa, csb):
        def stage1(x1, lo, hi, wait):
            def body(c, carry):
                cols = pl.ds(pl.multiple_of(c * XC, XC), XC)
                if wait:
                    pltpu.make_async_copy(axt_hbm.at[:, cols], axt.at[:, cols], sem.at[1 + c]).wait()
                x1[:, cols] = _dot(fd[lo:hi, :], axt[:, cols], NN)
                return carry
            if wait:
                jax.lax.fori_loop(0, 4, body, 0)
            else:
                for c in range(4):
                    x1[:, c * XC:(c + 1) * XC] = _dot(fd[lo:hi, :], axt[:, c * XC:(c + 1) * XC], NN)

        def fwd16(x1, rm, n, unroll):
            def group(r0):
                zs = [(x1[pl.ds(r0, 8), c * LN:(c + 1) * LN], x1[pl.ds(n + r0, 8), c * LN:(c + 1) * LN])
                      for c in range(R16)]
                ys = _fft(zs, -1)
                for r in range(R16):
                    re, im = ys[r]
                    if r:
                        tr, ti = tw[0, r], tw[1, r]
                        re, im = re * tr - im * ti, re * ti + im * tr
                    rm[r, pl.ds(r0, 8), 0:LN] = re
                    rm[r, pl.ds(r0, 8), LN:2 * LN] = im

            if unroll:
                for r0 in range(0, n, 8):
                    group(r0)
            else:
                def body(g, carry):
                    group(pl.multiple_of(g * 8, 8))
                    return carry
                jax.lax.fori_loop(0, n // 8, body, 0)
            if n < LN:
                rm[:, n:LN, :] = jnp.zeros((R16, LN - n, 2 * LN), f32)

        def wprep(ws, lo, hi):
            for p, wt in enumerate((wrt, wit)):
                for c in range(R16):
                    t = wt[lo:hi, c * LN:(c + 1) * LN].astype(f32).T
                    if hi - lo < LN:
                        t = jnp.concatenate([t, jnp.zeros((LN, LN - (hi - lo)), f32)], axis=1)
                    ws[p, c * LN:(c + 1) * LN, :] = t

        def stage23(rm, ws, cs):
            x = _dot(l2[...], rm[...].reshape(R16 * LN, 2 * LN).astype(bf16), NT)
            for r in range(R16):
                xr, xi = x[0:LN, r * LN:(r + 1) * LN], x[LN:2 * LN, r * LN:(r + 1) * LN]
                wr = ws[0, pl.ds(r, LN, stride=R16), :]
                wi = ws[1, pl.ds(r, LN, stride=R16), :]
                g = jnp.concatenate([xr * wr - xi * wi, xr * wi + xi * wr], axis=1).astype(bf16)
                c = _dot(l3[r], g, NN)
                cs[r, 0:LN, :] = c[0:LN, 0:LN] - c[LN:2 * LN, LN:2 * LN]
                cs[r, LN:2 * LN, :] = c[LN:2 * LN, 0:LN] + c[0:LN, LN:2 * LN]

        def inv16(cs, half):
            for r0 in range(0, LN, 8):
                zs = [(cs[r, r0:r0 + 8, :], cs[r, LN + r0:LN + r0 + 8, :]) for r in range(R16)]
                ys = _fft(zs, +1)
                for c in range(R16):
                    wall[PU + half, c * LN + r0:c * LN + r0 + 8, 0:LN] = ys[c][0].astype(bf16)
                    wall[PU + half, c * LN + r0:c * LN + r0 + 8, LN:2 * LN] = ys[c][1].astype(bf16)

        def stage4(half, prep):
            n = S // NP4
            for k in range(NP4):
                if do_b:
                    prep(k, NP4)
                y = _dot(l4[half * DM:(half + 1) * DM, :], wall[PU + half, k * n:(k + 1) * n, :], NT)
                if half:
                    ot[0:DM, k * n:(k + 1) * n] += y
                else:
                    ot[0:DM, k * n:(k + 1) * n] = y

        with scope('w0'):
            c_fda.wait()
        stage1(x1a, 0, 2 * LN, True)
        wait_all([c_fdb, c_tw])
        stage1(x1b, 2 * LN, 2 * LN + 2 * JB, False)
        fwd16(x1a, rma, LN, False)
        wait_all([c_l2, c_wrt, c_wit, c_l3])
        wprep(wsa, 0, LN)
        stage23(rma, wsa, csa)
        fwd16(x1b, rmb, JB, True)
        wprep(wsb, LN, J)
        stage23(rmb, wsb, csb)
        inv16(csa, 0)
        wait_all([c_bxt, c_l4, c_wq])
        stage4(0, x_prep)
        inv16(csb, 1)
        stage4(1, wq_prep)

    if do_a:
        pl.run_scoped(part_a,
                      pltpu.VMEM((2 * LN, S), f32), pltpu.VMEM((2 * JB, S), f32),
                      pltpu.VMEM((R16, LN, 2 * LN), f32), pltpu.VMEM((R16, LN, 2 * LN), f32),
                      pltpu.VMEM((2, S, LN), f32), pltpu.VMEM((2, S, LN), f32),
                      pltpu.VMEM((R16, 2 * LN, LN), f32), pltpu.VMEM((R16, 2 * LN, LN), f32))
    else:
        for c in cps[:-2]:
            c.wait()
        ot[0:DM, :] = jnp.zeros((DM, S), f32)
        if do_b:
            for k in range(NP4):
                x_prep(k, NP4)
                wq_prep(k, NP4)

    def ystep(c, carry):
        for k in range(OCH // LN):
            cols = pl.ds(pl.multiple_of(c * OCH + k * LN, LN), LN)
            ybuf[cols, :] = ot[0:YC, cols].astype(bf16).T
        return carry

    jax.lax.fori_loop(0, S // OCH, ystep, 0)
    c_y = pltpu.make_async_copy(ybuf, out_hbm.at[:, 0:YC], ysem.at[0])
    c_y.start()

    qscale = (D ** -0.5) * math.log2(math.e)

    wchunk(0, 0).wait()
    wchunk(1, 0).wait()

    def qstep(t, carry):
        if do_b:
            rq, rw = S // QPIECES, 2 * CCH // QPIECES
            for j in range(QPIECES):
                which, off = divmod(j * rw, CCH)
                r0 = pl.multiple_of(t * CCH + off, rw)
                src = (wuk_raw, wuv_raw)[which]
                wall[0:H, pl.ds(DM + which * DC + r0, rw), :] = jnp.swapaxes(src[pl.ds(r0, rw)], 0, 1)
                x = jnp.concatenate([wall[PX, j * rq:(j + 1) * rq, :], wall[PX + 1, j * rq:(j + 1) * rq, 0:DM - D]], axis=1)
                q_all[t, j * rq:(j + 1) * rq] = (_dot(x, wall[t, 0:DM, :], NN) * qscale).astype(bf16)

        @pl.when(t + 1 < H)
        def _():
            wchunk(0, t + 1).wait()
            wchunk(1, t + 1).wait()

        return carry

    with scope('P2'):
        jax.lax.fori_loop(0, H, qstep, 0)
    c_ckv.wait()
    c_wot.wait()

    def head(h, carry):
        with scope('head'):
            return head_body(h, carry)

    def head_body(h, carry):
        rr = jax.lax.broadcasted_iota(jnp.int32, (LN, LN), 0)
        cc = jax.lax.broadcasted_iota(jnp.int32, (LN, LN), 1)
        tri = cc <= rr
        neg = -1e30
        kv = {'K': [], 'U': []}
        scores, probs, ctxs = {}, {}, {}

        def rows(name, a, b):
            parts = []
            for lo, arr in sorted(kv[name], key=lambda x: x[0]):
                x, y = max(a, lo), min(b, lo + arr.shape[0])
                if x < y:
                    parts.append(arr[x - lo:y - lo])
            return _cat(parts, 0)

        for tok in HEAD_ORDER.split():
            kind, arg = tok[0], tok[1:]
            if kind in 'KU':
                a, b = map(int, arg.split('-')) if arg else (0, S // TQ)
                w0 = DM + (DC if kind == 'U' else 0)
                w = wall[h, w0:w0 + DC, :]
                kv[kind].append((a * TQ, _dot(ckv[a * TQ:b * TQ, :], w, NN).astype(bf16)))
                continue
            if kind == 'O':
                grp = [int(ch) for ch in arg]
                res = _dot(wot[h], _cat([ctxs[j] for j in grp], 0), NT)
                for n, j in enumerate(grp):
                    ot[DM:2 * DM, j * TQ:(j + 1) * TQ] += res[:, n * TQ:(n + 1) * TQ]
                continue
            i = int(arg)
            r0 = i * TQ
            lm = r0 + LN
            if kind == 'Q':
                q = q_all[h, r0:r0 + TQ, :]
                s = _dot(q, rows('K', 0, lm), NT)
                sx = jnp.where(tri, _dot(q[LN:], rows('K', lm, lm + LN), NT), neg)
                scores[i] = (s, sx)
            elif kind == 'S':
                s, sx = scores.pop(i)
                sd = jnp.where(tri, s[0:LN, r0:lm], neg)
                pt, lt = _softmax_rows(([s[0:LN, 0:r0]] if i else []) + [sd])
                pb, lb = _softmax_rows([s[LN:], sx])
                probs[i] = (jnp.concatenate([_cat(pt, 1), pb[0]], axis=0), pb[1], lt, lb)
            else:
                p, px, lt, lb = probs.pop(i)
                ctx = _dot(p, rows('U', 0, lm), NN)
                cx = _dot(px, rows('U', lm, lm + LN), NN)
                ctxs[i] = jnp.concatenate([ctx[0:LN] * (1.0 / lt), (ctx[LN:] + cx) * (1.0 / lb)],
                                          axis=0).astype(bf16)
        return carry

    if do_b:
        with scope('P3'):
            jax.lax.fori_loop(0, H, head, 0)

    def ocopy(c):
        rows = pl.ds(pl.multiple_of(c * OCH, OCH), OCH)
        return pltpu.make_async_copy(obuf.at[rows], out_hbm.at[rows, YC:2 * DM], osem.at[c])

    def ostep(c, carry):
        for k in range(OCH // LN):
            cols = pl.ds(pl.multiple_of(c * OCH + k * LN, LN), LN)
            obuf[cols, :] = ot[YC:2 * DM, cols].astype(bf16).T
        ocopy(c).start()
        return carry

    jax.lax.fori_loop(0, S // OCH, ostep, 0)
    c_y.wait()
    for c in range(S // OCH):
        ocopy(c).wait()


def _build(do_a=True, do_b=True, scopes=False, order=None):
    global HEAD_ORDER
    if order is not None:
        HEAD_ORDER = order
    def run(A_x, A_w_r, A_w_i, B_x, B_c_kv, B_w_q, B_w_uk, B_w_uv, B_w_o):
        axt = jnp.swapaxes(A_x, 1, 2).reshape(DM, S)
        bxt = jnp.swapaxes(B_x, 1, 2).reshape(DM, S)
        wrt = A_w_r.T
        wit = A_w_i.T
        ckv = B_c_kv.reshape(S, DC)
        wot = jnp.swapaxes(B_w_o, 1, 2)
        tabs = [jnp.asarray(t) for t in _tables()]
        args = (axt, wrt, wit, bxt, ckv, B_w_q, B_w_uk, B_w_uv, wot, *tabs)
        vm = pltpu.VMEM
        scratch = [
            vm((DM, S), bf16), vm((J, S), bf16), vm((J, S), bf16),
            vm(tabs[0].shape, bf16), vm(tabs[1].shape, bf16), vm(tabs[2].shape, f32),
            vm(tabs[3].shape, bf16), vm(tabs[4].shape, bf16),
            vm((DM, S), bf16), vm((S, DC), bf16),
            vm((DM, H, D), bf16),
            vm((DC, H, D), bf16), vm((DC, H, D), bf16), vm((H + 4, DM + 2 * DC, D), bf16),
            vm((H, DM, D), bf16), vm((H, S, D), bf16),
            vm((2 * DM, S), f32), vm((S, YC), bf16), vm((S, 2 * DM - YC), bf16),
            pltpu.SemaphoreType.DMA((16,)), pltpu.SemaphoreType.DMA((2, H)),
            pltpu.SemaphoreType.DMA((S // OCH,)), pltpu.SemaphoreType.DMA((1,)),
        ]
        out = pl.pallas_call(
            functools.partial(_kernel, do_a=do_a, do_b=do_b, scopes=scopes),
            in_specs=[pl.BlockSpec(memory_space=pl.ANY)] * len(args),
            out_specs=pl.BlockSpec(memory_space=pl.ANY),
            out_shape=jax.ShapeDtypeStruct((S, 2 * DM), bf16),
            scratch_shapes=scratch,
            compiler_params=pltpu.CompilerParams(vmem_limit_bytes=120 * 2**20),
        )(*args)
        return out.reshape(1, S, 2 * DM)

    return run


_run = _build()


@jax.jit
def pallas_concat_heads__spectral_gfnet__compressed_kv_cla__prompt_kernel(
    A_x: jax.Array,
    A_w_r: jax.Array,
    A_w_i: jax.Array,
    B_x: jax.Array,
    B_c_kv: jax.Array,
    B_w_q: jax.Array,
    B_w_uk: jax.Array,
    B_w_uv: jax.Array,
    B_w_o: jax.Array,
):
    return _run(A_x, A_w_r, A_w_i, B_x, B_c_kv, B_w_q, B_w_uk, B_w_uv, B_w_o)
```

```python
import contextlib
import functools
import math

import jax
import jax.numpy as jnp
import numpy as np
import jax.experimental.pallas as pl
import jax.experimental.pallas.tpu as pltpu

f32 = jnp.float32
bf16 = jnp.bfloat16

NN = (((1,), (0,)), ((), ()))
NT = (((1,), (1,)), ((), ()))

S = 2048
DM = 448
J = DM // 2 + 1
JB = 104
H = 16
D = 256
DC = 1024
R16 = 16
LN = 128
TQ = 256
CCH = DC // H
PX = H
PU = H + 2
YC = 384
HEAD_ORDER = ('U0-2 K0-8 U2-4 Q4 U4-8 Q1 S1 Q0 S4 V4 Q6 Q3 S0 V0 V1 S6 Q5 S5 S3 V6 Q7 S7 V3 V7 Q2 V5 O0 S2 V2 O76521 O4 O3')
OCH = 512
QPIECES = 16


def _dot(a, b, dn):
    return jax.lax.dot_general(a, b, dn, preferred_element_type=f32)


@functools.lru_cache(maxsize=None)
def _tables():
    j = np.arange(J)[:, None].astype(np.float64)
    d = np.arange(DM)[None, :].astype(np.float64)
    ang = 2.0 * np.pi * ((j * d) % DM) / DM
    cos, sin = np.cos(ang), np.sin(ang)
    fd = np.zeros((2 * LN + 2 * JB, DM), np.float64)
    fd[0:LN] = cos[0:LN]
    fd[LN:2 * LN] = -sin[0:LN]
    fd[2 * LN:2 * LN + J - LN] = cos[LN:]
    fd[2 * LN + JB:2 * LN + JB + J - LN] = -sin[LN:]

    m = np.arange(LN)[:, None].astype(np.float64)
    l = np.arange(LN)[None, :].astype(np.float64)
    a128 = 2.0 * np.pi * ((m * l) % LN) / LN
    fr, fi = np.cos(a128), -np.sin(a128)
    l2 = np.block([[fr, -fi], [fi, fr]])

    r = np.arange(R16)[:, None].astype(np.float64)
    at = 2.0 * np.pi * (r * l) / S
    tw = np.stack([np.cos(at), -np.sin(at)])
    tw = np.broadcast_to(tw[:, :, None, :], (2, R16, 8, LN)).copy()

    l3 = np.zeros((R16, 2 * LN, LN), np.float64)
    for rr in range(R16):
        a3 = 2.0 * np.pi * ((m * (rr + R16 * l)) % S) / S
        l3[rr] = np.concatenate([np.cos(a3), np.sin(a3)], axis=0)

    cj = np.full((J,), 2.0)
    cj[0] = 1.0
    cj[J - 1] = 1.0
    scale = cj[None, :] / float(S * DM)
    cr, ci = cos.T * scale, -sin.T * scale
    l4 = np.zeros((2, DM, 2 * LN), np.float64)
    l4[0, :, 0:LN] = cr[:, 0:LN]
    l4[0, :, LN:] = ci[:, 0:LN]
    l4[1, :, 0:J - LN] = cr[:, LN:]
    l4[1, :, LN:LN + J - LN] = ci[:, LN:]

    cast = lambda a, dt: np.asarray(a, np.float32).astype(dt)
    return (cast(fd, bf16), cast(l2, bf16), cast(tw, np.float32), cast(l3, bf16),
            cast(l4.reshape(2 * DM, 2 * LN), bf16))


def _cmul_const(z, k, n, sign):
    re, im = z
    k = k % n
    if k == 0:
        return re, im
    if 4 * k == n:
        return (-im, re) if sign > 0 else (im, -re)
    if 8 * k == n:
        c = math.sqrt(0.5)
        return ((re - im) * c, (re + im) * c) if sign > 0 else ((re + im) * c, (im - re) * c)
    if 8 * k == 3 * n:
        c = math.sqrt(0.5)
        return ((re + im) * (-c), (re - im) * c) if sign > 0 else ((im - re) * c, (re + im) * (-c))
    c = math.cos(2.0 * math.pi * k / n)
    s = sign * math.sin(2.0 * math.pi * k / n)
    return re * c - im * s, re * s + im * c


def _fft(zs, sign):
    n = len(zs)
    if n == 1:
        return zs
    ev = _fft(zs[0::2], sign)
    od = _fft(zs[1::2], sign)
    out = [None] * n
    for k in range(n // 2):
        if 4 * k == n:
            (er, ei), (orr, oi) = ev[k], od[k]
            if sign > 0:
                out[k] = (er - oi, ei + orr)
                out[k + n // 2] = (er + oi, ei - orr)
            else:
                out[k] = (er + oi, ei - orr)
                out[k + n // 2] = (er - oi, ei + orr)
            continue
        tr, ti = _cmul_const(od[k], k, n, sign)
        er, ei = ev[k]
        out[k] = (er + tr, ei + ti)
        out[k + n // 2] = (er - tr, ei - ti)
    return out


def _softmax_rows(segs):
    m = functools.reduce(jnp.maximum, [jnp.max(sg, axis=1, keepdims=True) for sg in segs])
    ps = [jnp.exp2(sg - m).astype(bf16) for sg in segs]
    l = functools.reduce(jnp.add, [jnp.sum(p.astype(f32), axis=1, keepdims=True) for p in ps])
    return ps, l


def _cat(parts, axis):
    return jnp.concatenate(parts, axis=axis) if len(parts) > 1 else parts[0]


def _kernel(axt_hbm, wrt_hbm, wit_hbm, bxt_hbm, ckv_hbm, wq_hbm, wuk_hbm, wuv_hbm, wot_hbm,
            fd_hbm, l2_hbm, tw_hbm, l3_hbm, l4_hbm,
            out_hbm,
            axt, wrt, wit, fd, l2, tw, l3, l4,
            bxt, ckv, wq_raw, wuk_raw, wuv_raw, wall, wot, q_all,
            ot, ybuf, obuf, sem, wsem, osem, ysem, *, do_a, do_b, scopes):
    scope = jax.named_scope if scopes else (lambda name: contextlib.nullcontext())
    XC = S // 4
    simple = ([(fd_hbm.at[0:2 * LN], fd.at[0:2 * LN])]
              + [(axt_hbm.at[:, c * XC:(c + 1) * XC], axt.at[:, c * XC:(c + 1) * XC]) for c in range(4)]
              + [(fd_hbm.at[2 * LN:], fd.at[2 * LN:]), (tw_hbm, tw), (l2_hbm, l2), (wrt_hbm, wrt), (wit_hbm, wit),
                 (l3_hbm, l3), (bxt_hbm, bxt), (l4_hbm, l4), (wq_hbm, wq_raw), (ckv_hbm, ckv), (wot_hbm, wot)])
    cps = [pltpu.make_async_copy(s, d, sem.at[i]) for i, (s, d) in enumerate(simple)]
    c_fda, c_axt = cps[0], cps[1:5]
    (c_fdb, c_tw, c_l2, c_wrt, c_wit, c_l3, c_bxt, c_l4, c_wq, c_ckv, c_wot) = cps[5:]

    def wchunk(which, t):
        src, dst = ((wuk_hbm, wuk_raw), (wuv_hbm, wuv_raw))[which]
        return pltpu.make_async_copy(src.at[pl.ds(t * CCH, CCH)], dst.at[pl.ds(t * CCH, CCH)], wsem.at[which, t])

    def issue(lo, hi):
        def body(i, carry):
            for k in range(lo, hi):
                pl.when(i == k)(cps[k].start)
            return carry
        jax.lax.fori_loop(lo, hi, body, 0)

    def wait_all(cs):
        def body(i, carry):
            for k, c in enumerate(cs):
                pl.when(i == k)(c.wait)
            return carry
        jax.lax.fori_loop(0, len(cs), body, 0)

    def issue_w(t, carry):
        wchunk(0, t).start()
        wchunk(1, t).start()
        return carry

    issue(0, len(cps) - 2)
    jax.lax.fori_loop(0, H, issue_w, 0)
    issue(len(cps) - 2, len(cps))

    def zero(i, carry):
        ot[pl.ds(pl.multiple_of(DM + i * 64, 64), 64), :] = jnp.zeros((64, S), f32)
        return carry

    jax.lax.fori_loop(0, DM // 64, zero, 0)

    def x_prep(k, n):
        w = S // n
        wall[PX, k * w:(k + 1) * w, :] = bxt[0:D, k * w:(k + 1) * w].T
        wall[PX + 1, k * w:(k + 1) * w, 0:DM - D] = bxt[D:DM, k * w:(k + 1) * w].T

    def wq_prep(k, n):
        g = DM // 16
        lo, hi = 16 * (k * g // n), 16 * ((k + 1) * g // n)
        wall[0:H, lo:hi, :] = jnp.swapaxes(wq_raw[lo:hi], 0, 1)

    def part_a(x1a, x1b, rma, rmb, wsa, wsb, csa, csb):
        def stage1(x1, lo, hi, wait):
            def body(c, carry):
                cols = pl.ds(pl.multiple_of(c * XC, XC), XC)
                if wait:
                    pltpu.make_async_copy(axt_hbm.at[:, cols], axt.at[:, cols], sem.at[1 + c]).wait()
                x1[:, cols] = _dot(fd[lo:hi, :], axt[:, cols], NN)
                return carry
            if wait:
                jax.lax.fori_loop(0, 4, body, 0)
            else:
                for c in range(4):
                    x1[:, c * XC:(c + 1) * XC] = _dot(fd[lo:hi, :], axt[:, c * XC:(c + 1) * XC], NN)

        def fwd16(x1, rm, n, r0):
            zs = [(x1[pl.ds(r0, 8), c * LN:(c + 1) * LN], x1[pl.ds(n + r0, 8), c * LN:(c + 1) * LN])
                  for c in range(R16)]
            ys = _fft(zs, -1)
            for r in range(R16):
                re, im = ys[r]
                if r:
                    tr, ti = tw[0, r], tw[1, r]
                    re, im = re * tr - im * ti, re * ti + im * tr
                rm[r, pl.ds(r0, 8), 0:LN] = re
                rm[r, pl.ds(r0, 8), LN:2 * LN] = im

        def wprep(ws, lo, hi, c):
            for p, wt in enumerate((wrt, wit)):
                t = wt[lo:hi, c * LN:(c + 1) * LN].astype(f32).T
                if hi - lo < LN:
                    t = jnp.concatenate([t, jnp.zeros((LN, LN - (hi - lo)), f32)], axis=1)
                ws[p, c * LN:(c + 1) * LN, :] = t

        def stage2(rm):
            return _dot(l2[...], rm[...].reshape(R16 * LN, 2 * LN).astype(bf16), NT)

        def stage3(x, ws, cs, r):
            xr, xi = x[0:LN, r * LN:(r + 1) * LN], x[LN:2 * LN, r * LN:(r + 1) * LN]
            wr = ws[0, pl.ds(r, LN, stride=R16), :]
            wi = ws[1, pl.ds(r, LN, stride=R16), :]
            g = jnp.concatenate([xr * wr - xi * wi, xr * wi + xi * wr], axis=1).astype(bf16)
            c = _dot(l3[r], g, NN)
            cs[r, 0:LN, :] = c[0:LN, 0:LN] - c[LN:2 * LN, LN:2 * LN]
            cs[r, LN:2 * LN, :] = c[LN:2 * LN, 0:LN] + c[0:LN, LN:2 * LN]

        def inv16(cs, half, r0):
            zs = [(cs[r, r0:r0 + 8, :], cs[r, LN + r0:LN + r0 + 8, :]) for r in range(R16)]
            ys = _fft(zs, +1)
            for c in range(R16):
                wall[PU + half, c * LN + r0:c * LN + r0 + 8, 0:LN] = ys[c][0].astype(bf16)
                wall[PU + half, c * LN + r0:c * LN + r0 + 8, LN:2 * LN] = ys[c][1].astype(bf16)

        def stage4(half, k):
            y = _dot(l4[half * DM:(half + 1) * DM, :], wall[PU + half, k * LN:(k + 1) * LN, :], NT)
            if half:
                ot[0:DM, k * LN:(k + 1) * LN] += y
            else:
                ot[0:DM, k * LN:(k + 1) * LN] = y

        with scope('w0'):
            c_fda.wait()
        stage1(x1a, 0, 2 * LN, True)
        wait_all([c_fdb, c_tw])
        stage1(x1b, 2 * LN, 2 * LN + 2 * JB, False)

        def fwd16a(g, carry):
            fwd16(x1a, rma, LN, pl.multiple_of(g * 8, 8))
            return carry

        def fwd16b(g, carry):
            fwd16(x1b, rmb, JB, pl.multiple_of(g * 8, 8))
            return carry

        jax.lax.fori_loop(0, LN // 8, fwd16a, 0)
        jax.lax.fori_loop(0, JB // 8, fwd16b, 0)
        wait_all([c_l2, c_wrt, c_wit, c_l3])
        rmb[:, JB:LN, :] = jnp.zeros((R16, LN - JB, 2 * LN), f32)
        for c in range(R16):
            wprep(wsa, 0, LN, c)
        xa = stage2(rma)
        for r in range(R16):
            stage3(xa, wsa, csa, r)
            wprep(wsb, LN, J, r)
        xb = stage2(rmb)
        for r in range(R16):
            stage3(xb, wsb, csb, r)
            inv16(csa, 0, r * 8)
        wait_all([c_bxt, c_l4, c_wq])
        for k in range(R16):
            if do_b:
                x_prep(k, R16)
            stage4(0, k)
            inv16(csb, 1, k * 8)
        for k in range(R16):
            if do_b:
                wq_prep(k, R16)
            stage4(1, k)

    if do_a:
        pl.run_scoped(part_a,
                      pltpu.VMEM((2 * LN, S), f32), pltpu.VMEM((2 * JB, S), f32),
                      pltpu.VMEM((R16, LN, 2 * LN), f32), pltpu.VMEM((R16, LN, 2 * LN), f32),
                      pltpu.VMEM((2, S, LN), f32), pltpu.VMEM((2, S, LN), f32),
                      pltpu.VMEM((R16, 2 * LN, LN), f32), pltpu.VMEM((R16, 2 * LN, LN), f32))
    else:
        for c in cps[:-2]:
            c.wait()
        ot[0:DM, :] = jnp.zeros((DM, S), f32)
        if do_b:
            for k in range(R16):
                x_prep(k, R16)
                wq_prep(k, R16)

    def ystep(c, carry):
        for k in range(OCH // LN):
            cols = pl.ds(pl.multiple_of(c * OCH + k * LN, LN), LN)
            ybuf[cols, :] = ot[0:YC, cols].astype(bf16).T
        return carry

    jax.lax.fori_loop(0, S // OCH, ystep, 0)
    c_y = pltpu.make_async_copy(ybuf, out_hbm.at[:, 0:YC], ysem.at[0])
    c_y.start()

    qscale = (D ** -0.5) * math.log2(math.e)

    wchunk(0, 0).wait()
    wchunk(1, 0).wait()

    def qstep(t, carry):
        if do_b:
            rq, rw = S // QPIECES, 2 * CCH // QPIECES
            for j in range(QPIECES):
                x = jnp.concatenate([wall[PX, j * rq:(j + 1) * rq, :], wall[PX + 1, j * rq:(j + 1) * rq, 0:DM - D]], axis=1)
                q_all[t, j * rq:(j + 1) * rq] = (_dot(x, wall[t, 0:DM, :], NN) * qscale).astype(bf16)
                which, off = divmod(j * rw, CCH)
                r0 = pl.multiple_of(t * CCH + off, rw)
                src = (wuk_raw, wuv_raw)[which]
                wall[0:H, pl.ds(DM + which * DC + r0, rw), :] = jnp.swapaxes(src[pl.ds(r0, rw)], 0, 1)

        @pl.when(t + 1 < H)
        def _():
            wchunk(0, t + 1).wait()
            wchunk(1, t + 1).wait()

        return carry

    with scope('P2'):
        jax.lax.fori_loop(0, H, qstep, 0)
    c_ckv.wait()
    c_wot.wait()

    def head(h, carry):
        with scope('head'):
            return head_body(h, carry)

    def head_body(h, carry):
        rr = jax.lax.broadcasted_iota(jnp.int32, (LN, LN), 0)
        cc = jax.lax.broadcasted_iota(jnp.int32, (LN, LN), 1)
        tri = cc <= rr
        neg = -1e30
        kv = {'K': [], 'U': []}
        scores, probs, ctxs = {}, {}, {}

        def rows(name, a, b):
            parts = []
            for lo, arr in sorted(kv[name], key=lambda x: x[0]):
                x, y = max(a, lo), min(b, lo + arr.shape[0])
                if x < y:
                    parts.append(arr[x - lo:y - lo])
            return _cat(parts, 0)

        for tok in HEAD_ORDER.split():
            kind, arg = tok[0], tok[1:]
            if kind in 'KU':
                a, b = map(int, arg.split('-')) if arg else (0, S // TQ)
                w0 = DM + (DC if kind == 'U' else 0)
                w = wall[h, w0:w0 + DC, :]
                kv[kind].append((a * TQ, _dot(ckv[a * TQ:b * TQ, :], w, NN).astype(bf16)))
                continue
            if kind == 'O':
                grp = [int(ch) for ch in arg]
                res = _dot(wot[h], _cat([ctxs[j] for j in grp], 0), NT)
                for n, j in enumerate(grp):
                    ot[DM:2 * DM, j * TQ:(j + 1) * TQ] += res[:, n * TQ:(n + 1) * TQ]
                continue
            i = int(arg)
            r0 = i * TQ
            lm = r0 + LN
            if kind == 'Q':
                q = q_all[h, r0:r0 + TQ, :]
                s = _dot(q, rows('K', 0, lm), NT)
                sx = jnp.where(tri, _dot(q[LN:], rows('K', lm, lm + LN), NT), neg)
                scores[i] = (s, sx)
            elif kind == 'S':
                s, sx = scores.pop(i)
                sd = jnp.where(tri, s[0:LN, r0:lm], neg)
                pt, lt = _softmax_rows(([s[0:LN, 0:r0]] if i else []) + [sd])
                pb, lb = _softmax_rows([s[LN:], sx])
                probs[i] = (jnp.concatenate([_cat(pt, 1), pb[0]], axis=0), pb[1], lt, lb)
            else:
                p, px, lt, lb = probs.pop(i)
                ctx = _dot(p, rows('U', 0, lm), NN)
                cx = _dot(px, rows('U', lm, lm + LN), NN)
                ctxs[i] = jnp.concatenate([ctx[0:LN] * (1.0 / lt), (ctx[LN:] + cx) * (1.0 / lb)],
                                          axis=0).astype(bf16)
        return carry

    if do_b:
        with scope('P3'):
            jax.lax.fori_loop(0, H, head, 0)

    def ocopy(c):
        rows = pl.ds(pl.multiple_of(c * OCH, OCH), OCH)
        return pltpu.make_async_copy(obuf.at[rows], out_hbm.at[rows, YC:2 * DM], osem.at[c])

    def ostep(c, carry):
        for k in range(OCH // LN):
            cols = pl.ds(pl.multiple_of(c * OCH + k * LN, LN), LN)
            obuf[cols, :] = ot[YC:2 * DM, cols].astype(bf16).T
        ocopy(c).start()
        return carry

    jax.lax.fori_loop(0, S // OCH, ostep, 0)
    c_y.wait()
    for c in range(S // OCH):
        ocopy(c).wait()


def _build(do_a=True, do_b=True, scopes=False, order=None):
    global HEAD_ORDER
    if order is not None:
        HEAD_ORDER = order
    def run(A_x, A_w_r, A_w_i, B_x, B_c_kv, B_w_q, B_w_uk, B_w_uv, B_w_o):
        axt = jnp.swapaxes(A_x, 1, 2).reshape(DM, S)
        bxt = jnp.swapaxes(B_x, 1, 2).reshape(DM, S)
        wrt = A_w_r.T
        wit = A_w_i.T
        ckv = B_c_kv.reshape(S, DC)
        wot = jnp.swapaxes(B_w_o, 1, 2)
        tabs = [jnp.asarray(t) for t in _tables()]
        args = (axt, wrt, wit, bxt, ckv, B_w_q, B_w_uk, B_w_uv, wot, *tabs)
        vm = pltpu.VMEM
        scratch = [
            vm((DM, S), bf16), vm((J, S), bf16), vm((J, S), bf16),
            vm(tabs[0].shape, bf16), vm(tabs[1].shape, bf16), vm(tabs[2].shape, f32),
            vm(tabs[3].shape, bf16), vm(tabs[4].shape, bf16),
            vm((DM, S), bf16), vm((S, DC), bf16),
            vm((DM, H, D), bf16),
            vm((DC, H, D), bf16), vm((DC, H, D), bf16), vm((H + 4, DM + 2 * DC, D), bf16),
            vm((H, DM, D), bf16), vm((H, S, D), bf16),
            vm((2 * DM, S), f32), vm((S, YC), bf16), vm((S, 2 * DM - YC), bf16),
            pltpu.SemaphoreType.DMA((16,)), pltpu.SemaphoreType.DMA((2, H)),
            pltpu.SemaphoreType.DMA((S // OCH,)), pltpu.SemaphoreType.DMA((1,)),
        ]
        out = pl.pallas_call(
            functools.partial(_kernel, do_a=do_a, do_b=do_b, scopes=scopes),
            in_specs=[pl.BlockSpec(memory_space=pl.ANY)] * len(args),
            out_specs=pl.BlockSpec(memory_space=pl.ANY),
            out_shape=jax.ShapeDtypeStruct((S, 2 * DM), bf16),
            scratch_shapes=scratch,
            compiler_params=pltpu.CompilerParams(vmem_limit_bytes=120 * 2**20),
        )(*args)
        return out.reshape(1, S, 2 * DM)

    return run


_run = _build()


@jax.jit
def pallas_concat_heads__spectral_gfnet__compressed_kv_cla__prompt_kernel(
    A_x: jax.Array,
    A_w_r: jax.Array,
    A_w_i: jax.Array,
    B_x: jax.Array,
    B_c_kv: jax.Array,
    B_w_q: jax.Array,
    B_w_uk: jax.Array,
    B_w_uv: jax.Array,
    B_w_o: jax.Array,
):
    return _run(A_x, A_w_r, A_w_i, B_x, B_c_kv, B_w_q, B_w_uk, B_w_uv, B_w_o)
```

```python
import contextlib
import functools
import math

import jax
import jax.numpy as jnp
import numpy as np
import jax.experimental.pallas as pl
import jax.experimental.pallas.tpu as pltpu

f32 = jnp.float32
bf16 = jnp.bfloat16

NN = (((1,), (0,)), ((), ()))
NT = (((1,), (1,)), ((), ()))

S = 2048
DM = 448
J = DM // 2 + 1
HD = DM // 2
JA = 120
JB = 112
H = 16
D = 256
DC = 1024
R16 = 16
LN = 128
TQ = 256
CCH = DC // H
PX = H
PU = H + 2
YC = 384
HEAD_ORDER = ('U0-2 K0-8 U2-4 Q4 U4-8 Q1 S1 Q0 S4 V4 Q6 Q3 S0 V0 V1 S6 Q5 S5 S3 V6 Q7 S7 V3 V7 Q2 V5 O0 S2 V2 O76521 O4 O3')
OCH = 512
QPIECES = 16


def _dot(a, b, dn):
    return jax.lax.dot_general(a, b, dn, preferred_element_type=f32)


@functools.lru_cache(maxsize=None)
def _tables():
    j = np.arange(J)[:, None].astype(np.float64)
    d = np.arange(DM)[None, :].astype(np.float64)
    ang = 2.0 * np.pi * ((j * d) % DM) / DM
    cos, sin = np.cos(ang), np.sin(ang)
    ne, no = (J + 1) // 2, J // 2
    fd = np.zeros((2 * JA + 2 * JB, HD), np.float64)
    fd[0:ne] = cos[0::2, 0:HD]
    fd[JA:JA + ne] = -sin[0::2, 0:HD]
    fd[2 * JA:2 * JA + no] = cos[1::2, 0:HD]
    fd[2 * JA + JB:2 * JA + JB + no] = -sin[1::2, 0:HD]

    m = np.arange(LN)[:, None].astype(np.float64)
    l = np.arange(LN)[None, :].astype(np.float64)
    a128 = 2.0 * np.pi * ((m * l) % LN) / LN
    fr, fi = np.cos(a128), -np.sin(a128)
    l2 = np.block([[fr, -fi], [fi, fr]])

    r = np.arange(R16)[:, None].astype(np.float64)
    at = 2.0 * np.pi * (r * l) / S
    tw = np.stack([np.cos(at), -np.sin(at)])
    tw = np.broadcast_to(tw[:, :, None, :], (2, R16, 8, LN)).copy()

    l3 = np.zeros((R16, 2 * LN, LN), np.float64)
    for rr in range(R16):
        a3 = 2.0 * np.pi * ((m * (rr + R16 * l)) % S) / S
        l3[rr] = np.concatenate([np.cos(a3), np.sin(a3)], axis=0)

    cj = np.full((J,), 2.0)
    cj[0] = 1.0
    cj[J - 1] = 1.0
    scale = cj[None, :] / float(S * DM)
    cr, ci = cos.T[0:HD] * scale, -sin.T[0:HD] * scale
    l4 = np.zeros((2, HD, 2 * LN), np.float64)
    l4[0, :, 0:ne] = cr[:, 0::2]
    l4[0, :, LN:LN + ne] = ci[:, 0::2]
    l4[1, :, 0:no] = cr[:, 1::2]
    l4[1, :, LN:LN + no] = ci[:, 1::2]

    cast = lambda a, dt: np.asarray(a, np.float32).astype(dt)
    return (cast(fd, bf16), cast(l2, bf16), cast(tw, np.float32), cast(l3, bf16),
            cast(l4.reshape(2 * HD, 2 * LN), bf16))


def _cmul_const(z, k, n, sign):
    re, im = z
    k = k % n
    if k == 0:
        return re, im
    if 4 * k == n:
        return (-im, re) if sign > 0 else (im, -re)
    if 8 * k == n:
        c = math.sqrt(0.5)
        return ((re - im) * c, (re + im) * c) if sign > 0 else ((re + im) * c, (im - re) * c)
    if 8 * k == 3 * n:
        c = math.sqrt(0.5)
        return ((re + im) * (-c), (re - im) * c) if sign > 0 else ((im - re) * c, (re + im) * (-c))
    c = math.cos(2.0 * math.pi * k / n)
    s = sign * math.sin(2.0 * math.pi * k / n)
    return re * c - im * s, re * s + im * c


def _fft(zs, sign):
    n = len(zs)
    if n == 1:
        return zs
    ev = _fft(zs[0::2], sign)
    od = _fft(zs[1::2], sign)
    out = [None] * n
    for k in range(n // 2):
        if 4 * k == n:
            (er, ei), (orr, oi) = ev[k], od[k]
            if sign > 0:
                out[k] = (er - oi, ei + orr)
                out[k + n // 2] = (er + oi, ei - orr)
            else:
                out[k] = (er + oi, ei - orr)
                out[k + n // 2] = (er - oi, ei + orr)
            continue
        tr, ti = _cmul_const(od[k], k, n, sign)
        er, ei = ev[k]
        out[k] = (er + tr, ei + ti)
        out[k + n // 2] = (er - tr, ei - ti)
    return out


def _softmax_rows(segs):
    m = functools.reduce(jnp.maximum, [jnp.max(sg, axis=1, keepdims=True) for sg in segs])
    ps = [jnp.exp2(sg - m).astype(bf16) for sg in segs]
    l = functools.reduce(jnp.add, [jnp.sum(p.astype(f32), axis=1, keepdims=True) for p in ps])
    return ps, l


def _cat(parts, axis):
    return jnp.concatenate(parts, axis=axis) if len(parts) > 1 else parts[0]


def _kernel(axt_hbm, wrt_hbm, wit_hbm, bxt_hbm, ckv_hbm, wq_hbm, wuk_hbm, wuv_hbm, wot_hbm,
            fd_hbm, l2_hbm, tw_hbm, l3_hbm, l4_hbm,
            out_hbm,
            axt, wrt, wit, fd, l2, tw, l3, l4,
            bxt, ckv, wq_raw, wuk_raw, wuv_raw, wall, wot, q_all,
            ot, ybuf, obuf, sem, wsem, osem, ysem, *, do_a, do_b, scopes):
    scope = jax.named_scope if scopes else (lambda name: contextlib.nullcontext())
    XC = S // 4
    simple = ([(fd_hbm, fd)]
              + [(axt_hbm.at[:, c * XC:(c + 1) * XC], axt.at[:, c * XC:(c + 1) * XC]) for c in range(4)]
              + [(tw_hbm, tw), (l2_hbm, l2), (wrt_hbm, wrt), (wit_hbm, wit),
                 (l3_hbm, l3), (bxt_hbm, bxt), (l4_hbm, l4), (wq_hbm, wq_raw), (ckv_hbm, ckv), (wot_hbm, wot)])
    cps = [pltpu.make_async_copy(s, d, sem.at[i]) for i, (s, d) in enumerate(simple)]
    c_fd = cps[0]
    (c_tw, c_l2, c_wrt, c_wit, c_l3, c_bxt, c_l4, c_wq, c_ckv, c_wot) = cps[5:]

    def wchunk(which, t):
        src, dst = ((wuk_hbm, wuk_raw), (wuv_hbm, wuv_raw))[which]
        return pltpu.make_async_copy(src.at[pl.ds(t * CCH, CCH)], dst.at[pl.ds(t * CCH, CCH)], wsem.at[which, t])

    def issue(lo, hi):
        def body(i, carry):
            for k in range(lo, hi):
                pl.when(i == k)(cps[k].start)
            return carry
        jax.lax.fori_loop(lo, hi, body, 0)

    def wait_all(cs):
        def body(i, carry):
            for k, c in enumerate(cs):
                pl.when(i == k)(c.wait)
            return carry
        jax.lax.fori_loop(0, len(cs), body, 0)

    def issue_w(t, carry):
        wchunk(0, t).start()
        wchunk(1, t).start()
        return carry

    issue(0, len(cps) - 2)
    jax.lax.fori_loop(0, H, issue_w, 0)
    issue(len(cps) - 2, len(cps))

    def zero(i, carry):
        ot[pl.ds(pl.multiple_of(DM + i * 64, 64), 64), :] = jnp.zeros((64, S), f32)
        return carry

    jax.lax.fori_loop(0, DM // 64, zero, 0)

    def x_prep(k, n):
        w = S // n
        wall[PX, k * w:(k + 1) * w, :] = bxt[0:D, k * w:(k + 1) * w].T
        wall[PX + 1, k * w:(k + 1) * w, 0:DM - D] = bxt[D:DM, k * w:(k + 1) * w].T

    def wq_prep(k, n):
        g = DM // 16
        lo, hi = 16 * (k * g // n), 16 * ((k + 1) * g // n)
        wall[0:H, lo:hi, :] = jnp.swapaxes(wq_raw[lo:hi], 0, 1)

    def part_a(x1a, x1b, rma, rmb, wsa, wsb, csa, csb):
        def stage1(c, carry):
            cols = pl.ds(pl.multiple_of(c * XC, XC), XC)
            pltpu.make_async_copy(axt_hbm.at[:, cols], axt.at[:, cols], sem.at[1 + c]).wait()
            lo, hi = axt[0:HD, cols].astype(f32), axt[HD:DM, cols].astype(f32)
            x1a[:, cols] = _dot(fd[0:2 * JA, :], (lo + hi).astype(bf16), NN)
            x1b[:, cols] = _dot(fd[2 * JA:, :], (lo - hi).astype(bf16), NN)
            return carry

        def fwd16(x1, rm, n, r0):
            zs = [(x1[pl.ds(r0, 8), c * LN:(c + 1) * LN], x1[pl.ds(n + r0, 8), c * LN:(c + 1) * LN])
                  for c in range(R16)]
            ys = _fft(zs, -1)
            for r in range(R16):
                re, im = ys[r]
                if r:
                    tr, ti = tw[0, r], tw[1, r]
                    re, im = re * tr - im * ti, re * ti + im * tr
                rm[r, pl.ds(r0, 8), 0:LN] = re
                rm[r, pl.ds(r0, 8), LN:2 * LN] = im

        def wprep(c):
            cols = slice(c * LN, (c + 1) * LN)
            row = jax.lax.broadcasted_iota(jnp.int32, (LN - JB, LN), 0)
            for p, wt in enumerate((wrt, wit)):
                u = pltpu.bitcast(wt[0:J - 1, cols], jnp.uint32)
                even = pltpu.bitcast(u << 16, f32)
                odd = pltpu.bitcast(u & jnp.uint32(0xFFFF0000), f32)
                last = jnp.broadcast_to(wt[J - 1:J, cols].astype(f32), (LN - JB, LN))
                wsa[p, cols, :] = jnp.concatenate([even, jnp.where(row == 0, last, 0.0)], axis=0).T
                wsb[p, cols, :] = jnp.concatenate([odd, jnp.zeros((LN - JB, LN), f32)], axis=0).T

        def stage2(rm):
            return _dot(l2[...], rm[...].reshape(R16 * LN, 2 * LN).astype(bf16), NT)

        def stage3(x, ws, cs, r):
            xr, xi = x[0:LN, r * LN:(r + 1) * LN], x[LN:2 * LN, r * LN:(r + 1) * LN]
            wr = ws[0, pl.ds(r, LN, stride=R16), :]
            wi = ws[1, pl.ds(r, LN, stride=R16), :]
            g = jnp.concatenate([xr * wr - xi * wi, xr * wi + xi * wr], axis=1).astype(bf16)
            c = _dot(l3[r], g, NN)
            cs[r, 0:LN, :] = c[0:LN, 0:LN] - c[LN:2 * LN, LN:2 * LN]
            cs[r, LN:2 * LN, :] = c[LN:2 * LN, 0:LN] + c[0:LN, LN:2 * LN]

        def inv16(cs, half, r0):
            zs = [(cs[r, r0:r0 + 8, :], cs[r, LN + r0:LN + r0 + 8, :]) for r in range(R16)]
            ys = _fft(zs, +1)
            for c in range(R16):
                wall[PU + half, c * LN + r0:c * LN + r0 + 8, 0:LN] = ys[c][0].astype(bf16)
                wall[PU + half, c * LN + r0:c * LN + r0 + 8, LN:2 * LN] = ys[c][1].astype(bf16)

        def stage4(half, k):
            cols = slice(k * LN, (k + 1) * LN)
            y = _dot(l4[half * HD:(half + 1) * HD, :], wall[PU + half, cols, :], NT)
            if half:
                ot[0:HD, cols] += y
                ot[HD:DM, cols] -= y
            else:
                ot[0:HD, cols] = y
                ot[HD:DM, cols] = y

        with scope('w0'):
            c_fd.wait()
        jax.lax.fori_loop(0, 4, stage1, 0)
        wait_all([c_tw])

        def fwd16a(g, carry):
            fwd16(x1a, rma, JA, pl.multiple_of(g * 8, 8))
            return carry

        def fwd16b(g, carry):
            fwd16(x1b, rmb, JB, pl.multiple_of(g * 8, 8))
            return carry

        jax.lax.fori_loop(0, JA // 8, fwd16a, 0)
        jax.lax.fori_loop(0, JB // 8, fwd16b, 0)
        wait_all([c_l2, c_wrt, c_wit, c_l3])
        rma[:, JA:LN, :] = jnp.zeros((R16, LN - JA, 2 * LN), f32)
        rmb[:, JB:LN, :] = jnp.zeros((R16, LN - JB, 2 * LN), f32)
        for c in range(R16):
            wprep(c)
        xa = stage2(rma)
        for r in range(R16):
            stage3(xa, wsa, csa, r)
        xb = stage2(rmb)
        for r in range(R16):
            stage3(xb, wsb, csb, r)
            inv16(csa, 0, r * 8)
        wait_all([c_bxt, c_l4, c_wq])
        for k in range(R16):
            if do_b:
                x_prep(k, R16)
            stage4(0, k)
            inv16(csb, 1, k * 8)
        for k in range(R16):
            if do_b:
                wq_prep(k, R16)
            stage4(1, k)

    if do_a:
        pl.run_scoped(part_a,
                      pltpu.VMEM((2 * JA, S), f32), pltpu.VMEM((2 * JB, S), f32),
                      pltpu.VMEM((R16, LN, 2 * LN), f32), pltpu.VMEM((R16, LN, 2 * LN), f32),
                      pltpu.VMEM((2, S, LN), f32), pltpu.VMEM((2, S, LN), f32),
                      pltpu.VMEM((R16, 2 * LN, LN), f32), pltpu.VMEM((R16, 2 * LN, LN), f32))
    else:
        for c in cps[:-2]:
            c.wait()
        ot[0:DM, :] = jnp.zeros((DM, S), f32)
        if do_b:
            for k in range(R16):
                x_prep(k, R16)
                wq_prep(k, R16)

    def ystep(c, carry):
        for k in range(OCH // LN):
            cols = pl.ds(pl.multiple_of(c * OCH + k * LN, LN), LN)
            ybuf[cols, :] = ot[0:YC, cols].astype(bf16).T
        return carry

    jax.lax.fori_loop(0, S // OCH, ystep, 0)
    c_y = pltpu.make_async_copy(ybuf, out_hbm.at[:, 0:YC], ysem.at[0])
    c_y.start()

    qscale = (D ** -0.5) * math.log2(math.e)

    wchunk(0, 0).wait()
    wchunk(1, 0).wait()

    def qstep(t, carry):
        if do_b:
            rq, rw = S // QPIECES, 2 * CCH // QPIECES
            for j in range(QPIECES):
                x = jnp.concatenate([wall[PX, j * rq:(j + 1) * rq, :], wall[PX + 1, j * rq:(j + 1) * rq, 0:DM - D]], axis=1)
                q_all[t, j * rq:(j + 1) * rq] = (_dot(x, wall[t, 0:DM, :], NN) * qscale).astype(bf16)
                which, off = divmod(j * rw, CCH)
                r0 = pl.multiple_of(t * CCH + off, rw)
                src = (wuk_raw, wuv_raw)[which]
                wall[0:H, pl.ds(DM + which * DC + r0, rw), :] = jnp.swapaxes(src[pl.ds(r0, rw)], 0, 1)

        @pl.when(t + 1 < H)
        def _():
            wchunk(0, t + 1).wait()
            wchunk(1, t + 1).wait()

        return carry

    with scope('P2'):
        jax.lax.fori_loop(0, H, qstep, 0)
    c_ckv.wait()
    c_wot.wait()

    def head(h, carry):
        with scope('head'):
            return head_body(h, carry)

    def head_body(h, carry):
        rr = jax.lax.broadcasted_iota(jnp.int32, (LN, LN), 0)
        cc = jax.lax.broadcasted_iota(jnp.int32, (LN, LN), 1)
        tri = cc <= rr
        neg = -1e30
        kv = {'K': [], 'U': []}
        scores, probs, ctxs = {}, {}, {}

        def rows(name, a, b):
            parts = []
            for lo, arr in sorted(kv[name], key=lambda x: x[0]):
                x, y = max(a, lo), min(b, lo + arr.shape[0])
                if x < y:
                    parts.append(arr[x - lo:y - lo])
            return _cat(parts, 0)

        for tok in HEAD_ORDER.split():
            kind, arg = tok[0], tok[1:]
            if kind in 'KU':
                a, b = map(int, arg.split('-')) if arg else (0, S // TQ)
                w0 = DM + (DC if kind == 'U' else 0)
                w = wall[h, w0:w0 + DC, :]
                kv[kind].append((a * TQ, _dot(ckv[a * TQ:b * TQ, :], w, NN).astype(bf16)))
                continue
            if kind == 'O':
                grp = [int(ch) for ch in arg]
                res = _dot(wot[h], _cat([ctxs[j] for j in grp], 0), NT)
                for n, j in enumerate(grp):
                    ot[DM:2 * DM, j * TQ:(j + 1) * TQ] += res[:, n * TQ:(n + 1) * TQ]
                continue
            i = int(arg)
            r0 = i * TQ
            lm = r0 + LN
            if kind == 'Q':
                q = q_all[h, r0:r0 + TQ, :]
                s = _dot(q, rows('K', 0, lm), NT)
                sx = jnp.where(tri, _dot(q[LN:], rows('K', lm, lm + LN), NT), neg)
                scores[i] = (s, sx)
            elif kind == 'S':
                s, sx = scores.pop(i)
                sd = jnp.where(tri, s[0:LN, r0:lm], neg)
                pt, lt = _softmax_rows(([s[0:LN, 0:r0]] if i else []) + [sd])
                pb, lb = _softmax_rows([s[LN:], sx])
                probs[i] = (jnp.concatenate([_cat(pt, 1), pb[0]], axis=0), pb[1], lt, lb)
            else:
                p, px, lt, lb = probs.pop(i)
                ctx = _dot(p, rows('U', 0, lm), NN)
                cx = _dot(px, rows('U', lm, lm + LN), NN)
                ctxs[i] = jnp.concatenate([ctx[0:LN] * (1.0 / lt), (ctx[LN:] + cx) * (1.0 / lb)],
                                          axis=0).astype(bf16)
        return carry

    if do_b:
        with scope('P3'):
            jax.lax.fori_loop(0, H, head, 0)

    def ocopy(c):
        rows = pl.ds(pl.multiple_of(c * OCH, OCH), OCH)
        return pltpu.make_async_copy(obuf.at[rows], out_hbm.at[rows, YC:2 * DM], osem.at[c])

    def ostep(c, carry):
        for k in range(OCH // LN):
            cols = pl.ds(pl.multiple_of(c * OCH + k * LN, LN), LN)
            obuf[cols, :] = ot[YC:2 * DM, cols].astype(bf16).T
        ocopy(c).start()
        return carry

    jax.lax.fori_loop(0, S // OCH, ostep, 0)
    c_y.wait()
    for c in range(S // OCH):
        ocopy(c).wait()


def _build(do_a=True, do_b=True, scopes=False, order=None):
    global HEAD_ORDER
    if order is not None:
        HEAD_ORDER = order
    def run(A_x, A_w_r, A_w_i, B_x, B_c_kv, B_w_q, B_w_uk, B_w_uv, B_w_o):
        axt = jnp.swapaxes(A_x, 1, 2).reshape(DM, S)
        bxt = jnp.swapaxes(B_x, 1, 2).reshape(DM, S)
        wrt = A_w_r.T
        wit = A_w_i.T
        ckv = B_c_kv.reshape(S, DC)
        wot = jnp.swapaxes(B_w_o, 1, 2)
        tabs = [jnp.asarray(t) for t in _tables()]
        args = (axt, wrt, wit, bxt, ckv, B_w_q, B_w_uk, B_w_uv, wot, *tabs)
        vm = pltpu.VMEM
        scratch = [
            vm((DM, S), bf16), vm((J, S), bf16), vm((J, S), bf16),
            vm(tabs[0].shape, bf16), vm(tabs[1].shape, bf16), vm(tabs[2].shape, f32),
            vm(tabs[3].shape, bf16), vm(tabs[4].shape, bf16),
            vm((DM, S), bf16), vm((S, DC), bf16),
            vm((DM, H, D), bf16),
            vm((DC, H, D), bf16), vm((DC, H, D), bf16), vm((H + 4, DM + 2 * DC, D), bf16),
            vm((H, DM, D), bf16), vm((H, S, D), bf16),
            vm((2 * DM, S), f32), vm((S, YC), bf16), vm((S, 2 * DM - YC), bf16),
            pltpu.SemaphoreType.DMA((15,)), pltpu.SemaphoreType.DMA((2, H)),
            pltpu.SemaphoreType.DMA((S // OCH,)), pltpu.SemaphoreType.DMA((1,)),
        ]
        out = pl.pallas_call(
            functools.partial(_kernel, do_a=do_a, do_b=do_b, scopes=scopes),
            in_specs=[pl.BlockSpec(memory_space=pl.ANY)] * len(args),
            out_specs=pl.BlockSpec(memory_space=pl.ANY),
            out_shape=jax.ShapeDtypeStruct((S, 2 * DM), bf16),
            scratch_shapes=scratch,
            compiler_params=pltpu.CompilerParams(vmem_limit_bytes=120 * 2**20),
        )(*args)
        return out.reshape(1, S, 2 * DM)

    return run


_run = _build()


@jax.jit
def pallas_concat_heads__spectral_gfnet__compressed_kv_cla__prompt_kernel(
    A_x: jax.Array,
    A_w_r: jax.Array,
    A_w_i: jax.Array,
    B_x: jax.Array,
    B_c_kv: jax.Array,
    B_w_q: jax.Array,
    B_w_uk: jax.Array,
    B_w_uv: jax.Array,
    B_w_o: jax.Array,
):
    return _run(A_x, A_w_r, A_w_i, B_x, B_c_kv, B_w_q, B_w_uk, B_w_uv, B_w_o)
```

```python
import contextlib
import functools
import math

import jax
import jax.numpy as jnp
import numpy as np
import jax.experimental.pallas as pl
import jax.experimental.pallas.tpu as pltpu

f32 = jnp.float32
bf16 = jnp.bfloat16

NN = (((1,), (0,)), ((), ()))
NT = (((1,), (1,)), ((), ()))

S = 2048
DM = 448
J = DM // 2 + 1
HD = DM // 2
JA = 120
JB = 112
H = 16
D = 256
DC = 1024
R16 = 16
LN = 128
TQ = 256
CCH = DC // H
PX = H
PU = H + 2
YC = 384
HEAD_ORDER = ('U0-2 K0-8 U2-4 Q4 U4-8 Q1 S1 Q0 S4 V4 Q6 Q3 S0 V0 V1 S6 Q5 S5 S3 V6 Q7 S7 V3 V7 Q2 V5 O0 S2 V2 O76521 O4 O3')
OCH = 512
QPIECES = 16


def _dot(a, b, dn):
    return jax.lax.dot_general(a, b, dn, preferred_element_type=f32)


@functools.lru_cache(maxsize=None)
def _tables():
    j = np.arange(J)[:, None].astype(np.float64)
    d = np.arange(DM)[None, :].astype(np.float64)
    ang = 2.0 * np.pi * ((j * d) % DM) / DM
    cos, sin = np.cos(ang), np.sin(ang)
    ne, no = (J + 1) // 2, J // 2
    fd = np.zeros((2 * JA + 2 * JB, HD), np.float64)
    fd[0:ne] = cos[0::2, 0:HD]
    fd[JA:JA + ne] = -sin[0::2, 0:HD]
    fd[2 * JA:2 * JA + no] = cos[1::2, 0:HD]
    fd[2 * JA + JB:2 * JA + JB + no] = -sin[1::2, 0:HD]

    m = np.arange(LN)[:, None].astype(np.float64)
    l = np.arange(LN)[None, :].astype(np.float64)
    a128 = 2.0 * np.pi * ((m * l) % LN) / LN
    fr, fi = np.cos(a128), -np.sin(a128)
    l2 = np.block([[fr, -fi], [fi, fr]])

    r = np.arange(R16)[:, None].astype(np.float64)
    at = 2.0 * np.pi * (r * l) / S
    tw = np.stack([np.cos(at), -np.sin(at)])
    tw = np.broadcast_to(tw[:, :, None, :], (2, R16, 8, LN)).copy()

    l3 = np.zeros((R16, 2 * LN, LN), np.float64)
    for rr in range(R16):
        a3 = 2.0 * np.pi * ((m * (rr + R16 * l)) % S) / S
        l3[rr] = np.concatenate([np.cos(a3), np.sin(a3)], axis=0)

    cj = np.full((J,), 2.0)
    cj[0] = 1.0
    cj[J - 1] = 1.0
    scale = cj[None, :] / float(S * DM)
    cr, ci = cos.T[0:HD] * scale, -sin.T[0:HD] * scale
    l4 = np.zeros((2, HD, 2 * LN), np.float64)
    l4[0, :, 0:ne] = cr[:, 0::2]
    l4[0, :, LN:LN + ne] = ci[:, 0::2]
    l4[1, :, 0:no] = cr[:, 1::2]
    l4[1, :, LN:LN + no] = ci[:, 1::2]

    cast = lambda a, dt: np.asarray(a, np.float32).astype(dt)
    return (cast(fd, bf16), cast(l2, bf16), cast(tw, np.float32), cast(l3, bf16),
            cast(l4.reshape(2 * HD, 2 * LN), bf16))


def _cmul_const(z, k, n, sign):
    re, im = z
    k = k % n
    if k == 0:
        return re, im
    if 4 * k == n:
        return (-im, re) if sign > 0 else (im, -re)
    if 8 * k == n:
        c = math.sqrt(0.5)
        return ((re - im) * c, (re + im) * c) if sign > 0 else ((re + im) * c, (im - re) * c)
    if 8 * k == 3 * n:
        c = math.sqrt(0.5)
        return ((re + im) * (-c), (re - im) * c) if sign > 0 else ((im - re) * c, (re + im) * (-c))
    c = math.cos(2.0 * math.pi * k / n)
    s = sign * math.sin(2.0 * math.pi * k / n)
    return re * c - im * s, re * s + im * c


def _fft(zs, sign):
    n = len(zs)
    if n == 1:
        return zs
    ev = _fft(zs[0::2], sign)
    od = _fft(zs[1::2], sign)
    out = [None] * n
    for k in range(n // 2):
        if 4 * k == n:
            (er, ei), (orr, oi) = ev[k], od[k]
            if sign > 0:
                out[k] = (er - oi, ei + orr)
                out[k + n // 2] = (er + oi, ei - orr)
            else:
                out[k] = (er + oi, ei - orr)
                out[k + n // 2] = (er - oi, ei + orr)
            continue
        tr, ti = _cmul_const(od[k], k, n, sign)
        er, ei = ev[k]
        out[k] = (er + tr, ei + ti)
        out[k + n // 2] = (er - tr, ei - ti)
    return out


def _softmax_rows(segs):
    m = functools.reduce(jnp.maximum, [jnp.max(sg, axis=1, keepdims=True) for sg in segs])
    ps = [jnp.exp2(sg - m).astype(bf16) for sg in segs]
    l = functools.reduce(jnp.add, [jnp.sum(p.astype(f32), axis=1, keepdims=True) for p in ps])
    return ps, l


def _cat(parts, axis):
    return jnp.concatenate(parts, axis=axis) if len(parts) > 1 else parts[0]


def _kernel(axt_hbm, wrt_hbm, wit_hbm, bxt_hbm, ckv_hbm, wq_hbm, wuk_hbm, wuv_hbm, wot_hbm,
            fd_hbm, l2_hbm, tw_hbm, l3_hbm, l4_hbm,
            out_hbm,
            axt, wrt, wit, fd, l2, tw, l3, l4,
            bxt, ckv, wq_raw, wuk_raw, wuv_raw, wall, wot, q_all,
            ot, ybuf, obuf, sem, wsem, osem, ysem, *, do_a, do_b, scopes):
    scope = jax.named_scope if scopes else (lambda name: contextlib.nullcontext())
    XC = S // 4
    simple = ([(fd_hbm, fd)]
              + [(axt_hbm.at[:, c * XC:(c + 1) * XC], axt.at[:, c * XC:(c + 1) * XC]) for c in range(4)]
              + [(tw_hbm, tw), (l2_hbm, l2), (wrt_hbm, wrt), (wit_hbm, wit),
                 (l3_hbm, l3), (bxt_hbm, bxt), (l4_hbm, l4), (wq_hbm, wq_raw), (ckv_hbm, ckv), (wot_hbm, wot)])
    cps = [pltpu.make_async_copy(s, d, sem.at[i]) for i, (s, d) in enumerate(simple)]
    c_fd = cps[0]
    (c_tw, c_l2, c_wrt, c_wit, c_l3, c_bxt, c_l4, c_wq, c_ckv, c_wot) = cps[5:]

    def wchunk(which, t):
        src, dst = ((wuk_hbm, wuk_raw), (wuv_hbm, wuv_raw))[which]
        return pltpu.make_async_copy(src.at[pl.ds(t * CCH, CCH)], dst.at[pl.ds(t * CCH, CCH)], wsem.at[which, t])

    def issue(lo, hi):
        def body(i, carry):
            for k in range(lo, hi):
                pl.when(i == k)(cps[k].start)
            return carry
        jax.lax.fori_loop(lo, hi, body, 0)

    def wait_all(cs):
        def body(i, carry):
            for k, c in enumerate(cs):
                pl.when(i == k)(c.wait)
            return carry
        jax.lax.fori_loop(0, len(cs), body, 0)

    def issue_w(t, carry):
        wchunk(0, t).start()
        wchunk(1, t).start()
        return carry

    issue(0, len(cps) - 2)
    jax.lax.fori_loop(0, H, issue_w, 0)
    issue(len(cps) - 2, len(cps))

    def zero(i, carry):
        ot[pl.ds(pl.multiple_of(DM + i * 64, 64), 64), :] = jnp.zeros((64, S), f32)
        return carry

    jax.lax.fori_loop(0, DM // 64, zero, 0)

    def x_prep(k, n):
        w = S // n
        wall[PX, k * w:(k + 1) * w, :] = bxt[0:D, k * w:(k + 1) * w].T
        wall[PX + 1, k * w:(k + 1) * w, 0:DM - D] = bxt[D:DM, k * w:(k + 1) * w].T

    def wq_prep(k, n):
        g = DM // 16
        lo, hi = 16 * (k * g // n), 16 * ((k + 1) * g // n)
        wall[0:H, lo:hi, :] = jnp.swapaxes(wq_raw[lo:hi], 0, 1)

    def part_a(x1a, x1b, rma, rmb, wsa, wsb, csa, csb):
        def stage1(c, carry):
            cols = pl.ds(pl.multiple_of(c * XC, XC), XC)
            pltpu.make_async_copy(axt_hbm.at[:, cols], axt.at[:, cols], sem.at[1 + c]).wait()
            lo, hi = axt[0:HD, cols].astype(f32), axt[HD:DM, cols].astype(f32)
            x1a[:, cols] = _dot(fd[0:2 * JA, :], (lo + hi).astype(bf16), NN)
            x1b[:, cols] = _dot(fd[2 * JA:, :], (lo - hi).astype(bf16), NN)
            return carry

        def fwd16(x1, rm, n, r0):
            zs = [(x1[pl.ds(r0, 8), c * LN:(c + 1) * LN], x1[pl.ds(n + r0, 8), c * LN:(c + 1) * LN])
                  for c in range(R16)]
            ys = _fft(zs, -1)
            for r in range(R16):
                re, im = ys[r]
                if r:
                    tr, ti = tw[0, r], tw[1, r]
                    re, im = re * tr - im * ti, re * ti + im * tr
                rm[r, pl.ds(r0, 8), 0:LN] = re
                rm[r, pl.ds(r0, 8), LN:2 * LN] = im

        def wprep(c):
            cols = slice(c * LN, (c + 1) * LN)
            row = jax.lax.broadcasted_iota(jnp.int32, (LN - JB, LN), 0)
            for p, wt in enumerate((wrt, wit)):
                u = pltpu.bitcast(wt[0:J - 1, cols], jnp.uint32)
                even = pltpu.bitcast(u << 16, f32)
                odd = pltpu.bitcast(u & jnp.uint32(0xFFFF0000), f32)
                last = jnp.broadcast_to(wt[J - 1:J, cols].astype(f32), (LN - JB, LN))
                wsa[p, cols, :] = jnp.concatenate([even, jnp.where(row == 0, last, 0.0)], axis=0).T
                wsb[p, cols, :] = jnp.concatenate([odd, jnp.zeros((LN - JB, LN), f32)], axis=0).T

        def stage2(rm):
            return _dot(l2[...], rm[...].reshape(R16 * LN, 2 * LN).astype(bf16), NT)

        def stage3(x, ws, cs, r):
            xr, xi = x[0:LN, r * LN:(r + 1) * LN], x[LN:2 * LN, r * LN:(r + 1) * LN]
            wr = ws[0, pl.ds(r, LN, stride=R16), :]
            wi = ws[1, pl.ds(r, LN, stride=R16), :]
            g = jnp.concatenate([xr * wr - xi * wi, xr * wi + xi * wr], axis=1).astype(bf16)
            c = _dot(l3[r], g, NN)
            cs[r, 0:LN, :] = c[0:LN, 0:LN] - c[LN:2 * LN, LN:2 * LN]
            cs[r, LN:2 * LN, :] = c[LN:2 * LN, 0:LN] + c[0:LN, LN:2 * LN]

        def inv16(cs, half, r0):
            zs = [(cs[r, r0:r0 + 8, :], cs[r, LN + r0:LN + r0 + 8, :]) for r in range(R16)]
            ys = _fft(zs, +1)
            for c in range(R16):
                wall[PU + half, c * LN + r0:c * LN + r0 + 8, 0:LN] = ys[c][0].astype(bf16)
                wall[PU + half, c * LN + r0:c * LN + r0 + 8, LN:2 * LN] = ys[c][1].astype(bf16)

        def stage4(half, k):
            cols = slice(k * LN, (k + 1) * LN)
            y = _dot(l4[half * HD:(half + 1) * HD, :], wall[PU + half, cols, :], NT)
            if half:
                ot[0:HD, cols] += y
                ot[HD:DM, cols] -= y
            else:
                ot[0:HD, cols] = y
                ot[HD:DM, cols] = y

        with scope('w0'):
            c_fd.wait()
        jax.lax.fori_loop(0, 4, stage1, 0)
        wait_all([c_tw])

        def fwd16a(g, carry):
            fwd16(x1a, rma, JA, pl.multiple_of(g * 8, 8))
            return carry

        def fwd16b(g, carry):
            fwd16(x1b, rmb, JB, pl.multiple_of(g * 8, 8))
            return carry

        jax.lax.fori_loop(0, JA // 8, fwd16a, 0)
        jax.lax.fori_loop(0, JB // 8, fwd16b, 0)
        wait_all([c_l2])
        rma[:, JA:LN, :] = jnp.zeros((R16, LN - JA, 2 * LN), f32)
        rmb[:, JB:LN, :] = jnp.zeros((R16, LN - JB, 2 * LN), f32)
        xa = stage2(rma)
        xb = stage2(rmb)
        wait_all([c_wrt, c_wit, c_l3])
        for c in range(R16):
            wprep(c)
        for r in range(R16):
            stage3(xa, wsa, csa, r)
        for r in range(R16):
            stage3(xb, wsb, csb, r)
            inv16(csa, 0, r * 8)
        wait_all([c_bxt, c_l4])
        for k in range(R16):
            if do_b:
                x_prep(k, R16)
            stage4(0, k)
            inv16(csb, 1, k * 8)
        wait_all([c_wq])
        for k in range(R16):
            if do_b:
                wq_prep(k, R16)
            stage4(1, k)

    if do_a:
        pl.run_scoped(part_a,
                      pltpu.VMEM((2 * JA, S), f32), pltpu.VMEM((2 * JB, S), f32),
                      pltpu.VMEM((R16, LN, 2 * LN), f32), pltpu.VMEM((R16, LN, 2 * LN), f32),
                      pltpu.VMEM((2, S, LN), f32), pltpu.VMEM((2, S, LN), f32),
                      pltpu.VMEM((R16, 2 * LN, LN), f32), pltpu.VMEM((R16, 2 * LN, LN), f32))
    else:
        for c in cps[:-2]:
            c.wait()
        ot[0:DM, :] = jnp.zeros((DM, S), f32)
        if do_b:
            for k in range(R16):
                x_prep(k, R16)
                wq_prep(k, R16)

    def ystep(c, carry):
        for k in range(OCH // LN):
            cols = pl.ds(pl.multiple_of(c * OCH + k * LN, LN), LN)
            ybuf[cols, :] = ot[0:YC, cols].astype(bf16).T
        return carry

    jax.lax.fori_loop(0, S // OCH, ystep, 0)
    c_y = pltpu.make_async_copy(ybuf, out_hbm.at[:, 0:YC], ysem.at[0])
    c_y.start()

    qscale = (D ** -0.5) * math.log2(math.e)

    wchunk(0, 0).wait()
    wchunk(1, 0).wait()

    def qstep(t, carry):
        if do_b:
            rq, rw = S // QPIECES, 2 * CCH // QPIECES
            for j in range(QPIECES):
                x = jnp.concatenate([wall[PX, j * rq:(j + 1) * rq, :], wall[PX + 1, j * rq:(j + 1) * rq, 0:DM - D]], axis=1)
                q_all[t, j * rq:(j + 1) * rq] = (_dot(x, wall[t, 0:DM, :], NN) * qscale).astype(bf16)
                which, off = divmod(j * rw, CCH)
                r0 = pl.multiple_of(t * CCH + off, rw)
                src = (wuk_raw, wuv_raw)[which]
                wall[0:H, pl.ds(DM + which * DC + r0, rw), :] = jnp.swapaxes(src[pl.ds(r0, rw)], 0, 1)

        @pl.when(t + 1 < H)
        def _():
            wchunk(0, t + 1).wait()
            wchunk(1, t + 1).wait()

        return carry

    with scope('P2'):
        jax.lax.fori_loop(0, H, qstep, 0)
    c_ckv.wait()
    c_wot.wait()

    def head(h, carry):
        with scope('head'):
            return head_body(h, carry)

    def head_body(h, carry):
        rr = jax.lax.broadcasted_iota(jnp.int32, (LN, LN), 0)
        cc = jax.lax.broadcasted_iota(jnp.int32, (LN, LN), 1)
        tri = cc <= rr
        neg = -1e30
        kv = {'K': [], 'U': []}
        scores, probs, ctxs = {}, {}, {}

        def rows(name, a, b):
            parts = []
            for lo, arr in sorted(kv[name], key=lambda x: x[0]):
                x, y = max(a, lo), min(b, lo + arr.shape[0])
                if x < y:
                    parts.append(arr[x - lo:y - lo])
            return _cat(parts, 0)

        for tok in HEAD_ORDER.split():
            kind, arg = tok[0], tok[1:]
            if kind in 'KU':
                a, b = map(int, arg.split('-')) if arg else (0, S // TQ)
                w0 = DM + (DC if kind == 'U' else 0)
                w = wall[h, w0:w0 + DC, :]
                kv[kind].append((a * TQ, _dot(ckv[a * TQ:b * TQ, :], w, NN).astype(bf16)))
                continue
            if kind == 'O':
                grp = [int(ch) for ch in arg]
                res = _dot(wot[h], _cat([ctxs[j] for j in grp], 0), NT)
                for n, j in enumerate(grp):
                    ot[DM:2 * DM, j * TQ:(j + 1) * TQ] += res[:, n * TQ:(n + 1) * TQ]
                continue
            i = int(arg)
            r0 = i * TQ
            lm = r0 + LN
            if kind == 'Q':
                q = q_all[h, r0:r0 + TQ, :]
                s = _dot(q, rows('K', 0, lm), NT)
                sx = jnp.where(tri, _dot(q[LN:], rows('K', lm, lm + LN), NT), neg)
                scores[i] = (s, sx)
            elif kind == 'S':
                s, sx = scores.pop(i)
                sd = jnp.where(tri, s[0:LN, r0:lm], neg)
                pt, lt = _softmax_rows(([s[0:LN, 0:r0]] if i else []) + [sd])
                pb, lb = _softmax_rows([s[LN:], sx])
                probs[i] = (jnp.concatenate([_cat(pt, 1), pb[0]], axis=0), pb[1], lt, lb)
            else:
                p, px, lt, lb = probs.pop(i)
                ctx = _dot(p, rows('U', 0, lm), NN)
                cx = _dot(px, rows('U', lm, lm + LN), NN)
                ctxs[i] = jnp.concatenate([ctx[0:LN] * (1.0 / lt), (ctx[LN:] + cx) * (1.0 / lb)],
                                          axis=0).astype(bf16)
        return carry

    if do_b:
        with scope('P3'):
            jax.lax.fori_loop(0, H, head, 0)

    def ocopy(c):
        rows = pl.ds(pl.multiple_of(c * OCH, OCH), OCH)
        return pltpu.make_async_copy(obuf.at[rows], out_hbm.at[rows, YC:2 * DM], osem.at[c])

    def ostep(c, carry):
        for k in range(OCH // LN):
            cols = pl.ds(pl.multiple_of(c * OCH + k * LN, LN), LN)
            obuf[cols, :] = ot[YC:2 * DM, cols].astype(bf16).T
        ocopy(c).start()
        return carry

    jax.lax.fori_loop(0, S // OCH, ostep, 0)
    c_y.wait()
    for c in range(S // OCH):
        ocopy(c).wait()


def _build(do_a=True, do_b=True, scopes=False, order=None):
    global HEAD_ORDER
    if order is not None:
        HEAD_ORDER = order
    def run(A_x, A_w_r, A_w_i, B_x, B_c_kv, B_w_q, B_w_uk, B_w_uv, B_w_o):
        axt = jnp.swapaxes(A_x, 1, 2).reshape(DM, S)
        bxt = jnp.swapaxes(B_x, 1, 2).reshape(DM, S)
        wrt = A_w_r.T
        wit = A_w_i.T
        ckv = B_c_kv.reshape(S, DC)
        wot = jnp.swapaxes(B_w_o, 1, 2)
        tabs = [jnp.asarray(t) for t in _tables()]
        args = (axt, wrt, wit, bxt, ckv, B_w_q, B_w_uk, B_w_uv, wot, *tabs)
        vm = pltpu.VMEM
        scratch = [
            vm((DM, S), bf16), vm((J, S), bf16), vm((J, S), bf16),
            vm(tabs[0].shape, bf16), vm(tabs[1].shape, bf16), vm(tabs[2].shape, f32),
            vm(tabs[3].shape, bf16), vm(tabs[4].shape, bf16),
            vm((DM, S), bf16), vm((S, DC), bf16),
            vm((DM, H, D), bf16),
            vm((DC, H, D), bf16), vm((DC, H, D), bf16), vm((H + 4, DM + 2 * DC, D), bf16),
            vm((H, DM, D), bf16), vm((H, S, D), bf16),
            vm((2 * DM, S), f32), vm((S, YC), bf16), vm((S, 2 * DM - YC), bf16),
            pltpu.SemaphoreType.DMA((15,)), pltpu.SemaphoreType.DMA((2, H)),
            pltpu.SemaphoreType.DMA((S // OCH,)), pltpu.SemaphoreType.DMA((1,)),
        ]
        out = pl.pallas_call(
            functools.partial(_kernel, do_a=do_a, do_b=do_b, scopes=scopes),
            in_specs=[pl.BlockSpec(memory_space=pl.ANY)] * len(args),
            out_specs=pl.BlockSpec(memory_space=pl.ANY),
            out_shape=jax.ShapeDtypeStruct((S, 2 * DM), bf16),
            scratch_shapes=scratch,
            compiler_params=pltpu.CompilerParams(vmem_limit_bytes=120 * 2**20),
        )(*args)
        return out.reshape(1, S, 2 * DM)

    return run


_run = _build()


@jax.jit
def pallas_concat_heads__spectral_gfnet__compressed_kv_cla__prompt_kernel(
    A_x: jax.Array,
    A_w_r: jax.Array,
    A_w_i: jax.Array,
    B_x: jax.Array,
    B_c_kv: jax.Array,
    B_w_q: jax.Array,
    B_w_uk: jax.Array,
    B_w_uv: jax.Array,
    B_w_o: jax.Array,
):
    return _run(A_x, A_w_r, A_w_i, B_x, B_c_kv, B_w_q, B_w_uk, B_w_uv, B_w_o)
```

```python
import contextlib
import functools
import math

import jax
import jax.numpy as jnp
import numpy as np
import jax.experimental.pallas as pl
import jax.experimental.pallas.tpu as pltpu

f32 = jnp.float32
bf16 = jnp.bfloat16

NN = (((1,), (0,)), ((), ()))
NT = (((1,), (1,)), ((), ()))

S = 2048
DM = 448
J = DM // 2 + 1
HD = DM // 2
JA = 120
JB = 112
H = 16
D = 256
DC = 1024
R16 = 16
LN = 128
TQ = 256
CCH = DC // H
PX = H
PU = H + 2
YC = 384
HEAD_ORDER = ('U0-2 K0-8 U2-4 Q4 U4-8 Q1 S1 Q0 S4 V4 Q6 Q3 S0 V0 V1 S6 Q5 S5 S3 V6 Q7 S7 V3 V7 Q2 V5 O0 S2 V2 O76521 O4 O3')
OCH = 512
QHEADS = 2
QPIECES = 16


def _dot(a, b, dn):
    return jax.lax.dot_general(a, b, dn, preferred_element_type=f32)


@functools.lru_cache(maxsize=None)
def _tables():
    j = np.arange(J)[:, None].astype(np.float64)
    d = np.arange(DM)[None, :].astype(np.float64)
    ang = 2.0 * np.pi * ((j * d) % DM) / DM
    cos, sin = np.cos(ang), np.sin(ang)
    ne, no = (J + 1) // 2, J // 2
    fd = np.zeros((2 * JA + 2 * JB, HD), np.float64)
    fd[0:ne] = cos[0::2, 0:HD]
    fd[JA:JA + ne] = -sin[0::2, 0:HD]
    fd[2 * JA:2 * JA + no] = cos[1::2, 0:HD]
    fd[2 * JA + JB:2 * JA + JB + no] = -sin[1::2, 0:HD]

    m = np.arange(LN)[:, None].astype(np.float64)
    l = np.arange(LN)[None, :].astype(np.float64)
    a128 = 2.0 * np.pi * ((m * l) % LN) / LN
    fr, fi = np.cos(a128), -np.sin(a128)
    l2 = np.block([[fr, -fi], [fi, fr]])

    r = np.arange(R16)[:, None].astype(np.float64)
    at = 2.0 * np.pi * (r * l) / S
    tw = np.stack([np.cos(at), -np.sin(at)])
    tw = np.broadcast_to(tw[:, :, None, :], (2, R16, 8, LN)).copy()

    l3 = np.zeros((R16, 2 * LN, LN), np.float64)
    for rr in range(R16):
        a3 = 2.0 * np.pi * ((m * (rr + R16 * l)) % S) / S
        l3[rr] = np.concatenate([np.cos(a3), np.sin(a3)], axis=0)

    cj = np.full((J,), 2.0)
    cj[0] = 1.0
    cj[J - 1] = 1.0
    scale = cj[None, :] / float(S * DM)
    cr, ci = cos.T[0:HD] * scale, -sin.T[0:HD] * scale
    l4 = np.zeros((2, HD, 2 * LN), np.float64)
    l4[0, :, 0:ne] = cr[:, 0::2]
    l4[0, :, LN:LN + ne] = ci[:, 0::2]
    l4[1, :, 0:no] = cr[:, 1::2]
    l4[1, :, LN:LN + no] = ci[:, 1::2]

    cast = lambda a, dt: np.asarray(a, np.float32).astype(dt)
    return (cast(fd, bf16), cast(l2, bf16), cast(tw, np.float32), cast(l3, bf16),
            cast(l4.reshape(2 * HD, 2 * LN), bf16))


def _cmul_const(z, k, n, sign):
    re, im = z
    k = k % n
    if k == 0:
        return re, im
    if 4 * k == n:
        return (-im, re) if sign > 0 else (im, -re)
    if 8 * k == n:
        c = math.sqrt(0.5)
        return ((re - im) * c, (re + im) * c) if sign > 0 else ((re + im) * c, (im - re) * c)
    if 8 * k == 3 * n:
        c = math.sqrt(0.5)
        return ((re + im) * (-c), (re - im) * c) if sign > 0 else ((im - re) * c, (re + im) * (-c))
    c = math.cos(2.0 * math.pi * k / n)
    s = sign * math.sin(2.0 * math.pi * k / n)
    return re * c - im * s, re * s + im * c


def _fft(zs, sign):
    n = len(zs)
    if n == 1:
        return zs
    ev = _fft(zs[0::2], sign)
    od = _fft(zs[1::2], sign)
    out = [None] * n
    for k in range(n // 2):
        if 4 * k == n:
            (er, ei), (orr, oi) = ev[k], od[k]
            if sign > 0:
                out[k] = (er - oi, ei + orr)
                out[k + n // 2] = (er + oi, ei - orr)
            else:
                out[k] = (er + oi, ei - orr)
                out[k + n // 2] = (er - oi, ei + orr)
            continue
        tr, ti = _cmul_const(od[k], k, n, sign)
        er, ei = ev[k]
        out[k] = (er + tr, ei + ti)
        out[k + n // 2] = (er - tr, ei - ti)
    return out


def _softmax_rows(segs):
    m = functools.reduce(jnp.maximum, [jnp.max(sg, axis=1, keepdims=True) for sg in segs])
    ps = [jnp.exp2(sg - m).astype(bf16) for sg in segs]
    l = functools.reduce(jnp.add, [jnp.sum(p.astype(f32), axis=1, keepdims=True) for p in ps])
    return ps, l


def _cat(parts, axis):
    return jnp.concatenate(parts, axis=axis) if len(parts) > 1 else parts[0]


def _kernel(axt_hbm, wrt_hbm, wit_hbm, bxt_hbm, ckv_hbm, wq_hbm, wuk_hbm, wuv_hbm, wot_hbm,
            fd_hbm, l2_hbm, tw_hbm, l3_hbm, l4_hbm,
            out_hbm,
            axt, wrt, wit, fd, l2, tw, l3, l4,
            bxt, ckv, wq_raw, wuk_raw, wuv_raw, wall, wot, q_all,
            ot, ybuf, obuf, sem, wsem, osem, ysem, *, do_a, do_b, scopes):
    scope = jax.named_scope if scopes else (lambda name: contextlib.nullcontext())
    XC = S // 4
    simple = ([(fd_hbm, fd)]
              + [(axt_hbm.at[:, c * XC:(c + 1) * XC], axt.at[:, c * XC:(c + 1) * XC]) for c in range(4)]
              + [(tw_hbm, tw), (l2_hbm, l2), (wrt_hbm, wrt), (wit_hbm, wit),
                 (l3_hbm, l3), (bxt_hbm, bxt), (l4_hbm, l4), (wq_hbm, wq_raw), (ckv_hbm, ckv), (wot_hbm, wot)])
    cps = [pltpu.make_async_copy(s, d, sem.at[i]) for i, (s, d) in enumerate(simple)]
    c_fd = cps[0]
    (c_tw, c_l2, c_wrt, c_wit, c_l3, c_bxt, c_l4, c_wq, c_ckv, c_wot) = cps[5:]

    def wchunk(which, t):
        src, dst = ((wuk_hbm, wuk_raw), (wuv_hbm, wuv_raw))[which]
        return pltpu.make_async_copy(src.at[pl.ds(t * CCH, CCH)], dst.at[pl.ds(t * CCH, CCH)], wsem.at[which, t])

    def issue(lo, hi):
        def body(i, carry):
            for k in range(lo, hi):
                pl.when(i == k)(cps[k].start)
            return carry
        jax.lax.fori_loop(lo, hi, body, 0)

    def wait_all(cs):
        def body(i, carry):
            for k, c in enumerate(cs):
                pl.when(i == k)(c.wait)
            return carry
        jax.lax.fori_loop(0, max(2, len(cs)), body, 0)

    def issue_w(t, carry):
        wchunk(0, t).start()
        wchunk(1, t).start()
        return carry

    with scope('issue'):
        issue(0, len(cps) - 2)
        jax.lax.fori_loop(0, H, issue_w, 0)
        issue(len(cps) - 2, len(cps))

    def zero(i, carry):
        ot[pl.ds(pl.multiple_of(DM + i * 64, 64), 64), :] = jnp.zeros((64, S), f32)
        return carry

    with scope('zero'):
        jax.lax.fori_loop(0, DM // 64, zero, 0)

    def x_prep(k, n):
        w = S // n
        wall[PX, k * w:(k + 1) * w, :] = bxt[0:D, k * w:(k + 1) * w].T
        wall[PX + 1, k * w:(k + 1) * w, 0:DM - D] = bxt[D:DM, k * w:(k + 1) * w].T

    def wq_prep(k, n):
        g = DM // 16
        lo, hi = 16 * (k * g // n), 16 * ((k + 1) * g // n)
        wall[0:H, lo:hi, :] = jnp.swapaxes(wq_raw[lo:hi], 0, 1)

    def part_a(x1a, x1b, rma, rmb, wsa, wsb, csa, csb):
        def stage1(c, carry):
            cols = pl.ds(pl.multiple_of(c * XC, XC), XC)
            pltpu.make_async_copy(axt_hbm.at[:, cols], axt.at[:, cols], sem.at[1 + c]).wait()
            lo, hi = axt[0:HD, cols].astype(f32), axt[HD:DM, cols].astype(f32)
            x1a[:, cols] = _dot(fd[0:2 * JA, :], (lo + hi).astype(bf16), NN)
            x1b[:, cols] = _dot(fd[2 * JA:, :], (lo - hi).astype(bf16), NN)
            return carry

        def fwd16(x1, rm, n, r0):
            zs = [(x1[pl.ds(r0, 8), c * LN:(c + 1) * LN], x1[pl.ds(n + r0, 8), c * LN:(c + 1) * LN])
                  for c in range(R16)]
            ys = _fft(zs, -1)
            for r in range(R16):
                re, im = ys[r]
                if r:
                    tr, ti = tw[0, r], tw[1, r]
                    re, im = re * tr - im * ti, re * ti + im * tr
                rm[r, pl.ds(r0, 8), 0:LN] = re
                rm[r, pl.ds(r0, 8), LN:2 * LN] = im

        def wprep(c):
            cols = slice(c * LN, (c + 1) * LN)
            row = jax.lax.broadcasted_iota(jnp.int32, (LN - JB, LN), 0)
            for p, wt in enumerate((wrt, wit)):
                u = pltpu.bitcast(wt[0:J - 1, cols], jnp.uint32)
                even = pltpu.bitcast(u << 16, f32)
                odd = pltpu.bitcast(u & jnp.uint32(0xFFFF0000), f32)
                last = jnp.broadcast_to(wt[J - 1:J, cols].astype(f32), (LN - JB, LN))
                wsa[p, cols, :] = jnp.concatenate([even, jnp.where(row == 0, last, 0.0)], axis=0).T
                wsb[p, cols, :] = jnp.concatenate([odd, jnp.zeros((LN - JB, LN), f32)], axis=0).T

        def stage2(rm):
            return _dot(l2[...], rm[...].reshape(R16 * LN, 2 * LN).astype(bf16), NT)

        def stage3(x, ws, cs, r):
            xr, xi = x[0:LN, r * LN:(r + 1) * LN], x[LN:2 * LN, r * LN:(r + 1) * LN]
            wr = ws[0, pl.ds(r, LN, stride=R16), :]
            wi = ws[1, pl.ds(r, LN, stride=R16), :]
            g = jnp.concatenate([xr * wr - xi * wi, xr * wi + xi * wr], axis=1).astype(bf16)
            c = _dot(l3[r], g, NN)
            cs[r, 0:LN, :] = c[0:LN, 0:LN] - c[LN:2 * LN, LN:2 * LN]
            cs[r, LN:2 * LN, :] = c[LN:2 * LN, 0:LN] + c[0:LN, LN:2 * LN]

        def inv16(cs, half, r0):
            zs = [(cs[r, r0:r0 + 8, :], cs[r, LN + r0:LN + r0 + 8, :]) for r in range(R16)]
            ys = _fft(zs, +1)
            for c in range(R16):
                wall[PU + half, c * LN + r0:c * LN + r0 + 8, 0:LN] = ys[c][0].astype(bf16)
                wall[PU + half, c * LN + r0:c * LN + r0 + 8, LN:2 * LN] = ys[c][1].astype(bf16)

        def stage4(half, k):
            cols = slice(k * LN, (k + 1) * LN)
            y = _dot(l4[half * HD:(half + 1) * HD, :], wall[PU + half, cols, :], NT)
            if half:
                ot[0:HD, cols] += y
                ot[HD:DM, cols] -= y
            else:
                ot[0:HD, cols] = y
                ot[HD:DM, cols] = y

        with scope('w0'):
            c_fd.wait()
        with scope('S1'):
            jax.lax.fori_loop(0, 4, stage1, 0)
        with scope('wt_tw'):
            wait_all([c_tw])

        def fwd16a(g, carry):
            fwd16(x1a, rma, JA, pl.multiple_of(g * 8, 8))
            return carry

        def fwd16b(g, carry):
            fwd16(x1b, rmb, JB, pl.multiple_of(g * 8, 8))
            return carry

        with scope('F16'):
            jax.lax.fori_loop(0, JA // 8, fwd16a, 0)
            jax.lax.fori_loop(0, JB // 8, fwd16b, 0)
        with scope('wt_l2'):
            wait_all([c_l2])
        rma[:, JA:LN, :] = jnp.zeros((R16, LN - JA, 2 * LN), f32)
        rmb[:, JB:LN, :] = jnp.zeros((R16, LN - JB, 2 * LN), f32)
        xa = stage2(rma)
        xb = stage2(rmb)
        with scope('wt_W'):
            wait_all([c_wrt, c_wit, c_l3])
        for c in range(R16):
            wprep(c)
        for r in range(R16):
            stage3(xa, wsa, csa, r)
        for r in range(R16):
            stage3(xb, wsb, csb, r)
            inv16(csa, 0, r * 8)
        with scope('wt_x'):
            wait_all([c_bxt, c_l4])
        for k in range(R16):
            if do_b:
                x_prep(k, R16)
            stage4(0, k)
            inv16(csb, 1, k * 8)
        with scope('wt_wq'):
            wait_all([c_wq])
        for k in range(R16):
            if do_b:
                wq_prep(k, R16)
            stage4(1, k)

    if do_a:
        pl.run_scoped(part_a,
                      pltpu.VMEM((2 * JA, S), f32), pltpu.VMEM((2 * JB, S), f32),
                      pltpu.VMEM((R16, LN, 2 * LN), f32), pltpu.VMEM((R16, LN, 2 * LN), f32),
                      pltpu.VMEM((2, S, LN), f32), pltpu.VMEM((2, S, LN), f32),
                      pltpu.VMEM((R16, 2 * LN, LN), f32), pltpu.VMEM((R16, 2 * LN, LN), f32))
    else:
        for c in cps[:-2]:
            c.wait()
        ot[0:DM, :] = jnp.zeros((DM, S), f32)
        if do_b:
            for k in range(R16):
                x_prep(k, R16)
                wq_prep(k, R16)

    def ystep(c, carry):
        for k in range(OCH // LN):
            cols = pl.ds(pl.multiple_of(c * OCH + k * LN, LN), LN)
            ybuf[cols, :] = ot[0:YC, cols].astype(bf16).T
        return carry

    with scope('Y'):
        jax.lax.fori_loop(0, S // OCH, ystep, 0)
    c_y = pltpu.make_async_copy(ybuf, out_hbm.at[:, 0:YC], ysem.at[0])
    c_y.start()

    qscale = (D ** -0.5) * math.log2(math.e)

    with scope('wt_c0'):
        for u in range(QHEADS):
            wchunk(0, u).wait()
            wchunk(1, u).wait()

    def qstep(tt, carry):
        if do_b:
            rq, rw = S // QPIECES, 2 * CCH // QPIECES
            for u in range(QHEADS):
                t = tt * QHEADS + u
                for j in range(QPIECES):
                    x = jnp.concatenate([wall[PX, j * rq:(j + 1) * rq, :], wall[PX + 1, j * rq:(j + 1) * rq, 0:DM - D]],
                                        axis=1)
                    q_all[t, j * rq:(j + 1) * rq] = (_dot(x, wall[t, 0:DM, :], NN) * qscale).astype(bf16)
                    which, off = divmod(j * rw, CCH)
                    r0 = pl.multiple_of(t * CCH + off, rw)
                    src = (wuk_raw, wuv_raw)[which]
                    wall[0:H, pl.ds(DM + which * DC + r0, rw), :] = jnp.swapaxes(src[pl.ds(r0, rw)], 0, 1)

        @pl.when(tt + 1 < H // QHEADS)
        def _():
            for u in range(QHEADS):
                wchunk(0, (tt + 1) * QHEADS + u).wait()
                wchunk(1, (tt + 1) * QHEADS + u).wait()

        return carry

    with scope('P2'):
        jax.lax.fori_loop(0, H // QHEADS, qstep, 0)
    with scope('wt_ckv'):
        c_ckv.wait()
        c_wot.wait()

    def head(h, carry):
        with scope('head'):
            return head_body(h, carry)

    def head_body(h, carry):
        rr = jax.lax.broadcasted_iota(jnp.int32, (LN, LN), 0)
        cc = jax.lax.broadcasted_iota(jnp.int32, (LN, LN), 1)
        tri = cc <= rr
        neg = -1e9 * math.log2(math.e)
        kv = {'K': [], 'U': []}
        scores, probs, ctxs = {}, {}, {}

        def rows(name, a, b):
            parts = []
            for lo, arr in sorted(kv[name], key=lambda x: x[0]):
                x, y = max(a, lo), min(b, lo + arr.shape[0])
                if x < y:
                    parts.append(arr[x - lo:y - lo])
            return _cat(parts, 0)

        for tok in HEAD_ORDER.split():
            kind, arg = tok[0], tok[1:]
            if kind in 'KU':
                a, b = map(int, arg.split('-')) if arg else (0, S // TQ)
                w0 = DM + (DC if kind == 'U' else 0)
                w = wall[h, w0:w0 + DC, :]
                kv[kind].append((a * TQ, _dot(ckv[a * TQ:b * TQ, :], w, NN).astype(bf16)))
                continue
            if kind == 'O':
                grp = [int(ch) for ch in arg]
                res = _dot(wot[h], _cat([ctxs[j] for j in grp], 0), NT)
                for n, j in enumerate(grp):
                    ot[DM:2 * DM, j * TQ:(j + 1) * TQ] += res[:, n * TQ:(n + 1) * TQ]
                continue
            i = int(arg)
            r0 = i * TQ
            lm = r0 + LN
            if kind == 'Q':
                q = q_all[h, r0:r0 + TQ, :]
                s = _dot(q, rows('K', 0, lm), NT)
                sx = jnp.where(tri, _dot(q[LN:], rows('K', lm, lm + LN), NT), neg)
                scores[i] = (s, sx)
            elif kind == 'S':
                s, sx = scores.pop(i)
                sd = jnp.where(tri, s[0:LN, r0:lm], neg)
                pt, lt = _softmax_rows(([s[0:LN, 0:r0]] if i else []) + [sd])
                pb, lb = _softmax_rows([s[LN:], sx])
                probs[i] = (jnp.concatenate([_cat(pt, 1), pb[0]], axis=0), pb[1], lt, lb)
            else:
                p, px, lt, lb = probs.pop(i)
                ctx = _dot(p, rows('U', 0, lm), NN)
                cx = _dot(px, rows('U', lm, lm + LN), NN)
                ctxs[i] = jnp.concatenate([ctx[0:LN] * (1.0 / lt), (ctx[LN:] + cx) * (1.0 / lb)],
                                          axis=0).astype(bf16)
        return carry

    if do_b:
        with scope('P3'):
            jax.lax.fori_loop(0, H, head, 0)

    def ocopy(c):
        rows = pl.ds(pl.multiple_of(c * OCH, OCH), OCH)
        return pltpu.make_async_copy(obuf.at[rows], out_hbm.at[rows, YC:2 * DM], osem.at[c])

    def ostep(c, carry):
        for k in range(OCH // LN):
            cols = pl.ds(pl.multiple_of(c * OCH + k * LN, LN), LN)
            obuf[cols, :] = ot[YC:2 * DM, cols].astype(bf16).T
        ocopy(c).start()
        return carry

    with scope('fin'):
        jax.lax.fori_loop(0, S // OCH, ostep, 0)
    with scope('wt_out'):
        c_y.wait()
        for c in range(S // OCH):
            ocopy(c).wait()


def _build(do_a=True, do_b=True, scopes=False, order=None):
    global HEAD_ORDER
    if order is not None:
        HEAD_ORDER = order
    def run(A_x, A_w_r, A_w_i, B_x, B_c_kv, B_w_q, B_w_uk, B_w_uv, B_w_o):
        axt = jnp.swapaxes(A_x, 1, 2).reshape(DM, S)
        bxt = jnp.swapaxes(B_x, 1, 2).reshape(DM, S)
        wrt = A_w_r.T
        wit = A_w_i.T
        ckv = B_c_kv.reshape(S, DC)
        wot = jnp.swapaxes(B_w_o, 1, 2)
        tabs = [jnp.asarray(t) for t in _tables()]
        args = (axt, wrt, wit, bxt, ckv, B_w_q, B_w_uk, B_w_uv, wot, *tabs)
        vm = pltpu.VMEM
        scratch = [
            vm((DM, S), bf16), vm((J, S), bf16), vm((J, S), bf16),
            vm(tabs[0].shape, bf16), vm(tabs[1].shape, bf16), vm(tabs[2].shape, f32),
            vm(tabs[3].shape, bf16), vm(tabs[4].shape, bf16),
            vm((DM, S), bf16), vm((S, DC), bf16),
            vm((DM, H, D), bf16),
            vm((DC, H, D), bf16), vm((DC, H, D), bf16), vm((H + 4, DM + 2 * DC, D), bf16),
            vm((H, DM, D), bf16), vm((H, S, D), bf16),
            vm((2 * DM, S), f32), vm((S, YC), bf16), vm((S, 2 * DM - YC), bf16),
            pltpu.SemaphoreType.DMA((15,)), pltpu.SemaphoreType.DMA((2, H)),
            pltpu.SemaphoreType.DMA((S // OCH,)), pltpu.SemaphoreType.DMA((1,)),
        ]
        out = pl.pallas_call(
            functools.partial(_kernel, do_a=do_a, do_b=do_b, scopes=scopes),
            in_specs=[pl.BlockSpec(memory_space=pl.ANY)] * len(args),
            out_specs=pl.BlockSpec(memory_space=pl.ANY),
            out_shape=jax.ShapeDtypeStruct((S, 2 * DM), bf16),
            scratch_shapes=scratch,
            compiler_params=pltpu.CompilerParams(vmem_limit_bytes=120 * 2**20),
        )(*args)
        return out.reshape(1, S, 2 * DM)

    return run


_run = _build()


@jax.jit
def pallas_concat_heads__spectral_gfnet__compressed_kv_cla__prompt_kernel(
    A_x: jax.Array,
    A_w_r: jax.Array,
    A_w_i: jax.Array,
    B_x: jax.Array,
    B_c_kv: jax.Array,
    B_w_q: jax.Array,
    B_w_uk: jax.Array,
    B_w_uv: jax.Array,
    B_w_o: jax.Array,
):
    return _run(A_x, A_w_r, A_w_i, B_x, B_c_kv, B_w_q, B_w_uk, B_w_uv, B_w_o)
```

```python
import contextlib
import functools
import math

import jax
import jax.numpy as jnp
import numpy as np
import jax.experimental.pallas as pl
import jax.experimental.pallas.tpu as pltpu

f32 = jnp.float32
bf16 = jnp.bfloat16

NN = (((1,), (0,)), ((), ()))
NT = (((1,), (1,)), ((), ()))

S = 2048
DM = 448
J = DM // 2 + 1
HD = DM // 2
JA = 120
JB = 112
H = 16
D = 256
DC = 1024
R16 = 16
LN = 128
TQ = 256
CCH = DC // H
PX = H
PU = H + 2
YC = 384
HEAD_ORDER = ('U0-2 K0-8 U2-4 Q4 U4-8 Q1 S1 Q0 S4 V4 Q6 Q3 S0 V0 V1 S6 Q5 S5 S3 V6 Q7 S7 V3 V7 Q2 V5 O0 S2 V2 O76521 O4 O3')
OCH = 512
QHEADS = 2
QPIECES = 16


def _dot(a, b, dn):
    return jax.lax.dot_general(a, b, dn, preferred_element_type=f32)


@functools.lru_cache(maxsize=None)
def _tables():
    j = np.arange(J)[:, None].astype(np.float64)
    d = np.arange(DM)[None, :].astype(np.float64)
    ang = 2.0 * np.pi * ((j * d) % DM) / DM
    cos, sin = np.cos(ang), np.sin(ang)
    ne, no = (J + 1) // 2, J // 2
    fd = np.zeros((2 * JA + 2 * JB, HD), np.float64)
    fd[0:ne] = cos[0::2, 0:HD]
    fd[JA:JA + ne] = -sin[0::2, 0:HD]
    fd[2 * JA:2 * JA + no] = cos[1::2, 0:HD]
    fd[2 * JA + JB:2 * JA + JB + no] = -sin[1::2, 0:HD]

    m = np.arange(LN)[:, None].astype(np.float64)
    l = np.arange(LN)[None, :].astype(np.float64)
    a128 = 2.0 * np.pi * ((m * l) % LN) / LN
    fr, fi = np.cos(a128), -np.sin(a128)
    l2 = np.block([[fr, -fi], [fi, fr]])

    r = np.arange(R16)[:, None].astype(np.float64)
    at = 2.0 * np.pi * (r * l) / S
    tw = np.stack([np.cos(at), -np.sin(at)])
    tw = np.broadcast_to(tw[:, :, None, :], (2, R16, 8, LN)).copy()

    l3 = np.zeros((R16, 2 * LN, LN), np.float64)
    for rr in range(R16):
        a3 = 2.0 * np.pi * ((m * (rr + R16 * l)) % S) / S
        l3[rr] = np.concatenate([np.cos(a3), np.sin(a3)], axis=0)

    cj = np.full((J,), 2.0)
    cj[0] = 1.0
    cj[J - 1] = 1.0
    scale = cj[None, :] / float(S * DM)
    cr, ci = cos.T[0:HD] * scale, -sin.T[0:HD] * scale
    l4 = np.zeros((2, HD, 2 * LN), np.float64)
    l4[0, :, 0:ne] = cr[:, 0::2]
    l4[0, :, LN:LN + ne] = ci[:, 0::2]
    l4[1, :, 0:no] = cr[:, 1::2]
    l4[1, :, LN:LN + no] = ci[:, 1::2]

    cast = lambda a, dt: np.asarray(a, np.float32).astype(dt)
    return (cast(fd, bf16), cast(l2, bf16), cast(tw, np.float32), cast(l3, bf16),
            cast(l4.reshape(2 * HD, 2 * LN), bf16))


def _cmul_const(z, k, n, sign):
    re, im = z
    k = k % n
    if k == 0:
        return re, im
    if 4 * k == n:
        return (-im, re) if sign > 0 else (im, -re)
    if 8 * k == n:
        c = math.sqrt(0.5)
        return ((re - im) * c, (re + im) * c) if sign > 0 else ((re + im) * c, (im - re) * c)
    if 8 * k == 3 * n:
        c = math.sqrt(0.5)
        return ((re + im) * (-c), (re - im) * c) if sign > 0 else ((im - re) * c, (re + im) * (-c))
    c = math.cos(2.0 * math.pi * k / n)
    s = sign * math.sin(2.0 * math.pi * k / n)
    return re * c - im * s, re * s + im * c


def _fft(zs, sign):
    n = len(zs)
    if n == 1:
        return zs
    ev = _fft(zs[0::2], sign)
    od = _fft(zs[1::2], sign)
    out = [None] * n
    for k in range(n // 2):
        if 4 * k == n:
            (er, ei), (orr, oi) = ev[k], od[k]
            if sign > 0:
                out[k] = (er - oi, ei + orr)
                out[k + n // 2] = (er + oi, ei - orr)
            else:
                out[k] = (er + oi, ei - orr)
                out[k + n // 2] = (er - oi, ei + orr)
            continue
        tr, ti = _cmul_const(od[k], k, n, sign)
        er, ei = ev[k]
        out[k] = (er + tr, ei + ti)
        out[k + n // 2] = (er - tr, ei - ti)
    return out


def _softmax_rows(segs):
    m = functools.reduce(jnp.maximum, [jnp.max(sg, axis=1, keepdims=True) for sg in segs])
    ps = [jnp.exp2(sg - m).astype(bf16) for sg in segs]
    l = functools.reduce(jnp.add, [jnp.sum(p.astype(f32), axis=1, keepdims=True) for p in ps])
    return ps, l


def _cat(parts, axis):
    return jnp.concatenate(parts, axis=axis) if len(parts) > 1 else parts[0]


def _kernel(axt_hbm, wrt_hbm, wit_hbm, bxt_hbm, ckv_hbm, wq_hbm, wuk_hbm, wuv_hbm, wot_hbm,
            fd_hbm, l2_hbm, tw_hbm, l3_hbm, l4_hbm,
            out_hbm,
            axt, wrt, wit, fd, l2, tw, l3, l4,
            bxt, ckv, wq_raw, wuk_raw, wuv_raw, wall, wot, q_all,
            ot, ybuf, obuf, sem, wsem, osem, ysem, *, do_a, do_b, scopes):
    scope = jax.named_scope if scopes else (lambda name: contextlib.nullcontext())
    XC = S // 4
    simple = ([(fd_hbm, fd)]
              + [(axt_hbm.at[:, c * XC:(c + 1) * XC], axt.at[:, c * XC:(c + 1) * XC]) for c in range(4)]
              + [(tw_hbm, tw), (l2_hbm, l2), (wrt_hbm, wrt), (wit_hbm, wit),
                 (l3_hbm, l3), (bxt_hbm, bxt), (l4_hbm, l4), (wq_hbm, wq_raw), (ckv_hbm, ckv), (wot_hbm, wot)])
    cps = [pltpu.make_async_copy(s, d, sem.at[i]) for i, (s, d) in enumerate(simple)]
    c_fd = cps[0]
    (c_tw, c_l2, c_wrt, c_wit, c_l3, c_bxt, c_l4, c_wq, c_ckv, c_wot) = cps[5:]

    def wchunk(which, t):
        src, dst = ((wuk_hbm, wuk_raw), (wuv_hbm, wuv_raw))[which]
        return pltpu.make_async_copy(src.at[pl.ds(t * CCH, CCH)], dst.at[pl.ds(t * CCH, CCH)], wsem.at[which, t])

    def issue(lo, hi):
        def body(i, carry):
            for k in range(lo, hi):
                pl.when(i == k)(cps[k].start)
            return carry
        jax.lax.fori_loop(lo, hi, body, 0)

    def wait_all(cs):
        def body(i, carry):
            for k, c in enumerate(cs):
                pl.when(i == k)(c.wait)
            return carry
        jax.lax.fori_loop(0, max(2, len(cs)), body, 0)

    def issue_w(t, carry):
        wchunk(0, t).start()
        wchunk(1, t).start()
        return carry

    with scope('issue'):
        issue(0, len(cps) - 2)
        jax.lax.fori_loop(0, H, issue_w, 0)
        issue(len(cps) - 2, len(cps))

    def zero(i, carry):
        ot[pl.ds(pl.multiple_of(DM + i * 64, 64), 64), :] = jnp.zeros((64, S), f32)
        return carry

    with scope('zero'):
        jax.lax.fori_loop(0, DM // 64, zero, 0)

    def x_prep(k, n):
        w = S // n
        wall[PX, k * w:(k + 1) * w, :] = bxt[0:D, k * w:(k + 1) * w].T
        wall[PX + 1, k * w:(k + 1) * w, 0:DM - D] = bxt[D:DM, k * w:(k + 1) * w].T

    def wq_prep(k, n):
        g = DM // 16
        lo, hi = 16 * (k * g // n), 16 * ((k + 1) * g // n)
        wall[0:H, lo:hi, :] = jnp.swapaxes(wq_raw[lo:hi], 0, 1)

    def part_a(x1a, x1b, rma, rmb, wsa, wsb, csa, csb):
        def stage1(c, carry):
            cols = pl.ds(pl.multiple_of(c * XC, XC), XC)
            pltpu.make_async_copy(axt_hbm.at[:, cols], axt.at[:, cols], sem.at[1 + c]).wait()
            lo, hi = axt[0:HD, cols].astype(f32), axt[HD:DM, cols].astype(f32)
            x1a[:, cols] = _dot(fd[0:2 * JA, :], (lo + hi).astype(bf16), NN)
            x1b[:, cols] = _dot(fd[2 * JA:, :], (lo - hi).astype(bf16), NN)
            return carry

        def fwd16(x1, rm, n, r0):
            zs = [(x1[pl.ds(r0, 8), c * LN:(c + 1) * LN], x1[pl.ds(n + r0, 8), c * LN:(c + 1) * LN])
                  for c in range(R16)]
            ys = _fft(zs, -1)
            for r in range(R16):
                re, im = ys[r]
                if r:
                    tr, ti = tw[0, r], tw[1, r]
                    re, im = re * tr - im * ti, re * ti + im * tr
                rm[r, pl.ds(r0, 8), 0:LN] = re
                rm[r, pl.ds(r0, 8), LN:2 * LN] = im

        def wprep(c):
            cols = slice(c * LN, (c + 1) * LN)
            row = jax.lax.broadcasted_iota(jnp.int32, (LN - JB, LN), 0)
            for p, wt in enumerate((wrt, wit)):
                u = pltpu.bitcast(wt[0:J - 1, cols], jnp.uint32)
                even = pltpu.bitcast(u << 16, f32)
                odd = pltpu.bitcast(u & jnp.uint32(0xFFFF0000), f32)
                last = jnp.broadcast_to(wt[J - 1:J, cols].astype(f32), (LN - JB, LN))
                wsa[p, cols, :] = jnp.concatenate([even, jnp.where(row == 0, last, 0.0)], axis=0).T
                wsb[p, cols, :] = jnp.concatenate([odd, jnp.zeros((LN - JB, LN), f32)], axis=0).T

        def stage2(rm, k):
            return _dot(l2[...], rm[4 * k:4 * k + 4].reshape(4 * LN, 2 * LN).astype(bf16), NT)

        def stage3(x, ws, cs, r):
            x = x[r // 4]
            c0 = (r % 4) * LN
            xr, xi = x[0:LN, c0:c0 + LN], x[LN:2 * LN, c0:c0 + LN]
            wr = ws[0, pl.ds(r, LN, stride=R16), :]
            wi = ws[1, pl.ds(r, LN, stride=R16), :]
            g = jnp.concatenate([xr * wr - xi * wi, xr * wi + xi * wr], axis=1).astype(bf16)
            c = _dot(l3[r], g, NN)
            cs[r, 0:LN, :] = c[0:LN, 0:LN] - c[LN:2 * LN, LN:2 * LN]
            cs[r, LN:2 * LN, :] = c[LN:2 * LN, 0:LN] + c[0:LN, LN:2 * LN]

        def inv16(cs, half, r0):
            zs = [(cs[r, r0:r0 + 8, :], cs[r, LN + r0:LN + r0 + 8, :]) for r in range(R16)]
            ys = _fft(zs, +1)
            for c in range(R16):
                wall[PU + half, c * LN + r0:c * LN + r0 + 8, 0:LN] = ys[c][0].astype(bf16)
                wall[PU + half, c * LN + r0:c * LN + r0 + 8, LN:2 * LN] = ys[c][1].astype(bf16)

        def stage4(half, k):
            cols = slice(k * LN, (k + 1) * LN)
            y = _dot(l4[half * HD:(half + 1) * HD, :], wall[PU + half, cols, :], NT)
            if half:
                ot[0:HD, cols] += y
                ot[HD:DM, cols] -= y
            else:
                ot[0:HD, cols] = y
                ot[HD:DM, cols] = y

        with scope('w0'):
            c_fd.wait()
        with scope('S1'):
            jax.lax.fori_loop(0, 4, stage1, 0)
        with scope('wt_tw'):
            wait_all([c_tw])

        def fwd16a(g, carry):
            fwd16(x1a, rma, JA, pl.multiple_of(g * 8, 8))
            return carry

        def fwd16b(g, carry):
            fwd16(x1b, rmb, JB, pl.multiple_of(g * 8, 8))
            return carry

        with scope('F16'):
            jax.lax.fori_loop(0, JA // 8, fwd16a, 0)
            jax.lax.fori_loop(0, JB // 8, fwd16b, 0)
        with scope('wt_l2'):
            wait_all([c_l2, c_wrt, c_wit])
        rma[:, JA:LN, :] = jnp.zeros((R16, LN - JA, 2 * LN), f32)
        rmb[:, JB:LN, :] = jnp.zeros((R16, LN - JB, 2 * LN), f32)
        xa, xb = [], []
        for k in range(8):
            wprep(2 * k)
            wprep(2 * k + 1)
            (xa, xb)[k // 4].append(stage2((rma, rmb)[k // 4], k % 4))
        with scope('wt_W'):
            wait_all([c_l3])
        for r in range(R16):
            stage3(xa, wsa, csa, r)
        for r in range(R16):
            stage3(xb, wsb, csb, r)
            inv16(csa, 0, r * 8)
        with scope('wt_x'):
            wait_all([c_bxt, c_l4])
        for k in range(R16):
            if do_b:
                x_prep(k, R16)
            stage4(0, k)
            inv16(csb, 1, k * 8)
        with scope('wt_wq'):
            wait_all([c_wq])
        for k in range(R16):
            if do_b:
                wq_prep(k, R16)
            stage4(1, k)

    if do_a:
        pl.run_scoped(part_a,
                      pltpu.VMEM((2 * JA, S), f32), pltpu.VMEM((2 * JB, S), f32),
                      pltpu.VMEM((R16, LN, 2 * LN), f32), pltpu.VMEM((R16, LN, 2 * LN), f32),
                      pltpu.VMEM((2, S, LN), f32), pltpu.VMEM((2, S, LN), f32),
                      pltpu.VMEM((R16, 2 * LN, LN), f32), pltpu.VMEM((R16, 2 * LN, LN), f32))
    else:
        for c in cps[:-2]:
            c.wait()
        ot[0:DM, :] = jnp.zeros((DM, S), f32)
        if do_b:
            for k in range(R16):
                x_prep(k, R16)
                wq_prep(k, R16)

    def ystep(c, carry):
        for k in range(OCH // LN):
            cols = pl.ds(pl.multiple_of(c * OCH + k * LN, LN), LN)
            ybuf[cols, :] = ot[0:YC, cols].astype(bf16).T
        return carry

    with scope('Y'):
        jax.lax.fori_loop(0, S // OCH, ystep, 0)
    c_y = pltpu.make_async_copy(ybuf, out_hbm.at[:, 0:YC], ysem.at[0])
    c_y.start()

    qscale = (D ** -0.5) * math.log2(math.e)

    with scope('wt_c0'):
        for u in range(QHEADS):
            wchunk(0, u).wait()
            wchunk(1, u).wait()

    def qstep(tt, carry):
        if do_b:
            rq, rw = S // QPIECES, 2 * CCH // QPIECES
            for u in range(QHEADS):
                t = tt * QHEADS + u
                for j in range(QPIECES):
                    x = jnp.concatenate([wall[PX, j * rq:(j + 1) * rq, :], wall[PX + 1, j * rq:(j + 1) * rq, 0:DM - D]],
                                        axis=1)
                    q_all[t, j * rq:(j + 1) * rq] = (_dot(x, wall[t, 0:DM, :], NN) * qscale).astype(bf16)
                    which, off = divmod(j * rw, CCH)
                    r0 = pl.multiple_of(t * CCH + off, rw)
                    src = (wuk_raw, wuv_raw)[which]
                    wall[0:H, pl.ds(DM + which * DC + r0, rw), :] = jnp.swapaxes(src[pl.ds(r0, rw)], 0, 1)

        @pl.when(tt + 1 < H // QHEADS)
        def _():
            for u in range(QHEADS):
                wchunk(0, (tt + 1) * QHEADS + u).wait()
                wchunk(1, (tt + 1) * QHEADS + u).wait()

        return carry

    with scope('P2'):
        jax.lax.fori_loop(0, H // QHEADS, qstep, 0)
    with scope('wt_ckv'):
        c_ckv.wait()
        c_wot.wait()

    def head(h, carry):
        with scope('head'):
            return head_body(h, carry)

    def head_body(h, carry):
        rr = jax.lax.broadcasted_iota(jnp.int32, (LN, LN), 0)
        cc = jax.lax.broadcasted_iota(jnp.int32, (LN, LN), 1)
        tri = cc <= rr
        neg = -1e9 * math.log2(math.e)
        kv = {'K': [], 'U': []}
        scores, probs, ctxs = {}, {}, {}

        def rows(name, a, b):
            parts = []
            for lo, arr in sorted(kv[name], key=lambda x: x[0]):
                x, y = max(a, lo), min(b, lo + arr.shape[0])
                if x < y:
                    parts.append(arr[x - lo:y - lo])
            return _cat(parts, 0)

        for tok in HEAD_ORDER.split():
            kind, arg = tok[0], tok[1:]
            if kind in 'KU':
                a, b = map(int, arg.split('-')) if arg else (0, S // TQ)
                w0 = DM + (DC if kind == 'U' else 0)
                w = wall[h, w0:w0 + DC, :]
                kv[kind].append((a * TQ, _dot(ckv[a * TQ:b * TQ, :], w, NN).astype(bf16)))
                continue
            if kind == 'O':
                grp = [int(ch) for ch in arg]
                res = _dot(wot[h], _cat([ctxs[j] for j in grp], 0), NT)
                for n, j in enumerate(grp):
                    ot[DM:2 * DM, j * TQ:(j + 1) * TQ] += res[:, n * TQ:(n + 1) * TQ]
                continue
            i = int(arg)
            r0 = i * TQ
            lm = r0 + LN
            if kind == 'Q':
                q = q_all[h, r0:r0 + TQ, :]
                s = _dot(q, rows('K', 0, lm), NT)
                sx = jnp.where(tri, _dot(q[LN:], rows('K', lm, lm + LN), NT), neg)
                scores[i] = (s, sx)
            elif kind == 'S':
                s, sx = scores.pop(i)
                sd = jnp.where(tri, s[0:LN, r0:lm], neg)
                pt, lt = _softmax_rows(([s[0:LN, 0:r0]] if i else []) + [sd])
                pb, lb = _softmax_rows([s[LN:], sx])
                probs[i] = (jnp.concatenate([_cat(pt, 1), pb[0]], axis=0), pb[1], lt, lb)
            else:
                p, px, lt, lb = probs.pop(i)
                ctx = _dot(p, rows('U', 0, lm), NN)
                cx = _dot(px, rows('U', lm, lm + LN), NN)
                ctxs[i] = jnp.concatenate([ctx[0:LN] * (1.0 / lt), (ctx[LN:] + cx) * (1.0 / lb)],
                                          axis=0).astype(bf16)
        return carry

    if do_b:
        with scope('P3'):
            jax.lax.fori_loop(0, H, head, 0)

    def ocopy(c):
        rows = pl.ds(pl.multiple_of(c * OCH, OCH), OCH)
        return pltpu.make_async_copy(obuf.at[rows], out_hbm.at[rows, YC:2 * DM], osem.at[c])

    def ostep(c, carry):
        for k in range(OCH // LN):
            cols = pl.ds(pl.multiple_of(c * OCH + k * LN, LN), LN)
            obuf[cols, :] = ot[YC:2 * DM, cols].astype(bf16).T
        ocopy(c).start()
        return carry

    with scope('fin'):
        jax.lax.fori_loop(0, S // OCH, ostep, 0)
    with scope('wt_out'):
        c_y.wait()
        for c in range(S // OCH):
            ocopy(c).wait()


def _build(do_a=True, do_b=True, scopes=False, order=None):
    global HEAD_ORDER
    if order is not None:
        HEAD_ORDER = order
    def run(A_x, A_w_r, A_w_i, B_x, B_c_kv, B_w_q, B_w_uk, B_w_uv, B_w_o):
        axt = jnp.swapaxes(A_x, 1, 2).reshape(DM, S)
        bxt = jnp.swapaxes(B_x, 1, 2).reshape(DM, S)
        wrt = A_w_r.T
        wit = A_w_i.T
        ckv = B_c_kv.reshape(S, DC)
        wot = jnp.swapaxes(B_w_o, 1, 2)
        tabs = [jnp.asarray(t) for t in _tables()]
        args = (axt, wrt, wit, bxt, ckv, B_w_q, B_w_uk, B_w_uv, wot, *tabs)
        vm = pltpu.VMEM
        scratch = [
            vm((DM, S), bf16), vm((J, S), bf16), vm((J, S), bf16),
            vm(tabs[0].shape, bf16), vm(tabs[1].shape, bf16), vm(tabs[2].shape, f32),
            vm(tabs[3].shape, bf16), vm(tabs[4].shape, bf16),
            vm((DM, S), bf16), vm((S, DC), bf16),
            vm((DM, H, D), bf16),
            vm((DC, H, D), bf16), vm((DC, H, D), bf16), vm((H + 4, DM + 2 * DC, D), bf16),
            vm((H, DM, D), bf16), vm((H, S, D), bf16),
            vm((2 * DM, S), f32), vm((S, YC), bf16), vm((S, 2 * DM - YC), bf16),
            pltpu.SemaphoreType.DMA((15,)), pltpu.SemaphoreType.DMA((2, H)),
            pltpu.SemaphoreType.DMA((S // OCH,)), pltpu.SemaphoreType.DMA((1,)),
        ]
        out = pl.pallas_call(
            functools.partial(_kernel, do_a=do_a, do_b=do_b, scopes=scopes),
            in_specs=[pl.BlockSpec(memory_space=pl.ANY)] * len(args),
            out_specs=pl.BlockSpec(memory_space=pl.ANY),
            out_shape=jax.ShapeDtypeStruct((S, 2 * DM), bf16),
            scratch_shapes=scratch,
            compiler_params=pltpu.CompilerParams(vmem_limit_bytes=120 * 2**20),
        )(*args)
        return out.reshape(1, S, 2 * DM)

    return run


_run = _build()


@jax.jit
def pallas_concat_heads__spectral_gfnet__compressed_kv_cla__prompt_kernel(
    A_x: jax.Array,
    A_w_r: jax.Array,
    A_w_i: jax.Array,
    B_x: jax.Array,
    B_c_kv: jax.Array,
    B_w_q: jax.Array,
    B_w_uk: jax.Array,
    B_w_uv: jax.Array,
    B_w_o: jax.Array,
):
    return _run(A_x, A_w_r, A_w_i, B_x, B_c_kv, B_w_q, B_w_uk, B_w_uv, B_w_o)
```

```python
import contextlib
import functools
import math

import jax
import jax.numpy as jnp
import numpy as np
import jax.experimental.pallas as pl
import jax.experimental.pallas.tpu as pltpu

f32 = jnp.float32
bf16 = jnp.bfloat16

NN = (((1,), (0,)), ((), ()))
NT = (((1,), (1,)), ((), ()))

S = 2048
DM = 448
J = DM // 2 + 1
HD = DM // 2
JA = 120
JB = 112
H = 16
D = 256
DC = 1024
R16 = 16
LN = 128
TQ = 256
CCH = DC // H
PX = H
YC = 384
HEAD_ORDER = ('U0-2 K0-8 U2-4 Q4 U4-8 Q1 S1 Q0 S4 V4 Q6 Q3 S0 V0 V1 S6 Q5 S5 S3 V6 Q7 S7 V3 V7 Q2 V5 O0 S2 V2 O76521 O4 O3')
OCH = 512
QHEADS = 2
QPIECES = 16


def _dot(a, b, dn):
    return jax.lax.dot_general(a, b, dn, preferred_element_type=f32)


@functools.lru_cache(maxsize=None)
def _tables():
    j = np.arange(J)[:, None].astype(np.float64)
    d = np.arange(DM)[None, :].astype(np.float64)
    ang = 2.0 * np.pi * ((j * d) % DM) / DM
    cos, sin = np.cos(ang), np.sin(ang)
    ne, no = (J + 1) // 2, J // 2
    fd = np.zeros((2 * JA + 2 * JB, HD), np.float64)
    fd[0:ne] = cos[0::2, 0:HD]
    fd[JA:JA + ne] = -sin[0::2, 0:HD]
    fd[2 * JA:2 * JA + no] = cos[1::2, 0:HD]
    fd[2 * JA + JB:2 * JA + JB + no] = -sin[1::2, 0:HD]

    m = np.arange(LN)[:, None].astype(np.float64)
    l = np.arange(LN)[None, :].astype(np.float64)
    a128 = 2.0 * np.pi * ((m * l) % LN) / LN
    fr, fi = np.cos(a128), -np.sin(a128)
    l2 = np.block([[fr, -fi], [fi, fr]])

    r = np.arange(R16)[:, None].astype(np.float64)
    at = 2.0 * np.pi * (r * l) / S
    tw = np.stack([np.cos(at), -np.sin(at)])
    tw = np.broadcast_to(tw[:, :, None, :], (2, R16, 8, LN)).copy()

    l3 = np.zeros((R16, 2 * LN, LN), np.float64)
    for rr in range(R16):
        a3 = 2.0 * np.pi * ((m * (rr + R16 * l)) % S) / S
        l3[rr] = np.concatenate([np.cos(a3), np.sin(a3)], axis=0)

    cj = np.full((J,), 2.0)
    cj[0] = 1.0
    cj[J - 1] = 1.0
    scale = cj[None, :] / float(S * DM)
    cr, ci = cos.T[0:HD] * scale, -sin.T[0:HD] * scale
    l4 = np.zeros((2, HD, 2 * LN), np.float64)
    l4[0, :, 0:ne] = cr[:, 0::2]
    l4[0, :, LN:LN + ne] = ci[:, 0::2]
    l4[1, :, 0:no] = cr[:, 1::2]
    l4[1, :, LN:LN + no] = ci[:, 1::2]

    cast = lambda a, dt: np.asarray(a, np.float32).astype(dt)
    return (cast(fd, bf16), cast(l2, bf16), cast(tw, np.float32), cast(l3, bf16),
            cast(l4.reshape(2 * HD, 2 * LN), bf16))


def _cmul_const(z, k, n, sign):
    re, im = z
    k = k % n
    if k == 0:
        return re, im
    if 4 * k == n:
        return (-im, re) if sign > 0 else (im, -re)
    if 8 * k == n:
        c = math.sqrt(0.5)
        return ((re - im) * c, (re + im) * c) if sign > 0 else ((re + im) * c, (im - re) * c)
    if 8 * k == 3 * n:
        c = math.sqrt(0.5)
        return ((re + im) * (-c), (re - im) * c) if sign > 0 else ((im - re) * c, (re + im) * (-c))
    c = math.cos(2.0 * math.pi * k / n)
    s = sign * math.sin(2.0 * math.pi * k / n)
    return re * c - im * s, re * s + im * c


def _fft(zs, sign):
    n = len(zs)
    if n == 1:
        return zs
    ev = _fft(zs[0::2], sign)
    od = _fft(zs[1::2], sign)
    out = [None] * n
    for k in range(n // 2):
        if 4 * k == n:
            (er, ei), (orr, oi) = ev[k], od[k]
            if sign > 0:
                out[k] = (er - oi, ei + orr)
                out[k + n // 2] = (er + oi, ei - orr)
            else:
                out[k] = (er + oi, ei - orr)
                out[k + n // 2] = (er - oi, ei + orr)
            continue
        tr, ti = _cmul_const(od[k], k, n, sign)
        er, ei = ev[k]
        out[k] = (er + tr, ei + ti)
        out[k + n // 2] = (er - tr, ei - ti)
    return out


def _softmax_rows(segs):
    m = functools.reduce(jnp.maximum, [jnp.max(sg, axis=1, keepdims=True) for sg in segs])
    ps = [jnp.exp2(sg - m).astype(bf16) for sg in segs]
    l = functools.reduce(jnp.add, [jnp.sum(p.astype(f32), axis=1, keepdims=True) for p in ps])
    return ps, l


def _cat(parts, axis):
    return jnp.concatenate(parts, axis=axis) if len(parts) > 1 else parts[0]


def _kernel(axt_hbm, wrt_hbm, wit_hbm, bxt_hbm, ckv_hbm, wq_hbm, wuk_hbm, wuv_hbm, wot_hbm,
            fd_hbm, l2_hbm, tw_hbm, l3_hbm, l4_hbm,
            out_hbm,
            axt, wrt, wit, fd, l2, tw, l3, l4,
            bxt, ckv, wq_raw, wuk_raw, wuv_raw, wall, wot, q_all,
            ot, ybuf, obuf, sem, wsem, osem, ysem, *, do_a, do_b, scopes):
    scope = jax.named_scope if scopes else (lambda name: contextlib.nullcontext())
    XC = S // 4
    simple = ([(fd_hbm, fd)]
              + [(axt_hbm.at[:, c * XC:(c + 1) * XC], axt.at[:, c * XC:(c + 1) * XC]) for c in range(4)]
              + [(tw_hbm, tw), (l2_hbm, l2), (wrt_hbm, wrt), (wit_hbm, wit),
                 (l3_hbm, l3), (l4_hbm, l4), (wq_hbm, wq_raw), (bxt_hbm, bxt), (ckv_hbm, ckv), (wot_hbm, wot)])
    cps = [pltpu.make_async_copy(s, d, sem.at[i]) for i, (s, d) in enumerate(simple)]
    c_fd = cps[0]
    (c_tw, c_l2, c_wrt, c_wit, c_l3, c_l4, c_wq, c_bxt, c_ckv, c_wot) = cps[5:]

    def wchunk(which, t):
        src, dst = ((wuk_hbm, wuk_raw), (wuv_hbm, wuv_raw))[which]
        return pltpu.make_async_copy(src.at[pl.ds(t * CCH, CCH)], dst.at[pl.ds(t * CCH, CCH)], wsem.at[which, t])

    def issue(lo, hi):
        def body(i, carry):
            for k in range(lo, hi):
                pl.when(i == k)(cps[k].start)
            return carry
        jax.lax.fori_loop(lo, hi, body, 0)

    def wait_all(cs):
        def body(i, carry):
            for k, c in enumerate(cs):
                pl.when(i == k)(c.wait)
            return carry
        jax.lax.fori_loop(0, max(2, len(cs)), body, 0)

    def issue_w(t, carry):
        wchunk(0, t).start()
        wchunk(1, t).start()
        return carry

    with scope('issue'):
        issue(0, len(cps) - 2)
        jax.lax.fori_loop(0, H, issue_w, 0)
        issue(len(cps) - 2, len(cps))

    def zero(i, carry):
        ot[pl.ds(pl.multiple_of(DM + i * 64, 64), 64), :] = jnp.zeros((64, S), f32)
        return carry

    with scope('zero'):
        jax.lax.fori_loop(0, DM // 64, zero, 0)

    def x_prep(k, n):
        w = S // n
        wall[PX, k * w:(k + 1) * w, :] = bxt[0:D, k * w:(k + 1) * w].T
        wall[PX + 1, k * w:(k + 1) * w, 0:DM - D] = bxt[D:DM, k * w:(k + 1) * w].T

    def wq_prep(k, n):
        g = DM // 16
        lo, hi = 16 * (k * g // n), 16 * ((k + 1) * g // n)
        wall[0:H, lo:hi, :] = jnp.swapaxes(wq_raw[lo:hi], 0, 1)

    def part_a(x1a, x1b, rma, rmb, wsa, wsb, csa, csb, us):
        def stage1(c, carry):
            cols = pl.ds(pl.multiple_of(c * XC, XC), XC)
            pltpu.make_async_copy(axt_hbm.at[:, cols], axt.at[:, cols], sem.at[1 + c]).wait()
            lo, hi = axt[0:HD, cols].astype(f32), axt[HD:DM, cols].astype(f32)
            x1a[:, cols] = _dot(fd[0:2 * JA, :], (lo + hi).astype(bf16), NN)
            x1b[:, cols] = _dot(fd[2 * JA:, :], (lo - hi).astype(bf16), NN)
            return carry

        def fwd16(x1, rm, n, r0):
            zs = [(x1[pl.ds(r0, 8), c * LN:(c + 1) * LN], x1[pl.ds(n + r0, 8), c * LN:(c + 1) * LN])
                  for c in range(R16)]
            ys = _fft(zs, -1)
            for r in range(R16):
                re, im = ys[r]
                if r:
                    tr, ti = tw[0, r], tw[1, r]
                    re, im = re * tr - im * ti, re * ti + im * tr
                rm[r, pl.ds(r0, 8), 0:LN] = re
                rm[r, pl.ds(r0, 8), LN:2 * LN] = im

        def wprep(c):
            cols = slice(c * LN, (c + 1) * LN)
            row = jax.lax.broadcasted_iota(jnp.int32, (LN - JB, LN), 0)
            for p, wt in enumerate((wrt, wit)):
                u = pltpu.bitcast(wt[0:J - 1, cols], jnp.uint32)
                even = pltpu.bitcast(u << 16, f32)
                odd = pltpu.bitcast(u & jnp.uint32(0xFFFF0000), f32)
                last = jnp.broadcast_to(wt[J - 1:J, cols].astype(f32), (LN - JB, LN))
                wsa[p, cols, :] = jnp.concatenate([even, jnp.where(row == 0, last, 0.0)], axis=0).T
                wsb[p, cols, :] = jnp.concatenate([odd, jnp.zeros((LN - JB, LN), f32)], axis=0).T

        def stage2(rm, k):
            return _dot(l2[...], rm[4 * k:4 * k + 4].reshape(4 * LN, 2 * LN).astype(bf16), NT)

        def stage3(x, ws, cs, r):
            x = x[r // 4]
            c0 = (r % 4) * LN
            xr, xi = x[0:LN, c0:c0 + LN], x[LN:2 * LN, c0:c0 + LN]
            wr = ws[0, pl.ds(r, LN, stride=R16), :]
            wi = ws[1, pl.ds(r, LN, stride=R16), :]
            g = jnp.concatenate([xr * wr - xi * wi, xr * wi + xi * wr], axis=1).astype(bf16)
            c = _dot(l3[r], g, NN)
            cs[r, 0:LN, :] = c[0:LN, 0:LN] - c[LN:2 * LN, LN:2 * LN]
            cs[r, LN:2 * LN, :] = c[LN:2 * LN, 0:LN] + c[0:LN, LN:2 * LN]

        def inv16(cs, half, r0):
            zs = [(cs[r, r0:r0 + 8, :], cs[r, LN + r0:LN + r0 + 8, :]) for r in range(R16)]
            ys = _fft(zs, +1)
            for c in range(R16):
                us[half, c * LN + r0:c * LN + r0 + 8, 0:LN] = ys[c][0].astype(bf16)
                us[half, c * LN + r0:c * LN + r0 + 8, LN:2 * LN] = ys[c][1].astype(bf16)

        def stage4(half, k):
            cols = slice(k * LN, (k + 1) * LN)
            y = _dot(l4[half * HD:(half + 1) * HD, :], us[half, cols, :], NT)
            if half:
                ot[0:HD, cols] += y
                ot[HD:DM, cols] -= y
            else:
                ot[0:HD, cols] = y
                ot[HD:DM, cols] = y

        with scope('w0'):
            c_fd.wait()
        with scope('S1'):
            jax.lax.fori_loop(0, 4, stage1, 0)
        with scope('wt_tw'):
            wait_all([c_tw])

        def fwd16a(g, carry):
            fwd16(x1a, rma, JA, pl.multiple_of(g * 8, 8))
            return carry

        def fwd16b(g, carry):
            fwd16(x1b, rmb, JB, pl.multiple_of(g * 8, 8))
            return carry

        with scope('F16'):
            jax.lax.fori_loop(0, JA // 8, fwd16a, 0)
            jax.lax.fori_loop(0, JB // 8, fwd16b, 0)
        with scope('wt_l2'):
            wait_all([c_l2, c_wrt, c_wit])
        rma[:, JA:LN, :] = jnp.zeros((R16, LN - JA, 2 * LN), f32)
        rmb[:, JB:LN, :] = jnp.zeros((R16, LN - JB, 2 * LN), f32)
        xa, xb = [], []
        for k in range(8):
            wprep(2 * k)
            wprep(2 * k + 1)
            (xa, xb)[k // 4].append(stage2((rma, rmb)[k // 4], k % 4))
        with scope('wt_W'):
            wait_all([c_l3, c_l4])
        for r in range(R16):
            stage3(xa, wsa, csa, r)
        for r in range(R16):
            stage3(xb, wsb, csb, r)
            inv16(csa, 0, r * 8)
        for k in range(R16):
            stage4(0, k)
            inv16(csb, 1, k * 8)
        with scope('wt_wq'):
            wait_all([c_wq])
        for k in range(R16):
            if do_b:
                wq_prep(k, R16)
            stage4(1, k)

    if do_a:
        pl.run_scoped(part_a,
                      pltpu.VMEM((2 * JA, S), f32), pltpu.VMEM((2 * JB, S), f32),
                      pltpu.VMEM((R16, LN, 2 * LN), f32), pltpu.VMEM((R16, LN, 2 * LN), f32),
                      pltpu.VMEM((2, S, LN), f32), pltpu.VMEM((2, S, LN), f32),
                      pltpu.VMEM((R16, 2 * LN, LN), f32), pltpu.VMEM((R16, 2 * LN, LN), f32),
                      pltpu.VMEM((2, S, 2 * LN), bf16))
    else:
        for c in cps[:-3]:
            c.wait()
        ot[0:DM, :] = jnp.zeros((DM, S), f32)
        if do_b:
            for k in range(R16):
                wq_prep(k, R16)

    with scope('wt_x'):
        wait_all([c_bxt])
    for k in range(R16):
        cols = slice(k * LN, (k + 1) * LN)
        ybuf[cols, :] = ot[0:YC, cols].astype(bf16).T
        if do_b:
            x_prep(k, R16)
    c_y = pltpu.make_async_copy(ybuf, out_hbm.at[:, 0:YC], ysem.at[0])
    c_y.start()

    qscale = (D ** -0.5) * math.log2(math.e)

    with scope('wt_c0'):
        for u in range(QHEADS):
            wchunk(0, u).wait()
            wchunk(1, u).wait()

    def qstep(tt, carry):
        if do_b:
            rq, rw = S // QPIECES, 2 * CCH // QPIECES
            for u in range(QHEADS):
                t = tt * QHEADS + u
                for j in range(QPIECES):
                    x = jnp.concatenate([wall[PX, j * rq:(j + 1) * rq, :], wall[PX + 1, j * rq:(j + 1) * rq, 0:DM - D]],
                                        axis=1)
                    q_all[t, j * rq:(j + 1) * rq] = (_dot(x, wall[t, 0:DM, :], NN) * qscale).astype(bf16)
                    which, off = divmod(j * rw, CCH)
                    r0 = pl.multiple_of(t * CCH + off, rw)
                    src = (wuk_raw, wuv_raw)[which]
                    wall[0:H, pl.ds(DM + which * DC + r0, rw), :] = jnp.swapaxes(src[pl.ds(r0, rw)], 0, 1)

        @pl.when(tt + 1 < H // QHEADS)
        def _():
            for u in range(QHEADS):
                wchunk(0, (tt + 1) * QHEADS + u).wait()
                wchunk(1, (tt + 1) * QHEADS + u).wait()

        return carry

    with scope('P2'):
        jax.lax.fori_loop(0, H // QHEADS, qstep, 0)
    with scope('wt_ckv'):
        c_ckv.wait()
        c_wot.wait()

    def head(h, carry):
        with scope('head'):
            return head_body(h, carry)

    def head_body(h, carry):
        rr = jax.lax.broadcasted_iota(jnp.int32, (LN, LN), 0)
        cc = jax.lax.broadcasted_iota(jnp.int32, (LN, LN), 1)
        tri = cc <= rr
        neg = -1e9 * math.log2(math.e)
        kv = {'K': [], 'U': []}
        scores, probs, ctxs = {}, {}, {}

        def rows(name, a, b):
            parts = []
            for lo, arr in sorted(kv[name], key=lambda x: x[0]):
                x, y = max(a, lo), min(b, lo + arr.shape[0])
                if x < y:
                    parts.append(arr[x - lo:y - lo])
            return _cat(parts, 0)

        for tok in HEAD_ORDER.split():
            kind, arg = tok[0], tok[1:]
            if kind in 'KU':
                a, b = map(int, arg.split('-')) if arg else (0, S // TQ)
                w0 = DM + (DC if kind == 'U' else 0)
                w = wall[h, w0:w0 + DC, :]
                kv[kind].append((a * TQ, _dot(ckv[a * TQ:b * TQ, :], w, NN).astype(bf16)))
                continue
            if kind == 'O':
                grp = [int(ch) for ch in arg]
                res = _dot(wot[h], _cat([ctxs[j] for j in grp], 0), NT)
                for n, j in enumerate(grp):
                    ot[DM:2 * DM, j * TQ:(j + 1) * TQ] += res[:, n * TQ:(n + 1) * TQ]
                continue
            i = int(arg)
            r0 = i * TQ
            lm = r0 + LN
            if kind == 'Q':
                q = q_all[h, r0:r0 + TQ, :]
                s = _dot(q, rows('K', 0, lm), NT)
                sx = jnp.where(tri, _dot(q[LN:], rows('K', lm, lm + LN), NT), neg)
                scores[i] = (s, sx)
            elif kind == 'S':
                s, sx = scores.pop(i)
                sd = jnp.where(tri, s[0:LN, r0:lm], neg)
                pt, lt = _softmax_rows(([s[0:LN, 0:r0]] if i else []) + [sd])
                pb, lb = _softmax_rows([s[LN:], sx])
                probs[i] = (jnp.concatenate([_cat(pt, 1), pb[0]], axis=0), pb[1], lt, lb)
            else:
                p, px, lt, lb = probs.pop(i)
                ctx = _dot(p, rows('U', 0, lm), NN)
                cx = _dot(px, rows('U', lm, lm + LN), NN)
                ctxs[i] = jnp.concatenate([ctx[0:LN] * (1.0 / lt), (ctx[LN:] + cx) * (1.0 / lb)],
                                          axis=0).astype(bf16)
        return carry

    if do_b:
        with scope('P3'):
            jax.lax.fori_loop(0, H, head, 0)

    def ocopy(c):
        rows = pl.ds(pl.multiple_of(c * OCH, OCH), OCH)
        return pltpu.make_async_copy(obuf.at[rows], out_hbm.at[rows, YC:2 * DM], osem.at[c])

    def ostep(c, carry):
        for k in range(OCH // LN):
            cols = pl.ds(pl.multiple_of(c * OCH + k * LN, LN), LN)
            obuf[cols, :] = ot[YC:2 * DM, cols].astype(bf16).T
        ocopy(c).start()
        return carry

    with scope('fin'):
        jax.lax.fori_loop(0, S // OCH, ostep, 0)
    with scope('wt_out'):
        c_y.wait()
        for c in range(S // OCH):
            ocopy(c).wait()


def _build(do_a=True, do_b=True, scopes=False, order=None):
    global HEAD_ORDER
    if order is not None:
        HEAD_ORDER = order
    def run(A_x, A_w_r, A_w_i, B_x, B_c_kv, B_w_q, B_w_uk, B_w_uv, B_w_o):
        axt = jnp.swapaxes(A_x, 1, 2).reshape(DM, S)
        bxt = jnp.swapaxes(B_x, 1, 2).reshape(DM, S)
        wrt = A_w_r.T
        wit = A_w_i.T
        ckv = B_c_kv.reshape(S, DC)
        wot = jnp.swapaxes(B_w_o, 1, 2)
        tabs = [jnp.asarray(t) for t in _tables()]
        args = (axt, wrt, wit, bxt, ckv, B_w_q, B_w_uk, B_w_uv, wot, *tabs)
        vm = pltpu.VMEM
        scratch = [
            vm((DM, S), bf16), vm((J, S), bf16), vm((J, S), bf16),
            vm(tabs[0].shape, bf16), vm(tabs[1].shape, bf16), vm(tabs[2].shape, f32),
            vm(tabs[3].shape, bf16), vm(tabs[4].shape, bf16),
            vm((DM, S), bf16), vm((S, DC), bf16),
            vm((DM, H, D), bf16),
            vm((DC, H, D), bf16), vm((DC, H, D), bf16), vm((H + 2, DM + 2 * DC, D), bf16),
            vm((H, DM, D), bf16), vm((H, S, D), bf16),
            vm((2 * DM, S), f32), vm((S, YC), bf16), vm((S, 2 * DM - YC), bf16),
            pltpu.SemaphoreType.DMA((15,)), pltpu.SemaphoreType.DMA((2, H)),
            pltpu.SemaphoreType.DMA((S // OCH,)), pltpu.SemaphoreType.DMA((1,)),
        ]
        out = pl.pallas_call(
            functools.partial(_kernel, do_a=do_a, do_b=do_b, scopes=scopes),
            in_specs=[pl.BlockSpec(memory_space=pl.ANY)] * len(args),
            out_specs=pl.BlockSpec(memory_space=pl.ANY),
            out_shape=jax.ShapeDtypeStruct((S, 2 * DM), bf16),
            scratch_shapes=scratch,
            compiler_params=pltpu.CompilerParams(vmem_limit_bytes=120 * 2**20),
        )(*args)
        return out.reshape(1, S, 2 * DM)

    return run


_run = _build()


@jax.jit
def pallas_concat_heads__spectral_gfnet__compressed_kv_cla__prompt_kernel(
    A_x: jax.Array,
    A_w_r: jax.Array,
    A_w_i: jax.Array,
    B_x: jax.Array,
    B_c_kv: jax.Array,
    B_w_q: jax.Array,
    B_w_uk: jax.Array,
    B_w_uv: jax.Array,
    B_w_o: jax.Array,
):
    return _run(A_x, A_w_r, A_w_i, B_x, B_c_kv, B_w_q, B_w_uk, B_w_uv, B_w_o)
```

```python
import contextlib
import functools
import math

import jax
import jax.numpy as jnp
import numpy as np
import jax.experimental.pallas as pl
import jax.experimental.pallas.tpu as pltpu

f32 = jnp.float32
bf16 = jnp.bfloat16

NN = (((1,), (0,)), ((), ()))
NT = (((1,), (1,)), ((), ()))

S = 2048
DM = 448
J = DM // 2 + 1
HD = DM // 2
JA = 120
JB = 112
H = 16
D = 256
DC = 1024
R16 = 16
LN = 128
TQ = 256
CCH = DC // H
PX = H
YC = 384
HEAD_ORDER = ('K0-8 U0-3 Q4 U4-8 U3-4 Q1 S1 Q0 S4 V4 Q6 Q3 S0 V0 V1 S6 Q5 S3 V6 S5 Q7 S7 V3 V7 Q2 V5 O0 S2 V2 O7521 O34 O6')
OCH = 256
QHEADS = 2
QPIECES = 16


def _dot(a, b, dn):
    return jax.lax.dot_general(a, b, dn, preferred_element_type=f32)


@functools.lru_cache(maxsize=None)
def _tables():
    j = np.arange(J)[:, None].astype(np.float64)
    d = np.arange(DM)[None, :].astype(np.float64)
    ang = 2.0 * np.pi * ((j * d) % DM) / DM
    cos, sin = np.cos(ang), np.sin(ang)
    ne, no = (J + 1) // 2, J // 2
    fd = np.zeros((2 * JA + 2 * JB, HD), np.float64)
    fd[0:ne] = cos[0::2, 0:HD]
    fd[JA:JA + ne] = -sin[0::2, 0:HD]
    fd[2 * JA:2 * JA + no] = cos[1::2, 0:HD]
    fd[2 * JA + JB:2 * JA + JB + no] = -sin[1::2, 0:HD]

    m = np.arange(LN)[:, None].astype(np.float64)
    l = np.arange(LN)[None, :].astype(np.float64)
    a128 = 2.0 * np.pi * ((m * l) % LN) / LN
    fr, fi = np.cos(a128), -np.sin(a128)
    l2 = np.block([[fr, -fi], [fi, fr]])

    r = np.arange(R16)[:, None].astype(np.float64)
    at = 2.0 * np.pi * (r * l) / S
    tw = np.stack([np.cos(at), -np.sin(at)])
    tw = np.broadcast_to(tw[:, :, None, :], (2, R16, 8, LN)).copy()

    l3 = np.zeros((R16, 2 * LN, LN), np.float64)
    for rr in range(R16):
        a3 = 2.0 * np.pi * ((m * (rr + R16 * l)) % S) / S
        l3[rr] = np.concatenate([np.cos(a3), np.sin(a3)], axis=0)

    cj = np.full((J,), 2.0)
    cj[0] = 1.0
    cj[J - 1] = 1.0
    scale = cj[None, :] / float(S * DM)
    cr, ci = cos.T[0:HD] * scale, -sin.T[0:HD] * scale
    l4 = np.zeros((2, HD, 2 * LN), np.float64)
    l4[0, :, 0:ne] = cr[:, 0::2]
    l4[0, :, LN:LN + ne] = ci[:, 0::2]
    l4[1, :, 0:no] = cr[:, 1::2]
    l4[1, :, LN:LN + no] = ci[:, 1::2]

    cast = lambda a, dt: np.asarray(a, np.float32).astype(dt)
    return (cast(fd, bf16), cast(l2, bf16), cast(tw, np.float32), cast(l3, bf16),
            cast(l4.reshape(2 * HD, 2 * LN), bf16))


def _cmul_const(z, k, n, sign):
    re, im = z
    k = k % n
    if k == 0:
        return re, im
    if 4 * k == n:
        return (-im, re) if sign > 0 else (im, -re)
    if 8 * k == n:
        c = math.sqrt(0.5)
        return ((re - im) * c, (re + im) * c) if sign > 0 else ((re + im) * c, (im - re) * c)
    if 8 * k == 3 * n:
        c = math.sqrt(0.5)
        return ((re + im) * (-c), (re - im) * c) if sign > 0 else ((im - re) * c, (re + im) * (-c))
    c = math.cos(2.0 * math.pi * k / n)
    s = sign * math.sin(2.0 * math.pi * k / n)
    return re * c - im * s, re * s + im * c


def _fft(zs, sign):
    n = len(zs)
    if n == 1:
        return zs
    ev = _fft(zs[0::2], sign)
    od = _fft(zs[1::2], sign)
    out = [None] * n
    for k in range(n // 2):
        if 4 * k == n:
            (er, ei), (orr, oi) = ev[k], od[k]
            if sign > 0:
                out[k] = (er - oi, ei + orr)
                out[k + n // 2] = (er + oi, ei - orr)
            else:
                out[k] = (er + oi, ei - orr)
                out[k + n // 2] = (er - oi, ei + orr)
            continue
        tr, ti = _cmul_const(od[k], k, n, sign)
        er, ei = ev[k]
        out[k] = (er + tr, ei + ti)
        out[k + n // 2] = (er - tr, ei - ti)
    return out


def _softmax_rows(segs):
    m = functools.reduce(jnp.maximum, [jnp.max(sg, axis=1, keepdims=True) for sg in segs])
    ps = [jnp.exp2(sg - m).astype(bf16) for sg in segs]
    l = functools.reduce(jnp.add, [jnp.sum(p.astype(f32), axis=1, keepdims=True) for p in ps])
    return ps, l


def _cat(parts, axis):
    return jnp.concatenate(parts, axis=axis) if len(parts) > 1 else parts[0]


def _kernel(axt_hbm, wrt_hbm, wit_hbm, bxt_hbm, ckv_hbm, wq_hbm, wuk_hbm, wuv_hbm, wot_hbm,
            fd_hbm, l2_hbm, tw_hbm, l3_hbm, l4_hbm,
            out_hbm,
            axt, wrt, wit, fd, l2, tw, l3, l4,
            bxt, ckv, wq_raw, wuk_raw, wuv_raw, wall, wot, q_all,
            ot, ybuf, obuf, sem, wsem, osem, ysem, *, do_a, do_b, scopes):
    scope = jax.named_scope if scopes else (lambda name: contextlib.nullcontext())
    XC = S // 4
    simple = ([(fd_hbm, fd)]
              + [(axt_hbm.at[:, c * XC:(c + 1) * XC], axt.at[:, c * XC:(c + 1) * XC]) for c in range(4)]
              + [(tw_hbm, tw), (l2_hbm, l2), (wrt_hbm, wrt), (wit_hbm, wit),
                 (l3_hbm, l3), (l4_hbm, l4), (wq_hbm, wq_raw), (bxt_hbm, bxt), (ckv_hbm, ckv), (wot_hbm, wot)])
    cps = [pltpu.make_async_copy(s, d, sem.at[i]) for i, (s, d) in enumerate(simple)]
    c_fd = cps[0]
    (c_tw, c_l2, c_wrt, c_wit, c_l3, c_l4, c_wq, c_bxt, c_ckv, c_wot) = cps[5:]

    def wchunk(which, t):
        src, dst = ((wuk_hbm, wuk_raw), (wuv_hbm, wuv_raw))[which]
        return pltpu.make_async_copy(src.at[pl.ds(t * CCH, CCH)], dst.at[pl.ds(t * CCH, CCH)], wsem.at[which, t])

    def issue(lo, hi):
        def body(i, carry):
            for k in range(lo, hi):
                pl.when(i == k)(cps[k].start)
            return carry
        jax.lax.fori_loop(lo, hi, body, 0)

    def wait_all(cs):
        def body(i, carry):
            for k, c in enumerate(cs):
                pl.when(i == k)(c.wait)
            return carry
        jax.lax.fori_loop(0, max(2, len(cs)), body, 0)

    def issue_w(t, carry):
        wchunk(0, t).start()
        wchunk(1, t).start()
        return carry

    with scope('issue'):
        issue(0, len(cps) - 2)
        jax.lax.fori_loop(0, H, issue_w, 0)
        issue(len(cps) - 2, len(cps))

    def zero(i, carry):
        ot[pl.ds(pl.multiple_of(DM + i * 64, 64), 64), :] = jnp.zeros((64, S), f32)
        return carry

    with scope('zero'):
        jax.lax.fori_loop(0, DM // 64, zero, 0)

    def x_prep(k):
        rr = jax.lax.broadcasted_iota(jnp.int32, (LN, LN), 0)
        cc = jax.lax.broadcasted_iota(jnp.int32, (LN, LN), 1)
        eye = jnp.where(rr == cc, 1.0, 0.0).astype(bf16)
        x = _dot(eye, bxt[:, k * LN:(k + 1) * LN], NT).astype(bf16)
        wall[PX, k * LN:(k + 1) * LN, :] = x[:, 0:D]
        wall[PX + 1, k * LN:(k + 1) * LN, 0:DM - D] = x[:, D:DM]

    def wq_prep(k, n):
        g = DM // 16
        lo, hi = 16 * (k * g // n), 16 * ((k + 1) * g // n)
        wall[0:H, lo:hi, :] = jnp.swapaxes(wq_raw[lo:hi], 0, 1)

    def part_a(x1a, x1b, rma, rmb, wsa, wsb, csa, csb, us):
        def stage1(c, carry):
            cols = pl.ds(pl.multiple_of(c * XC, XC), XC)
            pltpu.make_async_copy(axt_hbm.at[:, cols], axt.at[:, cols], sem.at[1 + c]).wait()
            lo, hi = axt[0:HD, cols].astype(f32), axt[HD:DM, cols].astype(f32)
            x1a[:, cols] = _dot(fd[0:2 * JA, :], (lo + hi).astype(bf16), NN)
            x1b[:, cols] = _dot(fd[2 * JA:, :], (lo - hi).astype(bf16), NN)
            return carry

        def fwd16(x1, rm, n, r0):
            zs = [(x1[pl.ds(r0, 8), c * LN:(c + 1) * LN], x1[pl.ds(n + r0, 8), c * LN:(c + 1) * LN])
                  for c in range(R16)]
            ys = _fft(zs, -1)
            for r in range(R16):
                re, im = ys[r]
                if r:
                    tr, ti = tw[0, r], tw[1, r]
                    re, im = re * tr - im * ti, re * ti + im * tr
                rm[r, pl.ds(r0, 8), 0:LN] = re
                rm[r, pl.ds(r0, 8), LN:2 * LN] = im

        def wprep(c):
            cols = slice(c * LN, (c + 1) * LN)
            row = jax.lax.broadcasted_iota(jnp.int32, (LN - JB, LN), 0)
            for p, wt in enumerate((wrt, wit)):
                u = pltpu.bitcast(wt[0:J - 1, cols], jnp.uint32)
                even = pltpu.bitcast(u << 16, f32)
                odd = pltpu.bitcast(u & jnp.uint32(0xFFFF0000), f32)
                last = jnp.broadcast_to(wt[J - 1:J, cols].astype(f32), (LN - JB, LN))
                wsa[p, cols, :] = jnp.concatenate([even, jnp.where(row == 0, last, 0.0)], axis=0).T
                wsb[p, cols, :] = jnp.concatenate([odd, jnp.zeros((LN - JB, LN), f32)], axis=0).T

        def stage2(rm, k):
            return _dot(l2[...], rm[4 * k:4 * k + 4].reshape(4 * LN, 2 * LN).astype(bf16), NT)

        def stage3(x, ws, cs, r):
            x = x[r // 4]
            c0 = (r % 4) * LN
            xr, xi = x[0:LN, c0:c0 + LN], x[LN:2 * LN, c0:c0 + LN]
            wr = ws[0, pl.ds(r, LN, stride=R16), :]
            wi = ws[1, pl.ds(r, LN, stride=R16), :]
            g = jnp.concatenate([xr * wr - xi * wi, xr * wi + xi * wr], axis=1).astype(bf16)
            c = _dot(l3[r], g, NN)
            cs[r, 0:LN, :] = c[0:LN, 0:LN] - c[LN:2 * LN, LN:2 * LN]
            cs[r, LN:2 * LN, :] = c[LN:2 * LN, 0:LN] + c[0:LN, LN:2 * LN]

        def inv16(cs, half, r0):
            zs = [(cs[r, r0:r0 + 8, :], cs[r, LN + r0:LN + r0 + 8, :]) for r in range(R16)]
            ys = _fft(zs, +1)
            for c in range(R16):
                us[half, c * LN + r0:c * LN + r0 + 8, 0:LN] = ys[c][0].astype(bf16)
                us[half, c * LN + r0:c * LN + r0 + 8, LN:2 * LN] = ys[c][1].astype(bf16)

        def stage4(half, k):
            cols = slice(k * LN, (k + 1) * LN)
            y = _dot(l4[half * HD:(half + 1) * HD, :], us[half, cols, :], NT)
            if half:
                ot[0:HD, cols] += y
                ot[HD:DM, cols] -= y
            else:
                ot[0:HD, cols] = y
                ot[HD:DM, cols] = y

        with scope('w0'):
            c_fd.wait()
        with scope('S1'):
            jax.lax.fori_loop(0, 4, stage1, 0)
        with scope('wt_tw'):
            wait_all([c_tw])

        def fwd16a(g, carry):
            fwd16(x1a, rma, JA, pl.multiple_of(g * 8, 8))
            return carry

        def fwd16b(g, carry):
            fwd16(x1b, rmb, JB, pl.multiple_of(g * 8, 8))
            return carry

        with scope('F16'):
            jax.lax.fori_loop(0, JA // 8, fwd16a, 0)
            jax.lax.fori_loop(0, JB // 8, fwd16b, 0)
        with scope('wt_l2'):
            wait_all([c_l2, c_wrt, c_wit])
        rma[:, JA:LN, :] = jnp.zeros((R16, LN - JA, 2 * LN), f32)
        rmb[:, JB:LN, :] = jnp.zeros((R16, LN - JB, 2 * LN), f32)
        xa, xb = [], []
        for k in range(8):
            wprep(2 * k)
            wprep(2 * k + 1)
            (xa, xb)[k // 4].append(stage2((rma, rmb)[k // 4], k % 4))
        with scope('wt_W'):
            wait_all([c_l3, c_l4])
        for r in range(R16):
            stage3(xa, wsa, csa, r)
        for r in range(R16):
            stage3(xb, wsb, csb, r)
            inv16(csa, 0, r * 8)
        for k in range(R16):
            stage4(0, k)
            inv16(csb, 1, k * 8)
        with scope('wt_wq'):
            wait_all([c_wq])
        for k in range(R16):
            if do_b:
                wq_prep(k, R16)
            stage4(1, k)

    if do_a:
        pl.run_scoped(part_a,
                      pltpu.VMEM((2 * JA, S), f32), pltpu.VMEM((2 * JB, S), f32),
                      pltpu.VMEM((R16, LN, 2 * LN), f32), pltpu.VMEM((R16, LN, 2 * LN), f32),
                      pltpu.VMEM((2, S, LN), f32), pltpu.VMEM((2, S, LN), f32),
                      pltpu.VMEM((R16, 2 * LN, LN), f32), pltpu.VMEM((R16, 2 * LN, LN), f32),
                      pltpu.VMEM((2, S, 2 * LN), bf16))
    else:
        for c in cps[:-3]:
            c.wait()
        ot[0:DM, :] = jnp.zeros((DM, S), f32)
        if do_b:
            for k in range(R16):
                wq_prep(k, R16)

    with scope('wt_x'):
        wait_all([c_bxt])
    for k in range(R16):
        cols = slice(k * LN, (k + 1) * LN)
        ybuf[cols, :] = ot[0:YC, cols].astype(bf16).T
        if do_b:
            x_prep(k)
    c_y = pltpu.make_async_copy(ybuf, out_hbm.at[:, 0:YC], ysem.at[0])
    c_y.start()

    qscale = (D ** -0.5) * math.log2(math.e)

    with scope('wt_c0'):
        for u in range(QHEADS):
            wchunk(0, u).wait()
            wchunk(1, u).wait()

    def qstep(tt, carry):
        if do_b:
            rq, rw = S // QPIECES, 2 * CCH // QPIECES
            for u in range(QHEADS):
                t = tt * QHEADS + u
                for j in range(QPIECES):
                    x = jnp.concatenate([wall[PX, j * rq:(j + 1) * rq, :], wall[PX + 1, j * rq:(j + 1) * rq, 0:DM - D]],
                                        axis=1)
                    q_all[t, j * rq:(j + 1) * rq] = (_dot(x, wall[t, 0:DM, :], NN) * qscale).astype(bf16)
                    which, off = divmod(j * rw, CCH)
                    r0 = pl.multiple_of(t * CCH + off, rw)
                    src = (wuk_raw, wuv_raw)[which]
                    wall[0:H, pl.ds(DM + which * DC + r0, rw), :] = jnp.swapaxes(src[pl.ds(r0, rw)], 0, 1)

        @pl.when(tt + 1 < H // QHEADS)
        def _():
            for u in range(QHEADS):
                wchunk(0, (tt + 1) * QHEADS + u).wait()
                wchunk(1, (tt + 1) * QHEADS + u).wait()

        return carry

    with scope('P2'):
        jax.lax.fori_loop(0, H // QHEADS, qstep, 0)
    with scope('wt_ckv'):
        c_ckv.wait()
        c_wot.wait()

    def head(h, carry):
        with scope('head'):
            return head_body(h, carry)

    def head_body(h, carry):
        rr = jax.lax.broadcasted_iota(jnp.int32, (LN, LN), 0)
        cc = jax.lax.broadcasted_iota(jnp.int32, (LN, LN), 1)
        tri = cc <= rr
        neg = -1e9 * math.log2(math.e)
        kv = {'K': [], 'U': []}
        scores, probs, ctxs = {}, {}, {}

        def rows(name, a, b):
            parts = []
            for lo, arr in sorted(kv[name], key=lambda x: x[0]):
                x, y = max(a, lo), min(b, lo + arr.shape[0])
                if x < y:
                    parts.append(arr[x - lo:y - lo])
            return _cat(parts, 0)

        for tok in HEAD_ORDER.split():
            kind, arg = tok[0], tok[1:]
            if kind in 'KU':
                a, b = map(int, arg.split('-')) if arg else (0, S // TQ)
                w0 = DM + (DC if kind == 'U' else 0)
                w = wall[h, w0:w0 + DC, :]
                kv[kind].append((a * TQ, _dot(ckv[a * TQ:b * TQ, :], w, NN).astype(bf16)))
                continue
            if kind == 'O':
                grp = [int(ch) for ch in arg]
                res = _dot(wot[h], _cat([ctxs[j] for j in grp], 0), NT)
                for n, j in enumerate(grp):
                    ot[DM:2 * DM, j * TQ:(j + 1) * TQ] += res[:, n * TQ:(n + 1) * TQ]
                continue
            i = int(arg)
            r0 = i * TQ
            lm = r0 + LN
            if kind == 'Q':
                q = q_all[h, r0:r0 + TQ, :]
                s = _dot(q, rows('K', 0, lm), NT)
                sx = jnp.where(tri, _dot(q[LN:], rows('K', lm, lm + LN), NT), neg)
                scores[i] = (s, sx)
            elif kind == 'S':
                s, sx = scores.pop(i)
                sd = jnp.where(tri, s[0:LN, r0:lm], neg)
                pt, lt = _softmax_rows(([s[0:LN, 0:r0]] if i else []) + [sd])
                pb, lb = _softmax_rows([s[LN:], sx])
                probs[i] = (jnp.concatenate([_cat(pt, 1), pb[0]], axis=0), pb[1], lt, lb)
            else:
                p, px, lt, lb = probs.pop(i)
                ctx = _dot(p, rows('U', 0, lm), NN)
                cx = _dot(px, rows('U', lm, lm + LN), NN)
                ctxs[i] = jnp.concatenate([ctx[0:LN] * (1.0 / lt), (ctx[LN:] + cx) * (1.0 / lb)],
                                          axis=0).astype(bf16)
        return carry

    if do_b:
        with scope('P3'):
            jax.lax.fori_loop(0, H, head, 0)

    def ocopy(c):
        rows = pl.ds(pl.multiple_of(c * OCH, OCH), OCH)
        return pltpu.make_async_copy(obuf.at[rows], out_hbm.at[rows, YC:2 * DM], osem.at[c])

    def ostep(c, carry):
        for k in range(OCH // LN):
            cols = pl.ds(pl.multiple_of(c * OCH + k * LN, LN), LN)
            obuf[cols, :] = ot[YC:2 * DM, cols].astype(bf16).T
        ocopy(c).start()
        return carry

    with scope('fin'):
        jax.lax.fori_loop(0, S // OCH, ostep, 0)
    with scope('wt_out'):
        c_y.wait()
        for c in range(S // OCH):
            ocopy(c).wait()


def _build(do_a=True, do_b=True, scopes=False, order=None):
    global HEAD_ORDER
    if order is not None:
        HEAD_ORDER = order
    def run(A_x, A_w_r, A_w_i, B_x, B_c_kv, B_w_q, B_w_uk, B_w_uv, B_w_o):
        axt = jnp.swapaxes(A_x, 1, 2).reshape(DM, S)
        bxt = jnp.swapaxes(B_x, 1, 2).reshape(DM, S)
        wrt = A_w_r.T
        wit = A_w_i.T
        ckv = B_c_kv.reshape(S, DC)
        wot = jnp.swapaxes(B_w_o, 1, 2)
        tabs = [jnp.asarray(t) for t in _tables()]
        args = (axt, wrt, wit, bxt, ckv, B_w_q, B_w_uk, B_w_uv, wot, *tabs)
        vm = pltpu.VMEM
        scratch = [
            vm((DM, S), bf16), vm((J, S), bf16), vm((J, S), bf16),
            vm(tabs[0].shape, bf16), vm(tabs[1].shape, bf16), vm(tabs[2].shape, f32),
            vm(tabs[3].shape, bf16), vm(tabs[4].shape, bf16),
            vm((DM, S), bf16), vm((S, DC), bf16),
            vm((DM, H, D), bf16),
            vm((DC, H, D), bf16), vm((DC, H, D), bf16), vm((H + 2, DM + 2 * DC, D), bf16),
            vm((H, DM, D), bf16), vm((H, S, D), bf16),
            vm((2 * DM, S), f32), vm((S, YC), bf16), vm((S, 2 * DM - YC), bf16),
            pltpu.SemaphoreType.DMA((15,)), pltpu.SemaphoreType.DMA((2, H)),
            pltpu.SemaphoreType.DMA((S // OCH,)), pltpu.SemaphoreType.DMA((1,)),
        ]
        out = pl.pallas_call(
            functools.partial(_kernel, do_a=do_a, do_b=do_b, scopes=scopes),
            in_specs=[pl.BlockSpec(memory_space=pl.ANY)] * len(args),
            out_specs=pl.BlockSpec(memory_space=pl.ANY),
            out_shape=jax.ShapeDtypeStruct((S, 2 * DM), bf16),
            scratch_shapes=scratch,
            compiler_params=pltpu.CompilerParams(vmem_limit_bytes=120 * 2**20),
        )(*args)
        return out.reshape(1, S, 2 * DM)

    return run


_run = _build()


@jax.jit
def pallas_concat_heads__spectral_gfnet__compressed_kv_cla__prompt_kernel(
    A_x: jax.Array,
    A_w_r: jax.Array,
    A_w_i: jax.Array,
    B_x: jax.Array,
    B_c_kv: jax.Array,
    B_w_q: jax.Array,
    B_w_uk: jax.Array,
    B_w_uv: jax.Array,
    B_w_o: jax.Array,
):
    return _run(A_x, A_w_r, A_w_i, B_x, B_c_kv, B_w_q, B_w_uk, B_w_uv, B_w_o)
```

```python
import contextlib
import functools
import math

import jax
import jax.numpy as jnp
import numpy as np
import jax.experimental.pallas as pl
import jax.experimental.pallas.tpu as pltpu

f32 = jnp.float32
bf16 = jnp.bfloat16

NN = (((1,), (0,)), ((), ()))
NT = (((1,), (1,)), ((), ()))

S = 2048
DM = 448
J = DM // 2 + 1
HD = DM // 2
JA = 120
JB = 112
H = 16
D = 256
DC = 1024
R16 = 16
LN = 128
TQ = 256
CCH = DC // H
PX = H
YC = 384
HEAD_ORDER = ('K0-8 U0-3 Q4 U4-8 U3-4 Q1 S1 Q0 S4 V4 Q6 Q3 S0 V0 V1 S6 Q5 S3 V6 S5 Q7 S7 V3 V7 Q2 V5 O0 S2 V2 O7521 O34 O6')
NWQ = 14
OCH = 256
QHEADS = 2
QPIECES = 16


def _dot(a, b, dn):
    return jax.lax.dot_general(a, b, dn, preferred_element_type=f32)


@functools.lru_cache(maxsize=None)
def _tables():
    j = np.arange(J)[:, None].astype(np.float64)
    d = np.arange(DM)[None, :].astype(np.float64)
    ang = 2.0 * np.pi * ((j * d) % DM) / DM
    cos, sin = np.cos(ang), np.sin(ang)
    ne, no = (J + 1) // 2, J // 2
    fd = np.zeros((2 * JA + 2 * JB, HD), np.float64)
    fd[0:ne] = cos[0::2, 0:HD]
    fd[JA:JA + ne] = -sin[0::2, 0:HD]
    fd[2 * JA:2 * JA + no] = cos[1::2, 0:HD]
    fd[2 * JA + JB:2 * JA + JB + no] = -sin[1::2, 0:HD]

    m = np.arange(LN)[:, None].astype(np.float64)
    l = np.arange(LN)[None, :].astype(np.float64)
    a128 = 2.0 * np.pi * ((m * l) % LN) / LN
    fr, fi = np.cos(a128), -np.sin(a128)
    l2 = np.block([[fr, -fi], [fi, fr]])

    r = np.arange(R16)[:, None].astype(np.float64)
    at = 2.0 * np.pi * (r * l) / S
    tw = np.stack([np.cos(at), -np.sin(at)])
    tw = np.broadcast_to(tw[:, :, None, :], (2, R16, 8, LN)).copy()

    l3 = np.zeros((R16, 2 * LN, LN), np.float64)
    for rr in range(R16):
        a3 = 2.0 * np.pi * ((m * (rr + R16 * l)) % S) / S
        l3[rr] = np.concatenate([np.cos(a3), np.sin(a3)], axis=0)

    cj = np.full((J,), 2.0)
    cj[0] = 1.0
    cj[J - 1] = 1.0
    scale = cj[None, :] / float(S * DM)
    cr, ci = cos.T[0:HD] * scale, -sin.T[0:HD] * scale
    l4 = np.zeros((2, HD, 2 * LN), np.float64)
    l4[0, :, 0:ne] = cr[:, 0::2]
    l4[0, :, LN:LN + ne] = ci[:, 0::2]
    l4[1, :, 0:no] = cr[:, 1::2]
    l4[1, :, LN:LN + no] = ci[:, 1::2]

    cast = lambda a, dt: np.asarray(a, np.float32).astype(dt)
    return (cast(fd, bf16), cast(l2, bf16), cast(tw, np.float32), cast(l3, bf16),
            cast(l4.reshape(2 * HD, 2 * LN), bf16))


def _cmul_const(z, k, n, sign):
    re, im = z
    k = k % n
    if k == 0:
        return re, im
    if 4 * k == n:
        return (-im, re) if sign > 0 else (im, -re)
    if 8 * k == n:
        c = math.sqrt(0.5)
        return ((re - im) * c, (re + im) * c) if sign > 0 else ((re + im) * c, (im - re) * c)
    if 8 * k == 3 * n:
        c = math.sqrt(0.5)
        return ((re + im) * (-c), (re - im) * c) if sign > 0 else ((im - re) * c, (re + im) * (-c))
    c = math.cos(2.0 * math.pi * k / n)
    s = sign * math.sin(2.0 * math.pi * k / n)
    return re * c - im * s, re * s + im * c


def _fft(zs, sign):
    n = len(zs)
    if n == 1:
        return zs
    ev = _fft(zs[0::2], sign)
    od = _fft(zs[1::2], sign)
    out = [None] * n
    for k in range(n // 2):
        if 4 * k == n:
            (er, ei), (orr, oi) = ev[k], od[k]
            if sign > 0:
                out[k] = (er - oi, ei + orr)
                out[k + n // 2] = (er + oi, ei - orr)
            else:
                out[k] = (er + oi, ei - orr)
                out[k + n // 2] = (er - oi, ei + orr)
            continue
        tr, ti = _cmul_const(od[k], k, n, sign)
        er, ei = ev[k]
        out[k] = (er + tr, ei + ti)
        out[k + n // 2] = (er - tr, ei - ti)
    return out


def _softmax_rows(segs):
    m = functools.reduce(jnp.maximum, [jnp.max(sg, axis=1, keepdims=True) for sg in segs])
    ps = [jnp.exp2(sg - m).astype(bf16) for sg in segs]
    l = functools.reduce(jnp.add, [jnp.sum(p.astype(f32), axis=1, keepdims=True) for p in ps])
    return ps, l


def _cat(parts, axis):
    return jnp.concatenate(parts, axis=axis) if len(parts) > 1 else parts[0]


def _kernel(axt_hbm, wrt_hbm, wit_hbm, bxt_hbm, ckv_hbm, wq_hbm, wuk_hbm, wuv_hbm, wot_hbm,
            fd_hbm, l2_hbm, tw_hbm, l3_hbm, l4_hbm,
            out_hbm,
            axt, wrt, wit, fd, l2, tw, l3, l4,
            bxt, ckv, wq_raw, wuk_raw, wuv_raw, wall, wot, q_all,
            ot, ybuf, obuf, sem, wsem, osem, ysem, *, do_a, do_b, scopes):
    scope = jax.named_scope if scopes else (lambda name: contextlib.nullcontext())
    XC = S // 4
    simple = ([(fd_hbm, fd)]
              + [(axt_hbm.at[:, c * XC:(c + 1) * XC], axt.at[:, c * XC:(c + 1) * XC]) for c in range(4)]
              + [(tw_hbm, tw), (l2_hbm, l2), (wrt_hbm, wrt), (wit_hbm, wit),
                 (l3_hbm, l3), (l4_hbm, l4), (wq_hbm, wq_raw), (bxt_hbm, bxt), (ckv_hbm, ckv), (wot_hbm, wot)])
    cps = [pltpu.make_async_copy(s, d, sem.at[i]) for i, (s, d) in enumerate(simple)]
    c_fd = cps[0]
    (c_tw, c_l2, c_wrt, c_wit, c_l3, c_l4, c_wq, c_bxt, c_ckv, c_wot) = cps[5:]

    def wchunk(which, t):
        src, dst = ((wuk_hbm, wuk_raw), (wuv_hbm, wuv_raw))[which]
        return pltpu.make_async_copy(src.at[pl.ds(t * CCH, CCH)], dst.at[pl.ds(t * CCH, CCH)], wsem.at[which, t])

    def issue(lo, hi):
        def body(i, carry):
            for k in range(lo, hi):
                pl.when(i == k)(cps[k].start)
            return carry
        jax.lax.fori_loop(lo, hi, body, 0)

    def wait_all(cs):
        def body(i, carry):
            for k, c in enumerate(cs):
                pl.when(i == k)(c.wait)
            return carry
        jax.lax.fori_loop(0, max(2, len(cs)), body, 0)

    def issue_w(t, carry):
        wchunk(0, t).start()
        wchunk(1, t).start()
        return carry

    with scope('issue'):
        issue(0, len(cps) - 2)
        jax.lax.fori_loop(0, H, issue_w, 0)
        issue(len(cps) - 2, len(cps))

    def zero(i, carry):
        ot[pl.ds(pl.multiple_of(DM + i * 64, 64), 64), :] = jnp.zeros((64, S), f32)
        return carry

    with scope('zero'):
        jax.lax.fori_loop(0, DM // 64, zero, 0)

    def x_prep(k):
        rr = jax.lax.broadcasted_iota(jnp.int32, (LN, LN), 0)
        cc = jax.lax.broadcasted_iota(jnp.int32, (LN, LN), 1)
        eye = jnp.where(rr == cc, 1.0, 0.0).astype(bf16)
        x = _dot(eye, bxt[:, k * LN:(k + 1) * LN], NT).astype(bf16)
        wall[PX, k * LN:(k + 1) * LN, :] = x[:, 0:D]
        wall[PX + 1, k * LN:(k + 1) * LN, 0:DM - D] = x[:, D:DM]

    def wq_prep(k):
        n = DM // NWQ
        wall[0:H, k * n:(k + 1) * n, :] = jnp.swapaxes(wq_raw[k * n:(k + 1) * n], 0, 1)

    def part_a(x1a, x1b, rma, rmb, wsa, wsb, csa, csb, us):
        def stage1(c, carry):
            cols = pl.ds(pl.multiple_of(c * XC, XC), XC)
            pltpu.make_async_copy(axt_hbm.at[:, cols], axt.at[:, cols], sem.at[1 + c]).wait()
            lo, hi = axt[0:HD, cols].astype(f32), axt[HD:DM, cols].astype(f32)
            x1a[:, cols] = _dot(fd[0:2 * JA, :], (lo + hi).astype(bf16), NN)
            x1b[:, cols] = _dot(fd[2 * JA:, :], (lo - hi).astype(bf16), NN)
            return carry

        def fwd16(x1, rm, n, r0):
            zs = [(x1[pl.ds(r0, 8), c * LN:(c + 1) * LN], x1[pl.ds(n + r0, 8), c * LN:(c + 1) * LN])
                  for c in range(R16)]
            ys = _fft(zs, -1)
            for r in range(R16):
                re, im = ys[r]
                if r:
                    tr, ti = tw[0, r], tw[1, r]
                    re, im = re * tr - im * ti, re * ti + im * tr
                rm[r, pl.ds(r0, 8), 0:LN] = re
                rm[r, pl.ds(r0, 8), LN:2 * LN] = im

        def wprep(c):
            cols = slice(c * LN, (c + 1) * LN)
            row = jax.lax.broadcasted_iota(jnp.int32, (LN - JB, LN), 0)
            for p, wt in enumerate((wrt, wit)):
                u = pltpu.bitcast(wt[0:J - 1, cols], jnp.uint32)
                even = pltpu.bitcast(u << 16, f32)
                odd = pltpu.bitcast(u & jnp.uint32(0xFFFF0000), f32)
                last = jnp.broadcast_to(wt[J - 1:J, cols].astype(f32), (LN - JB, LN))
                wsa[p, cols, :] = jnp.concatenate([even, jnp.where(row == 0, last, 0.0)], axis=0).T
                wsb[p, cols, :] = jnp.concatenate([odd, jnp.zeros((LN - JB, LN), f32)], axis=0).T

        def stage2(rm, k):
            return _dot(l2[...], rm[4 * k:4 * k + 4].reshape(4 * LN, 2 * LN).astype(bf16), NT)

        def stage3(x, ws, cs, r):
            x = x[r // 4]
            c0 = (r % 4) * LN
            xr, xi = x[0:LN, c0:c0 + LN], x[LN:2 * LN, c0:c0 + LN]
            wr = ws[0, pl.ds(r, LN, stride=R16), :]
            wi = ws[1, pl.ds(r, LN, stride=R16), :]
            g = jnp.concatenate([xr * wr - xi * wi, xr * wi + xi * wr], axis=1).astype(bf16)
            c = _dot(l3[r], g, NN)
            cs[r, 0:LN, :] = c[0:LN, 0:LN] - c[LN:2 * LN, LN:2 * LN]
            cs[r, LN:2 * LN, :] = c[LN:2 * LN, 0:LN] + c[0:LN, LN:2 * LN]

        def inv16(cs, half, r0):
            zs = [(cs[r, r0:r0 + 8, :], cs[r, LN + r0:LN + r0 + 8, :]) for r in range(R16)]
            ys = _fft(zs, +1)
            for c in range(R16):
                us[half, c * LN + r0:c * LN + r0 + 8, 0:LN] = ys[c][0].astype(bf16)
                us[half, c * LN + r0:c * LN + r0 + 8, LN:2 * LN] = ys[c][1].astype(bf16)

        def stage4(half, k):
            cols = slice(k * LN, (k + 1) * LN)
            y = _dot(l4[half * HD:(half + 1) * HD, :], us[half, cols, :], NT)
            if half:
                ot[0:HD, cols] += y
                ot[HD:DM, cols] -= y
            else:
                ot[0:HD, cols] = y
                ot[HD:DM, cols] = y

        with scope('w0'):
            c_fd.wait()
        with scope('S1'):
            jax.lax.fori_loop(0, 4, stage1, 0)
        with scope('wt_tw'):
            wait_all([c_tw])

        def fwd16a(g, carry):
            fwd16(x1a, rma, JA, pl.multiple_of(g * 8, 8))
            return carry

        def fwd16b(g, carry):
            fwd16(x1b, rmb, JB, pl.multiple_of(g * 8, 8))
            return carry

        with scope('F16'):
            jax.lax.fori_loop(0, JA // 8, fwd16a, 0)
            jax.lax.fori_loop(0, JB // 8, fwd16b, 0)
        with scope('wt_l2'):
            wait_all([c_l2, c_wrt, c_wit])
        rma[:, JA:LN, :] = jnp.zeros((R16, LN - JA, 2 * LN), f32)
        rmb[:, JB:LN, :] = jnp.zeros((R16, LN - JB, 2 * LN), f32)
        xa, xb = [], []
        for k in range(8):
            wprep(2 * k)
            wprep(2 * k + 1)
            (xa, xb)[k // 4].append(stage2((rma, rmb)[k // 4], k % 4))
        with scope('wt_W'):
            wait_all([c_l3, c_l4])
        for r in range(R16):
            stage3(xa, wsa, csa, r)
        for r in range(R16):
            stage3(xb, wsb, csb, r)
            inv16(csa, 0, r * 8)
        for k in range(R16):
            stage4(0, k)
            inv16(csb, 1, k * 8)
        with scope('wt_wq'):
            wait_all([c_wq])
        done = 0
        for k in range(R16):
            while do_b and done * R16 < (k + 1) * NWQ and done < NWQ:
                wq_prep(done)
                done += 1
            stage4(1, k)

    if do_a:
        pl.run_scoped(part_a,
                      pltpu.VMEM((2 * JA, S), f32), pltpu.VMEM((2 * JB, S), f32),
                      pltpu.VMEM((R16, LN, 2 * LN), f32), pltpu.VMEM((R16, LN, 2 * LN), f32),
                      pltpu.VMEM((2, S, LN), f32), pltpu.VMEM((2, S, LN), f32),
                      pltpu.VMEM((R16, 2 * LN, LN), f32), pltpu.VMEM((R16, 2 * LN, LN), f32),
                      pltpu.VMEM((2, S, 2 * LN), bf16))
    else:
        for c in cps[:-3]:
            c.wait()
        ot[0:DM, :] = jnp.zeros((DM, S), f32)
        if do_b:
            for k in range(R16):
                wq_prep(k % NWQ)

    with scope('wt_x'):
        wait_all([c_bxt])
    for k in range(R16):
        cols = slice(k * LN, (k + 1) * LN)
        ybuf[cols, :] = ot[0:YC, cols].astype(bf16).T
        if do_b:
            x_prep(k)
    c_y = pltpu.make_async_copy(ybuf, out_hbm.at[:, 0:YC], ysem.at[0])
    c_y.start()

    qscale = (D ** -0.5) * math.log2(math.e)

    with scope('wt_c0'):
        for u in range(QHEADS):
            wchunk(0, u).wait()
            wchunk(1, u).wait()

    def qstep(tt, carry):
        if do_b:
            rq, rw = S // QPIECES, 2 * CCH // QPIECES
            for u in range(QHEADS):
                t = tt * QHEADS + u
                for j in range(QPIECES):
                    x = jnp.concatenate([wall[PX, j * rq:(j + 1) * rq, :], wall[PX + 1, j * rq:(j + 1) * rq, 0:DM - D]],
                                        axis=1)
                    q_all[t, j * rq:(j + 1) * rq] = (_dot(x, wall[t, 0:DM, :], NN) * qscale).astype(bf16)
                    which, off = divmod(j * rw, CCH)
                    r0 = pl.multiple_of(t * CCH + off, rw)
                    src = (wuk_raw, wuv_raw)[which]
                    wall[0:H, pl.ds(DM + which * DC + r0, rw), :] = jnp.swapaxes(src[pl.ds(r0, rw)], 0, 1)

        @pl.when(tt + 1 < H // QHEADS)
        def _():
            for u in range(QHEADS):
                wchunk(0, (tt + 1) * QHEADS + u).wait()
                wchunk(1, (tt + 1) * QHEADS + u).wait()

        return carry

    with scope('P2'):
        jax.lax.fori_loop(0, H // QHEADS, qstep, 0)
    with scope('wt_ckv'):
        c_ckv.wait()
        c_wot.wait()

    def head(h, carry):
        with scope('head'):
            return head_body(h, carry)

    def head_body(h, carry):
        rr = jax.lax.broadcasted_iota(jnp.int32, (LN, LN), 0)
        cc = jax.lax.broadcasted_iota(jnp.int32, (LN, LN), 1)
        tri = cc <= rr
        neg = -1e9 * math.log2(math.e)
        kv = {'K': [], 'U': []}
        scores, probs, ctxs = {}, {}, {}

        def rows(name, a, b):
            parts = []
            for lo, arr in sorted(kv[name], key=lambda x: x[0]):
                x, y = max(a, lo), min(b, lo + arr.shape[0])
                if x < y:
                    parts.append(arr[x - lo:y - lo])
            return _cat(parts, 0)

        for tok in HEAD_ORDER.split():
            kind, arg = tok[0], tok[1:]
            if kind in 'KU':
                a, b = map(int, arg.split('-')) if arg else (0, S // TQ)
                w0 = DM + (DC if kind == 'U' else 0)
                w = wall[h, w0:w0 + DC, :]
                kv[kind].append((a * TQ, _dot(ckv[a * TQ:b * TQ, :], w, NN).astype(bf16)))
                continue
            if kind == 'O':
                grp = [int(ch) for ch in arg]
                res = _dot(wot[h], _cat([ctxs[j] for j in grp], 0), NT)
                for n, j in enumerate(grp):
                    ot[DM:2 * DM, j * TQ:(j + 1) * TQ] += res[:, n * TQ:(n + 1) * TQ]
                continue
            i = int(arg)
            r0 = i * TQ
            lm = r0 + LN
            if kind == 'Q':
                q = q_all[h, r0:r0 + TQ, :]
                s = _dot(q, rows('K', 0, lm), NT)
                sx = jnp.where(tri, _dot(q[LN:], rows('K', lm, lm + LN), NT), neg)
                scores[i] = (s, sx)
            elif kind == 'S':
                s, sx = scores.pop(i)
                sd = jnp.where(tri, s[0:LN, r0:lm], neg)
                pt, lt = _softmax_rows(([s[0:LN, 0:r0]] if i else []) + [sd])
                pb, lb = _softmax_rows([s[LN:], sx])
                probs[i] = (jnp.concatenate([_cat(pt, 1), pb[0]], axis=0), pb[1], lt, lb)
            else:
                p, px, lt, lb = probs.pop(i)
                ctx = _dot(p, rows('U', 0, lm), NN)
                cx = _dot(px, rows('U', lm, lm + LN), NN)
                ctxs[i] = jnp.concatenate([ctx[0:LN] * (1.0 / lt), (ctx[LN:] + cx) * (1.0 / lb)],
                                          axis=0).astype(bf16)
        return carry

    if do_b:
        with scope('P3'):
            jax.lax.fori_loop(0, H, head, 0)

    def ocopy(c):
        rows = pl.ds(pl.multiple_of(c * OCH, OCH), OCH)
        return pltpu.make_async_copy(obuf.at[rows], out_hbm.at[rows, YC:2 * DM], osem.at[c])

    def ostep(c, carry):
        for k in range(OCH // LN):
            cols = pl.ds(pl.multiple_of(c * OCH + k * LN, LN), LN)
            obuf[cols, :] = ot[YC:2 * DM, cols].astype(bf16).T
        ocopy(c).start()
        return carry

    with scope('fin'):
        jax.lax.fori_loop(0, S // OCH, ostep, 0)
    with scope('wt_out'):
        c_y.wait()
        for c in range(S // OCH):
            ocopy(c).wait()


def _build(do_a=True, do_b=True, scopes=False, order=None):
    global HEAD_ORDER
    if order is not None:
        HEAD_ORDER = order
    def run(A_x, A_w_r, A_w_i, B_x, B_c_kv, B_w_q, B_w_uk, B_w_uv, B_w_o):
        axt = jnp.swapaxes(A_x, 1, 2).reshape(DM, S)
        bxt = jnp.swapaxes(B_x, 1, 2).reshape(DM, S)
        wrt = A_w_r.T
        wit = A_w_i.T
        ckv = B_c_kv.reshape(S, DC)
        wot = jnp.swapaxes(B_w_o, 1, 2)
        tabs = [jnp.asarray(t) for t in _tables()]
        args = (axt, wrt, wit, bxt, ckv, B_w_q, B_w_uk, B_w_uv, wot, *tabs)
        vm = pltpu.VMEM
        scratch = [
            vm((DM, S), bf16), vm((J, S), bf16), vm((J, S), bf16),
            vm(tabs[0].shape, bf16), vm(tabs[1].shape, bf16), vm(tabs[2].shape, f32),
            vm(tabs[3].shape, bf16), vm(tabs[4].shape, bf16),
            vm((DM, S), bf16), vm((S, DC), bf16),
            vm((DM, H, D), bf16),
            vm((DC, H, D), bf16), vm((DC, H, D), bf16), vm((H + 2, DM + 2 * DC, D), bf16),
            vm((H, DM, D), bf16), vm((H, S, D), bf16),
            vm((2 * DM, S), f32), vm((S, YC), bf16), vm((S, 2 * DM - YC), bf16),
            pltpu.SemaphoreType.DMA((15,)), pltpu.SemaphoreType.DMA((2, H)),
            pltpu.SemaphoreType.DMA((S // OCH,)), pltpu.SemaphoreType.DMA((1,)),
        ]
        out = pl.pallas_call(
            functools.partial(_kernel, do_a=do_a, do_b=do_b, scopes=scopes),
            in_specs=[pl.BlockSpec(memory_space=pl.ANY)] * len(args),
            out_specs=pl.BlockSpec(memory_space=pl.ANY),
            out_shape=jax.ShapeDtypeStruct((S, 2 * DM), bf16),
            scratch_shapes=scratch,
            compiler_params=pltpu.CompilerParams(vmem_limit_bytes=120 * 2**20),
        )(*args)
        return out.reshape(1, S, 2 * DM)

    return run


_run = _build()


@jax.jit
def pallas_concat_heads__spectral_gfnet__compressed_kv_cla__prompt_kernel(
    A_x: jax.Array,
    A_w_r: jax.Array,
    A_w_i: jax.Array,
    B_x: jax.Array,
    B_c_kv: jax.Array,
    B_w_q: jax.Array,
    B_w_uk: jax.Array,
    B_w_uv: jax.Array,
    B_w_o: jax.Array,
):
    return _run(A_x, A_w_r, A_w_i, B_x, B_c_kv, B_w_q, B_w_uk, B_w_uv, B_w_o)
```

```python
import contextlib
import functools
import math

import jax
import jax.numpy as jnp
import numpy as np
import jax.experimental.pallas as pl
import jax.experimental.pallas.tpu as pltpu

f32 = jnp.float32
bf16 = jnp.bfloat16

NN = (((1,), (0,)), ((), ()))
NT = (((1,), (1,)), ((), ()))

S = 2048
DM = 448
J = DM // 2 + 1
HD = DM // 2
JA = 120
JB = 112
H = 16
D = 256
DC = 1024
R16 = 16
LN = 128
TQ = 256
CCH = DC // H
PX = H
YC = 384
HEAD_ORDER = ('K0-8 U0-3 Q4 U4-8 U3-4 Q1 S1 Q0 S4 V4 Q6 Q3 S0 V0 V1 S6 Q5 S3 V6 S5 Q7 S7 V3 V7 Q2 V5 O0 S2 V2 O7521 O34 O6')
NWQ = 14
OCH = 256
QHEADS = 2
QPIECES = 16


def _dot(a, b, dn):
    return jax.lax.dot_general(a, b, dn, preferred_element_type=f32)


@functools.lru_cache(maxsize=None)
def _tables():
    j = np.arange(J)[:, None].astype(np.float64)
    d = np.arange(DM)[None, :].astype(np.float64)
    ang = 2.0 * np.pi * ((j * d) % DM) / DM
    cos, sin = np.cos(ang), np.sin(ang)
    ne, no = (J + 1) // 2, J // 2
    fd = np.zeros((2 * JA + 2 * JB, HD), np.float64)
    fd[0:ne] = cos[0::2, 0:HD]
    fd[JA:JA + ne] = -sin[0::2, 0:HD]
    fd[2 * JA:2 * JA + no] = cos[1::2, 0:HD]
    fd[2 * JA + JB:2 * JA + JB + no] = -sin[1::2, 0:HD]

    m = np.arange(LN)[:, None].astype(np.float64)
    l = np.arange(LN)[None, :].astype(np.float64)
    a128 = 2.0 * np.pi * ((m * l) % LN) / LN
    fr, fi = np.cos(a128), -np.sin(a128)
    l2 = np.block([[fr, -fi], [fi, fr]])

    r = np.arange(R16)[:, None].astype(np.float64)
    at = 2.0 * np.pi * (r * l) / S
    tw = np.stack([np.cos(at), -np.sin(at)])
    tw = np.broadcast_to(tw[:, :, None, :], (2, R16, 8, LN)).copy()

    l3 = np.zeros((R16, 2 * LN, LN), np.float64)
    for rr in range(R16):
        a3 = 2.0 * np.pi * ((m * (rr + R16 * l)) % S) / S
        l3[rr] = np.concatenate([np.cos(a3), np.sin(a3)], axis=0)

    cj = np.full((J,), 2.0)
    cj[0] = 1.0
    cj[J - 1] = 1.0
    scale = cj[None, :] / float(S * DM)
    cr, ci = cos.T[0:HD] * scale, -sin.T[0:HD] * scale
    l4 = np.zeros((2, HD, 2 * LN), np.float64)
    l4[0, :, 0:ne] = cr[:, 0::2]
    l4[0, :, LN:LN + ne] = ci[:, 0::2]
    l4[1, :, 0:no] = cr[:, 1::2]
    l4[1, :, LN:LN + no] = ci[:, 1::2]

    cast = lambda a, dt: np.asarray(a, np.float32).astype(dt)
    return (cast(fd, bf16), cast(l2, bf16), cast(tw, np.float32), cast(l3, bf16),
            cast(l4.reshape(2 * HD, 2 * LN), bf16))


def _cmul_const(z, k, n, sign):
    re, im = z
    k = k % n
    if k == 0:
        return re, im
    if 4 * k == n:
        return (-im, re) if sign > 0 else (im, -re)
    if 8 * k == n:
        c = math.sqrt(0.5)
        return ((re - im) * c, (re + im) * c) if sign > 0 else ((re + im) * c, (im - re) * c)
    if 8 * k == 3 * n:
        c = math.sqrt(0.5)
        return ((re + im) * (-c), (re - im) * c) if sign > 0 else ((im - re) * c, (re + im) * (-c))
    c = math.cos(2.0 * math.pi * k / n)
    s = sign * math.sin(2.0 * math.pi * k / n)
    return re * c - im * s, re * s + im * c


def _fft(zs, sign):
    n = len(zs)
    if n == 1:
        return zs
    ev = _fft(zs[0::2], sign)
    od = _fft(zs[1::2], sign)
    out = [None] * n
    for k in range(n // 2):
        if 4 * k == n:
            (er, ei), (orr, oi) = ev[k], od[k]
            if sign > 0:
                out[k] = (er - oi, ei + orr)
                out[k + n // 2] = (er + oi, ei - orr)
            else:
                out[k] = (er + oi, ei - orr)
                out[k + n // 2] = (er - oi, ei + orr)
            continue
        tr, ti = _cmul_const(od[k], k, n, sign)
        er, ei = ev[k]
        out[k] = (er + tr, ei + ti)
        out[k + n // 2] = (er - tr, ei - ti)
    return out


def _softmax_rows(segs):
    m = functools.reduce(jnp.maximum, [jnp.max(sg, axis=1, keepdims=True) for sg in segs])
    ps = [jnp.exp2(sg - m).astype(bf16) for sg in segs]
    l = functools.reduce(jnp.add, [jnp.sum(p.astype(f32), axis=1, keepdims=True) for p in ps])
    return ps, l


def _cat(parts, axis):
    return jnp.concatenate(parts, axis=axis) if len(parts) > 1 else parts[0]


def _kernel(axt_hbm, wrt_hbm, wit_hbm, bxt_hbm, ckv_hbm, wq_hbm, wuk_hbm, wuv_hbm, wot_hbm,
            fd_hbm, l2_hbm, tw_hbm, l3_hbm, l4_hbm,
            out_hbm,
            axt, wrt, wit, fd, l2, tw, l3, l4,
            bxt, ckv, wq_raw, wuk_raw, wuv_raw, wall, wot, q_all,
            ot, ybuf, obuf, sem, wsem, osem, ysem, *, do_a, do_b, scopes):
    scope = jax.named_scope if scopes else (lambda name: contextlib.nullcontext())
    XC = S // 4
    simple = ([(fd_hbm, fd)]
              + [(axt_hbm.at[:, c * XC:(c + 1) * XC], axt.at[:, c * XC:(c + 1) * XC]) for c in range(4)]
              + [(tw_hbm, tw), (l2_hbm, l2), (wrt_hbm, wrt), (wit_hbm, wit),
                 (l3_hbm, l3), (l4_hbm, l4), (wq_hbm, wq_raw), (bxt_hbm, bxt), (ckv_hbm, ckv), (wot_hbm, wot)])
    cps = [pltpu.make_async_copy(s, d, sem.at[i]) for i, (s, d) in enumerate(simple)]
    c_fd = cps[0]
    (c_tw, c_l2, c_wrt, c_wit, c_l3, c_l4, c_wq, c_bxt, c_ckv, c_wot) = cps[5:]

    def wchunk(which, t):
        src, dst = ((wuk_hbm, wuk_raw), (wuv_hbm, wuv_raw))[which]
        return pltpu.make_async_copy(src.at[pl.ds(t * CCH, CCH)], dst.at[pl.ds(t * CCH, CCH)], wsem.at[which, t])

    def issue(lo, hi):
        def body(i, carry):
            for k in range(lo, hi):
                pl.when(i == k)(cps[k].start)
            return carry
        jax.lax.fori_loop(lo, hi, body, 0)

    def wait_all(cs):
        def body(i, carry):
            for k, c in enumerate(cs):
                pl.when(i == k)(c.wait)
            return carry
        jax.lax.fori_loop(0, max(2, len(cs)), body, 0)

    def issue_w(t, carry):
        wchunk(0, t).start()
        wchunk(1, t).start()
        return carry

    with scope('issue'):
        issue(0, len(cps) - 2)
        jax.lax.fori_loop(0, H, issue_w, 0)
        issue(len(cps) - 2, len(cps))

    def zero(i, carry):
        ot[pl.ds(pl.multiple_of(DM + i * 64, 64), 64), :] = jnp.zeros((64, S), f32)
        return carry

    with scope('zero'):
        jax.lax.fori_loop(0, DM // 64, zero, 0)

    def x_prep(k):
        rr = jax.lax.broadcasted_iota(jnp.int32, (LN, LN), 0)
        cc = jax.lax.broadcasted_iota(jnp.int32, (LN, LN), 1)
        eye = jnp.where(rr == cc, 1.0, 0.0).astype(bf16)
        x = _dot(eye, bxt[:, k * LN:(k + 1) * LN], NT).astype(bf16)
        wall[PX, k * LN:(k + 1) * LN, :] = x[:, 0:D]
        wall[PX + 1, k * LN:(k + 1) * LN, 0:DM - D] = x[:, D:DM]

    def wq_prep(k):
        n = DM // NWQ
        wall[0:H, k * n:(k + 1) * n, :] = jnp.swapaxes(wq_raw[k * n:(k + 1) * n], 0, 1)

    def part_a(x1a, x1b, rma, rmb, wsa, wsb, csa, csb, us):
        def stage1(c, carry):
            cols = pl.ds(pl.multiple_of(c * XC, XC), XC)
            pltpu.make_async_copy(axt_hbm.at[:, cols], axt.at[:, cols], sem.at[1 + c]).wait()
            lo, hi = axt[0:HD, cols].astype(f32), axt[HD:DM, cols].astype(f32)
            x1a[:, cols] = _dot(fd[0:2 * JA, :], (lo + hi).astype(bf16), NN)
            x1b[:, cols] = _dot(fd[2 * JA:, :], (lo - hi).astype(bf16), NN)
            return carry

        def fwd16(x1, rm, n, r0):
            zs = [(x1[pl.ds(r0, 8), c * LN:(c + 1) * LN], x1[pl.ds(n + r0, 8), c * LN:(c + 1) * LN])
                  for c in range(R16)]
            ys = _fft(zs, -1)
            for r in range(R16):
                re, im = ys[r]
                if r:
                    tr, ti = tw[0, r], tw[1, r]
                    re, im = re * tr - im * ti, re * ti + im * tr
                rm[r, pl.ds(r0, 8), 0:LN] = re
                rm[r, pl.ds(r0, 8), LN:2 * LN] = im

        def wprep(c):
            cols = slice(c * LN, (c + 1) * LN)
            row = jax.lax.broadcasted_iota(jnp.int32, (LN - JB, LN), 0)
            for p, wt in enumerate((wrt, wit)):
                u = pltpu.bitcast(wt[0:J - 1, cols], jnp.uint32)
                even = pltpu.bitcast(u << 16, f32)
                odd = pltpu.bitcast(u & jnp.uint32(0xFFFF0000), f32)
                last = jnp.broadcast_to(wt[J - 1:J, cols].astype(f32), (LN - JB, LN))
                wsa[p, cols, :] = jnp.concatenate([even, jnp.where(row == 0, last, 0.0)], axis=0).T
                wsb[p, cols, :] = jnp.concatenate([odd, jnp.zeros((LN - JB, LN), f32)], axis=0).T

        def stage2(rm, k):
            return _dot(l2[...], rm[4 * k:4 * k + 4].reshape(4 * LN, 2 * LN).astype(bf16), NT)

        def stage3(x, ws, cs, r):
            x = x[r // 4]
            c0 = (r % 4) * LN
            xr, xi = x[0:LN, c0:c0 + LN], x[LN:2 * LN, c0:c0 + LN]
            wr = ws[0, pl.ds(r, LN, stride=R16), :]
            wi = ws[1, pl.ds(r, LN, stride=R16), :]
            g = jnp.concatenate([xr * wr - xi * wi, xr * wi + xi * wr], axis=1).astype(bf16)
            c = _dot(l3[r], g, NN)
            cs[r, 0:LN, :] = c[0:LN, 0:LN] - c[LN:2 * LN, LN:2 * LN]
            cs[r, LN:2 * LN, :] = c[LN:2 * LN, 0:LN] + c[0:LN, LN:2 * LN]

        def inv16(cs, half, r0):
            zs = [(cs[r, r0:r0 + 8, :], cs[r, LN + r0:LN + r0 + 8, :]) for r in range(R16)]
            ys = _fft(zs, +1)
            for c in range(R16):
                us[half, c * LN + r0:c * LN + r0 + 8, 0:LN] = ys[c][0].astype(bf16)
                us[half, c * LN + r0:c * LN + r0 + 8, LN:2 * LN] = ys[c][1].astype(bf16)

        def stage4(half, k):
            cols = slice(k * LN, (k + 1) * LN)
            y = _dot(l4[half * HD:(half + 1) * HD, :], us[half, cols, :], NT)
            if half:
                e = ot[0:HD, cols]
                ot[0:HD, cols] = e + y
                ot[HD:DM, cols] = e - y
            else:
                ot[0:HD, cols] = y

        with scope('w0'):
            c_fd.wait()
        with scope('S1'):
            jax.lax.fori_loop(0, 4, stage1, 0)
        with scope('wt_tw'):
            wait_all([c_tw])

        def fwd16a(g, carry):
            fwd16(x1a, rma, JA, pl.multiple_of(g * 8, 8))
            return carry

        def fwd16b(g, carry):
            fwd16(x1b, rmb, JB, pl.multiple_of(g * 8, 8))
            return carry

        with scope('F16'):
            jax.lax.fori_loop(0, JA // 8, fwd16a, 0)
            jax.lax.fori_loop(0, JB // 8, fwd16b, 0)
        with scope('wt_l2'):
            wait_all([c_l2, c_wrt, c_wit])
        rma[:, JA:LN, :] = jnp.zeros((R16, LN - JA, 2 * LN), f32)
        rmb[:, JB:LN, :] = jnp.zeros((R16, LN - JB, 2 * LN), f32)
        xa, xb = [], []
        for k in range(8):
            wprep(2 * k)
            wprep(2 * k + 1)
            (xa, xb)[k // 4].append(stage2((rma, rmb)[k // 4], k % 4))
        with scope('wt_W'):
            wait_all([c_l3, c_l4])
        for r in range(R16):
            stage3(xa, wsa, csa, r)
        for r in range(R16):
            stage3(xb, wsb, csb, r)
            inv16(csa, 0, r * 8)
        for k in range(R16):
            stage4(0, k)
            inv16(csb, 1, k * 8)
        with scope('wt_wq'):
            wait_all([c_wq])
        done = 0
        for k in range(R16):
            while do_b and done * R16 < (k + 1) * NWQ and done < NWQ:
                wq_prep(done)
                done += 1
            stage4(1, k)

    if do_a:
        pl.run_scoped(part_a,
                      pltpu.VMEM((2 * JA, S), f32), pltpu.VMEM((2 * JB, S), f32),
                      pltpu.VMEM((R16, LN, 2 * LN), f32), pltpu.VMEM((R16, LN, 2 * LN), f32),
                      pltpu.VMEM((2, S, LN), f32), pltpu.VMEM((2, S, LN), f32),
                      pltpu.VMEM((R16, 2 * LN, LN), f32), pltpu.VMEM((R16, 2 * LN, LN), f32),
                      pltpu.VMEM((2, S, 2 * LN), bf16))
    else:
        for c in cps[:-3]:
            c.wait()
        ot[0:DM, :] = jnp.zeros((DM, S), f32)
        if do_b:
            for k in range(R16):
                wq_prep(k % NWQ)

    with scope('wt_x'):
        wait_all([c_bxt])
    for k in range(R16):
        cols = slice(k * LN, (k + 1) * LN)
        ybuf[cols, :] = ot[0:YC, cols].astype(bf16).T
        if do_b:
            x_prep(k)
    c_y = pltpu.make_async_copy(ybuf, out_hbm.at[:, 0:YC], ysem.at[0])
    c_y.start()

    qscale = (D ** -0.5) * math.log2(math.e)

    with scope('wt_c0'):
        for u in range(QHEADS):
            wchunk(0, u).wait()
            wchunk(1, u).wait()

    def qstep(tt, carry):
        if do_b:
            rq, rw = S // QPIECES, 2 * CCH // QPIECES
            for u in range(QHEADS):
                t = tt * QHEADS + u
                for j in range(QPIECES):
                    x = jnp.concatenate([wall[PX, j * rq:(j + 1) * rq, :], wall[PX + 1, j * rq:(j + 1) * rq, 0:DM - D]],
                                        axis=1)
                    q_all[t, j * rq:(j + 1) * rq] = (_dot(x, wall[t, 0:DM, :], NN) * qscale).astype(bf16)
                    which, off = divmod(j * rw, CCH)
                    r0 = pl.multiple_of(t * CCH + off, rw)
                    src = (wuk_raw, wuv_raw)[which]
                    wall[0:H, pl.ds(DM + which * DC + r0, rw), :] = jnp.swapaxes(src[pl.ds(r0, rw)], 0, 1)

        @pl.when(tt + 1 < H // QHEADS)
        def _():
            for u in range(QHEADS):
                wchunk(0, (tt + 1) * QHEADS + u).wait()
                wchunk(1, (tt + 1) * QHEADS + u).wait()

        return carry

    with scope('P2'):
        jax.lax.fori_loop(0, H // QHEADS, qstep, 0)
    with scope('wt_ckv'):
        c_ckv.wait()
        c_wot.wait()

    def head(h, carry):
        with scope('head'):
            return head_body(h, carry)

    def head_body(h, carry):
        rr = jax.lax.broadcasted_iota(jnp.int32, (LN, LN), 0)
        cc = jax.lax.broadcasted_iota(jnp.int32, (LN, LN), 1)
        tri = cc <= rr
        neg = -1e9 * math.log2(math.e)
        kv = {'K': [], 'U': []}
        scores, probs, ctxs = {}, {}, {}

        def rows(name, a, b):
            parts = []
            for lo, arr in sorted(kv[name], key=lambda x: x[0]):
                x, y = max(a, lo), min(b, lo + arr.shape[0])
                if x < y:
                    parts.append(arr[x - lo:y - lo])
            return _cat(parts, 0)

        for tok in HEAD_ORDER.split():
            kind, arg = tok[0], tok[1:]
            if kind in 'KU':
                a, b = map(int, arg.split('-')) if arg else (0, S // TQ)
                w0 = DM + (DC if kind == 'U' else 0)
                w = wall[h, w0:w0 + DC, :]
                kv[kind].append((a * TQ, _dot(ckv[a * TQ:b * TQ, :], w, NN).astype(bf16)))
                continue
            if kind == 'O':
                grp = [int(ch) for ch in arg]
                res = _dot(wot[h], _cat([ctxs[j] for j in grp], 0), NT)
                for n, j in enumerate(grp):
                    ot[DM:2 * DM, j * TQ:(j + 1) * TQ] += res[:, n * TQ:(n + 1) * TQ]
                continue
            i = int(arg)
            r0 = i * TQ
            lm = r0 + LN
            if kind == 'Q':
                q = q_all[h, r0:r0 + TQ, :]
                s = _dot(q, rows('K', 0, lm), NT)
                sx = jnp.where(tri, _dot(q[LN:], rows('K', lm, lm + LN), NT), neg)
                scores[i] = (s, sx)
            elif kind in 'STB':
                s, sx = scores[i]
                if kind in 'ST':
                    sd = jnp.where(tri, s[0:LN, r0:lm], neg)
                    pt, lt = _softmax_rows(([s[0:LN, 0:r0]] if i else []) + [sd])
                    probs[i, 0] = (_cat(pt, 1), lt)
                if kind in 'SB':
                    probs[i, 1] = _softmax_rows([s[LN:], sx])
            else:
                (pt, lt), ((pb, px), lb) = probs.pop((i, 0)), probs.pop((i, 1))
                ctx = _dot(jnp.concatenate([pt, pb], axis=0), rows('U', 0, lm), NN)
                cx = _dot(px, rows('U', lm, lm + LN), NN)
                ctxs[i] = jnp.concatenate([ctx[0:LN] * (1.0 / lt), (ctx[LN:] + cx) * (1.0 / lb)],
                                          axis=0).astype(bf16)
        return carry

    if do_b:
        with scope('P3'):
            jax.lax.fori_loop(0, H, head, 0)

    def ocopy(c):
        rows = pl.ds(pl.multiple_of(c * OCH, OCH), OCH)
        return pltpu.make_async_copy(obuf.at[rows], out_hbm.at[rows, YC:2 * DM], osem.at[c])

    def ostep(c, carry):
        for k in range(OCH // LN):
            cols = pl.ds(pl.multiple_of(c * OCH + k * LN, LN), LN)
            obuf[cols, :] = ot[YC:2 * DM, cols].astype(bf16).T
        ocopy(c).start()
        return carry

    with scope('fin'):
        jax.lax.fori_loop(0, S // OCH, ostep, 0)
    with scope('wt_out'):
        c_y.wait()
        for c in range(S // OCH):
            ocopy(c).wait()


def _build(do_a=True, do_b=True, scopes=False, order=None):
    global HEAD_ORDER
    if order is not None:
        HEAD_ORDER = order
    def run(A_x, A_w_r, A_w_i, B_x, B_c_kv, B_w_q, B_w_uk, B_w_uv, B_w_o):
        axt = jnp.swapaxes(A_x, 1, 2).reshape(DM, S)
        bxt = jnp.swapaxes(B_x, 1, 2).reshape(DM, S)
        wrt = A_w_r.T
        wit = A_w_i.T
        ckv = B_c_kv.reshape(S, DC)
        wot = jnp.swapaxes(B_w_o, 1, 2)
        tabs = [jnp.asarray(t) for t in _tables()]
        args = (axt, wrt, wit, bxt, ckv, B_w_q, B_w_uk, B_w_uv, wot, *tabs)
        vm = pltpu.VMEM
        scratch = [
            vm((DM, S), bf16), vm((J, S), bf16), vm((J, S), bf16),
            vm(tabs[0].shape, bf16), vm(tabs[1].shape, bf16), vm(tabs[2].shape, f32),
            vm(tabs[3].shape, bf16), vm(tabs[4].shape, bf16),
            vm((DM, S), bf16), vm((S, DC), bf16),
            vm((DM, H, D), bf16),
            vm((DC, H, D), bf16), vm((DC, H, D), bf16), vm((H + 2, DM + 2 * DC, D), bf16),
            vm((H, DM, D), bf16), vm((H, S, D), bf16),
            vm((2 * DM, S), f32), vm((S, YC), bf16), vm((S, 2 * DM - YC), bf16),
            pltpu.SemaphoreType.DMA((15,)), pltpu.SemaphoreType.DMA((2, H)),
            pltpu.SemaphoreType.DMA((S // OCH,)), pltpu.SemaphoreType.DMA((1,)),
        ]
        out = pl.pallas_call(
            functools.partial(_kernel, do_a=do_a, do_b=do_b, scopes=scopes),
            in_specs=[pl.BlockSpec(memory_space=pl.ANY)] * len(args),
            out_specs=pl.BlockSpec(memory_space=pl.ANY),
            out_shape=jax.ShapeDtypeStruct((S, 2 * DM), bf16),
            scratch_shapes=scratch,
            compiler_params=pltpu.CompilerParams(vmem_limit_bytes=120 * 2**20),
        )(*args)
        return out.reshape(1, S, 2 * DM)

    return run


_run = _build()


@jax.jit
def pallas_concat_heads__spectral_gfnet__compressed_kv_cla__prompt_kernel(
    A_x: jax.Array,
    A_w_r: jax.Array,
    A_w_i: jax.Array,
    B_x: jax.Array,
    B_c_kv: jax.Array,
    B_w_q: jax.Array,
    B_w_uk: jax.Array,
    B_w_uv: jax.Array,
    B_w_o: jax.Array,
):
    return _run(A_x, A_w_r, A_w_i, B_x, B_c_kv, B_w_q, B_w_uk, B_w_uv, B_w_o)
```

```python
import contextlib
import functools
import math

import jax
import jax.numpy as jnp
import numpy as np
import jax.experimental.pallas as pl
import jax.experimental.pallas.tpu as pltpu

f32 = jnp.float32
bf16 = jnp.bfloat16

NN = (((1,), (0,)), ((), ()))
NT = (((1,), (1,)), ((), ()))

S = 2048
DM = 448
J = DM // 2 + 1
HD = DM // 2
JA = 120
JB = 112
H = 16
D = 256
DC = 1024
R16 = 16
LN = 128
TQ = 256
CCH = DC // H
PX = H
YC = 384
HEAD_ORDER = ('K0-2 U0-3 U3-5 U5-6 K2-8 Q1 T1 B1 Q4 Q0 U6-8 T4 B4 V4 Q6 Q3 B6 T0 B0 V0 V1 T3 Q5 T5 Q7 T7 B5 T6 V6 B3 B7 '
              'V3 V7 Q2 V5 O0 T2 B2 V2 O75213 O4 O6')
NWQ = 14
OCH = 256
QHEADS = 2
QPIECES = 16


def _dot(a, b, dn):
    return jax.lax.dot_general(a, b, dn, preferred_element_type=f32)


@functools.lru_cache(maxsize=None)
def _tables():
    j = np.arange(J)[:, None].astype(np.float64)
    d = np.arange(DM)[None, :].astype(np.float64)
    ang = 2.0 * np.pi * ((j * d) % DM) / DM
    cos, sin = np.cos(ang), np.sin(ang)
    ne, no = (J + 1) // 2, J // 2
    fd = np.zeros((2 * JA + 2 * JB, HD), np.float64)
    fd[0:ne] = cos[0::2, 0:HD]
    fd[JA:JA + ne] = -sin[0::2, 0:HD]
    fd[2 * JA:2 * JA + no] = cos[1::2, 0:HD]
    fd[2 * JA + JB:2 * JA + JB + no] = -sin[1::2, 0:HD]

    m = np.arange(LN)[:, None].astype(np.float64)
    l = np.arange(LN)[None, :].astype(np.float64)
    a128 = 2.0 * np.pi * ((m * l) % LN) / LN
    fr, fi = np.cos(a128), -np.sin(a128)
    l2 = np.block([[fr, -fi], [fi, fr]])

    r = np.arange(R16)[:, None].astype(np.float64)
    at = 2.0 * np.pi * (r * l) / S
    tw = np.stack([np.cos(at), -np.sin(at)])
    tw = np.broadcast_to(tw[:, :, None, :], (2, R16, 8, LN)).copy()

    l3 = np.zeros((R16, 2 * LN, LN), np.float64)
    for rr in range(R16):
        a3 = 2.0 * np.pi * ((m * (rr + R16 * l)) % S) / S
        l3[rr] = np.concatenate([np.cos(a3), np.sin(a3)], axis=0)

    cj = np.full((J,), 2.0)
    cj[0] = 1.0
    cj[J - 1] = 1.0
    scale = cj[None, :] / float(S * DM)
    cr, ci = cos.T[0:HD] * scale, -sin.T[0:HD] * scale
    l4 = np.zeros((2, HD, 2 * LN), np.float64)
    l4[0, :, 0:ne] = cr[:, 0::2]
    l4[0, :, LN:LN + ne] = ci[:, 0::2]
    l4[1, :, 0:no] = cr[:, 1::2]
    l4[1, :, LN:LN + no] = ci[:, 1::2]

    def packed(a):
        h = np.asarray(a, np.float32).astype(bf16).view(np.uint16).astype(np.uint32)
        return h[..., 0::2, :] | (h[..., 1::2, :] << 16)

    return (packed(fd), packed(l2), np.asarray(tw, np.float32), packed(l3), packed(l4.reshape(2 * HD, 2 * LN)))


def _cmul_const(z, k, n, sign):
    re, im = z
    k = k % n
    if k == 0:
        return re, im
    if 4 * k == n:
        return (-im, re) if sign > 0 else (im, -re)
    if 8 * k == n:
        c = math.sqrt(0.5)
        return ((re - im) * c, (re + im) * c) if sign > 0 else ((re + im) * c, (im - re) * c)
    if 8 * k == 3 * n:
        c = math.sqrt(0.5)
        return ((re + im) * (-c), (re - im) * c) if sign > 0 else ((im - re) * c, (re + im) * (-c))
    c = math.cos(2.0 * math.pi * k / n)
    s = sign * math.sin(2.0 * math.pi * k / n)
    return re * c - im * s, re * s + im * c


def _fft(zs, sign):
    n = len(zs)
    if n == 1:
        return zs
    ev = _fft(zs[0::2], sign)
    od = _fft(zs[1::2], sign)
    out = [None] * n
    for k in range(n // 2):
        if 4 * k == n:
            (er, ei), (orr, oi) = ev[k], od[k]
            if sign > 0:
                out[k] = (er - oi, ei + orr)
                out[k + n // 2] = (er + oi, ei - orr)
            else:
                out[k] = (er + oi, ei - orr)
                out[k + n // 2] = (er - oi, ei + orr)
            continue
        tr, ti = _cmul_const(od[k], k, n, sign)
        er, ei = ev[k]
        out[k] = (er + tr, ei + ti)
        out[k + n // 2] = (er - tr, ei - ti)
    return out


def _softmax_rows(segs):
    m = functools.reduce(jnp.maximum, [jnp.max(sg, axis=1, keepdims=True) for sg in segs])
    ps = [jnp.exp2(sg - m).astype(bf16) for sg in segs]
    l = functools.reduce(jnp.add, [jnp.sum(p.astype(f32), axis=1, keepdims=True) for p in ps])
    return ps, l


def _bf(x):
    return pltpu.bitcast(x, bf16)


def _cat(parts, axis):
    return jnp.concatenate(parts, axis=axis) if len(parts) > 1 else parts[0]


def _kernel(axt_hbm, wrt_hbm, wit_hbm, bxt_hbm, ckv_hbm, wq_hbm, wuk_hbm, wuv_hbm, wot_hbm,
            fd_hbm, l2_hbm, tw_hbm, l3_hbm, l4_hbm,
            out_hbm,
            axt, wrt, wit, fd, l2, tw, l3, l4,
            bxt, ckv, wq_raw, wuk_raw, wuv_raw, wall, wot, q_all,
            ot, ybuf, obuf, sem, wsem, osem, ysem, *, do_a, do_b, scopes):
    scope = jax.named_scope if scopes else (lambda name: contextlib.nullcontext())
    XC = S // 4
    simple = ([(fd_hbm, fd)]
              + [(axt_hbm.at[:, c * XC:(c + 1) * XC], axt.at[:, c * XC:(c + 1) * XC]) for c in range(4)]
              + [(tw_hbm, tw), (l2_hbm, l2), (wrt_hbm, wrt), (wit_hbm, wit),
                 (l3_hbm, l3), (l4_hbm, l4), (wq_hbm, wq_raw), (bxt_hbm, bxt), (ckv_hbm, ckv), (wot_hbm, wot)])
    cps = [pltpu.make_async_copy(s, d, sem.at[i]) for i, (s, d) in enumerate(simple)]
    c_fd = cps[0]
    (c_tw, c_l2, c_wrt, c_wit, c_l3, c_l4, c_wq, c_bxt, c_ckv, c_wot) = cps[5:]

    def wchunk(which, t):
        src, dst = ((wuk_hbm, wuk_raw), (wuv_hbm, wuv_raw))[which]
        return pltpu.make_async_copy(src.at[pl.ds(t * CCH, CCH)], dst.at[pl.ds(t * CCH, CCH)], wsem.at[which, t])

    def issue(lo, hi):
        def body(i, carry):
            for k in range(lo, hi):
                pl.when(i == k)(cps[k].start)
            return carry
        jax.lax.fori_loop(lo, hi, body, 0)

    def wait_all(cs):
        def body(i, carry):
            for k, c in enumerate(cs):
                pl.when(i == k)(c.wait)
            return carry
        jax.lax.fori_loop(0, max(2, len(cs)), body, 0)

    def issue_w(t, carry):
        wchunk(0, t).start()
        wchunk(1, t).start()
        return carry

    with scope('issue'):
        issue(0, len(cps) - 2)
        jax.lax.fori_loop(0, H, issue_w, 0)
        issue(len(cps) - 2, len(cps))

    def zero(i, carry):
        ot[pl.ds(pl.multiple_of(DM + i * 64, 64), 64), :] = jnp.zeros((64, S), f32)
        return carry

    with scope('zero'):
        jax.lax.fori_loop(0, DM // 64, zero, 0)

    def x_prep(k):
        rr = jax.lax.broadcasted_iota(jnp.int32, (LN, LN), 0)
        cc = jax.lax.broadcasted_iota(jnp.int32, (LN, LN), 1)
        eye = jnp.where(rr == cc, 1.0, 0.0).astype(bf16)
        x = _dot(eye, bxt[:, k * LN:(k + 1) * LN], NT).astype(bf16)
        wall[PX, k * LN:(k + 1) * LN, :] = x[:, 0:D]
        wall[PX + 1, k * LN:(k + 1) * LN, 0:DM - D] = x[:, D:DM]

    def wq_prep(k):
        n = DM // NWQ
        wall[0:H, k * n:(k + 1) * n, :] = jnp.swapaxes(wq_raw[k * n:(k + 1) * n], 0, 1)

    def part_a(x1a, x1b, rma, rmb, wsa, wsb, csa, csb, us):
        def stage1(c, carry):
            cols = pl.ds(pl.multiple_of(c * XC, XC), XC)
            pltpu.make_async_copy(axt_hbm.at[:, cols], axt.at[:, cols], sem.at[1 + c]).wait()
            lo, hi = axt[0:HD, cols].astype(f32), axt[HD:DM, cols].astype(f32)
            x1a[:, cols] = _dot(_bf(fd[0:JA, :]), (lo + hi).astype(bf16), NN)
            x1b[:, cols] = _dot(_bf(fd[JA:, :]), (lo - hi).astype(bf16), NN)
            return carry

        def fwd16(x1, rm, n, r0):
            zs = [(x1[pl.ds(r0, 8), c * LN:(c + 1) * LN], x1[pl.ds(n + r0, 8), c * LN:(c + 1) * LN])
                  for c in range(R16)]
            ys = _fft(zs, -1)
            for r in range(R16):
                re, im = ys[r]
                if r:
                    tr, ti = tw[0, r], tw[1, r]
                    re, im = re * tr - im * ti, re * ti + im * tr
                rm[r, pl.ds(r0, 8), 0:LN] = re
                rm[r, pl.ds(r0, 8), LN:2 * LN] = im

        def wprep(c):
            cols = slice(c * LN, (c + 1) * LN)
            row = jax.lax.broadcasted_iota(jnp.int32, (LN - JB, LN), 0)
            for p, wt in enumerate((wrt, wit)):
                u = pltpu.bitcast(wt[0:J - 1, cols], jnp.uint32)
                even = pltpu.bitcast(u << 16, f32)
                odd = pltpu.bitcast(u & jnp.uint32(0xFFFF0000), f32)
                last = jnp.broadcast_to(wt[J - 1:J, cols].astype(f32), (LN - JB, LN))
                wsa[p, cols, :] = jnp.concatenate([even, jnp.where(row == 0, last, 0.0)], axis=0).T
                wsb[p, cols, :] = jnp.concatenate([odd, jnp.zeros((LN - JB, LN), f32)], axis=0).T

        def stage2(rm, k):
            return _dot(_bf(l2[...]), rm[4 * k:4 * k + 4].reshape(4 * LN, 2 * LN).astype(bf16), NT)

        def stage3(x, ws, cs, r):
            x = x[r // 4]
            c0 = (r % 4) * LN
            xr, xi = x[0:LN, c0:c0 + LN], x[LN:2 * LN, c0:c0 + LN]
            wr = ws[0, pl.ds(r, LN, stride=R16), :]
            wi = ws[1, pl.ds(r, LN, stride=R16), :]
            g = jnp.concatenate([xr * wr - xi * wi, xr * wi + xi * wr], axis=1).astype(bf16)
            c = _dot(_bf(l3[r]), g, NN)
            cs[r, 0:LN, :] = c[0:LN, 0:LN] - c[LN:2 * LN, LN:2 * LN]
            cs[r, LN:2 * LN, :] = c[LN:2 * LN, 0:LN] + c[0:LN, LN:2 * LN]

        def inv16(cs, half, r0):
            zs = [(cs[r, r0:r0 + 8, :], cs[r, LN + r0:LN + r0 + 8, :]) for r in range(R16)]
            ys = _fft(zs, +1)
            for c in range(R16):
                us[half, c * LN + r0:c * LN + r0 + 8, 0:LN] = ys[c][0].astype(bf16)
                us[half, c * LN + r0:c * LN + r0 + 8, LN:2 * LN] = ys[c][1].astype(bf16)

        def stage4(half, k):
            cols = slice(k * LN, (k + 1) * LN)
            y = _dot(_bf(l4[half * HD // 2:(half + 1) * HD // 2, :]), us[half, cols, :], NT)
            if half:
                e = ot[0:HD, cols]
                ot[0:HD, cols] = e + y
                ot[HD:DM, cols] = e - y
            else:
                ot[0:HD, cols] = y

        with scope('w0'):
            c_fd.wait()
        with scope('S1'):
            jax.lax.fori_loop(0, 4, stage1, 0)
        with scope('wt_tw'):
            wait_all([c_tw])

        def fwd16a(g, carry):
            fwd16(x1a, rma, JA, pl.multiple_of(g * 8, 8))
            return carry

        def fwd16b(g, carry):
            fwd16(x1b, rmb, JB, pl.multiple_of(g * 8, 8))
            return carry

        with scope('F16'):
            jax.lax.fori_loop(0, JA // 8, fwd16a, 0)
            jax.lax.fori_loop(0, JB // 8, fwd16b, 0)
        with scope('wt_l2'):
            wait_all([c_l2, c_wrt, c_wit])
        rma[:, JA:LN, :] = jnp.zeros((R16, LN - JA, 2 * LN), f32)
        rmb[:, JB:LN, :] = jnp.zeros((R16, LN - JB, 2 * LN), f32)
        xa, xb = [], []
        for k in range(8):
            wprep(2 * k)
            wprep(2 * k + 1)
            (xa, xb)[k // 4].append(stage2((rma, rmb)[k // 4], k % 4))
        with scope('wt_W'):
            wait_all([c_l3, c_l4])
        for r in range(R16):
            stage3(xa, wsa, csa, r)
        for r in range(R16):
            stage3(xb, wsb, csb, r)
            inv16(csa, 0, r * 8)
        for k in range(R16):
            stage4(0, k)
            inv16(csb, 1, k * 8)
        with scope('wt_wq'):
            wait_all([c_wq])
        done = 0
        for k in range(R16):
            while do_b and done * R16 < (k + 1) * NWQ and done < NWQ:
                wq_prep(done)
                done += 1
            stage4(1, k)

    if do_a:
        pl.run_scoped(part_a,
                      pltpu.VMEM((2 * JA, S), f32), pltpu.VMEM((2 * JB, S), f32),
                      pltpu.VMEM((R16, LN, 2 * LN), f32), pltpu.VMEM((R16, LN, 2 * LN), f32),
                      pltpu.VMEM((2, S, LN), f32), pltpu.VMEM((2, S, LN), f32),
                      pltpu.VMEM((R16, 2 * LN, LN), f32), pltpu.VMEM((R16, 2 * LN, LN), f32),
                      pltpu.VMEM((2, S, 2 * LN), bf16))
    else:
        for c in cps[:-3]:
            c.wait()
        ot[0:DM, :] = jnp.zeros((DM, S), f32)
        if do_b:
            for k in range(R16):
                wq_prep(k % NWQ)

    with scope('wt_x'):
        wait_all([c_bxt])
    for k in range(R16):
        cols = slice(k * LN, (k + 1) * LN)
        ybuf[cols, :] = ot[0:YC, cols].astype(bf16).T
        if do_b:
            x_prep(k)
    c_y = pltpu.make_async_copy(ybuf, out_hbm.at[:, 0:YC], ysem.at[0])
    c_y.start()

    qscale = (D ** -0.5) * math.log2(math.e)

    with scope('wt_c0'):
        for u in range(QHEADS):
            wchunk(0, u).wait()
            wchunk(1, u).wait()

    def qstep(tt, carry):
        if do_b:
            rq, rw = S // QPIECES, 2 * CCH // QPIECES
            for u in range(QHEADS):
                t = tt * QHEADS + u
                for j in range(QPIECES):
                    x = jnp.concatenate([wall[PX, j * rq:(j + 1) * rq, :], wall[PX + 1, j * rq:(j + 1) * rq, 0:DM - D]],
                                        axis=1)
                    q_all[t, j * rq:(j + 1) * rq] = (_dot(x, wall[t, 0:DM, :], NN) * qscale).astype(bf16)
                    which, off = divmod(j * rw, CCH)
                    r0 = pl.multiple_of(t * CCH + off, rw)
                    src = (wuk_raw, wuv_raw)[which]
                    wall[0:H, pl.ds(DM + which * DC + r0, rw), :] = jnp.swapaxes(src[pl.ds(r0, rw)], 0, 1)

        @pl.when(tt + 1 < H // QHEADS)
        def _():
            for u in range(QHEADS):
                wchunk(0, (tt + 1) * QHEADS + u).wait()
                wchunk(1, (tt + 1) * QHEADS + u).wait()

        return carry

    with scope('P2'):
        jax.lax.fori_loop(0, H // QHEADS, qstep, 0)
    with scope('wt_ckv'):
        c_ckv.wait()
        c_wot.wait()

    def head(h, carry):
        with scope('head'):
            return head_body(h, carry)

    def head_body(h, carry):
        rr = jax.lax.broadcasted_iota(jnp.int32, (LN, LN), 0)
        cc = jax.lax.broadcasted_iota(jnp.int32, (LN, LN), 1)
        tri = cc <= rr
        neg = -1e9 * math.log2(math.e)
        kv = {'K': [], 'U': []}
        scores, probs, ctxs = {}, {}, {}

        def rows(name, a, b):
            parts = []
            for lo, arr in sorted(kv[name], key=lambda x: x[0]):
                x, y = max(a, lo), min(b, lo + arr.shape[0])
                if x < y:
                    parts.append(arr[x - lo:y - lo])
            return _cat(parts, 0)

        for tok in HEAD_ORDER.split():
            kind, arg = tok[0], tok[1:]
            if kind in 'KU':
                a, b = map(int, arg.split('-')) if arg else (0, S // TQ)
                w0 = DM + (DC if kind == 'U' else 0)
                w = wall[h, w0:w0 + DC, :]
                kv[kind].append((a * TQ, _dot(ckv[a * TQ:b * TQ, :], w, NN).astype(bf16)))
                continue
            if kind == 'O':
                grp = [int(ch) for ch in arg]
                res = _dot(wot[h], _cat([ctxs[j] for j in grp], 0), NT)
                for n, j in enumerate(grp):
                    ot[DM:2 * DM, j * TQ:(j + 1) * TQ] += res[:, n * TQ:(n + 1) * TQ]
                continue
            i = int(arg)
            r0 = i * TQ
            lm = r0 + LN
            if kind == 'Q':
                q = q_all[h, r0:r0 + TQ, :]
                s = _dot(q, rows('K', 0, lm), NT)
                sx = jnp.where(tri, _dot(q[LN:], rows('K', lm, lm + LN), NT), neg)
                scores[i] = (s, sx)
            elif kind in 'STB':
                s, sx = scores[i]
                if kind in 'ST':
                    sd = jnp.where(tri, s[0:LN, r0:lm], neg)
                    pt, lt = _softmax_rows(([s[0:LN, 0:r0]] if i else []) + [sd])
                    probs[i, 0] = (_cat(pt, 1), lt)
                if kind in 'SB':
                    probs[i, 1] = _softmax_rows([s[LN:], sx])
            else:
                (pt, lt), ((pb, px), lb) = probs.pop((i, 0)), probs.pop((i, 1))
                ctx = _dot(jnp.concatenate([pt, pb], axis=0), rows('U', 0, lm), NN)
                cx = _dot(px, rows('U', lm, lm + LN), NN)
                ctxs[i] = jnp.concatenate([ctx[0:LN] * (1.0 / lt), (ctx[LN:] + cx) * (1.0 / lb)],
                                          axis=0).astype(bf16)
        return carry

    if do_b:
        with scope('P3'):
            jax.lax.fori_loop(0, H, head, 0)

    def ocopy(c):
        rows = pl.ds(pl.multiple_of(c * OCH, OCH), OCH)
        return pltpu.make_async_copy(obuf.at[rows], out_hbm.at[rows, YC:2 * DM], osem.at[c])

    def ostep(c, carry):
        for k in range(OCH // LN):
            cols = pl.ds(pl.multiple_of(c * OCH + k * LN, LN), LN)
            obuf[cols, :] = ot[YC:2 * DM, cols].astype(bf16).T
        ocopy(c).start()
        return carry

    with scope('fin'):
        jax.lax.fori_loop(0, S // OCH, ostep, 0)
    with scope('wt_out'):
        c_y.wait()
        for c in range(S // OCH):
            ocopy(c).wait()


def _build(do_a=True, do_b=True, scopes=False, order=None):
    global HEAD_ORDER
    if order is not None:
        HEAD_ORDER = order
    def run(A_x, A_w_r, A_w_i, B_x, B_c_kv, B_w_q, B_w_uk, B_w_uv, B_w_o):
        axt = jnp.swapaxes(A_x, 1, 2).reshape(DM, S)
        bxt = jnp.swapaxes(B_x, 1, 2).reshape(DM, S)
        wrt = A_w_r.T
        wit = A_w_i.T
        ckv = B_c_kv.reshape(S, DC)
        wot = jnp.swapaxes(B_w_o, 1, 2)
        tabs = [jnp.asarray(t) for t in _tables()]
        args = (axt, wrt, wit, bxt, ckv, B_w_q, B_w_uk, B_w_uv, wot, *tabs)
        vm = pltpu.VMEM
        scratch = [
            vm((DM, S), bf16), vm((J, S), bf16), vm((J, S), bf16),
            *[vm(t.shape, t.dtype) for t in tabs],
            vm((DM, S), bf16), vm((S, DC), bf16),
            vm((DM, H, D), bf16),
            vm((DC, H, D), bf16), vm((DC, H, D), bf16), vm((H + 2, DM + 2 * DC, D), bf16),
            vm((H, DM, D), bf16), vm((H, S, D), bf16),
            vm((2 * DM, S), f32), vm((S, YC), bf16), vm((S, 2 * DM - YC), bf16),
            pltpu.SemaphoreType.DMA((15,)), pltpu.SemaphoreType.DMA((2, H)),
            pltpu.SemaphoreType.DMA((S // OCH,)), pltpu.SemaphoreType.DMA((1,)),
        ]
        out = pl.pallas_call(
            functools.partial(_kernel, do_a=do_a, do_b=do_b, scopes=scopes),
            in_specs=[pl.BlockSpec(memory_space=pl.ANY)] * len(args),
            out_specs=pl.BlockSpec(memory_space=pl.ANY),
            out_shape=jax.ShapeDtypeStruct((S, 2 * DM), bf16),
            scratch_shapes=scratch,
            compiler_params=pltpu.CompilerParams(vmem_limit_bytes=120 * 2**20),
        )(*args)
        return out.reshape(1, S, 2 * DM)

    return run


_run = _build()


@jax.jit
def pallas_concat_heads__spectral_gfnet__compressed_kv_cla__prompt_kernel(
    A_x: jax.Array,
    A_w_r: jax.Array,
    A_w_i: jax.Array,
    B_x: jax.Array,
    B_c_kv: jax.Array,
    B_w_q: jax.Array,
    B_w_uk: jax.Array,
    B_w_uv: jax.Array,
    B_w_o: jax.Array,
):
    return _run(A_x, A_w_r, A_w_i, B_x, B_c_kv, B_w_q, B_w_uk, B_w_uv, B_w_o)
```

```python
import contextlib
import functools
import math

import jax
import jax.numpy as jnp
import numpy as np
import jax.experimental.pallas as pl
import jax.experimental.pallas.tpu as pltpu

f32 = jnp.float32
bf16 = jnp.bfloat16

NN = (((1,), (0,)), ((), ()))
NT = (((1,), (1,)), ((), ()))

S = 2048
DM = 448
J = DM // 2 + 1
HD = DM // 2
JA = 120
JB = 112
H = 16
D = 256
DC = 1024
R16 = 16
LN = 128
TQ = 256
CCH = DC // H
PX = H
YC = 384
HEAD_ORDER = ('K0-2 U0-3 U3-5 U5-6 K2-8 Q1 T1 B1 Q4 Q0 U6-8 T4 B4 V4 Q6 Q3 B6 T0 B0 V0 V1 T3 Q5 T5 Q7 T7 B5 T6 V6 B3 B7 '
              'V3 V7 Q2 V5 O0 T2 B2 V2 O75213 O4 O6')
NWQ = 14
OCH = 256
QHEADS = 2
QPIECES = 16


def _dot(a, b, dn):
    return jax.lax.dot_general(a, b, dn, preferred_element_type=f32)


@functools.lru_cache(maxsize=None)
def _tables():
    j = np.arange(J)[:, None].astype(np.float64)
    d = np.arange(DM)[None, :].astype(np.float64)
    ang = 2.0 * np.pi * ((j * d) % DM) / DM
    cos, sin = np.cos(ang), np.sin(ang)
    ne, no = (J + 1) // 2, J // 2
    fd = np.zeros((2 * JA + 2 * JB, HD), np.float64)
    fd[0:ne] = cos[0::2, 0:HD]
    fd[JA:JA + ne] = -sin[0::2, 0:HD]
    fd[2 * JA:2 * JA + no] = cos[1::2, 0:HD]
    fd[2 * JA + JB:2 * JA + JB + no] = -sin[1::2, 0:HD]

    m = np.arange(LN)[:, None].astype(np.float64)
    l = np.arange(LN)[None, :].astype(np.float64)
    a128 = 2.0 * np.pi * ((m * l) % LN) / LN
    fr, fi = np.cos(a128), -np.sin(a128)
    l2 = np.block([[fr, -fi], [fi, fr]])

    r = np.arange(R16)[:, None].astype(np.float64)
    at = 2.0 * np.pi * (r * l) / S
    tw = np.stack([np.cos(at), -np.sin(at)])
    tw = np.broadcast_to(tw[:, :, None, :], (2, R16, 8, LN)).copy()

    l3 = np.zeros((R16, 2 * LN, LN), np.float64)
    for rr in range(R16):
        a3 = 2.0 * np.pi * ((m * (rr + R16 * l)) % S) / S
        l3[rr] = np.concatenate([np.cos(a3), np.sin(a3)], axis=0)

    cj = np.full((J,), 2.0)
    cj[0] = 1.0
    cj[J - 1] = 1.0
    scale = cj[None, :] / float(S * DM)
    cr, ci = cos.T[0:HD] * scale, -sin.T[0:HD] * scale
    l4 = np.zeros((2, HD, 2 * LN), np.float64)
    l4[0, :, 0:ne] = cr[:, 0::2]
    l4[0, :, LN:LN + ne] = ci[:, 0::2]
    l4[1, :, 0:no] = cr[:, 1::2]
    l4[1, :, LN:LN + no] = ci[:, 1::2]

    def packed(a):
        h = np.asarray(a, np.float32).astype(bf16).view(np.uint16).astype(np.uint32)
        return h[..., 0::2, :] | (h[..., 1::2, :] << 16)

    return (packed(fd), packed(l2), np.asarray(tw, np.float32), packed(l3), packed(l4.reshape(2 * HD, 2 * LN)))


def _cmul_const(z, k, n, sign):
    re, im = z
    k = k % n
    if k == 0:
        return re, im
    if 4 * k == n:
        return (-im, re) if sign > 0 else (im, -re)
    if 8 * k == n:
        c = math.sqrt(0.5)
        return ((re - im) * c, (re + im) * c) if sign > 0 else ((re + im) * c, (im - re) * c)
    if 8 * k == 3 * n:
        c = math.sqrt(0.5)
        return ((re + im) * (-c), (re - im) * c) if sign > 0 else ((im - re) * c, (re + im) * (-c))
    c = math.cos(2.0 * math.pi * k / n)
    s = sign * math.sin(2.0 * math.pi * k / n)
    return re * c - im * s, re * s + im * c


def _fft(zs, sign):
    n = len(zs)
    if n == 1:
        return zs
    ev = _fft(zs[0::2], sign)
    od = _fft(zs[1::2], sign)
    out = [None] * n
    for k in range(n // 2):
        if 4 * k == n:
            (er, ei), (orr, oi) = ev[k], od[k]
            if sign > 0:
                out[k] = (er - oi, ei + orr)
                out[k + n // 2] = (er + oi, ei - orr)
            else:
                out[k] = (er + oi, ei - orr)
                out[k + n // 2] = (er - oi, ei + orr)
            continue
        tr, ti = _cmul_const(od[k], k, n, sign)
        er, ei = ev[k]
        out[k] = (er + tr, ei + ti)
        out[k + n // 2] = (er - tr, ei - ti)
    return out


def _softmax_rows(segs):
    m = functools.reduce(jnp.maximum, [jnp.max(sg, axis=1, keepdims=True) for sg in segs])
    ps = [jnp.exp2(sg - m).astype(bf16) for sg in segs]
    l = functools.reduce(jnp.add, [jnp.sum(p.astype(f32), axis=1, keepdims=True) for p in ps])
    return ps, l


def _bf(x):
    return pltpu.bitcast(x, bf16)


def _cat(parts, axis):
    return jnp.concatenate(parts, axis=axis) if len(parts) > 1 else parts[0]


def _kernel(axt_hbm, wrt_hbm, wit_hbm, bxt_hbm, ckv_hbm, wq_hbm, wuk_hbm, wuv_hbm, wot_hbm,
            fd_hbm, l2_hbm, tw_hbm, l3_hbm, l4_hbm,
            out_hbm,
            axt, wrt, wit, fd, l2, tw, l3, l4,
            bxt, ckv, wq_raw, wuk_raw, wuv_raw, wall, wot, q_all,
            ot, ybuf, obuf, sem, wsem, osem, ysem, *, do_a, do_b, scopes):
    scope = jax.named_scope if scopes else (lambda name: contextlib.nullcontext())
    XC = S // 4
    simple = ([(fd_hbm, fd)]
              + [(axt_hbm.at[:, c * XC:(c + 1) * XC], axt.at[:, c * XC:(c + 1) * XC]) for c in range(4)]
              + [(tw_hbm, tw), (l2_hbm, l2), (wrt_hbm, wrt), (wit_hbm, wit),
                 (l3_hbm, l3), (l4_hbm, l4), (wq_hbm, wq_raw), (bxt_hbm, bxt), (ckv_hbm, ckv), (wot_hbm, wot)])
    cps = [pltpu.make_async_copy(s, d, sem.at[i]) for i, (s, d) in enumerate(simple)]
    c_fd = cps[0]
    (c_tw, c_l2, c_wrt, c_wit, c_l3, c_l4, c_wq, c_bxt, c_ckv, c_wot) = cps[5:]

    def wchunk(which, t):
        src, dst = ((wuk_hbm, wuk_raw), (wuv_hbm, wuv_raw))[which]
        return pltpu.make_async_copy(src.at[pl.ds(t * CCH, CCH)], dst.at[pl.ds(t * CCH, CCH)], wsem.at[which, t])

    def issue(lo, hi):
        def body(i, carry):
            for k in range(lo, hi):
                pl.when(i == k)(cps[k].start)
            return carry
        jax.lax.fori_loop(lo, hi, body, 0)

    def wait_all(cs):
        def body(i, carry):
            for k, c in enumerate(cs):
                pl.when(i == k)(c.wait)
            return carry
        jax.lax.fori_loop(0, max(2, len(cs)), body, 0)

    def issue_w(t, carry):
        wchunk(0, t).start()
        wchunk(1, t).start()
        ot[DM:2 * DM, pl.ds(pl.multiple_of(t * LN, LN), LN)] = jnp.zeros((DM, LN), f32)
        return carry

    with scope('issue'):
        issue(0, len(cps) - 2)
        jax.lax.fori_loop(0, H, issue_w, 0)
        issue(len(cps) - 2, len(cps))

    def x_prep(k):
        rr = jax.lax.broadcasted_iota(jnp.int32, (LN, LN), 0)
        cc = jax.lax.broadcasted_iota(jnp.int32, (LN, LN), 1)
        eye = jnp.where(rr == cc, 1.0, 0.0).astype(bf16)
        x = _dot(eye, bxt[:, k * LN:(k + 1) * LN], NT).astype(bf16)
        wall[PX, k * LN:(k + 1) * LN, :] = x[:, 0:D]
        wall[PX + 1, k * LN:(k + 1) * LN, 0:DM - D] = x[:, D:DM]

    def wq_prep(k):
        n = DM // NWQ
        wall[0:H, k * n:(k + 1) * n, :] = jnp.swapaxes(wq_raw[k * n:(k + 1) * n], 0, 1)

    def part_a(x1a, x1b, rma, rmb, wsa, wsb, csa, csb, us):
        def stage1(c, carry):
            cols = pl.ds(pl.multiple_of(c * XC, XC), XC)
            pltpu.make_async_copy(axt_hbm.at[:, cols], axt.at[:, cols], sem.at[1 + c]).wait()
            lo, hi = axt[0:HD, cols].astype(f32), axt[HD:DM, cols].astype(f32)
            x1a[:, cols] = _dot(_bf(fd[0:JA, :]), (lo + hi).astype(bf16), NN)
            x1b[:, cols] = _dot(_bf(fd[JA:, :]), (lo - hi).astype(bf16), NN)
            return carry

        def fwd16(x1, rm, n, r0):
            zs = [(x1[pl.ds(r0, 8), c * LN:(c + 1) * LN], x1[pl.ds(n + r0, 8), c * LN:(c + 1) * LN])
                  for c in range(R16)]
            ys = _fft(zs, -1)
            for r in range(R16):
                re, im = ys[r]
                if r:
                    tr, ti = tw[0, r], tw[1, r]
                    re, im = re * tr - im * ti, re * ti + im * tr
                rm[r, pl.ds(r0, 8), 0:LN] = re
                rm[r, pl.ds(r0, 8), LN:2 * LN] = im

        def wprep(c):
            cols = slice(c * LN, (c + 1) * LN)
            row = jax.lax.broadcasted_iota(jnp.int32, (LN - JB, LN), 0)
            for p, wt in enumerate((wrt, wit)):
                u = pltpu.bitcast(wt[0:J - 1, cols], jnp.uint32)
                even = pltpu.bitcast(u << 16, f32)
                odd = pltpu.bitcast(u & jnp.uint32(0xFFFF0000), f32)
                last = jnp.broadcast_to(wt[J - 1:J, cols].astype(f32), (LN - JB, LN))
                wsa[p, cols, :] = jnp.concatenate([even, jnp.where(row == 0, last, 0.0)], axis=0).T
                wsb[p, cols, :] = jnp.concatenate([odd, jnp.zeros((LN - JB, LN), f32)], axis=0).T

        def stage2(rm, k):
            return _dot(_bf(l2[...]), rm[4 * k:4 * k + 4].reshape(4 * LN, 2 * LN).astype(bf16), NT)

        def stage3(x, ws, cs, r):
            x = x[r // 4]
            c0 = (r % 4) * LN
            xr, xi = x[0:LN, c0:c0 + LN], x[LN:2 * LN, c0:c0 + LN]
            wr = ws[0, pl.ds(r, LN, stride=R16), :]
            wi = ws[1, pl.ds(r, LN, stride=R16), :]
            g = jnp.concatenate([xr * wr - xi * wi, xr * wi + xi * wr], axis=1).astype(bf16)
            c = _dot(_bf(l3[r]), g, NN)
            cs[r, 0:LN, :] = c[0:LN, 0:LN] - c[LN:2 * LN, LN:2 * LN]
            cs[r, LN:2 * LN, :] = c[LN:2 * LN, 0:LN] + c[0:LN, LN:2 * LN]

        def inv16(cs, half, r0):
            zs = [(cs[r, r0:r0 + 8, :], cs[r, LN + r0:LN + r0 + 8, :]) for r in range(R16)]
            ys = _fft(zs, +1)
            for c in range(R16):
                us[half, c * LN + r0:c * LN + r0 + 8, 0:LN] = ys[c][0].astype(bf16)
                us[half, c * LN + r0:c * LN + r0 + 8, LN:2 * LN] = ys[c][1].astype(bf16)

        def stage4(half, k):
            cols = slice(k * LN, (k + 1) * LN)
            y = _dot(_bf(l4[half * HD // 2:(half + 1) * HD // 2, :]), us[half, cols, :], NT)
            if half:
                e = ot[0:HD, cols]
                ot[0:HD, cols] = e + y
                ot[HD:DM, cols] = e - y
            else:
                ot[0:HD, cols] = y

        with scope('w0'):
            c_fd.wait()
        with scope('S1'):
            jax.lax.fori_loop(0, 4, stage1, 0)
        with scope('wt_tw'):
            wait_all([c_tw])

        def fwd16a(g, carry):
            fwd16(x1a, rma, JA, pl.multiple_of(g * 8, 8))
            return carry

        def fwd16b(g, carry):
            fwd16(x1b, rmb, JB, pl.multiple_of(g * 8, 8))
            return carry

        with scope('F16'):
            jax.lax.fori_loop(0, JA // 8, fwd16a, 0)
            jax.lax.fori_loop(0, JB // 8, fwd16b, 0)
        with scope('wt_l2'):
            wait_all([c_l2, c_wrt, c_wit])
        rma[:, JA:LN, :] = jnp.zeros((R16, LN - JA, 2 * LN), f32)
        rmb[:, JB:LN, :] = jnp.zeros((R16, LN - JB, 2 * LN), f32)
        xa, xb = [], []
        for k in range(8):
            wprep(2 * k)
            wprep(2 * k + 1)
            (xa, xb)[k // 4].append(stage2((rma, rmb)[k // 4], k % 4))
        with scope('wt_W'):
            wait_all([c_l3, c_l4])
        for r in range(R16):
            stage3(xa, wsa, csa, r)
        for r in range(R16):
            stage3(xb, wsb, csb, r)
            inv16(csa, 0, r * 8)
        for k in range(R16):
            stage4(0, k)
            inv16(csb, 1, k * 8)
        with scope('wt_wq'):
            wait_all([c_wq])
        done = 0
        for k in range(R16):
            while do_b and done * R16 < (k + 1) * NWQ and done < NWQ:
                wq_prep(done)
                done += 1
            stage4(1, k)

    if do_a:
        pl.run_scoped(part_a,
                      pltpu.VMEM((2 * JA, S), f32), pltpu.VMEM((2 * JB, S), f32),
                      pltpu.VMEM((R16, LN, 2 * LN), f32), pltpu.VMEM((R16, LN, 2 * LN), f32),
                      pltpu.VMEM((2, S, LN), f32), pltpu.VMEM((2, S, LN), f32),
                      pltpu.VMEM((R16, 2 * LN, LN), f32), pltpu.VMEM((R16, 2 * LN, LN), f32),
                      pltpu.VMEM((2, S, 2 * LN), bf16))
    else:
        for c in cps[:-3]:
            c.wait()
        ot[0:DM, :] = jnp.zeros((DM, S), f32)
        if do_b:
            for k in range(R16):
                wq_prep(k % NWQ)

    with scope('wt_x'):
        wait_all([c_bxt])
    for k in range(R16):
        cols = slice(k * LN, (k + 1) * LN)
        ybuf[cols, :] = ot[0:YC, cols].astype(bf16).T
        if do_b:
            x_prep(k)
    c_y = pltpu.make_async_copy(ybuf, out_hbm.at[:, 0:YC], ysem.at[0])
    c_y.start()

    qscale = (D ** -0.5) * math.log2(math.e)

    with scope('wt_c0'):
        for u in range(QHEADS):
            wchunk(0, u).wait()
            wchunk(1, u).wait()

    def qstep(tt, carry):
        if do_b:
            rq, rw = S // QPIECES, 2 * CCH // QPIECES
            for u in range(QHEADS):
                t = tt * QHEADS + u
                for j in range(QPIECES):
                    x = jnp.concatenate([wall[PX, j * rq:(j + 1) * rq, :], wall[PX + 1, j * rq:(j + 1) * rq, 0:DM - D]],
                                        axis=1)
                    q_all[t, j * rq:(j + 1) * rq] = (_dot(x, wall[t, 0:DM, :], NN) * qscale).astype(bf16)
                    which, off = divmod(j * rw, CCH)
                    r0 = pl.multiple_of(t * CCH + off, rw)
                    src = (wuk_raw, wuv_raw)[which]
                    wall[0:H, pl.ds(DM + which * DC + r0, rw), :] = jnp.swapaxes(src[pl.ds(r0, rw)], 0, 1)

        @pl.when(tt + 1 < H // QHEADS)
        def _():
            for u in range(QHEADS):
                wchunk(0, (tt + 1) * QHEADS + u).wait()
                wchunk(1, (tt + 1) * QHEADS + u).wait()

        return carry

    with scope('P2'):
        jax.lax.fori_loop(0, H // QHEADS, qstep, 0)
    with scope('wt_ckv'):
        c_ckv.wait()
        c_wot.wait()

    def head(h, carry):
        with scope('head'):
            return head_body(h, carry)

    def head_body(h, carry):
        rr = jax.lax.broadcasted_iota(jnp.int32, (LN, LN), 0)
        cc = jax.lax.broadcasted_iota(jnp.int32, (LN, LN), 1)
        tri = cc <= rr
        neg = -1e9 * math.log2(math.e)
        kv = {'K': [], 'U': []}
        scores, probs, ctxs = {}, {}, {}

        def rows(name, a, b):
            parts = []
            for lo, arr in sorted(kv[name], key=lambda x: x[0]):
                x, y = max(a, lo), min(b, lo + arr.shape[0])
                if x < y:
                    parts.append(arr[x - lo:y - lo])
            return _cat(parts, 0)

        for tok in HEAD_ORDER.split():
            kind, arg = tok[0], tok[1:]
            if kind in 'KU':
                a, b = map(int, arg.split('-')) if arg else (0, S // TQ)
                w0 = DM + (DC if kind == 'U' else 0)
                w = wall[h, w0:w0 + DC, :]
                kv[kind].append((a * TQ, _dot(ckv[a * TQ:b * TQ, :], w, NN).astype(bf16)))
                continue
            if kind == 'O':
                grp = [int(ch) for ch in arg]
                res = _dot(wot[h], _cat([ctxs[j] for j in grp], 0), NT)
                for n, j in enumerate(grp):
                    ot[DM:2 * DM, j * TQ:(j + 1) * TQ] += res[:, n * TQ:(n + 1) * TQ]
                continue
            i = int(arg)
            r0 = i * TQ
            lm = r0 + LN
            if kind == 'Q':
                q = q_all[h, r0:r0 + TQ, :]
                s = _dot(q, rows('K', 0, lm), NT)
                sx = jnp.where(tri, _dot(q[LN:], rows('K', lm, lm + LN), NT), neg)
                scores[i] = (s, sx)
            elif kind in 'STB':
                s, sx = scores[i]
                if kind in 'ST':
                    sd = jnp.where(tri, s[0:LN, r0:lm], neg)
                    pt, lt = _softmax_rows(([s[0:LN, 0:r0]] if i else []) + [sd])
                    probs[i, 0] = (_cat(pt, 1), lt)
                if kind in 'SB':
                    probs[i, 1] = _softmax_rows([s[LN:], sx])
            else:
                (pt, lt), ((pb, px), lb) = probs.pop((i, 0)), probs.pop((i, 1))
                ctx = _dot(jnp.concatenate([pt, pb], axis=0), rows('U', 0, lm), NN)
                cx = _dot(px, rows('U', lm, lm + LN), NN)
                ctxs[i] = jnp.concatenate([ctx[0:LN] * (1.0 / lt), (ctx[LN:] + cx) * (1.0 / lb)],
                                          axis=0).astype(bf16)
        return carry

    if do_b:
        with scope('P3'):
            jax.lax.fori_loop(0, H, head, 0)

    def ocopy(c):
        rows = pl.ds(pl.multiple_of(c * OCH, OCH), OCH)
        return pltpu.make_async_copy(obuf.at[rows], out_hbm.at[rows, YC:2 * DM], osem.at[c])

    def ostep(c, carry):
        for k in range(OCH // LN):
            cols = pl.ds(pl.multiple_of(c * OCH + k * LN, LN), LN)
            obuf[cols, :] = ot[YC:2 * DM, cols].astype(bf16).T
        ocopy(c).start()
        return carry

    with scope('fin'):
        jax.lax.fori_loop(0, S // OCH, ostep, 0)
    with scope('wt_out'):
        c_y.wait()
        for c in range(S // OCH):
            ocopy(c).wait()


def _build(do_a=True, do_b=True, scopes=False, order=None):
    global HEAD_ORDER
    if order is not None:
        HEAD_ORDER = order
    def run(A_x, A_w_r, A_w_i, B_x, B_c_kv, B_w_q, B_w_uk, B_w_uv, B_w_o):
        axt = jnp.swapaxes(A_x, 1, 2).reshape(DM, S)
        bxt = jnp.swapaxes(B_x, 1, 2).reshape(DM, S)
        wrt = A_w_r.T
        wit = A_w_i.T
        ckv = B_c_kv.reshape(S, DC)
        wot = jnp.swapaxes(B_w_o, 1, 2)
        tabs = [jnp.asarray(t) for t in _tables()]
        args = (axt, wrt, wit, bxt, ckv, B_w_q, B_w_uk, B_w_uv, wot, *tabs)
        vm = pltpu.VMEM
        scratch = [
            vm((DM, S), bf16), vm((J, S), bf16), vm((J, S), bf16),
            *[vm(t.shape, t.dtype) for t in tabs],
            vm((DM, S), bf16), vm((S, DC), bf16),
            vm((DM, H, D), bf16),
            vm((DC, H, D), bf16), vm((DC, H, D), bf16), vm((H + 2, DM + 2 * DC, D), bf16),
            vm((H, DM, D), bf16), vm((H, S, D), bf16),
            vm((2 * DM, S), f32), vm((S, YC), bf16), vm((S, 2 * DM - YC), bf16),
            pltpu.SemaphoreType.DMA((15,)), pltpu.SemaphoreType.DMA((2, H)),
            pltpu.SemaphoreType.DMA((S // OCH,)), pltpu.SemaphoreType.DMA((1,)),
        ]
        out = pl.pallas_call(
            functools.partial(_kernel, do_a=do_a, do_b=do_b, scopes=scopes),
            in_specs=[pl.BlockSpec(memory_space=pl.ANY)] * len(args),
            out_specs=pl.BlockSpec(memory_space=pl.ANY),
            out_shape=jax.ShapeDtypeStruct((S, 2 * DM), bf16),
            scratch_shapes=scratch,
            compiler_params=pltpu.CompilerParams(vmem_limit_bytes=120 * 2**20),
        )(*args)
        return out.reshape(1, S, 2 * DM)

    return run


_run = _build()


@jax.jit
def pallas_concat_heads__spectral_gfnet__compressed_kv_cla__prompt_kernel(
    A_x: jax.Array,
    A_w_r: jax.Array,
    A_w_i: jax.Array,
    B_x: jax.Array,
    B_c_kv: jax.Array,
    B_w_q: jax.Array,
    B_w_uk: jax.Array,
    B_w_uv: jax.Array,
    B_w_o: jax.Array,
):
    return _run(A_x, A_w_r, A_w_i, B_x, B_c_kv, B_w_q, B_w_uk, B_w_uv, B_w_o)
```

```python
import contextlib
import functools
import math

import jax
import jax.numpy as jnp
import numpy as np
import jax.experimental.pallas as pl
import jax.experimental.pallas.tpu as pltpu

f32 = jnp.float32
bf16 = jnp.bfloat16

NN = (((1,), (0,)), ((), ()))
NT = (((1,), (1,)), ((), ()))

S = 2048
DM = 448
J = DM // 2 + 1
HD = DM // 2
JA = 120
JB = 112
H = 16
D = 256
DC = 1024
R16 = 16
LN = 128
TQ = 256
CCH = DC // H
PX = H
YC = 384
HEAD_ORDER = ('K0-2 U0-3 U3-6 K2-8 Q1 T1 B1 Q4 U6-8 Q0 T4 B4 V4 Q6 B0 Q3 B6 T0 V0 T3 V1 Q5 T5 Q7 B5 T6 V6 B3 T7 B7 '
              'V3 V7 Q2 V5 O0 T2 B2 V2 O75213 O4 O6')
NWQ = 14
OCH = 256
QHEADS = 2
QPIECES = 16


def _dot(a, b, dn):
    return jax.lax.dot_general(a, b, dn, preferred_element_type=f32)


@functools.lru_cache(maxsize=None)
def _tables():
    j = np.arange(J)[:, None].astype(np.float64)
    d = np.arange(DM)[None, :].astype(np.float64)
    ang = 2.0 * np.pi * ((j * d) % DM) / DM
    cos, sin = np.cos(ang), np.sin(ang)
    ne, no = (J + 1) // 2, J // 2
    fd = np.zeros((2 * JA + 2 * JB, HD), np.float64)
    fd[0:ne] = cos[0::2, 0:HD]
    fd[JA:JA + ne] = -sin[0::2, 0:HD]
    fd[2 * JA:2 * JA + no] = cos[1::2, 0:HD]
    fd[2 * JA + JB:2 * JA + JB + no] = -sin[1::2, 0:HD]

    m = np.arange(LN)[:, None].astype(np.float64)
    l = np.arange(LN)[None, :].astype(np.float64)
    a128 = 2.0 * np.pi * ((m * l) % LN) / LN
    fr, fi = np.cos(a128), -np.sin(a128)
    l2 = np.block([[fr, -fi], [fi, fr]])

    r = np.arange(R16)[:, None].astype(np.float64)
    at = 2.0 * np.pi * (r * l) / S
    tw = np.stack([np.cos(at), -np.sin(at)])
    tw = np.broadcast_to(tw[:, :, None, :], (2, R16, 8, LN)).copy()

    l3 = np.zeros((R16, 2 * LN, LN), np.float64)
    for rr in range(R16):
        a3 = 2.0 * np.pi * ((m * (rr + R16 * l)) % S) / S
        l3[rr] = np.concatenate([np.cos(a3), np.sin(a3)], axis=0)

    cj = np.full((J,), 2.0)
    cj[0] = 1.0
    cj[J - 1] = 1.0
    scale = cj[None, :] / float(S * DM)
    cr, ci = cos.T[0:HD] * scale, -sin.T[0:HD] * scale
    l4 = np.zeros((2, HD, 2 * LN), np.float64)
    l4[0, :, 0:ne] = cr[:, 0::2]
    l4[0, :, LN:LN + ne] = ci[:, 0::2]
    l4[1, :, 0:no] = cr[:, 1::2]
    l4[1, :, LN:LN + no] = ci[:, 1::2]

    def packed(a):
        h = np.asarray(a, np.float32).astype(bf16).view(np.uint16).astype(np.uint32)
        return h[..., 0::2, :] | (h[..., 1::2, :] << 16)

    return (packed(fd), packed(l2), np.asarray(tw, np.float32), packed(l3), packed(l4.reshape(2 * HD, 2 * LN)))


def _cmul_const(z, k, n, sign):
    re, im = z
    k = k % n
    if k == 0:
        return re, im
    if 4 * k == n:
        return (-im, re) if sign > 0 else (im, -re)
    if 8 * k == n:
        c = math.sqrt(0.5)
        return ((re - im) * c, (re + im) * c) if sign > 0 else ((re + im) * c, (im - re) * c)
    if 8 * k == 3 * n:
        c = math.sqrt(0.5)
        return ((re + im) * (-c), (re - im) * c) if sign > 0 else ((im - re) * c, (re + im) * (-c))
    c = math.cos(2.0 * math.pi * k / n)
    s = sign * math.sin(2.0 * math.pi * k / n)
    return re * c - im * s, re * s + im * c


def _fft(zs, sign):
    n = len(zs)
    if n == 1:
        return zs
    ev = _fft(zs[0::2], sign)
    od = _fft(zs[1::2], sign)
    out = [None] * n
    for k in range(n // 2):
        if 4 * k == n:
            (er, ei), (orr, oi) = ev[k], od[k]
            if sign > 0:
                out[k] = (er - oi, ei + orr)
                out[k + n // 2] = (er + oi, ei - orr)
            else:
                out[k] = (er + oi, ei - orr)
                out[k + n // 2] = (er - oi, ei + orr)
            continue
        tr, ti = _cmul_const(od[k], k, n, sign)
        er, ei = ev[k]
        out[k] = (er + tr, ei + ti)
        out[k + n // 2] = (er - tr, ei - ti)
    return out


def _softmax_rows(segs):
    m = functools.reduce(jnp.maximum, [jnp.max(sg, axis=1, keepdims=True) for sg in segs])
    ps = [jnp.exp2(sg - m).astype(bf16) for sg in segs]
    l = functools.reduce(jnp.add, [jnp.sum(p.astype(f32), axis=1, keepdims=True) for p in ps])
    return ps, l


def _bf(x):
    return pltpu.bitcast(x, bf16)


def _cat(parts, axis):
    return jnp.concatenate(parts, axis=axis) if len(parts) > 1 else parts[0]


def _kernel(axt_hbm, wrt_hbm, wit_hbm, bxt_hbm, ckv_hbm, wq_hbm, wuk_hbm, wuv_hbm, wot_hbm,
            fd_hbm, l2_hbm, tw_hbm, l3_hbm, l4_hbm,
            out_hbm,
            axt, wrt, wit, fd, l2, tw, l3, l4,
            bxt, ckv, wq_raw, wuk_raw, wuv_raw, wall, wot, q_all,
            ot, ybuf, obuf, sem, wsem, osem, ysem, *, do_a, do_b, scopes, order):
    scope = jax.named_scope if scopes else (lambda name: contextlib.nullcontext())
    XC = S // 4
    simple = ([(fd_hbm, fd)]
              + [(axt_hbm.at[:, c * XC:(c + 1) * XC], axt.at[:, c * XC:(c + 1) * XC]) for c in range(4)]
              + [(tw_hbm, tw), (l2_hbm, l2), (wrt_hbm, wrt), (wit_hbm, wit),
                 (l3_hbm, l3), (l4_hbm, l4), (wq_hbm, wq_raw), (bxt_hbm, bxt), (ckv_hbm, ckv), (wot_hbm, wot)])
    cps = [pltpu.make_async_copy(s, d, sem.at[i]) for i, (s, d) in enumerate(simple)]
    c_fd = cps[0]
    (c_tw, c_l2, c_wrt, c_wit, c_l3, c_l4, c_wq, c_bxt, c_ckv, c_wot) = cps[5:]

    def wchunk(which, t):
        src, dst = ((wuk_hbm, wuk_raw), (wuv_hbm, wuv_raw))[which]
        return pltpu.make_async_copy(src.at[pl.ds(t * CCH, CCH)], dst.at[pl.ds(t * CCH, CCH)], wsem.at[which, t])

    def issue(lo, hi):
        def body(i, carry):
            for k in range(lo, hi):
                pl.when(i == k)(cps[k].start)
            return carry
        jax.lax.fori_loop(lo, hi, body, 0)

    def wait_all(cs):
        def body(i, carry):
            for k, c in enumerate(cs):
                pl.when(i == k)(c.wait)
            return carry
        jax.lax.fori_loop(0, max(2, len(cs)), body, 0)

    def issue_w(t, carry):
        wchunk(0, t).start()
        wchunk(1, t).start()
        ot[DM:2 * DM, pl.ds(pl.multiple_of(t * LN, LN), LN)] = jnp.zeros((DM, LN), f32)
        return carry

    with scope('issue'):
        issue(0, len(cps) - 2)
        jax.lax.fori_loop(0, H, issue_w, 0)
        issue(len(cps) - 2, len(cps))

    def x_prep(k):
        rr = jax.lax.broadcasted_iota(jnp.int32, (LN, LN), 0)
        cc = jax.lax.broadcasted_iota(jnp.int32, (LN, LN), 1)
        eye = jnp.where(rr == cc, 1.0, 0.0).astype(bf16)
        x = _dot(eye, bxt[:, k * LN:(k + 1) * LN], NT).astype(bf16)
        wall[PX, k * LN:(k + 1) * LN, :] = x[:, 0:D]
        wall[PX + 1, k * LN:(k + 1) * LN, 0:DM - D] = x[:, D:DM]

    def wq_prep(k):
        n = DM // NWQ
        wall[0:H, k * n:(k + 1) * n, :] = jnp.swapaxes(wq_raw[k * n:(k + 1) * n], 0, 1)

    def part_a(x1a, x1b, rma, rmb, wsa, wsb, csa, csb, us):
        def stage1(c, carry):
            cols = pl.ds(pl.multiple_of(c * XC, XC), XC)
            pltpu.make_async_copy(axt_hbm.at[:, cols], axt.at[:, cols], sem.at[1 + c]).wait()
            lo, hi = axt[0:HD, cols].astype(f32), axt[HD:DM, cols].astype(f32)
            x1a[:, cols] = _dot(_bf(fd[0:JA, :]), (lo + hi).astype(bf16), NN)
            x1b[:, cols] = _dot(_bf(fd[JA:, :]), (lo - hi).astype(bf16), NN)
            return carry

        def fwd16(x1, rm, n, r0):
            zs = [(x1[pl.ds(r0, 8), c * LN:(c + 1) * LN], x1[pl.ds(n + r0, 8), c * LN:(c + 1) * LN])
                  for c in range(R16)]
            ys = _fft(zs, -1)
            for r in range(R16):
                re, im = ys[r]
                if r:
                    tr, ti = tw[0, r], tw[1, r]
                    re, im = re * tr - im * ti, re * ti + im * tr
                rm[r, pl.ds(r0, 8), 0:LN] = re
                rm[r, pl.ds(r0, 8), LN:2 * LN] = im

        def wprep(c):
            cols = slice(c * LN, (c + 1) * LN)
            row = jax.lax.broadcasted_iota(jnp.int32, (LN - JB, LN), 0)
            for p, wt in enumerate((wrt, wit)):
                u = pltpu.bitcast(wt[0:J - 1, cols], jnp.uint32)
                even = pltpu.bitcast(u << 16, f32)
                odd = pltpu.bitcast(u & jnp.uint32(0xFFFF0000), f32)
                last = jnp.broadcast_to(wt[J - 1:J, cols].astype(f32), (LN - JB, LN))
                wsa[p, cols, :] = jnp.concatenate([even, jnp.where(row == 0, last, 0.0)], axis=0).T
                wsb[p, cols, :] = jnp.concatenate([odd, jnp.zeros((LN - JB, LN), f32)], axis=0).T

        def stage2(rm, k):
            return _dot(_bf(l2[...]), rm[4 * k:4 * k + 4].reshape(4 * LN, 2 * LN).astype(bf16), NT)

        def stage3(x, ws, cs, r):
            x = x[r // 4]
            c0 = (r % 4) * LN
            xr, xi = x[0:LN, c0:c0 + LN], x[LN:2 * LN, c0:c0 + LN]
            wr = ws[0, pl.ds(r, LN, stride=R16), :]
            wi = ws[1, pl.ds(r, LN, stride=R16), :]
            g = jnp.concatenate([xr * wr - xi * wi, xr * wi + xi * wr], axis=1).astype(bf16)
            c = _dot(_bf(l3[r]), g, NN)
            cs[r, 0:LN, :] = c[0:LN, 0:LN] - c[LN:2 * LN, LN:2 * LN]
            cs[r, LN:2 * LN, :] = c[LN:2 * LN, 0:LN] + c[0:LN, LN:2 * LN]

        def inv16(cs, half, r0):
            zs = [(cs[r, r0:r0 + 8, :], cs[r, LN + r0:LN + r0 + 8, :]) for r in range(R16)]
            ys = _fft(zs, +1)
            for c in range(R16):
                us[half, c * LN + r0:c * LN + r0 + 8, 0:LN] = ys[c][0].astype(bf16)
                us[half, c * LN + r0:c * LN + r0 + 8, LN:2 * LN] = ys[c][1].astype(bf16)

        def stage4(half, k):
            cols = slice(k * LN, (k + 1) * LN)
            y = _dot(_bf(l4[half * HD // 2:(half + 1) * HD // 2, :]), us[half, cols, :], NT)
            if half:
                e = ot[0:HD, cols]
                ot[0:HD, cols] = e + y
                ot[HD:DM, cols] = e - y
            else:
                ot[0:HD, cols] = y

        with scope('w0'):
            c_fd.wait()
        with scope('S1'):
            jax.lax.fori_loop(0, 4, stage1, 0)
        with scope('wt_tw'):
            wait_all([c_tw])

        def fwd16a(g, carry):
            fwd16(x1a, rma, JA, pl.multiple_of(g * 8, 8))
            return carry

        def fwd16b(g, carry):
            fwd16(x1b, rmb, JB, pl.multiple_of(g * 8, 8))
            return carry

        with scope('F16'):
            jax.lax.fori_loop(0, JA // 8, fwd16a, 0)
            jax.lax.fori_loop(0, JB // 8, fwd16b, 0)
        with scope('wt_l2'):
            wait_all([c_l2, c_wrt, c_wit])
        rma[:, JA:LN, :] = jnp.zeros((R16, LN - JA, 2 * LN), f32)
        rmb[:, JB:LN, :] = jnp.zeros((R16, LN - JB, 2 * LN), f32)
        xa, xb = [], []
        for k in range(8):
            wprep(2 * k)
            wprep(2 * k + 1)
            (xa, xb)[k // 4].append(stage2((rma, rmb)[k // 4], k % 4))
        with scope('wt_W'):
            wait_all([c_l3, c_l4])
        for r in range(R16):
            stage3(xa, wsa, csa, r)
        for r in range(R16):
            stage3(xb, wsb, csb, r)
            inv16(csa, 0, r * 8)
        for k in range(R16):
            stage4(0, k)
            inv16(csb, 1, k * 8)
        with scope('wt_wq'):
            wait_all([c_wq])
        done = 0
        for k in range(R16):
            while do_b and done * R16 < (k + 1) * NWQ and done < NWQ:
                wq_prep(done)
                done += 1
            stage4(1, k)

    if do_a:
        pl.run_scoped(part_a,
                      pltpu.VMEM((2 * JA, S), f32), pltpu.VMEM((2 * JB, S), f32),
                      pltpu.VMEM((R16, LN, 2 * LN), f32), pltpu.VMEM((R16, LN, 2 * LN), f32),
                      pltpu.VMEM((2, S, LN), f32), pltpu.VMEM((2, S, LN), f32),
                      pltpu.VMEM((R16, 2 * LN, LN), f32), pltpu.VMEM((R16, 2 * LN, LN), f32),
                      pltpu.VMEM((2, S, 2 * LN), bf16))
    else:
        for c in cps[:-3]:
            c.wait()
        ot[0:DM, :] = jnp.zeros((DM, S), f32)
        if do_b:
            for k in range(R16):
                wq_prep(k % NWQ)

    with scope('wt_x'):
        wait_all([c_bxt])
    for k in range(R16):
        cols = slice(k * LN, (k + 1) * LN)
        ybuf[cols, :] = ot[0:YC, cols].astype(bf16).T
        if do_b:
            x_prep(k)
    c_y = pltpu.make_async_copy(ybuf, out_hbm.at[:, 0:YC], ysem.at[0])
    c_y.start()

    qscale = (D ** -0.5) * math.log2(math.e)

    with scope('wt_c0'):
        for u in range(QHEADS):
            wchunk(0, u).wait()
            wchunk(1, u).wait()

    def qstep(tt, carry):
        if do_b:
            rq, rw = S // QPIECES, 2 * CCH // QPIECES
            for u in range(QHEADS):
                t = tt * QHEADS + u
                for j in range(QPIECES):
                    x = jnp.concatenate([wall[PX, j * rq:(j + 1) * rq, :], wall[PX + 1, j * rq:(j + 1) * rq, 0:DM - D]],
                                        axis=1)
                    q_all[t, j * rq:(j + 1) * rq] = (_dot(x, wall[t, 0:DM, :], NN) * qscale).astype(bf16)
                    which, off = divmod(j * rw, CCH)
                    r0 = pl.multiple_of(t * CCH + off, rw)
                    src = (wuk_raw, wuv_raw)[which]
                    wall[0:H, pl.ds(DM + which * DC + r0, rw), :] = jnp.swapaxes(src[pl.ds(r0, rw)], 0, 1)

        @pl.when(tt + 1 < H // QHEADS)
        def _():
            for u in range(QHEADS):
                wchunk(0, (tt + 1) * QHEADS + u).wait()
                wchunk(1, (tt + 1) * QHEADS + u).wait()

        return carry

    with scope('P2'):
        jax.lax.fori_loop(0, H // QHEADS, qstep, 0)
    with scope('wt_ckv'):
        c_ckv.wait()
        c_wot.wait()

    def head(h, carry):
        with scope('head'):
            return head_body(h, carry)

    def head_body(h, carry):
        rr = jax.lax.broadcasted_iota(jnp.int32, (LN, LN), 0)
        cc = jax.lax.broadcasted_iota(jnp.int32, (LN, LN), 1)
        tri = cc <= rr
        neg = -1e9 * math.log2(math.e)
        kv = {'K': [], 'U': []}
        scores, probs, ctxs = {}, {}, {}

        def rows(name, a, b):
            parts = []
            for lo, arr in sorted(kv[name], key=lambda x: x[0]):
                x, y = max(a, lo), min(b, lo + arr.shape[0])
                if x < y:
                    parts.append(arr[x - lo:y - lo])
            return _cat(parts, 0)

        for tok in order.split():
            kind, arg = tok[0], tok[1:]
            if kind in 'KU':
                a, b = map(int, arg.split('-')) if arg else (0, S // TQ)
                w0 = DM + (DC if kind == 'U' else 0)
                w = wall[h, w0:w0 + DC, :]
                kv[kind].append((a * TQ, _dot(ckv[a * TQ:b * TQ, :], w, NN).astype(bf16)))
                continue
            if kind == 'O':
                grp = [int(ch) for ch in arg]
                res = _dot(wot[h], _cat([ctxs[j] for j in grp], 0), NT)
                for n, j in enumerate(grp):
                    ot[DM:2 * DM, j * TQ:(j + 1) * TQ] += res[:, n * TQ:(n + 1) * TQ]
                continue
            i = int(arg)
            r0 = i * TQ
            lm = r0 + LN
            if kind == 'Q':
                q = q_all[h, r0:r0 + TQ, :]
                s = _dot(q, rows('K', 0, lm), NT)
                sx = jnp.where(tri, _dot(q[LN:], rows('K', lm, lm + LN), NT), neg)
                scores[i] = (s, sx)
            elif kind in 'STB':
                s, sx = scores[i]
                if kind in 'ST':
                    sd = jnp.where(tri, s[0:LN, r0:lm], neg)
                    pt, lt = _softmax_rows(([s[0:LN, 0:r0]] if i else []) + [sd])
                    probs[i, 0] = (_cat(pt, 1), lt)
                if kind in 'SB':
                    probs[i, 1] = _softmax_rows([s[LN:], sx])
            else:
                (pt, lt), ((pb, px), lb) = probs.pop((i, 0)), probs.pop((i, 1))
                ctx = _dot(jnp.concatenate([pt, pb], axis=0), rows('U', 0, lm), NN)
                cx = _dot(px, rows('U', lm, lm + LN), NN)
                ctxs[i] = jnp.concatenate([ctx[0:LN] * (1.0 / lt), (ctx[LN:] + cx) * (1.0 / lb)],
                                          axis=0).astype(bf16)
        return carry

    if do_b:
        with scope('P3'):
            jax.lax.fori_loop(0, H, head, 0)

    def ocopy(c):
        rows = pl.ds(pl.multiple_of(c * OCH, OCH), OCH)
        return pltpu.make_async_copy(obuf.at[rows], out_hbm.at[rows, YC:2 * DM], osem.at[c])

    def ostep(c, carry):
        for k in range(OCH // LN):
            cols = pl.ds(pl.multiple_of(c * OCH + k * LN, LN), LN)
            obuf[cols, :] = ot[YC:2 * DM, cols].astype(bf16).T
        ocopy(c).start()
        return carry

    with scope('fin'):
        jax.lax.fori_loop(0, S // OCH, ostep, 0)
    with scope('wt_out'):
        c_y.wait()
        for c in range(S // OCH):
            ocopy(c).wait()


def _build(do_a=True, do_b=True, scopes=False, order=HEAD_ORDER):
    def run(A_x, A_w_r, A_w_i, B_x, B_c_kv, B_w_q, B_w_uk, B_w_uv, B_w_o):
        axt = jnp.swapaxes(A_x, 1, 2).reshape(DM, S)
        bxt = jnp.swapaxes(B_x, 1, 2).reshape(DM, S)
        wrt = A_w_r.T
        wit = A_w_i.T
        ckv = B_c_kv.reshape(S, DC)
        wot = jnp.swapaxes(B_w_o, 1, 2)
        tabs = [jnp.asarray(t) for t in _tables()]
        args = (axt, wrt, wit, bxt, ckv, B_w_q, B_w_uk, B_w_uv, wot, *tabs)
        vm = pltpu.VMEM
        scratch = [
            vm((DM, S), bf16), vm((J, S), bf16), vm((J, S), bf16),
            *[vm(t.shape, t.dtype) for t in tabs],
            vm((DM, S), bf16), vm((S, DC), bf16),
            vm((DM, H, D), bf16),
            vm((DC, H, D), bf16), vm((DC, H, D), bf16), vm((H + 2, DM + 2 * DC, D), bf16),
            vm((H, DM, D), bf16), vm((H, S, D), bf16),
            vm((2 * DM, S), f32), vm((S, YC), bf16), vm((S, 2 * DM - YC), bf16),
            pltpu.SemaphoreType.DMA((15,)), pltpu.SemaphoreType.DMA((2, H)),
            pltpu.SemaphoreType.DMA((S // OCH,)), pltpu.SemaphoreType.DMA((1,)),
        ]
        out = pl.pallas_call(
            functools.partial(_kernel, do_a=do_a, do_b=do_b, scopes=scopes, order=order),
            in_specs=[pl.BlockSpec(memory_space=pl.ANY)] * len(args),
            out_specs=pl.BlockSpec(memory_space=pl.ANY),
            out_shape=jax.ShapeDtypeStruct((S, 2 * DM), bf16),
            scratch_shapes=scratch,
            compiler_params=pltpu.CompilerParams(vmem_limit_bytes=120 * 2**20),
        )(*args)
        return out.reshape(1, S, 2 * DM)

    return run


_run = _build()


@jax.jit
def pallas_concat_heads__spectral_gfnet__compressed_kv_cla__prompt_kernel(
    A_x: jax.Array,
    A_w_r: jax.Array,
    A_w_i: jax.Array,
    B_x: jax.Array,
    B_c_kv: jax.Array,
    B_w_q: jax.Array,
    B_w_uk: jax.Array,
    B_w_uv: jax.Array,
    B_w_o: jax.Array,
):
    return _run(A_x, A_w_r, A_w_i, B_x, B_c_kv, B_w_q, B_w_uk, B_w_uv, B_w_o)
```

```python
import contextlib
import functools
import math

import jax
import jax.numpy as jnp
import numpy as np
import jax.experimental.pallas as pl
import jax.experimental.pallas.tpu as pltpu

f32 = jnp.float32
bf16 = jnp.bfloat16

NN = (((1,), (0,)), ((), ()))
NT = (((1,), (1,)), ((), ()))

S = 2048
DM = 448
J = DM // 2 + 1
HD = DM // 2
JA = 120
JB = 112
H = 16
D = 256
DC = 1024
R16 = 16
LN = 128
TQ = 256
CCH = DC // H
PX = H
YC = 384
HEAD_ORDER = ('K0-2 U0-3 U3-6 K2-8 Q1 T1 B1 Q4 U6-8 Q0 T4 B4 V4 Q6 B0 Q3 B6 T0 V0 T3 V1 Q5 T5 Q7 B5 T6 V6 B3 T7 B7 '
              'V3 V7 Q2 V5 O0 T2 B2 V2 O75213 O4 O6')
NWQ = 28
OCH = 256
QHEADS = 2
QPIECES = 16


def _dot(a, b, dn):
    return jax.lax.dot_general(a, b, dn, preferred_element_type=f32)


@functools.lru_cache(maxsize=None)
def _tables():
    j = np.arange(J)[:, None].astype(np.float64)
    d = np.arange(DM)[None, :].astype(np.float64)
    ang = 2.0 * np.pi * ((j * d) % DM) / DM
    cos, sin = np.cos(ang), np.sin(ang)
    ne, no = (J + 1) // 2, J // 2
    fd = np.zeros((2 * JA + 2 * JB, HD), np.float64)
    fd[0:ne] = cos[0::2, 0:HD]
    fd[JA:JA + ne] = -sin[0::2, 0:HD]
    fd[2 * JA:2 * JA + no] = cos[1::2, 0:HD]
    fd[2 * JA + JB:2 * JA + JB + no] = -sin[1::2, 0:HD]

    m = np.arange(LN)[:, None].astype(np.float64)
    l = np.arange(LN)[None, :].astype(np.float64)
    a128 = 2.0 * np.pi * ((m * l) % LN) / LN
    fr, fi = np.cos(a128), -np.sin(a128)
    l2 = np.block([[fr, -fi], [fi, fr]])

    r = np.arange(R16)[:, None].astype(np.float64)
    at = 2.0 * np.pi * (r * l) / S
    tw = np.stack([np.cos(at), -np.sin(at)])
    tw = np.broadcast_to(tw[:, :, None, :], (2, R16, 8, LN)).copy()

    l3 = np.zeros((R16, 2 * LN, LN), np.float64)
    for rr in range(R16):
        a3 = 2.0 * np.pi * ((m * (rr + R16 * l)) % S) / S
        l3[rr] = np.concatenate([np.cos(a3), np.sin(a3)], axis=0)

    cj = np.full((J,), 2.0)
    cj[0] = 1.0
    cj[J - 1] = 1.0
    scale = cj[None, :] / float(S * DM)
    cr, ci = cos.T[0:HD] * scale, -sin.T[0:HD] * scale
    l4 = np.zeros((2, HD, 2 * LN), np.float64)
    l4[0, :, 0:ne] = cr[:, 0::2]
    l4[0, :, LN:LN + ne] = ci[:, 0::2]
    l4[1, :, 0:no] = cr[:, 1::2]
    l4[1, :, LN:LN + no] = ci[:, 1::2]

    def packed(a):
        h = np.asarray(a, np.float32).astype(bf16).view(np.uint16).astype(np.uint32)
        return h[..., 0::2, :] | (h[..., 1::2, :] << 16)

    return (packed(fd), packed(l2), np.asarray(tw, np.float32), packed(l3), packed(l4.reshape(2 * HD, 2 * LN)))


def _cmul_const(z, k, n, sign):
    re, im = z
    k = k % n
    if k == 0:
        return re, im
    if 4 * k == n:
        return (-im, re) if sign > 0 else (im, -re)
    if 8 * k == n:
        c = math.sqrt(0.5)
        return ((re - im) * c, (re + im) * c) if sign > 0 else ((re + im) * c, (im - re) * c)
    if 8 * k == 3 * n:
        c = math.sqrt(0.5)
        return ((re + im) * (-c), (re - im) * c) if sign > 0 else ((im - re) * c, (re + im) * (-c))
    c = math.cos(2.0 * math.pi * k / n)
    s = sign * math.sin(2.0 * math.pi * k / n)
    return re * c - im * s, re * s + im * c


def _fft(zs, sign):
    n = len(zs)
    if n == 1:
        return zs
    ev = _fft(zs[0::2], sign)
    od = _fft(zs[1::2], sign)
    out = [None] * n
    for k in range(n // 2):
        if 4 * k == n:
            (er, ei), (orr, oi) = ev[k], od[k]
            if sign > 0:
                out[k] = (er - oi, ei + orr)
                out[k + n // 2] = (er + oi, ei - orr)
            else:
                out[k] = (er + oi, ei - orr)
                out[k + n // 2] = (er - oi, ei + orr)
            continue
        tr, ti = _cmul_const(od[k], k, n, sign)
        er, ei = ev[k]
        out[k] = (er + tr, ei + ti)
        out[k + n // 2] = (er - tr, ei - ti)
    return out


def _softmax_rows(segs):
    m = functools.reduce(jnp.maximum, [jnp.max(sg, axis=1, keepdims=True) for sg in segs])
    ps = [jnp.exp2(sg - m).astype(bf16) for sg in segs]
    l = functools.reduce(jnp.add, [jnp.sum(p.astype(f32), axis=1, keepdims=True) for p in ps])
    return ps, l


def _bf(x):
    return pltpu.bitcast(x, bf16)


def _cat(parts, axis):
    return jnp.concatenate(parts, axis=axis) if len(parts) > 1 else parts[0]


def _kernel(axt_hbm, wrt_hbm, wit_hbm, bxt_hbm, ckv_hbm, wq_hbm, wuk_hbm, wuv_hbm, wot_hbm,
            fd_hbm, l2_hbm, tw_hbm, l3_hbm, l4_hbm,
            out_hbm,
            axt, wrt, wit, fd, l2, tw, l3, l4,
            bxt, ckv, wq_raw, wuk_raw, wuv_raw, wall, wot, q_all,
            ot, ybuf, obuf, sem, wsem, osem, ysem, *, do_a, do_b, scopes, order):
    scope = jax.named_scope if scopes else (lambda name: contextlib.nullcontext())
    XC = S // 4
    simple = ([(fd_hbm, fd)]
              + [(axt_hbm.at[:, c * XC:(c + 1) * XC], axt.at[:, c * XC:(c + 1) * XC]) for c in range(4)]
              + [(tw_hbm, tw), (l2_hbm, l2), (wrt_hbm, wrt), (wit_hbm, wit),
                 (l3_hbm, l3), (l4_hbm, l4), (wq_hbm, wq_raw), (bxt_hbm, bxt), (ckv_hbm, ckv), (wot_hbm, wot)])
    cps = [pltpu.make_async_copy(s, d, sem.at[i]) for i, (s, d) in enumerate(simple)]
    c_fd = cps[0]
    (c_tw, c_l2, c_wrt, c_wit, c_l3, c_l4, c_wq, c_bxt, c_ckv, c_wot) = cps[5:]

    def wchunk(which, t):
        src, dst = ((wuk_hbm, wuk_raw), (wuv_hbm, wuv_raw))[which]
        return pltpu.make_async_copy(src.at[pl.ds(t * CCH, CCH)], dst.at[pl.ds(t * CCH, CCH)], wsem.at[which, t])

    def issue(lo, hi):
        def body(i, carry):
            for k in range(lo, hi):
                pl.when(i == k)(cps[k].start)
            return carry
        jax.lax.fori_loop(lo, hi, body, 0)

    def wait_all(cs):
        def body(i, carry):
            for k, c in enumerate(cs):
                pl.when(i == k)(c.wait)
            return carry
        jax.lax.fori_loop(0, max(2, len(cs)), body, 0)

    def issue_w(t, carry):
        wchunk(0, t).start()
        wchunk(1, t).start()
        ot[DM:2 * DM, pl.ds(pl.multiple_of(t * LN, LN), LN)] = jnp.zeros((DM, LN), f32)
        return carry

    with scope('issue'):
        issue(0, len(cps) - 2)
        jax.lax.fori_loop(0, H, issue_w, 0)
        issue(len(cps) - 2, len(cps))

    def x_prep(k):
        rr = jax.lax.broadcasted_iota(jnp.int32, (LN, LN), 0)
        cc = jax.lax.broadcasted_iota(jnp.int32, (LN, LN), 1)
        eye = jnp.where(rr == cc, 1.0, 0.0).astype(bf16)
        x = _dot(eye, bxt[:, k * LN:(k + 1) * LN], NT).astype(bf16)
        wall[PX, k * LN:(k + 1) * LN, :] = x[:, 0:D]
        wall[PX + 1, k * LN:(k + 1) * LN, 0:DM - D] = x[:, D:DM]

    def wq_prep(k):
        n = DM // NWQ
        wall[0:H, k * n:(k + 1) * n, :] = jnp.swapaxes(wq_raw[k * n:(k + 1) * n], 0, 1)

    def part_a(x1a, x1b, rma, rmb, wsa, wsb, csa, csb, us):
        def stage1(c, carry):
            cols = pl.ds(pl.multiple_of(c * XC, XC), XC)
            pltpu.make_async_copy(axt_hbm.at[:, cols], axt.at[:, cols], sem.at[1 + c]).wait()
            lo, hi = axt[0:HD, cols].astype(f32), axt[HD:DM, cols].astype(f32)
            x1a[:, cols] = _dot(_bf(fd[0:JA, :]), (lo + hi).astype(bf16), NN)
            x1b[:, cols] = _dot(_bf(fd[JA:, :]), (lo - hi).astype(bf16), NN)
            return carry

        def fwd16(x1, rm, n, r0):
            zs = [(x1[pl.ds(r0, 8), c * LN:(c + 1) * LN], x1[pl.ds(n + r0, 8), c * LN:(c + 1) * LN])
                  for c in range(R16)]
            ys = _fft(zs, -1)
            for r in range(R16):
                re, im = ys[r]
                if r:
                    tr, ti = tw[0, r], tw[1, r]
                    re, im = re * tr - im * ti, re * ti + im * tr
                rm[r, pl.ds(r0, 8), 0:LN] = re
                rm[r, pl.ds(r0, 8), LN:2 * LN] = im

        def wprep(c):
            cols = slice(c * LN, (c + 1) * LN)
            row = jax.lax.broadcasted_iota(jnp.int32, (LN - JB, LN), 0)
            for p, wt in enumerate((wrt, wit)):
                u = pltpu.bitcast(wt[0:J - 1, cols], jnp.uint32)
                even = pltpu.bitcast(u << 16, f32)
                odd = pltpu.bitcast(u & jnp.uint32(0xFFFF0000), f32)
                last = jnp.broadcast_to(wt[J - 1:J, cols].astype(f32), (LN - JB, LN))
                wsa[p, cols, :] = jnp.concatenate([even, jnp.where(row == 0, last, 0.0)], axis=0).T
                wsb[p, cols, :] = jnp.concatenate([odd, jnp.zeros((LN - JB, LN), f32)], axis=0).T

        def stage2(rm, k):
            return _dot(_bf(l2[...]), rm[4 * k:4 * k + 4].reshape(4 * LN, 2 * LN).astype(bf16), NT)

        def stage3(x, ws, cs, r):
            x = x[r // 4]
            c0 = (r % 4) * LN
            xr, xi = x[0:LN, c0:c0 + LN], x[LN:2 * LN, c0:c0 + LN]
            wr = ws[0, pl.ds(r, LN, stride=R16), :]
            wi = ws[1, pl.ds(r, LN, stride=R16), :]
            g = jnp.concatenate([xr * wr - xi * wi, xr * wi + xi * wr], axis=1).astype(bf16)
            c = _dot(_bf(l3[r]), g, NN)
            cs[r, 0:LN, :] = c[0:LN, 0:LN] - c[LN:2 * LN, LN:2 * LN]
            cs[r, LN:2 * LN, :] = c[LN:2 * LN, 0:LN] + c[0:LN, LN:2 * LN]

        def inv16(cs, half, r0):
            zs = [(cs[r, r0:r0 + 8, :], cs[r, LN + r0:LN + r0 + 8, :]) for r in range(R16)]
            ys = _fft(zs, +1)
            for c in range(R16):
                us[half, c * LN + r0:c * LN + r0 + 8, 0:LN] = ys[c][0].astype(bf16)
                us[half, c * LN + r0:c * LN + r0 + 8, LN:2 * LN] = ys[c][1].astype(bf16)

        def stage4(k):
            cols = slice(k * LN, (k + 1) * LN)
            e = _dot(_bf(l4[0:HD // 2, :]), us[0, cols, :], NT)
            o = _dot(_bf(l4[HD // 2:HD, :]), us[1, cols, :], NT)
            ot[0:HD, cols] = e + o
            ot[HD:DM, cols] = e - o

        with scope('w0'):
            c_fd.wait()
        with scope('S1'):
            jax.lax.fori_loop(0, 4, stage1, 0)
        with scope('wt_tw'):
            wait_all([c_tw])

        def fwd16a(g, carry):
            fwd16(x1a, rma, JA, pl.multiple_of(g * 8, 8))
            return carry

        def fwd16b(g, carry):
            fwd16(x1b, rmb, JB, pl.multiple_of(g * 8, 8))
            return carry

        with scope('F16'):
            jax.lax.fori_loop(0, JA // 8, fwd16a, 0)
            jax.lax.fori_loop(0, JB // 8, fwd16b, 0)
        with scope('wt_l2'):
            wait_all([c_l2, c_wrt, c_wit])
        rma[:, JA:LN, :] = jnp.zeros((R16, LN - JA, 2 * LN), f32)
        rmb[:, JB:LN, :] = jnp.zeros((R16, LN - JB, 2 * LN), f32)
        xa, xb = [], []
        for k in range(8):
            wprep(2 * k)
            wprep(2 * k + 1)
            (xa, xb)[k // 4].append(stage2((rma, rmb)[k // 4], k % 4))
        with scope('wt_W'):
            wait_all([c_l3, c_l4])
        for r in range(R16):
            stage3(xa, wsa, csa, r)
        for r in range(R16):
            stage3(xb, wsb, csb, r)
            inv16(csa, 0, r * 8)
        for k in range(R16):
            inv16(csb, 1, k * 8)
        with scope('wt_wq'):
            wait_all([c_wq])
        done = 0
        for k in range(R16):
            while do_b and done * R16 < (k + 1) * NWQ and done < NWQ:
                wq_prep(done)
                done += 1
            stage4(k)

    if do_a:
        pl.run_scoped(part_a,
                      pltpu.VMEM((2 * JA, S), f32), pltpu.VMEM((2 * JB, S), f32),
                      pltpu.VMEM((R16, LN, 2 * LN), f32), pltpu.VMEM((R16, LN, 2 * LN), f32),
                      pltpu.VMEM((2, S, LN), f32), pltpu.VMEM((2, S, LN), f32),
                      pltpu.VMEM((R16, 2 * LN, LN), f32), pltpu.VMEM((R16, 2 * LN, LN), f32),
                      pltpu.VMEM((2, S, 2 * LN), bf16))
    else:
        for c in cps[:-3]:
            c.wait()
        ot[0:DM, :] = jnp.zeros((DM, S), f32)
        if do_b:
            for k in range(NWQ):
                wq_prep(k)

    with scope('wt_x'):
        wait_all([c_bxt])
    for k in range(R16):
        cols = slice(k * LN, (k + 1) * LN)
        ybuf[cols, :] = ot[0:YC, cols].astype(bf16).T
        if do_b:
            x_prep(k)
    c_y = pltpu.make_async_copy(ybuf, out_hbm.at[:, 0:YC], ysem.at[0])
    c_y.start()

    qscale = (D ** -0.5) * math.log2(math.e)

    with scope('wt_c0'):
        for u in range(QHEADS):
            wchunk(0, u).wait()
            wchunk(1, u).wait()

    def qstep(tt, carry):
        if do_b:
            rq, rw = S // QPIECES, 2 * CCH // QPIECES
            for u in range(QHEADS):
                t = tt * QHEADS + u
                for j in range(QPIECES):
                    x = jnp.concatenate([wall[PX, j * rq:(j + 1) * rq, :], wall[PX + 1, j * rq:(j + 1) * rq, 0:DM - D]],
                                        axis=1)
                    q_all[t, j * rq:(j + 1) * rq] = (_dot(x, wall[t, 0:DM, :], NN) * qscale).astype(bf16)
                    which, off = divmod(j * rw, CCH)
                    r0 = pl.multiple_of(t * CCH + off, rw)
                    src = (wuk_raw, wuv_raw)[which]
                    wall[0:H, pl.ds(DM + which * DC + r0, rw), :] = jnp.swapaxes(src[pl.ds(r0, rw)], 0, 1)

        @pl.when(tt + 1 < H // QHEADS)
        def _():
            for u in range(QHEADS):
                wchunk(0, (tt + 1) * QHEADS + u).wait()
                wchunk(1, (tt + 1) * QHEADS + u).wait()

        return carry

    with scope('P2'):
        jax.lax.fori_loop(0, H // QHEADS, qstep, 0)
    with scope('wt_ckv'):
        c_ckv.wait()
        c_wot.wait()

    def head(h, carry):
        with scope('head'):
            return head_body(h, carry)

    def head_body(h, carry):
        rr = jax.lax.broadcasted_iota(jnp.int32, (LN, LN), 0)
        cc = jax.lax.broadcasted_iota(jnp.int32, (LN, LN), 1)
        tri = cc <= rr
        neg = -1e9 * math.log2(math.e)
        kv = {'K': [], 'U': []}
        scores, probs, ctxs = {}, {}, {}

        def rows(name, a, b):
            parts = []
            for lo, arr in sorted(kv[name], key=lambda x: x[0]):
                x, y = max(a, lo), min(b, lo + arr.shape[0])
                if x < y:
                    parts.append(arr[x - lo:y - lo])
            return _cat(parts, 0)

        for tok in order.split():
            kind, arg = tok[0], tok[1:]
            if kind in 'KU':
                a, b = map(int, arg.split('-')) if arg else (0, S // TQ)
                w0 = DM + (DC if kind == 'U' else 0)
                w = wall[h, w0:w0 + DC, :]
                kv[kind].append((a * TQ, _dot(ckv[a * TQ:b * TQ, :], w, NN).astype(bf16)))
                continue
            if kind == 'O':
                grp = [int(ch) for ch in arg]
                res = _dot(wot[h], _cat([ctxs[j] for j in grp], 0), NT)
                for n, j in enumerate(grp):
                    ot[DM:2 * DM, j * TQ:(j + 1) * TQ] += res[:, n * TQ:(n + 1) * TQ]
                continue
            i = int(arg)
            r0 = i * TQ
            lm = r0 + LN
            if kind == 'Q':
                q = q_all[h, r0:r0 + TQ, :]
                s = _dot(q, rows('K', 0, lm), NT)
                sx = jnp.where(tri, _dot(q[LN:], rows('K', lm, lm + LN), NT), neg)
                scores[i] = (s, sx)
            elif kind in 'STB':
                s, sx = scores[i]
                if kind in 'ST':
                    sd = jnp.where(tri, s[0:LN, r0:lm], neg)
                    pt, lt = _softmax_rows(([s[0:LN, 0:r0]] if i else []) + [sd])
                    probs[i, 0] = (_cat(pt, 1), lt)
                if kind in 'SB':
                    probs[i, 1] = _softmax_rows([s[LN:], sx])
            else:
                (pt, lt), ((pb, px), lb) = probs.pop((i, 0)), probs.pop((i, 1))
                ctx = _dot(jnp.concatenate([pt, pb], axis=0), rows('U', 0, lm), NN)
                cx = _dot(px, rows('U', lm, lm + LN), NN)
                ctxs[i] = jnp.concatenate([ctx[0:LN] * (1.0 / lt), (ctx[LN:] + cx) * (1.0 / lb)],
                                          axis=0).astype(bf16)
        return carry

    if do_b:
        with scope('P3'):
            jax.lax.fori_loop(0, H, head, 0)

    def ocopy(c):
        rows = pl.ds(pl.multiple_of(c * OCH, OCH), OCH)
        return pltpu.make_async_copy(obuf.at[rows], out_hbm.at[rows, YC:2 * DM], osem.at[c])

    def ostep(c, carry):
        for k in range(OCH // LN):
            cols = pl.ds(pl.multiple_of(c * OCH + k * LN, LN), LN)
            obuf[cols, :] = ot[YC:2 * DM, cols].astype(bf16).T
        ocopy(c).start()
        return carry

    with scope('fin'):
        jax.lax.fori_loop(0, S // OCH, ostep, 0)
    with scope('wt_out'):
        c_y.wait()
        for c in range(S // OCH):
            ocopy(c).wait()


def _build(do_a=True, do_b=True, scopes=False, order=HEAD_ORDER):
    def run(A_x, A_w_r, A_w_i, B_x, B_c_kv, B_w_q, B_w_uk, B_w_uv, B_w_o):
        axt = jnp.swapaxes(A_x, 1, 2).reshape(DM, S)
        bxt = jnp.swapaxes(B_x, 1, 2).reshape(DM, S)
        wrt = A_w_r.T
        wit = A_w_i.T
        ckv = B_c_kv.reshape(S, DC)
        wot = jnp.swapaxes(B_w_o, 1, 2)
        tabs = [jnp.asarray(t) for t in _tables()]
        args = (axt, wrt, wit, bxt, ckv, B_w_q, B_w_uk, B_w_uv, wot, *tabs)
        vm = pltpu.VMEM
        scratch = [
            vm((DM, S), bf16), vm((J, S), bf16), vm((J, S), bf16),
            *[vm(t.shape, t.dtype) for t in tabs],
            vm((DM, S), bf16), vm((S, DC), bf16),
            vm((DM, H, D), bf16),
            vm((DC, H, D), bf16), vm((DC, H, D), bf16), vm((H + 2, DM + 2 * DC, D), bf16),
            vm((H, DM, D), bf16), vm((H, S, D), bf16),
            vm((2 * DM, S), f32), vm((S, YC), bf16), vm((S, 2 * DM - YC), bf16),
            pltpu.SemaphoreType.DMA((15,)), pltpu.SemaphoreType.DMA((2, H)),
            pltpu.SemaphoreType.DMA((S // OCH,)), pltpu.SemaphoreType.DMA((1,)),
        ]
        out = pl.pallas_call(
            functools.partial(_kernel, do_a=do_a, do_b=do_b, scopes=scopes, order=order),
            in_specs=[pl.BlockSpec(memory_space=pl.ANY)] * len(args),
            out_specs=pl.BlockSpec(memory_space=pl.ANY),
            out_shape=jax.ShapeDtypeStruct((S, 2 * DM), bf16),
            scratch_shapes=scratch,
            compiler_params=pltpu.CompilerParams(vmem_limit_bytes=120 * 2**20),
        )(*args)
        return out.reshape(1, S, 2 * DM)

    return run


_run = _build()


@jax.jit
def pallas_concat_heads__spectral_gfnet__compressed_kv_cla__prompt_kernel(
    A_x: jax.Array,
    A_w_r: jax.Array,
    A_w_i: jax.Array,
    B_x: jax.Array,
    B_c_kv: jax.Array,
    B_w_q: jax.Array,
    B_w_uk: jax.Array,
    B_w_uv: jax.Array,
    B_w_o: jax.Array,
):
    return _run(A_x, A_w_r, A_w_i, B_x, B_c_kv, B_w_q, B_w_uk, B_w_uv, B_w_o)
```
